```python
import jax
import jax.numpy as jnp

def _softmax(x, axis=-1):
    return jax.nn.softmax(x, axis=axis)

def _gelu(x):
    return jax.nn.gelu(x, approximate=True)

def _silu(x):
    return jax.nn.silu(x)

def _sigmoid(x):
    return jax.nn.sigmoid(x)

def _layernorm(x, axis=-1, eps=1e-05):
    m = jnp.mean(x, axis=axis, keepdims=True)
    v = jnp.var(x, axis=axis, keepdims=True)
    return (x - m) / jnp.sqrt(v + eps)

def _scatter_add(tgt, idx, src, axis=0):
    return tgt.at[idx].add(src)

def _segment_sum(src, seg, n):
    return jax.ops.segment_sum(src, seg, n)

class _Rng:

    def __init__(self, key):
        self._k = key

    def _next(self):
        self._k, sub = jax.random.split(self._k)
        return sub

    def normal(self, shape):
        return jax.random.normal(self._next(), shape, dtype=jnp.bfloat16)

    def randint(self, lo, hi, shape):
        return jax.random.randint(self._next(), shape, lo, hi, dtype=jnp.int32)

    def uniform(self, shape, lo=0.0, hi=1.0):
        return jax.random.uniform(self._next(), shape, jnp.bfloat16, lo, hi)

    def permutation(self, n):
        return jax.random.permutation(self._next(), n)
kernel_name = 'parallel_sum__memory_aug_recurrent_mem_tr__moe_arch_mod__prompt'

def setup_inputs():
    _rng = _Rng(jax.random.key(int.from_bytes(__import__("os").urandom(4), "little")))
    _w = lambda a: (lambda t: t.astype(jnp.bfloat16) if jnp.issubdtype(t.dtype, jnp.floating) else t)(jnp.asarray(a))

    def _A_setup():
        B, S, Dm = (1, 2048, 1024)
        H, Dh = (32, 128)
        M, seg = (8, 32)
        seg = min(seg, S)
        S = S // seg * seg
        return {'x': _w((lambda *s: _rng.normal(s) * 0.05)(B, S, Dm)), 'mem0': _w((lambda *s: _rng.normal(s) * 0.05)(B, M, Dm)), 'Wq': _w((lambda *s: _rng.normal(s) * 0.05)(Dm, H, Dh) * Dm ** (-0.5)), 'Wk': _w((lambda *s: _rng.normal(s) * 0.05)(Dm, H, Dh) * Dm ** (-0.5)), 'Wv': _w((lambda *s: _rng.normal(s) * 0.05)(Dm, H, Dh) * Dm ** (-0.5)), 'Wo': _w((lambda *s: _rng.normal(s) * 0.05)(H, Dh, Dm) * (H * Dh) ** (-0.5)), 'seg_len': seg}
    _A_in = _A_setup()

    def _B_setup():
        B, S, D, F, C = (1, 2048, 1024, 3584, 2)
        return {'x': _w((lambda *s: _rng.normal(s) * 0.05)(B, S, D)), 'w_r': _w((lambda *s: _rng.normal(s) * 0.05)(D)), 'w_gate': _w((lambda *s: _rng.normal(s) * 0.05)(D, F)), 'w_up': _w((lambda *s: _rng.normal(s) * 0.05)(D, F)), 'w_down': _w((lambda *s: _rng.normal(s) * 0.05)(F, D))}
    _B_in = _B_setup()
    return {'A_x': _A_in['x'], 'A_mem0': _A_in['mem0'], 'A_Wq': _A_in['Wq'], 'A_Wk': _A_in['Wk'], 'A_Wv': _A_in['Wv'], 'A_Wo': _A_in['Wo'], 'A_seg_len': _A_in['seg_len'], 'B_x': _B_in['x'], 'B_w_r': _B_in['w_r'], 'B_w_gate': _B_in['w_gate'], 'B_w_up': _B_in['w_up'], 'B_w_down': _B_in['w_down']}

def reference(A_x, A_mem0, A_Wq, A_Wk, A_Wv, A_Wo, A_seg_len, B_x, B_w_r, B_w_gate, B_w_up, B_w_down):

    def _A_ref(x, mem0, Wq, Wk, Wv, Wo, seg_len):
        B, S, Dm = x.shape
        H, Dh = (Wq.shape[1], Wq.shape[2])
        M = mem0.shape[1]
        scale = Dh ** (-0.5)
        n_seg = S // seg_len
        L = M + seg_len
        idx = jnp.arange(L)
        mask = (idx[:, None] < M) | (idx[:, None] >= idx[None, :])
        mem = mem0
        outs = []
        for s in range(n_seg):
            xs = x[:, s * seg_len:(s + 1) * seg_len, :].copy()
            h = jnp.concatenate([mem, xs], axis=1)
            q = jnp.einsum('btd,dhe->bhte', h, Wq)
            k = jnp.einsum('btd,dhe->bhte', h, Wk)
            v = jnp.einsum('btd,dhe->bhte', h, Wv)
            scores = jnp.einsum('bhqe,bhke->bhqk', q, k) * scale
            scores = jnp.where(mask[None, None], scores, -1000000000.0)
            p = _softmax(scores, axis=-1)
            o = jnp.einsum('bhqk,bhke->bhqe', p, v)
            o = jnp.einsum('bhte,hed->btd', o, Wo)
            mem = o[:, :M, :].copy()
            outs.append(o[:, M:, :])
        return jnp.concatenate(outs, axis=1)

    def _B_ref(x, w_r, w_gate, w_up, w_down):
        B, S, D = x.shape
        C = 2
        r = x @ w_r
        idx = jnp.argsort(-r, axis=-1)[:, :C]
        idx_e = jnp.repeat(idx.reshape(B, C, 1), D, axis=2)
        x_sel = jnp.take_along_axis(x, idx_e, axis=1)
        g = _silu(x_sel @ w_gate)
        u = x_sel @ w_up
        y = g * u @ w_down
        r_sel = _sigmoid(jnp.take_along_axis(r, idx, axis=1))
        y = y * r_sel.reshape(B, C, 1)
        b_off = (jnp.arange(B) * S).reshape(B, 1)
        flat_idx = (idx + b_off).reshape(B * C)
        zero = (x * 0.0).reshape(B * S, D)
        upd = _scatter_add(zero, flat_idx, y.reshape(B * C, D), axis=0)
        return x + upd.reshape(B, S, D)
    x = A_x
    xn = _layernorm(x, axis=-1)
    return x + _A_ref(xn, A_mem0, A_Wq, A_Wk, A_Wv, A_Wo, A_seg_len) + _B_ref(xn, B_w_r, B_w_gate, B_w_up, B_w_down)
```

```python
import jax
import jax.numpy as jnp
from jax import lax
import jax.experimental.pallas as pl
import jax.experimental.pallas.tpu as pltpu

BF = jnp.bfloat16
U32 = jnp.uint32
F32 = jnp.float32

S = 2048
D = 1024
H = 32
DH = 128
MEM = 8
SEG = 32
NSEG = S // SEG
FF = 3584
KT = D // 128
FT = FF // 128
XS = 24
PRE = S - NSEG * XS
RING = 576
RING32 = RING // 2
NPAIR = H // 2
NCH = 12

LAG_QK = 1
LAG_PV = 4
N_PART = 4
H_SPLIT = 26
UNROLL = 2


def _b2u(x):
    return pltpu.bitcast(x, U32)


def _u2b(x):
    return pltpu.bitcast(x, BF)


def _dot(a, b):
    return jnp.dot(a, b, preferred_element_type=F32)


def _dot_nt(a, b):
    return lax.dot_general(a, b, (((1,), (1,)), ((), ())), preferred_element_type=F32)


def _rbf(x):
    return x.astype(BF).astype(F32)


def _kernel(x_hbm, mem0_hbm, wq_hbm, wk_hbm, wv_hbm, wo_hbm, wr_hbm, wg_hbm, wu_hbm, wd_hbm,
            out_hbm,
            x_s, xn_t, xn_pre, wqkv, wtmp0, wtmp1, wo_s, ring, oring, abuf, out_s, raw,
            wg_s, wu_s, wd_s, mem0_s, wr_s, r_s,
            sem_x, sem_w, sem_wo, sem_small, sem_ffn, sem_out):
    w32 = [w.bitcast(U32) for w in (wq_hbm, wk_hbm, wv_hbm)]
    wo32 = wo_hbm.bitcast(U32)
    wg32 = wg_hbm.bitcast(U32)
    wu32 = wu_hbm.bitcast(U32)
    wd32 = wd_hbm.bitcast(U32)

    x_first = pltpu.make_async_copy(x_hbm.at[pl.ds(0, PRE), :], x_s.at[pl.ds(0, PRE), :], sem_x.at[0])

    def x_piece(c):
        r0 = pl.multiple_of(PRE + 128 * c, 128)
        return pltpu.make_async_copy(x_hbm.at[pl.ds(r0, 128), :], x_s.at[pl.ds(r0, 128), :],
                                     sem_x.at[1 + c])

    def w_copies(m, c):
        g4 = pl.multiple_of(4 * (c % 4), 4)
        return [pltpu.make_async_copy(w32[m].at[:, par, pl.ds(g4, 4), :],
                                      raw.at[c, :, pl.ds(4 * par, 4), :], sem_w.at[c])
                for par in range(2)]

    def w_start(c):
        if isinstance(c, int):
            for cp in w_copies(c // 4, c):
                cp.start()
        else:
            for m in range(3):
                @pl.when(c // 4 == m)
                def _():
                    for cp in w_copies(m, c):
                        cp.start()

    def w_wait(c):
        for cp in w_copies(0, c):
            cp.wait()

    def wo_copy(n):
        c0 = pl.multiple_of(128 * n, 128)
        return pltpu.make_async_copy(wo32.at[:, pl.ds(c0, 128)], wo_s.at[n], sem_wo)

    small_copies = [pltpu.make_async_copy(mem0_hbm, mem0_s, sem_small.at[0]),
                    pltpu.make_async_copy(wr_hbm, wr_s, sem_small.at[1])]
    ffn_copies = (
        [pltpu.make_async_copy(wg32.at[:, pl.ds(128 * j, 128)], wg_s.at[j], sem_ffn) for j in range(FT)]
        + [pltpu.make_async_copy(wu32.at[:, pl.ds(128 * j, 128)], wu_s.at[j], sem_ffn) for j in range(FT)]
        + [pltpu.make_async_copy(wd32.at[:, pl.ds(128 * n, 128)], wd_s.at[n], sem_ffn) for n in range(KT)])

    x_first.start()
    for c in small_copies:
        c.start()
    w_start(0)

    eps_bf = 1.0013580322265625e-05

    def layernorm_rows(r0, dst_pre):
        for q in range(8):
            rq = pl.multiple_of(r0 + 16 * q, 16)
            xf = x_s[pl.ds(rq, 16), :].astype(F32)
            mean = jnp.sum(xf, axis=1, keepdims=True) * (1.0 / D)
            cen = xf - mean
            var = jnp.sum(cen * cen, axis=1, keepdims=True) * (1.0 / D)
            sd = _rbf(jnp.sqrt(_rbf(_rbf(var) + eps_bf)))
            xp = _b2u((_rbf(xf - _rbf(mean)) * (1.0 / sd)).astype(BF))
            hq = pl.multiple_of(rq // 2, 8)
            for k in range(KT):
                xn_t[k, pl.ds(hq, 8), :] = xp[:, 128 * k:128 * (k + 1)]
                if dst_pre:
                    xn_pre[k, pl.ds(hq, 8), :] = xp[:, 128 * k:128 * (k + 1)]

    def router_rows(blk, wr16):
        h0 = pl.multiple_of(64 * blk, 64)
        xb = jnp.concatenate([_u2b(xn_t[k, pl.ds(h0, 64), :]) for k in range(KT)], axis=1)
        r_s[pl.ds(blk, 1), :] = _dot_nt(wr16, xb)[0:1, :]

    small_copies[1].wait()
    wr16 = jnp.broadcast_to(wr_s[...].astype(F32).reshape(1, D), (16, D)).astype(BF)
    x_first.wait()

    def ln_body(c, carry):
        layernorm_rows(128 * c, True)
        return carry

    lax.fori_loop(0, PRE // 128, ln_body, 0)
    for c in range(PRE // 128 - 1):
        router_rows(c, wr16)

    raw2 = raw.reshape(NCH * 4096, 128)
    wtmp = (wtmp0, wtmp1)

    def relayout(c, j):
        view = raw2.at[pl.ds(pl.multiple_of(c * 4096, 4096), 4096), :]
        for blk in range(4):
            a = view[pl.ds(1024 * blk + j, 128, stride=8), :]
            b = view[pl.ds(1024 * blk + 4 + j, 128, stride=8), :]
            ev = (a & jnp.uint32(0xFFFF)) | (b << 16)
            od = (a >> 16) | (b & jnp.uint32(0xFFFF0000))
            rows = pl.ds(128 * blk, 128)
            wqkv[8 * c + 2 * j, rows, :] = ev
            wqkv[8 * c + 2 * j + 1, rows, :] = od
            wtmp[j % 2][0, rows, :] = ev
            wtmp[j % 2][1, rows, :] = od

    def pre_mm(c, j):
        for i in range(2):
            for q in range(PRE // 128):
                lhs = jnp.concatenate([_u2b(xn_pre[k, pl.ds(64 * q, 64), :]) for k in range(KT)], axis=1)
                y = _dot(lhs, _u2b(wtmp[j % 2][i]))
                ring[8 * c + 2 * j + i, pl.ds(32 + 64 * q, 64), :] = _b2u(y.astype(BF))

    w_wait(0)
    w_start(1)
    x_piece(0).start()
    relayout(0, 0)

    def pre_body(c, carry):
        for j in range(3):
            relayout(c, j + 1)
            pre_mm(c, j)
            if j == 0:
                router_rows(c + PRE // 128 - 1, wr16)

        @pl.when(c + 1 < NCH)
        def _():
            w_wait(c + 1)
        x_piece(c).wait()

        @pl.when(c + 2 < NCH)
        def _():
            w_start(c + 2)

        @pl.when(c + 1 < NCH)
        def _():
            x_piece(c + 1).start()

        @pl.when((c >= 2) & (c < 2 + KT))
        def _():
            wo_copy(c - 2).start()

        relayout(jnp.minimum(c + 1, NCH - 1), 0)
        layernorm_rows(PRE + 128 * c, False)
        pre_mm(c, 3)
        return carry

    lax.fori_loop(0, NCH, pre_body, 0)
    router_rows(S // 128 - 1, wr16)

    for c in ffn_copies:
        c.start()

    row = lax.broadcasted_iota(jnp.int32, (80, 80), 0)
    col = lax.broadcasted_iota(jnp.int32, (80, 80), 1)
    same_head = (jnp.where(row < 64, row >> 5, (row - 64) >> 3)
                 == jnp.where(col < 64, col >> 5, (col - 64) >> 3))
    allowed = same_head & ((col >= 64) | (row >= 64) | (col <= row))
    fill = jnp.where(same_head, -1e9, -jnp.inf).astype(F32)
    low_half = lax.broadcasted_iota(jnp.int32, (8, 128), 0) < 4
    scale = DH ** -0.5

    def one_step(s, mem):
        x_ld = pl.multiple_of(PRE // 2 + s * (XS // 2), 4)
        qkv_st = pl.multiple_of((s * (XS // 2)) % RING32, 4)
        qkv_ld = pl.multiple_of((s * (SEG // 2) + 32) % RING32, 16)
        o_st = pl.multiple_of((s * (SEG // 2)) % RING32, 16)
        o_ld = qkv_st
        a_st = pl.multiple_of(s * (XS // 2), 4)

        lk = []
        for k in range(KT):
            l0 = xn_t[k, pl.ds(x_ld, 8), :]
            l1 = jnp.where(low_half, xn_t[k, pl.ds(x_ld + 8, 8), :], mem[k])
            lk.append(_u2b(jnp.concatenate([l0, l1], axis=0)))
        lhs = jnp.concatenate(lk, axis=1)

        ymem = {}
        xs = {}
        probs = {}
        parts = {}

        def proj(h):
            for m in range(3):
                y = _dot(lhs, _u2b(wqkv[m * H + h]))
                ring[m * H + h, pl.ds(qkv_st, XS // 2), :] = _b2u(y.astype(BF))[0:XS // 2]
                ymem[(h, m)] = y[XS:XS + MEM]
                xs[(h, m)] = ring[m * H + h, pl.ds(qkv_ld, SEG // 2), :]

        def pair(p, m):
            a, b = 2 * p, 2 * p + 1
            mm = jnp.concatenate([ymem[(a, m)], ymem[(b, m)]], axis=0).astype(BF)
            return jnp.concatenate([_u2b(xs[(a, m)]), _u2b(xs[(b, m)]), mm], axis=0)

        def qk(p):
            sc = _dot_nt(pair(p, 0), pair(p, 1))
            sc = jnp.where(allowed, sc * scale, fill)
            e = jnp.exp(sc - jnp.max(sc, axis=1, keepdims=True))
            l = jnp.sum(e, axis=1, keepdims=True)
            r = pl.reciprocal(l, approx=True)
            r = r * (2.0 - l * r)
            probs[p] = (e * r).astype(BF)

        def pv(p):
            op = _b2u(_dot(probs[p], pair(p, 2)).astype(BF))
            om = op[32:40]
            for i, h in enumerate((2 * p, 2 * p + 1)):
                oring[h, pl.ds(o_st, SEG // 2), :] = op[16 * i:16 * i + 16]
                omh = om if i == 1 else pltpu.roll(om, 4, axis=0)
                a0 = oring[h, pl.ds(o_ld, 8), :]
                a1 = jnp.where(low_half, oring[h, pl.ds(o_ld + 8, 8), :], omh)
                parts[h] = _u2b(jnp.concatenate([a0, a1], axis=0))

        def after(t):
            for lag, fn in ((LAG_QK, qk), (LAG_PV, pv)):
                if (t - 1 - lag) % 2 == 0 and 0 <= (t - 1 - lag) // 2 < NPAIR:
                    fn((t - 1 - lag) // 2)

        for t in range(H):
            proj(t)
            after(t)
        t = H
        lhs_a = jnp.concatenate([parts[j] for j in range(H_SPLIT)], axis=1)
        acc = []
        for n in range(N_PART):
            acc.append(_dot(lhs_a, _u2b(wo_s[n, pl.ds(0, H_SPLIT * 64), :])))
            after(t)
            t += 1
        while t - 1 - LAG_PV <= 2 * (NPAIR - 1):
            after(t)
            t += 1
        lhs_b = jnp.concatenate([parts[j] for j in range(H_SPLIT, H)], axis=1)
        lhs_o = jnp.concatenate([lhs_a, lhs_b], axis=1)
        new_mem = [None] * KT

        def finish(n, y):
            yp = _b2u(y.astype(BF))
            abuf[n, pl.ds(a_st, XS // 2), :] = yp[0:XS // 2]
            new_mem[n] = yp[8:16]

        for n in range(N_PART, KT):
            finish(n, _dot(lhs_o, _u2b(wo_s[n])))
            if n == N_PART:
                for n2 in range(N_PART):
                    tail = _u2b(wo_s[n2, pl.ds(H_SPLIT * 64, (H - H_SPLIT) * 64), :])
                    finish(n2, _dot(lhs_b, tail) + acc[n2])
        return new_mem

    def body(i, mem):
        mem = list(mem)
        for u in range(UNROLL):
            mem = one_step(i * UNROLL + u, mem)
        return tuple(mem)

    small_copies[0].wait()
    for n in range(KT):
        wo_copy(n).wait()
    m0 = mem0_s[...].astype(F32)
    m0p = _b2u(jnp.concatenate([m0, m0], axis=0).astype(BF))
    lax.fori_loop(0, NSEG // UNROLL, body,
                  tuple(m0p[:, 128 * k:128 * (k + 1)] for k in range(KT)))

    early = S - PRE

    def combine(r0, nrows, n, a):
        h0 = r0 // 2 if isinstance(r0, int) else pl.multiple_of(r0 // 2, 8)
        xf = x_s[pl.ds(r0, nrows), pl.ds(128 * n, 128)].astype(F32)
        b = _u2b(xn_t[n, pl.ds(h0, nrows // 2), :]).astype(F32)
        out_s[pl.ds(r0, nrows), pl.ds(128 * n, 128)] = (_rbf(xf + a) + b).astype(BF)

    def combine_early(r0, nrows):
        h0 = r0 // 2 if isinstance(r0, int) else pl.multiple_of(r0 // 2, 8)
        for n in range(KT):
            combine(r0, nrows, n, _u2b(abuf[n, pl.ds(h0, nrows // 2), :]).astype(F32))

    for c in ffn_copies:
        c.wait()
    for e0 in range(0, early, 64):
        combine_early(e0, 64)

    r = _rbf(r_s[...])
    tok = (lax.broadcasted_iota(jnp.int32, (16, 128), 0) * 128
           + lax.broadcasted_iota(jnp.int32, (16, 128), 1))
    top1 = jnp.max(r)
    idx1 = jnp.min(jnp.where(r == top1, tok, S - 1))
    r2 = jnp.where(tok == idx1, -jnp.inf, r)
    top2 = jnp.max(r2)
    idx2 = jnp.min(jnp.where((r2 == top2) & (tok != idx1), tok, S - 1))

    def load_row(t):
        w = jnp.concatenate([xn_t[k, pl.ds(t // 2, 1), :] for k in range(KT)], axis=1)
        bits = jnp.where(t % 2 == 0, w << 16, w & jnp.uint32(0xFFFF0000))
        return pltpu.bitcast(bits, F32), w

    sel_row = lax.broadcasted_iota(jnp.int32, (16, D), 0)
    xs1, _ = load_row(idx1)
    xs2, _ = load_row(idx2)
    x_sel = jnp.where(sel_row == 0, xs1, jnp.where(sel_row == 1, xs2, 0.0)).astype(BF)
    hid = []
    for j in range(FT):
        g = _rbf(_dot(x_sel, _u2b(wg_s[j])))
        u = _rbf(_dot(x_sel, _u2b(wu_s[j])))
        hid.append((_rbf(g * _rbf(jax.nn.sigmoid(g))) * u).astype(BF))
    hid = jnp.concatenate(hid, axis=1)
    y = jnp.concatenate([_rbf(_dot(hid, _u2b(wd_s[n]))) for n in range(KT)], axis=1)
    gate = jnp.where(lax.broadcasted_iota(jnp.int32, (16, 1), 0) == 0, top1, top2)
    y = _rbf(y * _rbf(jax.nn.sigmoid(gate)))

    def patch_row(t, yrow):
        xr, w = load_row(t)
        bits = pltpu.bitcast(_rbf(xr + yrow), U32)
        w = jnp.where(t % 2 == 0,
                      (w & jnp.uint32(0xFFFF0000)) | (bits >> 16),
                      (w & jnp.uint32(0xFFFF)) | bits)
        for k in range(KT):
            xn_t[k, pl.ds(t // 2, 1), :] = w[:, 128 * k:128 * (k + 1)]

    patch_row(idx1, y[0:1])
    patch_row(idx2, y[1:2])
    for t in (idx1, idx2):
        combine_early(pl.multiple_of(jnp.minimum((t // 16) * 16, early - 16), 16), 16)

    def out_copy(r0, nrows, j):
        return pltpu.make_async_copy(out_s.at[pl.ds(r0, nrows), :], out_hbm.at[pl.ds(r0, nrows), :],
                                     sem_out.at[j])

    out_copy(0, early, 4).start()

    def epi_body(c, carry):
        r0 = pl.multiple_of(early + 128 * c, 128)
        p0 = pl.multiple_of((r0 % RING) // 2, 32)
        p1 = pl.multiple_of(((r0 + 64) % RING) // 2, 32)
        lhs = jnp.concatenate(
            [_u2b(jnp.concatenate([oring[h, pl.ds(p0, 32), :], oring[h, pl.ds(p1, 32), :]], axis=0))
             for h in range(H)], axis=1)
        for n in range(KT):
            combine(r0, 128, n, _rbf(_dot(lhs, _u2b(wo_s[n]))))
        out_copy(r0, 128, c).start()
        return carry

    lax.fori_loop(0, PRE // 128, epi_body, 0)
    out_copy(0, early, 4).wait()
    for c in range(PRE // 128):
        out_copy(early + 128 * c, 128, c).wait()


@jax.jit
def pallas_parallel_sum__memory_aug_recurrent_mem_tr__moe_arch_mod__prompt_kernel(
    A_x: jax.Array,
    A_mem0: jax.Array,
    A_Wq: jax.Array,
    A_Wk: jax.Array,
    A_Wv: jax.Array,
    A_Wo: jax.Array,
    A_seg_len: jax.Array,
    B_x: jax.Array,
    B_w_r: jax.Array,
    B_w_gate: jax.Array,
    B_w_up: jax.Array,
    B_w_down: jax.Array,
):
    del A_seg_len, B_x
    assert A_x.shape == (1, S, D) and A_mem0.shape == (1, MEM, D)
    assert A_Wq.shape == (D, H, DH) and A_Wo.shape == (H, DH, D)
    assert B_w_gate.shape == (D, FF) and B_w_down.shape == (FF, D)
    any_spec = pl.BlockSpec(memory_space=pl.ANY)
    out = pl.pallas_call(
        _kernel,
        out_shape=jax.ShapeDtypeStruct((S, D), BF),
        in_specs=[any_spec] * 10,
        out_specs=any_spec,
        scratch_shapes=[
            pltpu.VMEM((S, D), BF),
            pltpu.VMEM((KT, S // 2 + 8, 128), U32),
            pltpu.VMEM((KT, PRE // 2, 128), U32),
            pltpu.VMEM((3 * H, D // 2, 128), U32),
            pltpu.VMEM((2, D // 2, 128), U32),
            pltpu.VMEM((2, D // 2, 128), U32),
            pltpu.VMEM((KT, H * DH // 2, 128), U32),
            pltpu.VMEM((3 * H, RING32, 128), U32),
            pltpu.VMEM((H, RING32 + 8, 128), U32),
            pltpu.VMEM((KT, (S - PRE) // 2, 128), U32),
            pltpu.VMEM((S, D), BF),
            pltpu.VMEM((NCH, D // 2, 8, 128), U32),
            pltpu.VMEM((FT, D // 2, 128), U32),
            pltpu.VMEM((FT, D // 2, 128), U32),
            pltpu.VMEM((KT, FF // 2, 128), U32),
            pltpu.VMEM((MEM, D), BF),
            pltpu.VMEM((D,), BF),
            pltpu.VMEM((16, 128), F32),
            pltpu.SemaphoreType.DMA((1 + NCH,)),
            pltpu.SemaphoreType.DMA((NCH,)),
            pltpu.SemaphoreType.DMA(()),
            pltpu.SemaphoreType.DMA((2,)),
            pltpu.SemaphoreType.DMA(()),
            pltpu.SemaphoreType.DMA((5,)),
        ],
        compiler_params=pltpu.CompilerParams(vmem_limit_bytes=120 * 1024 * 1024),
    )(A_x.reshape(S, D), A_mem0.reshape(MEM, D), A_Wq.reshape(D // 2, 2, H, DH), A_Wk.reshape(D // 2, 2, H, DH),
      A_Wv.reshape(D // 2, 2, H, DH), A_Wo.reshape(H * DH, D),
      B_w_r, B_w_gate, B_w_up, B_w_down)
    return out.reshape(1, S, D)
```

```python
import jax
import jax.numpy as jnp
from jax import lax
import jax.experimental.pallas as pl
import jax.experimental.pallas.tpu as pltpu

BF = jnp.bfloat16
U32 = jnp.uint32
F32 = jnp.float32

S = 2048
D = 1024
H = 32
DH = 128
MEM = 8
SEG = 32
NSEG = S // SEG
FF = 3584
KT = D // 128
FT = FF // 128
XS = 24
PRE = S - NSEG * XS
RING = 576
RING32 = RING // 2
NPAIR = H // 2
NCH = 12
SEM_SMALL, SEM_X, SEM_W = 0, 2, 3 + NCH
SEM_WO, SEM_FFN, SEM_OUT = 3 + 2 * NCH, 4 + 2 * NCH, 5 + 2 * NCH
NSEM = SEM_OUT + 5

LAG_QK = 1
LAG_PV = 4
N_PART = 4
H_SPLIT = 26
UNROLL = 2


def _b2u(x):
    return pltpu.bitcast(x, U32)


def _u2b(x):
    return pltpu.bitcast(x, BF)


def _dot(a, b):
    return jnp.dot(a, b, preferred_element_type=F32)


def _dot_nt(a, b):
    return lax.dot_general(a, b, (((1,), (1,)), ((), ())), preferred_element_type=F32)


def _after(w, dep, zero):
    if dep is None:
        return w
    return jnp.concatenate([w[0:8] | (dep & zero), w[8:]], axis=0)


def _rbf(x):
    return x.astype(BF).astype(F32)


def _kernel(x_hbm, mem0_hbm, wq_hbm, wk_hbm, wv_hbm, wo_hbm, wr_hbm, wg_hbm, wu_hbm, wd_hbm,
            out_hbm,
            x_s, xn_t, xn_pre, wqkv, wo_s, ring, oring, abuf, out_s, raw,
            wg_s, wu_s, wd_s, mem0_s, wr_s, r_s, zero_s,
            sems):
    w32 = [w.bitcast(U32) for w in (wq_hbm, wk_hbm, wv_hbm)]
    wo32 = wo_hbm.bitcast(U32)
    wg32 = wg_hbm.bitcast(U32)
    wu32 = wu_hbm.bitcast(U32)
    wd32 = wd_hbm.bitcast(U32)

    x_first = pltpu.make_async_copy(x_hbm.at[pl.ds(0, PRE), :], x_s.at[pl.ds(0, PRE), :], sems.at[SEM_X])

    def x_piece(c):
        r0 = PRE + 128 * c if isinstance(c, int) else pl.multiple_of(PRE + 128 * c, 128)
        return pltpu.make_async_copy(x_hbm.at[pl.ds(r0, 128), :], x_s.at[pl.ds(r0, 128), :],
                                     sems.at[SEM_X + 1 + c])

    def w_copies(m, c):
        g4 = 4 * (c % 4) if isinstance(c, int) else 0
        return [pltpu.make_async_copy(w32[m].at[:, par, pl.ds(g4, 4), :],
                                      raw.at[c, :, pl.ds(4 * par, 4), :], sems.at[SEM_W + c])
                for par in range(2)]

    def w_wait(c):
        for cp in w_copies(0, c):
            cp.wait()

    def wo_copy(n):
        return pltpu.make_async_copy(wo32.at[:, pl.ds(128 * n, 128)], wo_s.at[n], sems.at[SEM_WO])

    small_copies = [pltpu.make_async_copy(mem0_hbm, mem0_s, sems.at[SEM_SMALL]),
                    pltpu.make_async_copy(wr_hbm, wr_s, sems.at[SEM_SMALL + 1])]
    ffn_copies = (
        [pltpu.make_async_copy(wg32.at[:, pl.ds(128 * j, 128)], wg_s.at[j], sems.at[SEM_FFN]) for j in range(FT)]
        + [pltpu.make_async_copy(wu32.at[:, pl.ds(128 * j, 128)], wu_s.at[j], sems.at[SEM_FFN]) for j in range(FT)]
        + [pltpu.make_async_copy(wd32.at[:, pl.ds(128 * n, 128)], wd_s.at[n], sems.at[SEM_FFN]) for n in range(KT)])

    zero_s[0] = 0
    x_first.start()
    for c in small_copies:
        c.start()
    for c in range(NCH):
        for cp in w_copies(c // 4, c):
            cp.start()
        x_piece(c).start()
    for n in range(KT):
        wo_copy(n).start()
    eps_bf = 1.0013580322265625e-05

    def layernorm16(rq, dst_pre):
        rq = pl.multiple_of(rq, 16)
        xf = x_s[pl.ds(rq, 16), :].astype(F32)
        mean = jnp.sum(xf, axis=1, keepdims=True) * (1.0 / D)
        cen = xf - mean
        var = jnp.sum(cen * cen, axis=1, keepdims=True) * (1.0 / D)
        sd = _rbf(jnp.sqrt(_rbf(_rbf(var) + eps_bf)))
        xp = _b2u((_rbf(xf - _rbf(mean)) * (1.0 / sd)).astype(BF))
        hq = pl.multiple_of(rq // 2, 8)
        for k in range(KT):
            xn_t[k, pl.ds(hq, 8), :] = xp[:, 128 * k:128 * (k + 1)]
            if dst_pre:
                xn_pre[k, pl.ds(hq, 8), :] = xp[:, 128 * k:128 * (k + 1)]

    def router_rows(blk, wr16):
        h0 = pl.multiple_of(64 * blk, 64)
        xb = jnp.concatenate([_u2b(xn_t[k, pl.ds(h0, 64), :]) for k in range(KT)], axis=1)
        r_s[pl.ds(blk, 1), :] = _dot_nt(wr16, xb)[0:1, :]

    zero = jnp.full((8, 128), zero_s[0], jnp.int32).astype(U32)
    x_first.wait()
    for c in small_copies:
        c.wait()
    wr16 = jnp.broadcast_to(wr_s[...].astype(F32).reshape(1, D), (16, D)).astype(BF)

    def ln_body(c, carry):
        for q in range(8):
            layernorm16(128 * c + 16 * q, True)
        return carry

    lax.fori_loop(0, PRE // 128, ln_body, 0)
    for c in range(PRE // 128):
        router_rows(c, wr16)

    raw2 = raw.reshape(NCH * 4096, 128)

    def relayout(c, j, k):
        view = raw2.at[pl.ds(pl.multiple_of(c * 4096, 4096), 4096), :]
        a = view[pl.ds(512 * k + j, 64, stride=8), :]
        b = view[pl.ds(512 * k + 4 + j, 64, stride=8), :]
        rows = pl.ds(64 * k, 64)
        wqkv[8 * c + 2 * j, rows, :] = (a & jnp.uint32(0xFFFF)) | (b << 16)
        wqkv[8 * c + 2 * j + 1, rows, :] = (a >> 16) | (b & jnp.uint32(0xFFFF0000))

    def pre_dot(c, j, k, dep=None):
        i, q = k // 4, k % 4
        lhs = jnp.concatenate([_u2b(xn_pre[kk, pl.ds(64 * q, 64), :]) for kk in range(KT)], axis=1)
        y = _dot(lhs, _u2b(_after(wqkv[8 * c + 2 * j + i], dep, zero)))
        ring[8 * c + 2 * j + i, pl.ds(32 + 64 * q, 64), :] = _b2u(y.astype(BF))

    w_wait(0)
    for k in range(8):
        relayout(0, 0, k)

    x_piece(0).wait()

    def pre_body(c, carry):
        r0 = PRE + 128 * c
        deps = {}
        for t in range(24):
            j, k = t // 8, t % 8
            pre_dot(c, j, k, deps.get(t))
            relayout(c, j + 1, k)
            if t % 3 == 0 and t // 3 < 7:
                for q in ((0, 1) if t == 0 else (t // 3 + 1,)):
                    layernorm16(r0 + 16 * q, False)
                    deps[t + 4] = xn_t[KT - 1, pl.ds(pl.multiple_of(r0 // 2 + 8 * q, 8), 8), :]

        @pl.when(c + 1 < NCH)
        def _():
            w_wait(c + 1)
            x_piece(c + 1).wait()

        cn = jnp.minimum(c + 1, NCH - 1)
        for k in range(8):
            pre_dot(c, 3, k)
            relayout(cn, 0, k)
            if k == 0:
                router_rows(c + PRE // 128, wr16)
        return carry

    lax.fori_loop(0, NCH, pre_body, 0)
    for c in ffn_copies:
        c.start()

    row = lax.broadcasted_iota(jnp.int32, (80, 80), 0)
    col = lax.broadcasted_iota(jnp.int32, (80, 80), 1)
    same_head = (jnp.where(row < 64, row >> 5, (row - 64) >> 3)
                 == jnp.where(col < 64, col >> 5, (col - 64) >> 3))
    allowed = same_head & ((col >= 64) | (row >= 64) | (col <= row))
    fill = jnp.where(same_head, -1e9, -jnp.inf).astype(F32)
    low_half = lax.broadcasted_iota(jnp.int32, (8, 128), 0) < 4
    scale = DH ** -0.5

    def one_step(s, mem):
        x_ld = pl.multiple_of(PRE // 2 + s * (XS // 2), 4)
        qkv_st = pl.multiple_of((s * (XS // 2)) % RING32, 4)
        qkv_ld = pl.multiple_of((s * (SEG // 2) + 32) % RING32, 16)
        o_st = pl.multiple_of((s * (SEG // 2)) % RING32, 16)
        o_ld = qkv_st
        a_st = pl.multiple_of(s * (XS // 2), 4)

        lk = []
        for k in range(KT):
            l0 = xn_t[k, pl.ds(x_ld, 8), :]
            l1 = jnp.where(low_half, xn_t[k, pl.ds(x_ld + 8, 8), :], mem[k])
            lk.append(_u2b(jnp.concatenate([l0, l1], axis=0)))
        lhs = jnp.concatenate(lk, axis=1)

        ymem = {}
        xs = {}
        probs = {}
        parts = {}

        def proj(h):
            for m in range(3):
                y = _dot(lhs, _u2b(wqkv[m * H + h]))
                ring[m * H + h, pl.ds(qkv_st, XS // 2), :] = _b2u(y.astype(BF))[0:XS // 2]
                ymem[(h, m)] = y[XS:XS + MEM]
                xs[(h, m)] = ring[m * H + h, pl.ds(qkv_ld, SEG // 2), :]

        def pair(p, m):
            a, b = 2 * p, 2 * p + 1
            mm = jnp.concatenate([ymem[(a, m)], ymem[(b, m)]], axis=0).astype(BF)
            return jnp.concatenate([_u2b(xs[(a, m)]), _u2b(xs[(b, m)]), mm], axis=0)

        def qk(p):
            sc = _dot_nt(pair(p, 0), pair(p, 1))
            sc = jnp.where(allowed, sc * scale, fill)
            e = jnp.exp(sc - jnp.max(sc, axis=1, keepdims=True))
            l = jnp.sum(e, axis=1, keepdims=True)
            r = pl.reciprocal(l, approx=True)
            r = r * (2.0 - l * r)
            probs[p] = (e * r).astype(BF)

        def pv(p):
            op = _b2u(_dot(probs[p], pair(p, 2)).astype(BF))
            om = op[32:40]
            for i, h in enumerate((2 * p, 2 * p + 1)):
                oring[h, pl.ds(o_st, SEG // 2), :] = op[16 * i:16 * i + 16]
                omh = om if i == 1 else pltpu.roll(om, 4, axis=0)
                a0 = oring[h, pl.ds(o_ld, 8), :]
                a1 = jnp.where(low_half, oring[h, pl.ds(o_ld + 8, 8), :], omh)
                parts[h] = _u2b(jnp.concatenate([a0, a1], axis=0))

        def after(t):
            for lag, fn in ((LAG_QK, qk), (LAG_PV, pv)):
                if (t - 1 - lag) % 2 == 0 and 0 <= (t - 1 - lag) // 2 < NPAIR:
                    fn((t - 1 - lag) // 2)

        for t in range(H):
            proj(t)
            after(t)
        t = H
        lhs_a = jnp.concatenate([parts[j] for j in range(H_SPLIT)], axis=1)
        acc = []
        for n in range(N_PART):
            acc.append(_dot(lhs_a, _u2b(wo_s[n, pl.ds(0, H_SPLIT * 64), :])))
            after(t)
            t += 1
        while t - 1 - LAG_PV <= 2 * (NPAIR - 1):
            after(t)
            t += 1
        lhs_b = jnp.concatenate([parts[j] for j in range(H_SPLIT, H)], axis=1)
        lhs_o = jnp.concatenate([lhs_a, lhs_b], axis=1)
        new_mem = [None] * KT

        def finish(n, y):
            yp = _b2u(y.astype(BF))
            abuf[n, pl.ds(a_st, XS // 2), :] = yp[0:XS // 2]
            new_mem[n] = yp[8:16]

        for n in range(N_PART, KT):
            finish(n, _dot(lhs_o, _u2b(wo_s[n])))
            if n == N_PART:
                for n2 in range(N_PART):
                    tail = _u2b(wo_s[n2, pl.ds(H_SPLIT * 64, (H - H_SPLIT) * 64), :])
                    finish(n2, _dot(lhs_b, tail) + acc[n2])
        return new_mem

    def body(i, mem):
        mem = list(mem)
        for u in range(UNROLL):
            mem = one_step(i * UNROLL + u, mem)
        return tuple(mem)

    for n in range(KT):
        wo_copy(n).wait()
    m0 = mem0_s[...].astype(F32)
    m0p = _b2u(jnp.concatenate([m0, m0], axis=0).astype(BF))
    lax.fori_loop(0, NSEG // UNROLL, body,
                  tuple(m0p[:, 128 * k:128 * (k + 1)] for k in range(KT)))

    early = S - PRE

    def combine(r0, nrows, n, a):
        h0 = r0 // 2 if isinstance(r0, int) else pl.multiple_of(r0 // 2, 8)
        xf = x_s[pl.ds(r0, nrows), pl.ds(128 * n, 128)].astype(F32)
        b = _u2b(xn_t[n, pl.ds(h0, nrows // 2), :]).astype(F32)
        out_s[pl.ds(r0, nrows), pl.ds(128 * n, 128)] = (_rbf(xf + a) + b).astype(BF)

    def combine_early(r0, nrows):
        h0 = r0 // 2 if isinstance(r0, int) else pl.multiple_of(r0 // 2, 8)
        for n in range(KT):
            combine(r0, nrows, n, _u2b(abuf[n, pl.ds(h0, nrows // 2), :]).astype(F32))

    for c in ffn_copies:
        c.wait()
    zrow = pl.multiple_of(zero_s[0], 16)

    def paced_combine(piece):
        if piece >= early // 64:
            return None
        combine_early(64 * piece, 64)
        return _b2u(out_s[pl.ds(zrow, 16), pl.ds(0, 128)])

    for piece in range(4):
        dep = paced_combine(piece)

    r = _rbf(r_s[...])
    tok = (lax.broadcasted_iota(jnp.int32, (16, 128), 0) * 128
           + lax.broadcasted_iota(jnp.int32, (16, 128), 1))
    top1 = jnp.max(r)
    idx1 = jnp.min(jnp.where(r == top1, tok, S - 1))
    r2 = jnp.where(tok == idx1, -jnp.inf, r)
    top2 = jnp.max(r2)
    idx2 = jnp.min(jnp.where((r2 == top2) & (tok != idx1), tok, S - 1))

    def load_row(t):
        w = jnp.concatenate([xn_t[k, pl.ds(t // 2, 1), :] for k in range(KT)], axis=1)
        bits = jnp.where(t % 2 == 0, w << 16, w & jnp.uint32(0xFFFF0000))
        return pltpu.bitcast(bits, F32), w

    sel_row = lax.broadcasted_iota(jnp.int32, (16, D), 0)
    xs1, _ = load_row(idx1)
    xs2, _ = load_row(idx2)
    x_sel = jnp.where(sel_row == 0, xs1, jnp.where(sel_row == 1, xs2, 0.0)).astype(BF)
    hid = []
    for j in range(FT):
        g = _rbf(_dot(x_sel, _u2b(_after(wg_s[j], dep, zero))))
        dep = paced_combine(4 + j)
        u = _rbf(_dot(x_sel, _u2b(wu_s[j])))
        hid.append((_rbf(g * _rbf(jax.nn.sigmoid(g))) * u).astype(BF))
    hid = jnp.concatenate(hid, axis=1)
    y = jnp.concatenate([_rbf(_dot(hid, _u2b(wd_s[n]))) for n in range(KT)], axis=1)
    gate = jnp.where(lax.broadcasted_iota(jnp.int32, (16, 1), 0) == 0, top1, top2)
    y = _rbf(y * _rbf(jax.nn.sigmoid(gate)))

    def patch_row(t, yrow):
        xr, w = load_row(t)
        bits = pltpu.bitcast(_rbf(xr + yrow), U32)
        w = jnp.where(t % 2 == 0,
                      (w & jnp.uint32(0xFFFF0000)) | (bits >> 16),
                      (w & jnp.uint32(0xFFFF)) | bits)
        for k in range(KT):
            xn_t[k, pl.ds(t // 2, 1), :] = w[:, 128 * k:128 * (k + 1)]

    patch_row(idx1, y[0:1])
    patch_row(idx2, y[1:2])
    for t in (idx1, idx2):
        combine_early(pl.multiple_of(jnp.minimum((t // 16) * 16, early - 16), 16), 16)

    def out_copy(r0, nrows, j):
        return pltpu.make_async_copy(out_s.at[pl.ds(r0, nrows), :], out_hbm.at[pl.ds(r0, nrows), :],
                                     sems.at[SEM_OUT + j])

    out_copy(0, early, 4).start()

    def epi_body(c, carry):
        r0 = pl.multiple_of(early + 128 * c, 128)
        p0 = pl.multiple_of((r0 % RING) // 2, 32)
        p1 = pl.multiple_of(((r0 + 64) % RING) // 2, 32)
        lhs = jnp.concatenate(
            [_u2b(jnp.concatenate([oring[h, pl.ds(p0, 32), :], oring[h, pl.ds(p1, 32), :]], axis=0))
             for h in range(H)], axis=1)
        for n in range(KT):
            combine(r0, 128, n, _rbf(_dot(lhs, _u2b(wo_s[n]))))
        out_copy(r0, 128, c).start()
        return carry

    lax.fori_loop(0, PRE // 128, epi_body, 0)
    out_copy(0, early, 4).wait()
    for c in range(PRE // 128):
        out_copy(early + 128 * c, 128, c).wait()


@jax.jit
def pallas_parallel_sum__memory_aug_recurrent_mem_tr__moe_arch_mod__prompt_kernel(
    A_x: jax.Array,
    A_mem0: jax.Array,
    A_Wq: jax.Array,
    A_Wk: jax.Array,
    A_Wv: jax.Array,
    A_Wo: jax.Array,
    A_seg_len: jax.Array,
    B_x: jax.Array,
    B_w_r: jax.Array,
    B_w_gate: jax.Array,
    B_w_up: jax.Array,
    B_w_down: jax.Array,
):
    del A_seg_len, B_x
    assert A_x.shape == (1, S, D) and A_mem0.shape == (1, MEM, D)
    assert A_Wq.shape == (D, H, DH) and A_Wo.shape == (H, DH, D)
    assert B_w_gate.shape == (D, FF) and B_w_down.shape == (FF, D)
    any_spec = pl.BlockSpec(memory_space=pl.ANY)
    out = pl.pallas_call(
        _kernel,
        out_shape=jax.ShapeDtypeStruct((S, D), BF),
        in_specs=[any_spec] * 10,
        out_specs=any_spec,
        scratch_shapes=[
            pltpu.VMEM((S, D), BF),
            pltpu.VMEM((KT, S // 2 + 8, 128), U32),
            pltpu.VMEM((KT, PRE // 2, 128), U32),
            pltpu.VMEM((3 * H, D // 2, 128), U32),
            pltpu.VMEM((KT, H * DH // 2, 128), U32),
            pltpu.VMEM((3 * H, RING32, 128), U32),
            pltpu.VMEM((H, RING32 + 8, 128), U32),
            pltpu.VMEM((KT, (S - PRE) // 2, 128), U32),
            pltpu.VMEM((S, D), BF),
            pltpu.VMEM((NCH, D // 2, 8, 128), U32),
            pltpu.VMEM((FT, D // 2, 128), U32),
            pltpu.VMEM((FT, D // 2, 128), U32),
            pltpu.VMEM((KT, FF // 2, 128), U32),
            pltpu.VMEM((MEM, D), BF),
            pltpu.VMEM((D,), BF),
            pltpu.VMEM((16, 128), F32),
            pltpu.SMEM((1,), jnp.int32),
            pltpu.SemaphoreType.DMA((NSEM,)),
        ],
        compiler_params=pltpu.CompilerParams(vmem_limit_bytes=120 * 1024 * 1024),
    )(A_x.reshape(S, D), A_mem0.reshape(MEM, D), A_Wq.reshape(D // 2, 2, H, DH), A_Wk.reshape(D // 2, 2, H, DH),
      A_Wv.reshape(D // 2, 2, H, DH), A_Wo.reshape(H * DH, D),
      B_w_r, B_w_gate, B_w_up, B_w_down)
    return out.reshape(1, S, D)
```

```python
import jax
import jax.numpy as jnp
from jax import lax
import jax.experimental.pallas as pl
import jax.experimental.pallas.tpu as pltpu

BF = jnp.bfloat16
U32 = jnp.uint32
F32 = jnp.float32

S = 2048
D = 1024
H = 32
DH = 128
MEM = 8
SEG = 32
NSEG = S // SEG
FF = 3584
KT = D // 128
FT = FF // 128
XS = 24
PRE = S - NSEG * XS
RING = 576
RING32 = RING // 2
NPAIR = H // 2
NCH = 12
SEM_SMALL, SEM_X, SEM_W = 0, 2, 3 + NCH
SEM_WO, SEM_FFN, SEM_OUT = 3 + 2 * NCH, 4 + 2 * NCH, 5 + 2 * NCH
NSEM = SEM_OUT + 9

LAG_QK = 1
LAG_PV = 4
N_PART = 4
H_SPLIT = 26
REL_SCHED = {0: [(0, 0), (0, 1)], 1: [(0, 2), (0, 3)], 2: [(0, 4)], 3: [(0, 5)], 4: [(0, 6)], 5: [(0, 7)]}
REL_SCHED.update({6 + k: [(1, k)] for k in range(8)})
UNROLL = 4


def _b2u(x):
    return pltpu.bitcast(x, U32)


def _u2b(x):
    return pltpu.bitcast(x, BF)


def _dot(a, b):
    return jnp.dot(a, b, preferred_element_type=F32)


def _dot_nt(a, b):
    return lax.dot_general(a, b, (((1,), (1,)), ((), ())), preferred_element_type=F32)


def _after(w, dep, zero):
    if not dep:
        return w
    d = dep[0]
    for e in dep[1:]:
        d = d | e
    return jnp.concatenate([w[0:8] | (d & zero), w[8:]], axis=0)


def _rbf(x):
    return x.astype(BF).astype(F32)


def _kernel(x_hbm, mem0_hbm, wq_hbm, wk_hbm, wv_hbm, wo_hbm, wr_hbm, wg_hbm, wu_hbm, wd_hbm,
            out_hbm,
            x_s, xn_t, xn_pre, hbuf, wqkv, wo_s, ring, oring, abuf, out_s, raw,
            wg_s, wu_s, wd_s, mem0_s, wr_s, r_s, xsel_s, gate_s, zero_s, idx_s,
            sems):
    w32 = [w.bitcast(U32) for w in (wq_hbm, wk_hbm, wv_hbm)]
    wo32 = wo_hbm.bitcast(U32)
    wg32 = wg_hbm.bitcast(U32)
    wu32 = wu_hbm.bitcast(U32)
    wd32 = wd_hbm.bitcast(U32)

    x_first = pltpu.make_async_copy(x_hbm.at[pl.ds(0, PRE), :], x_s.at[pl.ds(0, PRE), :], sems.at[SEM_X])

    def x_piece(c):
        r0 = PRE + 128 * c if isinstance(c, int) else pl.multiple_of(PRE + 128 * c, 128)
        return pltpu.make_async_copy(x_hbm.at[pl.ds(r0, 128), :], x_s.at[pl.ds(r0, 128), :],
                                     sems.at[SEM_X + 1 + c])

    def w_start(c):
        for par in range(2):
            pltpu.make_async_copy(w32[c // 4].at[:, par, pl.ds(4 * (c % 4), 4), :],
                                  raw.at[c, :, pl.ds(4 * par, 4), :], sems.at[SEM_W + c]).start()

    def w_wait(c):
        pltpu.make_async_copy(raw.at[c], raw.at[c], sems.at[SEM_W + c]).wait()

    def wo_copy(n):
        return pltpu.make_async_copy(wo32.at[:, pl.ds(128 * n, 128)], wo_s.at[n], sems.at[SEM_WO])

    small_copies = [pltpu.make_async_copy(mem0_hbm, mem0_s, sems.at[SEM_SMALL]),
                    pltpu.make_async_copy(wr_hbm, wr_s, sems.at[SEM_SMALL + 1])]
    ffn_copies = (
        [pltpu.make_async_copy(wg32.at[:, pl.ds(128 * j, 128)], wg_s.at[j], sems.at[SEM_FFN]) for j in range(FT)]
        + [pltpu.make_async_copy(wu32.at[:, pl.ds(128 * j, 128)], wu_s.at[j], sems.at[SEM_FFN]) for j in range(FT)]
        + [pltpu.make_async_copy(wd32.at[:, pl.ds(128 * n, 128)], wd_s.at[n], sems.at[SEM_FFN]) for n in range(KT)])

    zero_s[0] = 0
    x_first.start()
    for c in small_copies:
        c.start()
    for c in range(NCH):
        w_start(c)
        x_piece(c).start()
    for n in range(KT):
        wo_copy(n).start()
    eps_bf = 1.0013580322265625e-05

    def layernorm16(rq, dst_ref, dst_row):
        rq = pl.multiple_of(rq, 16)
        xf = x_s[pl.ds(rq, 16), :].astype(F32)
        mean = jnp.sum(xf, axis=1, keepdims=True) * (1.0 / D)
        cen = xf - mean
        var = jnp.sum(cen * cen, axis=1, keepdims=True) * (1.0 / D)
        sd = _rbf(jnp.sqrt(_rbf(_rbf(var) + eps_bf)))
        xp = _b2u((_rbf(xf - _rbf(mean)) * (1.0 / sd)).astype(BF))
        hq = pl.multiple_of(rq // 2, 8)
        dst_row = pl.multiple_of(dst_row, 8)
        for k in range(KT):
            xn_t[k, pl.ds(hq, 8), :] = xp[:, 128 * k:128 * (k + 1)]
            dst_ref[k, pl.ds(dst_row, 8), :] = xp[:, 128 * k:128 * (k + 1)]

    zero = jnp.full((8, 128), zero_s[0], jnp.int32).astype(U32)
    r_s[...] = jnp.full(r_s.shape, -jnp.inf, F32)
    x_first.wait()

    def ln_body(c, carry):
        for q in range(4):
            layernorm16(64 * c + 16 * q, xn_pre, 32 * c + 8 * q)
        return carry

    lax.fori_loop(0, PRE // 64, ln_body, 0)

    raw2 = raw.reshape(NCH * 4096, 128)

    def raw_view(p):
        return raw2.at[pl.ds((p // 4) * 4096 + p % 4, 4093), :]

    def relayout(src, dst, j, k):
        a = src[pl.ds(512 * k, 64, stride=8), :]
        b = src[pl.ds(512 * k + 4, 64, stride=8), :]
        rows = pl.ds(64 * k, 64)
        dst[2 * j, rows, :] = (a & jnp.uint32(0xFFFF)) | (b << 16)
        dst[2 * j + 1, rows, :] = (a >> 16) | (b & jnp.uint32(0xFFFF0000))

    def pre_dot(w_view, ring_view, j, k, dep=None):
        i, q = k // 4, k % 4
        lhs = jnp.concatenate([_u2b(xn_pre[kk, pl.ds(64 * q, 64), :]) for kk in range(KT)], axis=1)
        y = _dot(lhs, _u2b(_after(w_view[2 * j + i], dep, zero)))
        ring_view[2 * j + i, pl.ds(32 + 64 * q, 64), :] = _b2u(y.astype(BF))

    for c in small_copies:
        c.wait()
    w_wait(0)
    for k in range(8):
        relayout(raw_view(0), wqkv, 0, k)
    x_piece(0).wait()

    def pre_body(t, carry):
        @pl.when((t % 2 == 1) & (t < 2 * NCH - 1))
        def _():
            w_wait((t + 1) // 2)
            x_piece((t + 1) // 2).wait()

        deps = {}
        w_view = wqkv.at[pl.ds(4 * t, 6)]
        ring_view = ring.at[pl.ds(4 * t, 4)]
        srcs = (raw_view(2 * t + 1), raw_view(jnp.minimum(2 * t + 2, 4 * NCH - 1)))
        for v in range(16):
            j, k = v // 8, v % 8
            pre_dot(w_view, ring_view, j, k, deps.get(v))
            for jr, kr in REL_SCHED.get(v, ()):
                relayout(srcs[jr], w_view, jr + 1, kr)
                deps.setdefault(v + 2, []).append(w_view[2 * jr + 3, pl.ds(64 * kr + 56, 8), :])
            if v % 3 == 0 and v < 12:
                q = 4 * t + v // 3
                hrow = pl.multiple_of(32 * (q // 3) + 8 * (q % 3), 8)
                layernorm16(PRE + 16 * q, hbuf, hrow)
                deps.setdefault(v + 4, []).append(hbuf[KT - 1, pl.ds(hrow, 8), :])
        return carry

    lax.fori_loop(0, 2 * NCH, pre_body, 0)
    for c in ffn_copies:
        c.start()

    row = lax.broadcasted_iota(jnp.int32, (80, 80), 0)
    col = lax.broadcasted_iota(jnp.int32, (80, 80), 1)
    same_head = (jnp.where(row < 64, row >> 5, (row - 64) >> 3)
                 == jnp.where(col < 64, col >> 5, (col - 64) >> 3))
    allowed = same_head & ((col >= 64) | (row >= 64) | (col <= row))
    fill = jnp.where(same_head, -1e9, -jnp.inf).astype(F32)
    low_half = lax.broadcasted_iota(jnp.int32, (8, 128), 0) < 4
    high_half = jnp.logical_not(low_half)
    scale = DH ** -0.5
    wr16 = jnp.broadcast_to(wr_s[...].astype(F32).reshape(1, D), (16, D)).astype(BF)

    def load_row(t):
        w = jnp.concatenate([xn_t[k, pl.ds(t // 2, 1), :] for k in range(KT)], axis=1)
        bits = jnp.where(t % 2 == 0, w << 16, w & jnp.uint32(0xFFFF0000))
        return pltpu.bitcast(bits, F32), w

    def router(blk):
        h0 = pl.multiple_of(64 * blk, 64)
        xb = jnp.concatenate([_u2b(xn_t[k, pl.ds(h0, 64), :]) for k in range(KT)], axis=1)
        r_s[pl.ds(blk, 1), :] = _rbf(_dot_nt(wr16, xb)[0:1, :])
        r = r_s[...]
        tok = (lax.broadcasted_iota(jnp.int32, (16, 128), 0) * 128
               + lax.broadcasted_iota(jnp.int32, (16, 128), 1))
        top1 = jnp.max(r)
        idx1 = jnp.min(jnp.where(r == top1, tok, S - 1))
        r2 = jnp.where(tok == idx1, -jnp.inf, r)
        top2 = jnp.max(r2)
        idx2 = jnp.min(jnp.where((r2 == top2) & (tok != idx1), tok, S - 1))
        idx_s[0] = idx1
        idx_s[1] = idx2
        gate_s[...] = jnp.where(lax.broadcasted_iota(jnp.int32, (16, 128), 0) == 0, top1, top2)
        sel_row = lax.broadcasted_iota(jnp.int32, (16, D), 0)
        xs1, _ = load_row(idx1)
        xs2, _ = load_row(idx2)
        xsel_s[...] = _b2u(jnp.where(sel_row == 0, xs1, jnp.where(sel_row == 1, xs2, 0.0)).astype(BF))

    def one_step(i, u, mem):
        odd = u % 2
        s2 = i * (UNROLL // 2) + u // 2
        h_ld = pl.multiple_of(32 * s2, 32)
        r24 = pl.multiple_of((XS * s2) % RING32, 8)
        a24 = pl.multiple_of(XS * s2, 8)
        qkv_ld = pl.multiple_of((SEG * s2 + 32) % RING32, 32) + 16 * odd
        o_st = pl.multiple_of((SEG * s2) % RING32, 32) + 16 * odd
        m0 = 0 if odd else XS

        def with_mem(ref, idx, base, m):
            lo = ref[idx, pl.ds(base + 8 * odd, 8), :]
            hi = ref[idx, pl.ds(base + 8 + 8 * odd, 8), :]
            if odd:
                lo = jnp.where(low_half, m, lo)
            else:
                hi = jnp.where(low_half, hi, m)
            return _u2b(jnp.concatenate([lo, hi], axis=0))

        def store_tokens(ref, idx, base, yp):
            if odd:
                pltpu.store(ref.at[idx, pl.ds(base + 8, 8), :], yp[0:8], mask=high_half)
                ref[idx, pl.ds(base + 16, 8), :] = yp[8:16]
            else:
                ref[idx, pl.ds(base, 8), :] = yp[0:8]
                pltpu.store(ref.at[idx, pl.ds(base + 8, 8), :], yp[8:16], mask=low_half)

        lhs = jnp.concatenate([with_mem(hbuf, k, h_ld, mem[k]) for k in range(KT)], axis=1)

        ymem = {}
        xs = {}
        probs = {}
        parts = {}

        def proj(h):
            for m in range(3):
                y = _dot(lhs, _u2b(wqkv[m * H + h]))
                store_tokens(ring, m * H + h, r24, _b2u(y.astype(BF)))
                ymem[(h, m)] = y[m0:m0 + MEM]
                xs[(h, m)] = ring[m * H + h, pl.ds(qkv_ld, SEG // 2), :]

        def pair(p, m):
            a, b = 2 * p, 2 * p + 1
            mm = jnp.concatenate([ymem[(a, m)], ymem[(b, m)]], axis=0).astype(BF)
            return jnp.concatenate([_u2b(xs[(a, m)]), _u2b(xs[(b, m)]), mm], axis=0)

        def qk(p):
            sc = _dot_nt(pair(p, 0), pair(p, 1))
            sc = jnp.where(allowed, sc * scale, fill)
            e = jnp.exp(sc - jnp.max(sc, axis=1, keepdims=True))
            l = jnp.sum(e, axis=1, keepdims=True)
            r = pl.reciprocal(l, approx=True)
            r = r * (2.0 - l * r)
            probs[p] = (e * r).astype(BF)

        def pv(p):
            op = _b2u(_dot(probs[p], pair(p, 2)).astype(BF))
            om = op[32:40]
            om_sw = pltpu.roll(om, 4, axis=0)
            for j, h in enumerate((2 * p, 2 * p + 1)):
                oring[h, pl.ds(o_st, SEG // 2), :] = op[16 * j:16 * j + 16]
                parts[h] = with_mem(oring, h, r24, om if j != odd else om_sw)

        def after(t):
            for lag, fn in ((LAG_QK, qk), (LAG_PV, pv)):
                if (t - 1 - lag) % 2 == 0 and 0 <= (t - 1 - lag) // 2 < NPAIR:
                    fn((t - 1 - lag) // 2)

        for t in range(H):
            proj(t)
            after(t)
            if u == 0 and t == 0:
                router(i)
        t = H
        lhs_a = jnp.concatenate([parts[j] for j in range(H_SPLIT)], axis=1)
        acc = []
        for n in range(N_PART):
            acc.append(_dot(lhs_a, _u2b(wo_s[n, pl.ds(0, H_SPLIT * 64), :])))
            after(t)
            t += 1
        while t - 1 - LAG_PV <= 2 * (NPAIR - 1):
            after(t)
            t += 1
        lhs_b = jnp.concatenate([parts[j] for j in range(H_SPLIT, H)], axis=1)
        lhs_o = jnp.concatenate([lhs_a, lhs_b], axis=1)
        new_mem = [None] * KT

        def finish(n, y):
            store_tokens(abuf, n, a24, _b2u(y.astype(BF)))
            ym = y[m0:m0 + MEM]
            new_mem[n] = _b2u(jnp.concatenate([ym, ym], axis=0).astype(BF))

        for n in range(N_PART, KT):
            finish(n, _dot(lhs_o, _u2b(wo_s[n])))
            if n == N_PART:
                for n2 in range(N_PART):
                    tail = _u2b(wo_s[n2, pl.ds(H_SPLIT * 64, (H - H_SPLIT) * 64), :])
                    finish(n2, _dot(lhs_b, tail) + acc[n2])
        return new_mem

    def body(i, mem):
        mem = list(mem)
        for u in range(UNROLL):
            mem = one_step(i, u, mem)
        return tuple(mem)

    for n in range(KT):
        wo_copy(n).wait()
    mi = mem0_s[...].astype(F32)
    mip = _b2u(jnp.concatenate([mi, mi], axis=0).astype(BF))
    lax.fori_loop(0, NSEG // UNROLL, body,
                  tuple(mip[:, 128 * k:128 * (k + 1)] for k in range(KT)))

    early = S - PRE
    zrow = pl.multiple_of(zero_s[0], 16)
    FPER = 9

    def half_rows(r0):
        return r0 // 2 if isinstance(r0, int) else pl.multiple_of(r0 // 2, 8)

    def combine(r0, nrows, n, a):
        xf = x_s[pl.ds(r0, nrows), pl.ds(128 * n, 128)].astype(F32)
        b = _u2b(xn_t[n, pl.ds(half_rows(r0), nrows // 2), :]).astype(F32)
        out_s[pl.ds(r0, nrows), pl.ds(128 * n, 128)] = (_rbf(xf + a) + b).astype(BF)

    def combine_stored(r0, nrows):
        for n in range(KT):
            combine(r0, nrows, n, _u2b(abuf[n, pl.ds(half_rows(r0), nrows // 2), :]).astype(F32))

    def out_copy(r0, nrows, j):
        return pltpu.make_async_copy(out_s.at[pl.ds(r0, nrows), :], out_hbm.at[pl.ds(r0, nrows), :],
                                     sems.at[SEM_OUT + j])

    def ffn_groups(j0, count, y, done):
        x_sel = _u2b(xsel_s[...])
        hid = {}

        def up(w_ref, j, key):
            part = _dot(x_sel[:, 0:512], _u2b(w_ref[j, pl.ds(0, 256), :]))
            yield
            hid[key] = _rbf(_dot(x_sel[:, 512:1024], _u2b(w_ref[j, pl.ds(256, 256), :])) + part)
            yield

        def down(jj):
            g = hid[("g", jj)]
            hb = (_rbf(g * _rbf(jax.nn.sigmoid(g))) * hid[("u", jj)]).astype(BF)
            rows = pl.ds(pl.multiple_of(64 * (j0 + jj), 64), 64)
            for half in range(2):
                w = jnp.concatenate([_u2b(wd_s[4 * half + n, rows, :]) for n in range(4)], axis=1)
                y[half] = _dot(hb, w) + y[half]
                yield

        for jj in range(count + 1):
            if jj < count:
                yield from up(wg_s, j0 + jj, ("g", jj))
                yield from up(wu_s, j0 + jj, ("u", jj))
            elif count == 1:
                yield
                yield
            if jj >= 1:
                yield from down(jj - 1)
        done()

    def epi_chunk(r0, side, pieces, keep):
        p0 = (r0 % RING) // 2
        p1 = ((r0 + 64) % RING) // 2
        if not isinstance(r0, int):
            p0, p1 = pl.multiple_of(p0, 32), pl.multiple_of(p1, 32)
        deps = {}
        for n in range(KT):
            acc = None
            for g in range(8):
                lhs = jnp.concatenate(
                    [_u2b(jnp.concatenate([oring[h, pl.ds(p0, 32), :], oring[h, pl.ds(p1, 32), :]], axis=0))
                     for h in range(4 * g, 4 * g + 4)], axis=1)
                w = _after(wo_s[n, pl.ds(256 * g, 256), :], deps.get(8 * n + g), zero)
                y = _dot(lhs, _u2b(w))
                acc = y if acc is None else y + acc
                next(side, None)
                if pieces is not None and g % 4 == 0 and 8 * n + g < 56:
                    for e in ((0, 1, 2) if n == 0 and g == 0 else (2 * n + g // 4 + 2,)):
                        combine_stored(pieces + 32 * e, 32)
                    deps[8 * n + g + 6] = [_b2u(out_s[pl.ds(zrow, 16), pl.ds(0, 128)])]
            ab = acc.astype(BF)
            if keep:
                abuf[n, pl.ds(half_rows(r0), 64), :] = _b2u(ab)
            combine(r0, 128, n, ab.astype(F32))

    for c in ffn_copies:
        c.wait()

    def epi_body(c, y):
        y = list(y)
        r0 = pl.multiple_of(early + 128 * c, 128)
        e0 = pl.multiple_of(512 * c, 512)
        epi_chunk(r0, ffn_groups(FPER * c, FPER, y, lambda: None), e0, True)
        out_copy(r0, 128, c).start()
        out_copy(e0, 512, 4 + c).start()
        return tuple(y)

    y = list(lax.fori_loop(0, 3, epi_body, (jnp.zeros((16, 512), F32), jnp.zeros((16, 512), F32))))
    idx1 = idx_s[0]
    idx2 = idx_s[1]

    def patch_row(t, yrow):
        xr, w = load_row(t)
        bits = pltpu.bitcast(_rbf(xr + yrow), U32)
        w = jnp.where(t % 2 == 0,
                      (w & jnp.uint32(0xFFFF0000)) | (bits >> 16),
                      (w & jnp.uint32(0xFFFF)) | bits)
        for k in range(KT):
            xn_t[k, pl.ds(t // 2, 1), :] = w[:, 128 * k:128 * (k + 1)]

    def patch():
        gate = _rbf(jax.nn.sigmoid(gate_s[:, 0:1]))
        yy = _rbf(_rbf(jnp.concatenate(y, axis=1)) * gate)
        patch_row(idx1, yy[0:1])
        patch_row(idx2, yy[1:2])

    last = S - 128
    epi_chunk(last, ffn_groups(3 * FPER, 1, y, patch), None, False)
    out_copy(last, 128, 3).start()
    for c in range(3):
        out_copy(early + 128 * c, 128, c).wait()
        out_copy(512 * c, 512, 4 + c).wait()
    blk1 = jnp.minimum(idx1 // 16, last // 16 - 1)
    blk2 = jnp.minimum(idx2 // 16, last // 16 - 1)
    blk2 = jnp.where(blk2 == blk1, jnp.where(blk1 == 0, 1, blk1 - 1), blk2)
    fix = []
    for j, blk in enumerate((blk1, blk2)):
        r0 = pl.multiple_of(blk * 16, 16)
        combine_stored(r0, 16)
        fix.append(out_copy(r0, 16, 7 + j))
    for cp in fix:
        cp.start()
    out_copy(last, 128, 3).wait()
    for cp in fix:
        cp.wait()


@jax.jit
def pallas_parallel_sum__memory_aug_recurrent_mem_tr__moe_arch_mod__prompt_kernel(
    A_x: jax.Array,
    A_mem0: jax.Array,
    A_Wq: jax.Array,
    A_Wk: jax.Array,
    A_Wv: jax.Array,
    A_Wo: jax.Array,
    A_seg_len: jax.Array,
    B_x: jax.Array,
    B_w_r: jax.Array,
    B_w_gate: jax.Array,
    B_w_up: jax.Array,
    B_w_down: jax.Array,
):
    del A_seg_len, B_x
    assert A_x.shape == (1, S, D) and A_mem0.shape == (1, MEM, D)
    assert A_Wq.shape == (D, H, DH) and A_Wo.shape == (H, DH, D)
    assert B_w_gate.shape == (D, FF) and B_w_down.shape == (FF, D)
    any_spec = pl.BlockSpec(memory_space=pl.ANY)
    out = pl.pallas_call(
        _kernel,
        out_shape=jax.ShapeDtypeStruct((S, D), BF),
        in_specs=[any_spec] * 10,
        out_specs=any_spec,
        scratch_shapes=[
            pltpu.VMEM((S, D), BF),
            pltpu.VMEM((KT, S // 2, 128), U32),
            pltpu.VMEM((KT, PRE // 2, 128), U32),
            pltpu.VMEM((KT, 16 * NSEG, 128), U32),
            pltpu.VMEM((3 * H + 2, D // 2, 128), U32),
            pltpu.VMEM((KT, H * DH // 2, 128), U32),
            pltpu.VMEM((3 * H, RING32, 128), U32),
            pltpu.VMEM((H, RING32, 128), U32),
            pltpu.VMEM((KT, S // 2, 128), U32),
            pltpu.VMEM((S, D), BF),
            pltpu.VMEM((NCH, D // 2, 8, 128), U32),
            pltpu.VMEM((FT, D // 2, 128), U32),
            pltpu.VMEM((FT, D // 2, 128), U32),
            pltpu.VMEM((KT, FF // 2, 128), U32),
            pltpu.VMEM((MEM, D), BF),
            pltpu.VMEM((D,), BF),
            pltpu.VMEM((16, 128), F32),
            pltpu.VMEM((8, D), U32),
            pltpu.VMEM((16, 128), F32),
            pltpu.SMEM((1,), jnp.int32),
            pltpu.SMEM((2,), jnp.int32),
            pltpu.SemaphoreType.DMA((NSEM,)),
        ],
        compiler_params=pltpu.CompilerParams(vmem_limit_bytes=126 * 1024 * 1024),
    )(A_x.reshape(S, D), A_mem0.reshape(MEM, D), A_Wq.reshape(D // 2, 2, H, DH), A_Wk.reshape(D // 2, 2, H, DH),
      A_Wv.reshape(D // 2, 2, H, DH), A_Wo.reshape(H * DH, D),
      B_w_r, B_w_gate, B_w_up, B_w_down)
    return out.reshape(1, S, D)
```

```python
import jax
import jax.numpy as jnp
from jax import lax
import jax.experimental.pallas as pl
import jax.experimental.pallas.tpu as pltpu

BF = jnp.bfloat16
U32 = jnp.uint32
F32 = jnp.float32

S = 2048
D = 1024
H = 32
DH = 128
MEM = 8
SEG = 32
NSEG = S // SEG
FF = 3584
KT = D // 128
FT = FF // 128
XS = 24
PRE = S - NSEG * XS
RING = 576
RING32 = RING // 2
NPAIR = H // 2
NCH = 12
SEM_SMALL, SEM_X, SEM_W = 0, 2, 3 + NCH
SEM_WO, SEM_FFN, SEM_OUT = 3 + 2 * NCH, 4 + 2 * NCH, 5 + 2 * NCH
NSEM = SEM_OUT + 9

LAG_QK = 1
LAG_PV = 4
N_PART = 4
H_SPLIT = 26
REL_SCHED = {0: [(0, 0), (0, 1)], 1: [(0, 2), (0, 3)], 2: [(0, 4)], 3: [(0, 5)], 4: [(0, 6)], 5: [(0, 7)]}
REL_SCHED.update({6 + k: [(1, k)] for k in range(8)})
K_SPLIT = 1
LN_LAG = 5
UNROLL = 4


def _b2u(x):
    return pltpu.bitcast(x, U32)


def _u2b(x):
    return pltpu.bitcast(x, BF)


def _dot(a, b):
    return jnp.dot(a, b, preferred_element_type=F32)


def _dot_nt(a, b):
    return lax.dot_general(a, b, (((1,), (1,)), ((), ())), preferred_element_type=F32)


def _after(w, dep, zero):
    if not dep:
        return w
    d = dep[0]
    for e in dep[1:]:
        d = d | e
    return jnp.concatenate([w[0:8] | (d & zero), w[8:]], axis=0)


def _rbf(x):
    return x.astype(BF).astype(F32)


def _kernel(x_hbm, mem0_hbm, wq_hbm, wk_hbm, wv_hbm, wo_hbm, wr_hbm, wg_hbm, wu_hbm, wd_hbm,
            out_hbm,
            x_s, xn_t, xn_pre, hbuf, wqkv, wo_s, ring, oring, abuf, out_s, raw,
            wg_s, wu_s, wd_s, mem0_s, wr_s, wrf_s, r_s, xsel_s, gate_s, zero_s, idx_s,
            sems):
    w32 = [w.bitcast(U32) for w in (wq_hbm, wk_hbm, wv_hbm)]
    wo32 = wo_hbm.bitcast(U32)
    wg32 = wg_hbm.bitcast(U32)
    wu32 = wu_hbm.bitcast(U32)
    wd32 = wd_hbm.bitcast(U32)

    x_first = pltpu.make_async_copy(x_hbm.at[pl.ds(0, PRE), :], x_s.at[pl.ds(0, PRE), :], sems.at[SEM_X])

    def x_piece(c):
        r0 = PRE + 128 * c if isinstance(c, int) else pl.multiple_of(PRE + 128 * c, 128)
        return pltpu.make_async_copy(x_hbm.at[pl.ds(r0, 128), :], x_s.at[pl.ds(r0, 128), :],
                                     sems.at[SEM_X + 1 + c])

    def w_start(c):
        for par in range(2):
            pltpu.make_async_copy(w32[c // 4].at[:, par, pl.ds(4 * (c % 4), 4), :],
                                  raw.at[c, :, pl.ds(4 * par, 4), :], sems.at[SEM_W + c]).start()

    def w_wait(c):
        pltpu.make_async_copy(raw.at[c], raw.at[c], sems.at[SEM_W + c]).wait()

    def wo_copy(n):
        return pltpu.make_async_copy(wo32.at[:, pl.ds(128 * n, 128)], wo_s.at[n], sems.at[SEM_WO])

    small_copies = [pltpu.make_async_copy(mem0_hbm, mem0_s, sems.at[SEM_SMALL]),
                    pltpu.make_async_copy(wr_hbm, wr_s, sems.at[SEM_SMALL + 1])]
    ffn_copies = (
        [pltpu.make_async_copy(wg32.at[:, pl.ds(128 * j, 128)], wg_s.at[j], sems.at[SEM_FFN]) for j in range(FT)]
        + [pltpu.make_async_copy(wu32.at[:, pl.ds(128 * j, 128)], wu_s.at[j], sems.at[SEM_FFN]) for j in range(FT)]
        + [pltpu.make_async_copy(wd32.at[:, pl.ds(128 * n, 128)], wd_s.at[n], sems.at[SEM_FFN]) for n in range(KT)])

    zero_s[0] = 0
    x_first.start()
    for c in small_copies:
        c.start()
    for c in range(NCH):
        w_start(c)
        x_piece(c).start()
    for n in range(KT):
        wo_copy(n).start()
    eps_bf = 1.0013580322265625e-05

    def layernorm16(rq, dst_ref, dst_row, not_before=None):
        rq = pl.multiple_of(rq, 16)
        xf = x_s[pl.ds(rq, 16), :].astype(F32)
        if not_before is not None:
            x0 = _after(pltpu.bitcast(xf[:, 0:128], U32), [not_before], zero)
            xf = jnp.concatenate([pltpu.bitcast(x0, F32), xf[:, 128:]], axis=1)
        mean = jnp.sum(xf, axis=1, keepdims=True) * (1.0 / D)
        cen = xf - mean
        var = jnp.sum(cen * cen, axis=1, keepdims=True) * (1.0 / D)
        sd = _rbf(jnp.sqrt(_rbf(_rbf(var) + eps_bf)))
        xn = (_rbf(xf - _rbf(mean)) * (1.0 / sd)).astype(BF)
        wr = jnp.concatenate([wrf_s[...], wrf_s[...]], axis=0)
        score = _rbf(jnp.sum(xn.astype(F32) * wr, axis=1, keepdims=True))
        r_s[...] = jnp.where(lane16 == rq // 16, score, r_s[...])
        xp = _b2u(xn)
        hq = pl.multiple_of(rq // 2, 8)
        dst_row = pl.multiple_of(dst_row, 8)
        for k in range(KT):
            xn_t[k, pl.ds(hq, 8), :] = xp[:, 128 * k:128 * (k + 1)]
            dst_ref[k, pl.ds(dst_row, 8), :] = xp[:, 128 * k:128 * (k + 1)]

    zero = jnp.full((8, 128), zero_s[0], jnp.int32).astype(U32)
    r_s[...] = jnp.full(r_s.shape, -jnp.inf, F32)
    lane16 = lax.broadcasted_iota(jnp.int32, (16, 128), 1)
    x_first.wait()
    for c in small_copies:
        c.wait()
    wrf_s[...] = jnp.broadcast_to(wr_s[...].astype(F32).reshape(1, D), (8, D))

    def ln_body(c, carry):
        for q in range(8):
            layernorm16(128 * c + 16 * q, xn_pre, 64 * c + 8 * q)
        return carry

    lax.fori_loop(0, PRE // 128, ln_body, 0)

    raw2 = raw.reshape(NCH * 4096, 128)

    def raw_view(p):
        return raw2.at[pl.ds((p // 4) * 4096 + p % 4, 4093), :]

    def relayout(src, dst, j, k):
        a = src[pl.ds(512 * k, 64, stride=8), :]
        b = src[pl.ds(512 * k + 4, 64, stride=8), :]
        rows = pl.ds(64 * k, 64)
        dst[2 * j, rows, :] = (a & jnp.uint32(0xFFFF)) | (b << 16)
        dst[2 * j + 1, rows, :] = (a >> 16) | (b & jnp.uint32(0xFFFF0000))

    def pre_dot(w_view, ring_view, j, k, dep=None):
        i, q = k // 4, k % 4
        lhs = jnp.concatenate([_u2b(xn_pre[kk, pl.ds(64 * q, 64), :]) for kk in range(KT)], axis=1)
        y = _dot(lhs, _u2b(_after(w_view[2 * j + i], dep, zero)))
        yp = _b2u(y.astype(BF))
        ring_view[2 * j + i, pl.ds(32 + 64 * q, 64), :] = yp
        return yp[0:8]

    w_wait(0)
    for k in range(8):
        relayout(raw_view(0), wqkv, 0, k)
    x_piece(0).wait()

    def pre_body(t, carry):
        @pl.when((t % 2 == 1) & (t < 2 * NCH - 1))
        def _():
            w_wait((t + 1) // 2)
            x_piece((t + 1) // 2).wait()

        deps = {}
        w_view = wqkv.at[pl.ds(4 * t, 6)]
        ring_view = ring.at[pl.ds(4 * t, 4)]
        srcs = (raw_view(2 * t + 1), raw_view(jnp.minimum(2 * t + 2, 4 * NCH - 1)))
        for v in range(16):
            j, k = v // 8, v % 8
            done = pre_dot(w_view, ring_view, j, k, deps.get(v))
            for jr, kr in REL_SCHED.get(v, ()):
                relayout(srcs[jr], w_view, jr + 1, kr)
                deps.setdefault(v + 2, []).append(w_view[2 * jr + 3, pl.ds(64 * kr + 56, 8), :])
            if v % 3 == 0 and v < 12:
                q = 4 * t + v // 3
                hrow = pl.multiple_of(32 * (q // 3) + 8 * (q % 3), 8)
                layernorm16(PRE + 16 * q, hbuf, hrow, done if v else None)
                deps.setdefault(v + LN_LAG, []).append(hbuf[KT - 1, pl.ds(hrow, 8), :])
        return carry

    lax.fori_loop(0, 2 * NCH, pre_body, 0)
    for c in ffn_copies:
        c.start()

    row = lax.broadcasted_iota(jnp.int32, (80, 80), 0)
    col = lax.broadcasted_iota(jnp.int32, (80, 80), 1)
    same_head = (jnp.where(row < 64, row >> 5, (row - 64) >> 3)
                 == jnp.where(col < 64, col >> 5, (col - 64) >> 3))
    allowed = same_head & ((col >= 64) | (row >= 64) | (col <= row))
    fill = jnp.where(same_head, -1e9, -jnp.inf).astype(F32)
    low_half = lax.broadcasted_iota(jnp.int32, (8, 128), 0) < 4
    high_half = jnp.logical_not(low_half)
    scale = DH ** -0.5

    def load_row(t):
        w = jnp.concatenate([xn_t[k, pl.ds(t // 2, 1), :] for k in range(KT)], axis=1)
        bits = jnp.where(t % 2 == 0, w << 16, w & jnp.uint32(0xFFFF0000))
        return pltpu.bitcast(bits, F32), w

    def select_tokens():
        r = r_s[...]
        tok = lane16 * 16 + lax.broadcasted_iota(jnp.int32, (16, 128), 0)
        top1 = jnp.max(r)
        idx1 = jnp.min(jnp.where(r == top1, tok, S - 1))
        r2 = jnp.where(tok == idx1, -jnp.inf, r)
        top2 = jnp.max(r2)
        idx2 = jnp.min(jnp.where((r2 == top2) & (tok != idx1), tok, S - 1))
        idx_s[0] = idx1
        idx_s[1] = idx2
        gate_s[...] = jnp.where(lax.broadcasted_iota(jnp.int32, (16, 128), 0) == 0, top1, top2)
        sel_row = lax.broadcasted_iota(jnp.int32, (16, D), 0)
        xs1, _ = load_row(idx1)
        xs2, _ = load_row(idx2)
        xsel_s[...] = _b2u(jnp.where(sel_row == 0, xs1, jnp.where(sel_row == 1, xs2, 0.0)).astype(BF))

    def one_step(i, u, mem):
        odd = u % 2
        s2 = i * (UNROLL // 2) + u // 2
        h_ld = pl.multiple_of(32 * s2, 32)
        r24 = pl.multiple_of((XS * s2) % RING32, 8)
        a24 = pl.multiple_of(XS * s2, 8)
        qkv_ld = pl.multiple_of((SEG * s2 + 32) % RING32, 32) + 16 * odd
        o_st = pl.multiple_of((SEG * s2) % RING32, 32) + 16 * odd
        m0 = 0 if odd else XS

        def with_mem(ref, idx, base, m):
            lo = ref[idx, pl.ds(base + 8 * odd, 8), :]
            hi = ref[idx, pl.ds(base + 8 + 8 * odd, 8), :]
            if odd:
                lo = jnp.where(low_half, m, lo)
            else:
                hi = jnp.where(low_half, hi, m)
            return _u2b(jnp.concatenate([lo, hi], axis=0))

        def store_tokens(ref, idx, base, yp):
            if odd:
                pltpu.store(ref.at[idx, pl.ds(base + 8, 8), :], yp[0:8], mask=high_half)
                ref[idx, pl.ds(base + 16, 8), :] = yp[8:16]
            else:
                ref[idx, pl.ds(base, 8), :] = yp[0:8]
                pltpu.store(ref.at[idx, pl.ds(base + 8, 8), :], yp[8:16], mask=low_half)

        lk = [with_mem(hbuf, k, h_ld, mem[k]) for k in range(KT)]
        lhs = jnp.concatenate(lk, axis=1)

        ymem = {}
        xs = {}
        probs = {}
        parts = {}

        def proj(h):
            split = h < K_SPLIT and u > 0
            if split:
                lhs7 = jnp.concatenate(lk[:KT - 1], axis=1)
                head = [_dot(lhs7, _u2b(wqkv[m * H + h, pl.ds(0, 448), :])) for m in range(3)]
            for m in range(3):
                if split:
                    y = _dot(lk[KT - 1], _u2b(wqkv[m * H + h, pl.ds(448, 64), :])) + head[m]
                else:
                    y = _dot(lhs, _u2b(wqkv[m * H + h]))
                store_tokens(ring, m * H + h, r24, _b2u(y.astype(BF)))
                ymem[(h, m)] = y[m0:m0 + MEM]
                xs[(h, m)] = ring[m * H + h, pl.ds(qkv_ld, SEG // 2), :]

        def pair(p, m):
            a, b = 2 * p, 2 * p + 1
            mm = jnp.concatenate([ymem[(a, m)], ymem[(b, m)]], axis=0).astype(BF)
            return jnp.concatenate([_u2b(xs[(a, m)]), _u2b(xs[(b, m)]), mm], axis=0)

        def qk(p):
            sc = _dot_nt(pair(p, 0), pair(p, 1))
            sc = jnp.where(allowed, sc * scale, fill)
            e = jnp.exp(sc - jnp.max(sc, axis=1, keepdims=True))
            l = jnp.sum(e, axis=1, keepdims=True)
            r = pl.reciprocal(l, approx=True)
            r = r * (2.0 - l * r)
            probs[p] = (e * r).astype(BF)

        def pv(p):
            op = _b2u(_dot(probs[p], pair(p, 2)).astype(BF))
            om = op[32:40]
            om_sw = pltpu.roll(om, 4, axis=0)
            for j, h in enumerate((2 * p, 2 * p + 1)):
                oring[h, pl.ds(o_st, SEG // 2), :] = op[16 * j:16 * j + 16]
                parts[h] = with_mem(oring, h, r24, om if j != odd else om_sw)

        def after(t):
            for lag, fn in ((LAG_QK, qk), (LAG_PV, pv)):
                if (t - 1 - lag) % 2 == 0 and 0 <= (t - 1 - lag) // 2 < NPAIR:
                    fn((t - 1 - lag) // 2)

        for t in range(H):
            proj(t)
            after(t)
            if u == 0 and t == 8:
                select_tokens()
        t = H
        lhs_a = jnp.concatenate([parts[j] for j in range(H_SPLIT)], axis=1)
        acc = []
        for n in range(N_PART):
            acc.append(_dot(lhs_a, _u2b(wo_s[n, pl.ds(0, H_SPLIT * 64), :])))
            after(t)
            t += 1
        while t - 1 - LAG_PV <= 2 * (NPAIR - 1):
            after(t)
            t += 1
        lhs_b = jnp.concatenate([parts[j] for j in range(H_SPLIT, H)], axis=1)
        lhs_o = jnp.concatenate([lhs_a, lhs_b], axis=1)
        new_mem = [None] * KT

        def finish(n, y):
            store_tokens(abuf, n, a24, _b2u(y.astype(BF)))
            ym = y[m0:m0 + MEM]
            new_mem[n] = _b2u(jnp.concatenate([ym, ym], axis=0).astype(BF))

        for n in range(N_PART, KT):
            finish(n, _dot(lhs_o, _u2b(wo_s[n])))
            if n == N_PART:
                for n2 in range(N_PART):
                    tail = _u2b(wo_s[n2, pl.ds(H_SPLIT * 64, (H - H_SPLIT) * 64), :])
                    finish(n2, _dot(lhs_b, tail) + acc[n2])
        return new_mem

    def body(i, mem):
        mem = list(mem)
        for u in range(UNROLL):
            mem = one_step(i, u, mem)
        return tuple(mem)

    for n in range(KT):
        wo_copy(n).wait()
    mi = mem0_s[...].astype(F32)
    mip = _b2u(jnp.concatenate([mi, mi], axis=0).astype(BF))
    lax.fori_loop(0, NSEG // UNROLL, body,
                  tuple(mip[:, 128 * k:128 * (k + 1)] for k in range(KT)))

    early = S - PRE
    zrow = pl.multiple_of(zero_s[0], 16)
    FPER = 9

    def half_rows(r0):
        return r0 // 2 if isinstance(r0, int) else pl.multiple_of(r0 // 2, 8)

    def combine(r0, nrows, n, a):
        xf = x_s[pl.ds(r0, nrows), pl.ds(128 * n, 128)].astype(F32)
        b = _u2b(xn_t[n, pl.ds(half_rows(r0), nrows // 2), :]).astype(F32)
        out_s[pl.ds(r0, nrows), pl.ds(128 * n, 128)] = (_rbf(xf + a) + b).astype(BF)

    def combine_stored(r0, nrows):
        for n in range(KT):
            combine(r0, nrows, n, _u2b(abuf[n, pl.ds(half_rows(r0), nrows // 2), :]).astype(F32))

    def out_copy(r0, nrows, j):
        return pltpu.make_async_copy(out_s.at[pl.ds(r0, nrows), :], out_hbm.at[pl.ds(r0, nrows), :],
                                     sems.at[SEM_OUT + j])

    def ffn_groups(j0, count, y, done):
        x_sel = _u2b(xsel_s[...])
        hid = {}

        def up(w_ref, j, key):
            part = _dot(x_sel[:, 0:512], _u2b(w_ref[j, pl.ds(0, 256), :]))
            yield
            hid[key] = _rbf(_dot(x_sel[:, 512:1024], _u2b(w_ref[j, pl.ds(256, 256), :])) + part)
            yield

        def down(jj):
            g = hid[("g", jj)]
            hb = (_rbf(g * _rbf(jax.nn.sigmoid(g))) * hid[("u", jj)]).astype(BF)
            rows = pl.ds(pl.multiple_of(64 * (j0 + jj), 64), 64)
            for half in range(2):
                w = jnp.concatenate([_u2b(wd_s[4 * half + n, rows, :]) for n in range(4)], axis=1)
                y[half] = _dot(hb, w) + y[half]
                yield

        for jj in range(count + 1):
            if jj < count:
                yield from up(wg_s, j0 + jj, ("g", jj))
                yield from up(wu_s, j0 + jj, ("u", jj))
            elif count == 1:
                yield
                yield
            if jj >= 1:
                yield from down(jj - 1)
        done()

    def epi_chunk(r0, side, pieces, keep):
        p0 = (r0 % RING) // 2
        p1 = ((r0 + 64) % RING) // 2
        if not isinstance(r0, int):
            p0, p1 = pl.multiple_of(p0, 32), pl.multiple_of(p1, 32)
        deps = {}
        for n in range(KT):
            acc = None
            for g in range(8):
                lhs = jnp.concatenate(
                    [_u2b(jnp.concatenate([oring[h, pl.ds(p0, 32), :], oring[h, pl.ds(p1, 32), :]], axis=0))
                     for h in range(4 * g, 4 * g + 4)], axis=1)
                w = _after(wo_s[n, pl.ds(256 * g, 256), :], deps.get(8 * n + g), zero)
                y = _dot(lhs, _u2b(w))
                acc = y if acc is None else y + acc
                next(side, None)
                if pieces is not None and g % 4 == 0 and 8 * n + g < 56:
                    for e in ((0, 1, 2) if n == 0 and g == 0 else (2 * n + g // 4 + 2,)):
                        combine_stored(pieces + 32 * e, 32)
                    deps[8 * n + g + 6] = [_b2u(out_s[pl.ds(zrow, 16), pl.ds(0, 128)])]
            ab = acc.astype(BF)
            if keep:
                abuf[n, pl.ds(half_rows(r0), 64), :] = _b2u(ab)
            combine(r0, 128, n, ab.astype(F32))

    for c in ffn_copies:
        c.wait()

    def epi_body(c, y):
        y = list(y)
        r0 = pl.multiple_of(early + 128 * c, 128)
        e0 = pl.multiple_of(512 * c, 512)
        epi_chunk(r0, ffn_groups(FPER * c, FPER, y, lambda: None), e0, True)
        out_copy(r0, 128, c).start()
        out_copy(e0, 512, 4 + c).start()
        return tuple(y)

    y = list(lax.fori_loop(0, 3, epi_body, (jnp.zeros((16, 512), F32), jnp.zeros((16, 512), F32))))
    idx1 = idx_s[0]
    idx2 = idx_s[1]

    def patch_row(t, yrow):
        xr, w = load_row(t)
        bits = pltpu.bitcast(_rbf(xr + yrow), U32)
        w = jnp.where(t % 2 == 0,
                      (w & jnp.uint32(0xFFFF0000)) | (bits >> 16),
                      (w & jnp.uint32(0xFFFF)) | bits)
        for k in range(KT):
            xn_t[k, pl.ds(t // 2, 1), :] = w[:, 128 * k:128 * (k + 1)]

    def patch():
        gate = _rbf(jax.nn.sigmoid(gate_s[:, 0:1]))
        yy = _rbf(_rbf(jnp.concatenate(y, axis=1)) * gate)
        patch_row(idx1, yy[0:1])
        patch_row(idx2, yy[1:2])

    last = S - 128
    epi_chunk(last, ffn_groups(3 * FPER, 1, y, patch), None, False)
    out_copy(last, 128, 3).start()
    for c in range(3):
        out_copy(early + 128 * c, 128, c).wait()
        out_copy(512 * c, 512, 4 + c).wait()
    blk1 = jnp.minimum(idx1 // 16, last // 16 - 1)
    blk2 = jnp.minimum(idx2 // 16, last // 16 - 1)
    blk2 = jnp.where(blk2 == blk1, jnp.where(blk1 == 0, 1, blk1 - 1), blk2)
    fix = []
    for j, blk in enumerate((blk1, blk2)):
        r0 = pl.multiple_of(blk * 16, 16)
        combine_stored(r0, 16)
        fix.append(out_copy(r0, 16, 7 + j))
    for cp in fix:
        cp.start()
    out_copy(last, 128, 3).wait()
    for cp in fix:
        cp.wait()


@jax.jit
def pallas_parallel_sum__memory_aug_recurrent_mem_tr__moe_arch_mod__prompt_kernel(
    A_x: jax.Array,
    A_mem0: jax.Array,
    A_Wq: jax.Array,
    A_Wk: jax.Array,
    A_Wv: jax.Array,
    A_Wo: jax.Array,
    A_seg_len: jax.Array,
    B_x: jax.Array,
    B_w_r: jax.Array,
    B_w_gate: jax.Array,
    B_w_up: jax.Array,
    B_w_down: jax.Array,
):
    del A_seg_len, B_x
    assert A_x.shape == (1, S, D) and A_mem0.shape == (1, MEM, D)
    assert A_Wq.shape == (D, H, DH) and A_Wo.shape == (H, DH, D)
    assert B_w_gate.shape == (D, FF) and B_w_down.shape == (FF, D)
    any_spec = pl.BlockSpec(memory_space=pl.ANY)
    out = pl.pallas_call(
        _kernel,
        out_shape=jax.ShapeDtypeStruct((S, D), BF),
        in_specs=[any_spec] * 10,
        out_specs=any_spec,
        scratch_shapes=[
            pltpu.VMEM((S, D), BF),
            pltpu.VMEM((KT, S // 2, 128), U32),
            pltpu.VMEM((KT, PRE // 2, 128), U32),
            pltpu.VMEM((KT, 16 * NSEG, 128), U32),
            pltpu.VMEM((3 * H + 2, D // 2, 128), U32),
            pltpu.VMEM((KT, H * DH // 2, 128), U32),
            pltpu.VMEM((3 * H, RING32, 128), U32),
            pltpu.VMEM((H, RING32, 128), U32),
            pltpu.VMEM((KT, S // 2, 128), U32),
            pltpu.VMEM((S, D), BF),
            pltpu.VMEM((NCH, D // 2, 8, 128), U32),
            pltpu.VMEM((FT, D // 2, 128), U32),
            pltpu.VMEM((FT, D // 2, 128), U32),
            pltpu.VMEM((KT, FF // 2, 128), U32),
            pltpu.VMEM((MEM, D), BF),
            pltpu.VMEM((D,), BF),
            pltpu.VMEM((8, D), F32),
            pltpu.VMEM((16, 128), F32),
            pltpu.VMEM((8, D), U32),
            pltpu.VMEM((16, 128), F32),
            pltpu.SMEM((1,), jnp.int32),
            pltpu.SMEM((2,), jnp.int32),
            pltpu.SemaphoreType.DMA((NSEM,)),
        ],
        compiler_params=pltpu.CompilerParams(vmem_limit_bytes=126 * 1024 * 1024),
    )(A_x.reshape(S, D), A_mem0.reshape(MEM, D), A_Wq.reshape(D // 2, 2, H, DH), A_Wk.reshape(D // 2, 2, H, DH),
      A_Wv.reshape(D // 2, 2, H, DH), A_Wo.reshape(H * DH, D),
      B_w_r, B_w_gate, B_w_up, B_w_down)
    return out.reshape(1, S, D)
```

```python
import jax
import jax.numpy as jnp
from jax import lax
import jax.experimental.pallas as pl
import jax.experimental.pallas.tpu as pltpu

BF = jnp.bfloat16
U32 = jnp.uint32
F32 = jnp.float32

S = 2048
D = 1024
H = 32
DH = 128
MEM = 8
SEG = 32
NSEG = S // SEG
FF = 3584
KT = D // 128
FT = FF // 128
XS = 24
PRE = S - NSEG * XS
RING = 576
RING32 = RING // 2
NPAIR = H // 2
NCH = 12
NPRE = 16
SEM_SMALL, SEM_X, SEM_W = 0, 2, 3 + NPRE
SEM_WO, SEM_FFN, SEM_OUT = SEM_W + NCH, SEM_W + NCH + 1, SEM_W + NCH + 2
NSEM = SEM_OUT + 9

LAG_QK = 1
LAG_PV = 4
N_PART = 4
H_SPLIT = 26
REL_SCHED = {0: [(0, 0), (0, 1)], 1: [(0, 2), (0, 3)], 2: [(0, 4)], 3: [(0, 5)], 4: [(0, 6)], 5: [(0, 7)]}
REL_SCHED.update({6 + k: [(1, k)] for k in range(8)})
REL_SCHED.update({14 + k: [(2, k)] for k in range(8)})
K_SPLIT = 1
LN_LAG = 5
UNROLL = 4


def _b2u(x):
    return pltpu.bitcast(x, U32)


def _u2b(x):
    return pltpu.bitcast(x, BF)


def _dot(a, b):
    return jnp.dot(a, b, preferred_element_type=F32)


def _dot_nt(a, b):
    return lax.dot_general(a, b, (((1,), (1,)), ((), ())), preferred_element_type=F32)


def _after(w, dep, zero):
    if not dep:
        return w
    d = dep[0]
    for e in dep[1:]:
        d = d | e
    return jnp.concatenate([w[0:8] | (d & zero), w[8:]], axis=0)


def _rbf(x):
    return x.astype(BF).astype(F32)


def _kernel(x_hbm, mem0_hbm, wq_hbm, wk_hbm, wv_hbm, wo_hbm, wr_hbm, wg_hbm, wu_hbm, wd_hbm,
            out_hbm,
            x_s, xn_t, xn_pre, hbuf, wqkv, wo_s, ring, oring, abuf, out_s, raw,
            wg_s, wu_s, wd_s, mem0_s, wr_s, wrf_s, r_s, xsel_s, gate_s, zero_s, idx_s,
            sems):
    w32 = [w.bitcast(U32) for w in (wq_hbm, wk_hbm, wv_hbm)]
    wo32 = wo_hbm.bitcast(U32)
    wg32 = wg_hbm.bitcast(U32)
    wu32 = wu_hbm.bitcast(U32)
    wd32 = wd_hbm.bitcast(U32)

    x_first = pltpu.make_async_copy(x_hbm.at[pl.ds(0, PRE), :], x_s.at[pl.ds(0, PRE), :], sems.at[SEM_X])

    def x_piece(c):
        r0 = PRE + 96 * c if isinstance(c, int) else pl.multiple_of(PRE + 96 * c, 32)
        return pltpu.make_async_copy(x_hbm.at[pl.ds(r0, 96), :], x_s.at[pl.ds(r0, 96), :],
                                     sems.at[SEM_X + 1 + c])

    def w_start(c):
        for par in range(2):
            pltpu.make_async_copy(w32[c // 4].at[:, par, pl.ds(4 * (c % 4), 4), :],
                                  raw.at[c, :, pl.ds(4 * par, 4), :], sems.at[SEM_W + c]).start()

    def w_wait(c):
        pltpu.make_async_copy(raw.at[c], raw.at[c], sems.at[SEM_W + c]).wait()

    def wo_copy(n):
        return pltpu.make_async_copy(wo32.at[:, pl.ds(128 * n, 128)], wo_s.at[n], sems.at[SEM_WO])

    small_copies = [pltpu.make_async_copy(mem0_hbm, mem0_s, sems.at[SEM_SMALL]),
                    pltpu.make_async_copy(wr_hbm, wr_s, sems.at[SEM_SMALL + 1])]
    ffn_copies = (
        [pltpu.make_async_copy(wg32.at[:, pl.ds(128 * j, 128)], wg_s.at[j], sems.at[SEM_FFN]) for j in range(FT)]
        + [pltpu.make_async_copy(wu32.at[:, pl.ds(128 * j, 128)], wu_s.at[j], sems.at[SEM_FFN]) for j in range(FT)]
        + [pltpu.make_async_copy(wd32.at[:, pl.ds(128 * n, 128)], wd_s.at[n], sems.at[SEM_FFN]) for n in range(KT)])

    zero_s[0] = 0
    x_first.start()
    for c in small_copies:
        c.start()
    for c in range(NCH):
        w_start(c)
        for t in range(NPRE):
            if min(3 * t + 3, 4 * NCH - 1) // 4 == c + 1 or (c == 0 and t == 0):
                x_piece(t).start()
    for n in range(KT):
        wo_copy(n).start()
    eps_bf = 1.0013580322265625e-05

    def layernorm16(rq, dst_ref, dst_row, not_before=None):
        rq = pl.multiple_of(rq, 16)
        xf = x_s[pl.ds(rq, 16), :].astype(F32)
        if not_before is not None:
            x0 = _after(pltpu.bitcast(xf[:, 0:128], U32), [not_before], zero)
            xf = jnp.concatenate([pltpu.bitcast(x0, F32), xf[:, 128:]], axis=1)
        mean = jnp.sum(xf, axis=1, keepdims=True) * (1.0 / D)
        cen = xf - mean
        var = jnp.sum(cen * cen, axis=1, keepdims=True) * (1.0 / D)
        sd = _rbf(jnp.sqrt(_rbf(_rbf(var) + eps_bf)))
        xn = (_rbf(xf - _rbf(mean)) * (1.0 / sd)).astype(BF)
        wr = jnp.concatenate([wrf_s[...], wrf_s[...]], axis=0)
        score = _rbf(jnp.sum(xn.astype(F32) * wr, axis=1, keepdims=True))
        r_s[...] = jnp.where(lane16 == rq // 16, score, r_s[...])
        xp = _b2u(xn)
        hq = pl.multiple_of(rq // 2, 8)
        dst_row = pl.multiple_of(dst_row, 8)
        for k in range(KT):
            xn_t[k, pl.ds(hq, 8), :] = xp[:, 128 * k:128 * (k + 1)]
            dst_ref[k, pl.ds(dst_row, 8), :] = xp[:, 128 * k:128 * (k + 1)]

    zero = jnp.full((8, 128), zero_s[0], jnp.int32).astype(U32)
    r_s[...] = jnp.full(r_s.shape, -jnp.inf, F32)
    lane16 = lax.broadcasted_iota(jnp.int32, (16, 128), 1)
    x_first.wait()
    for c in small_copies:
        c.wait()
    wrf_s[...] = jnp.broadcast_to(wr_s[...].astype(F32).reshape(1, D), (8, D))

    def ln_body(c, carry):
        for q in range(8):
            layernorm16(128 * c + 16 * q, xn_pre, 64 * c + 8 * q)
        return carry

    lax.fori_loop(0, PRE // 128, ln_body, 0)

    raw2 = raw.reshape(NCH * 4096, 128)

    def raw_view(p):
        return raw2.at[pl.ds((p >> 2) * 4096 + (p & 3), 4093), :]

    def relayout(src, dst, j, k):
        a = src[pl.ds(512 * k, 64, stride=8), :]
        b = src[pl.ds(512 * k + 4, 64, stride=8), :]
        rows = pl.ds(64 * k, 64)
        dst[2 * j, rows, :] = (a & jnp.uint32(0xFFFF)) | (b << 16)
        dst[2 * j + 1, rows, :] = (a >> 16) | (b & jnp.uint32(0xFFFF0000))

    def pre_dot(w_view, ring_view, j, k, dep=None):
        i, q = k // 4, k % 4
        lhs = jnp.concatenate([_u2b(xn_pre[kk, pl.ds(64 * q, 64), :]) for kk in range(KT)], axis=1)
        y = _dot(lhs, _u2b(_after(w_view[2 * j + i], dep, zero)))
        yp = _b2u(y.astype(BF))
        ring_view[2 * j + i, pl.ds(32 + 64 * q, 64), :] = yp
        return yp[0:8]

    w_wait(0)
    for k in range(8):
        relayout(raw_view(0), wqkv, 0, k)

    def pre_body(t, carry):
        x_piece(t).wait()

        @pl.when(((t & 3) != 0) & (t < NPRE - 1))
        def _():
            w_wait((3 * t + 3) >> 2)

        deps = {}
        w_view = wqkv.at[pl.ds(6 * t, 8)]
        ring_view = ring.at[pl.ds(6 * t, 6)]
        srcs = [raw_view(jnp.minimum(3 * t + 1 + j, 4 * NCH - 1)) for j in range(3)]
        for v in range(24):
            j, k = v // 8, v % 8
            done = pre_dot(w_view, ring_view, j, k, deps.get(v))
            for jr, kr in REL_SCHED.get(v, ()):
                relayout(srcs[jr], w_view, jr + 1, kr)
                deps.setdefault(v + 2, []).append(w_view[2 * jr + 3, pl.ds(64 * kr + 56, 8), :])
            if v % 3 == 0 and v < 18:
                q = v // 3
                hrow = pl.multiple_of(64 * t, 64) + 32 * (q // 3) + 8 * (q % 3)
                layernorm16(PRE + 96 * t + 16 * q, hbuf, hrow, done if v else None)
                deps.setdefault(v + LN_LAG, []).append(hbuf[KT - 1, pl.ds(hrow, 8), :])
        return carry

    lax.fori_loop(0, NPRE, pre_body, 0)
    for c in ffn_copies:
        c.start()

    row = lax.broadcasted_iota(jnp.int32, (80, 80), 0)
    col = lax.broadcasted_iota(jnp.int32, (80, 80), 1)
    same_head = (jnp.where(row < 64, row >> 5, (row - 64) >> 3)
                 == jnp.where(col < 64, col >> 5, (col - 64) >> 3))
    allowed = same_head & ((col >= 64) | (row >= 64) | (col <= row))
    fill = jnp.where(same_head, -1e9, -jnp.inf).astype(F32)
    low_half = lax.broadcasted_iota(jnp.int32, (8, 128), 0) < 4
    high_half = jnp.logical_not(low_half)
    scale = DH ** -0.5

    def load_row(t):
        w = jnp.concatenate([xn_t[k, pl.ds(t // 2, 1), :] for k in range(KT)], axis=1)
        bits = jnp.where(t % 2 == 0, w << 16, w & jnp.uint32(0xFFFF0000))
        return pltpu.bitcast(bits, F32), w

    def select_tokens():
        r = r_s[...]
        tok = lane16 * 16 + lax.broadcasted_iota(jnp.int32, (16, 128), 0)
        top1 = jnp.max(r)
        idx1 = jnp.min(jnp.where(r == top1, tok, S - 1))
        r2 = jnp.where(tok == idx1, -jnp.inf, r)
        top2 = jnp.max(r2)
        idx2 = jnp.min(jnp.where((r2 == top2) & (tok != idx1), tok, S - 1))
        idx_s[0] = idx1
        idx_s[1] = idx2
        gate_s[...] = jnp.where(lax.broadcasted_iota(jnp.int32, (16, 128), 0) == 0, top1, top2)
        sel_row = lax.broadcasted_iota(jnp.int32, (16, D), 0)
        xs1, _ = load_row(idx1)
        xs2, _ = load_row(idx2)
        xsel_s[...] = _b2u(jnp.where(sel_row == 0, xs1, jnp.where(sel_row == 1, xs2, 0.0)).astype(BF))

    def one_step(i, u, mem):
        odd = u % 2
        s2 = i * (UNROLL // 2) + u // 2
        h_ld = pl.multiple_of(32 * s2, 32)
        r24 = pl.multiple_of((XS * s2) % RING32, 8)
        a24 = pl.multiple_of(XS * s2, 8)
        qkv_ld = pl.multiple_of((SEG * s2 + 32) % RING32, 32) + 16 * odd
        o_st = pl.multiple_of((SEG * s2) % RING32, 32) + 16 * odd
        m0 = 0 if odd else XS

        def with_mem(ref, idx, base, m):
            lo = ref[idx, pl.ds(base + 8 * odd, 8), :]
            hi = ref[idx, pl.ds(base + 8 + 8 * odd, 8), :]
            if odd:
                lo = jnp.where(low_half, m, lo)
            else:
                hi = jnp.where(low_half, hi, m)
            return _u2b(jnp.concatenate([lo, hi], axis=0))

        def store_tokens(ref, idx, base, yp):
            if odd:
                pltpu.store(ref.at[idx, pl.ds(base + 8, 8), :], yp[0:8], mask=high_half)
                ref[idx, pl.ds(base + 16, 8), :] = yp[8:16]
            else:
                ref[idx, pl.ds(base, 8), :] = yp[0:8]
                pltpu.store(ref.at[idx, pl.ds(base + 8, 8), :], yp[8:16], mask=low_half)

        lk = [with_mem(hbuf, k, h_ld, mem[k]) for k in range(KT)]
        lhs = jnp.concatenate(lk, axis=1)

        ymem = {}
        xs = {}
        probs = {}
        parts = {}

        def proj(h):
            split = h < K_SPLIT and u > 0
            if split:
                lhs7 = jnp.concatenate(lk[:KT - 1], axis=1)
                head = [_dot(lhs7, _u2b(wqkv[m * H + h, pl.ds(0, 448), :])) for m in range(3)]
            for m in range(3):
                if split:
                    y = _dot(lk[KT - 1], _u2b(wqkv[m * H + h, pl.ds(448, 64), :])) + head[m]
                else:
                    y = _dot(lhs, _u2b(wqkv[m * H + h]))
                store_tokens(ring, m * H + h, r24, _b2u(y.astype(BF)))
                ymem[(h, m)] = y[m0:m0 + MEM]
                xs[(h, m)] = ring[m * H + h, pl.ds(qkv_ld, SEG // 2), :]

        def pair(p, m):
            a, b = 2 * p, 2 * p + 1
            mm = jnp.concatenate([ymem[(a, m)], ymem[(b, m)]], axis=0).astype(BF)
            return jnp.concatenate([_u2b(xs[(a, m)]), _u2b(xs[(b, m)]), mm], axis=0)

        def qk(p):
            sc = _dot_nt(pair(p, 0), pair(p, 1))
            sc = jnp.where(allowed, sc * scale, fill)
            e = jnp.exp(sc - jnp.max(sc, axis=1, keepdims=True))
            l = jnp.sum(e, axis=1, keepdims=True)
            r = pl.reciprocal(l, approx=True)
            r = r * (2.0 - l * r)
            probs[p] = (e * r).astype(BF)

        def pv(p):
            op = _b2u(_dot(probs[p], pair(p, 2)).astype(BF))
            om = op[32:40]
            om_sw = pltpu.roll(om, 4, axis=0)
            for j, h in enumerate((2 * p, 2 * p + 1)):
                oring[h, pl.ds(o_st, SEG // 2), :] = op[16 * j:16 * j + 16]
                parts[h] = with_mem(oring, h, r24, om if j != odd else om_sw)

        def after(t):
            for lag, fn in ((LAG_QK, qk), (LAG_PV, pv)):
                if (t - 1 - lag) % 2 == 0 and 0 <= (t - 1 - lag) // 2 < NPAIR:
                    fn((t - 1 - lag) // 2)

        for t in range(H):
            proj(t)
            after(t)
            if u == 0 and t == 8:
                select_tokens()
        t = H
        lhs_a = jnp.concatenate([parts[j] for j in range(H_SPLIT)], axis=1)
        acc = []
        for n in range(N_PART):
            acc.append(_dot(lhs_a, _u2b(wo_s[n, pl.ds(0, H_SPLIT * 64), :])))
            after(t)
            t += 1
        while t - 1 - LAG_PV <= 2 * (NPAIR - 1):
            after(t)
            t += 1
        lhs_b = jnp.concatenate([parts[j] for j in range(H_SPLIT, H)], axis=1)
        lhs_o = jnp.concatenate([lhs_a, lhs_b], axis=1)
        new_mem = [None] * KT

        def finish(n, y):
            store_tokens(abuf, n, a24, _b2u(y.astype(BF)))
            ym = y[m0:m0 + MEM]
            new_mem[n] = _b2u(jnp.concatenate([ym, ym], axis=0).astype(BF))

        for n in range(N_PART, KT):
            finish(n, _dot(lhs_o, _u2b(wo_s[n])))
            if n == N_PART:
                for n2 in range(N_PART):
                    tail = _u2b(wo_s[n2, pl.ds(H_SPLIT * 64, (H - H_SPLIT) * 64), :])
                    finish(n2, _dot(lhs_b, tail) + acc[n2])
        return new_mem

    def body(i, mem):
        mem = list(mem)
        for u in range(UNROLL):
            mem = one_step(i, u, mem)
        return tuple(mem)

    for n in range(KT):
        wo_copy(n).wait()
    mi = mem0_s[...].astype(F32)
    mip = _b2u(jnp.concatenate([mi, mi], axis=0).astype(BF))
    lax.fori_loop(0, NSEG // UNROLL, body,
                  tuple(mip[:, 128 * k:128 * (k + 1)] for k in range(KT)))

    early = S - PRE
    zrow = pl.multiple_of(zero_s[0], 16)
    FPER = 9

    def half_rows(r0):
        return r0 // 2 if isinstance(r0, int) else pl.multiple_of(r0 // 2, 8)

    def combine(r0, nrows, n, a):
        xf = x_s[pl.ds(r0, nrows), pl.ds(128 * n, 128)].astype(F32)
        b = _u2b(xn_t[n, pl.ds(half_rows(r0), nrows // 2), :]).astype(F32)
        out_s[pl.ds(r0, nrows), pl.ds(128 * n, 128)] = (_rbf(xf + a) + b).astype(BF)

    def combine_stored(r0, nrows):
        for n in range(KT):
            combine(r0, nrows, n, _u2b(abuf[n, pl.ds(half_rows(r0), nrows // 2), :]).astype(F32))

    def out_copy(r0, nrows, j):
        return pltpu.make_async_copy(out_s.at[pl.ds(r0, nrows), :], out_hbm.at[pl.ds(r0, nrows), :],
                                     sems.at[SEM_OUT + j])

    def ffn_groups(j0, count, y, done):
        x_sel = _u2b(xsel_s[...])
        hid = {}

        def up(w_ref, j, key):
            part = _dot(x_sel[:, 0:512], _u2b(w_ref[j, pl.ds(0, 256), :]))
            yield
            hid[key] = _rbf(_dot(x_sel[:, 512:1024], _u2b(w_ref[j, pl.ds(256, 256), :])) + part)
            yield

        def down(jj):
            g = hid[("g", jj)]
            hb = (_rbf(g * _rbf(jax.nn.sigmoid(g))) * hid[("u", jj)]).astype(BF)
            rows = pl.ds(pl.multiple_of(64 * (j0 + jj), 64), 64)
            for half in range(2):
                w = jnp.concatenate([_u2b(wd_s[4 * half + n, rows, :]) for n in range(4)], axis=1)
                y[half] = _dot(hb, w) + y[half]
                yield

        for jj in range(count + 1):
            if jj < count:
                yield from up(wg_s, j0 + jj, ("g", jj))
                yield from up(wu_s, j0 + jj, ("u", jj))
            elif count == 1:
                yield
                yield
            if jj >= 1:
                yield from down(jj - 1)
        done()

    def epi_chunk(r0, side, pieces, keep):
        p0 = (r0 % RING) // 2
        p1 = ((r0 + 64) % RING) // 2
        if not isinstance(r0, int):
            p0, p1 = pl.multiple_of(p0, 32), pl.multiple_of(p1, 32)
        deps = {}
        for n in range(KT):
            acc = None
            for g in range(8):
                lhs = jnp.concatenate(
                    [_u2b(jnp.concatenate([oring[h, pl.ds(p0, 32), :], oring[h, pl.ds(p1, 32), :]], axis=0))
                     for h in range(4 * g, 4 * g + 4)], axis=1)
                w = _after(wo_s[n, pl.ds(256 * g, 256), :], deps.get(8 * n + g), zero)
                y = _dot(lhs, _u2b(w))
                acc = y if acc is None else y + acc
                next(side, None)
                if pieces is not None and g % 4 == 0 and 8 * n + g < 56:
                    for e in ((0, 1, 2) if n == 0 and g == 0 else (2 * n + g // 4 + 2,)):
                        combine_stored(pieces + 32 * e, 32)
                    deps[8 * n + g + 6] = [_b2u(out_s[pl.ds(zrow, 16), pl.ds(0, 128)])]
            ab = acc.astype(BF)
            if keep:
                abuf[n, pl.ds(half_rows(r0), 64), :] = _b2u(ab)
            combine(r0, 128, n, ab.astype(F32))

    for c in ffn_copies:
        c.wait()

    def epi_body(c, y):
        y = list(y)
        r0 = pl.multiple_of(early + 128 * c, 128)
        e0 = pl.multiple_of(512 * c, 512)
        epi_chunk(r0, ffn_groups(FPER * c, FPER, y, lambda: None), e0, True)
        out_copy(r0, 128, c).start()
        out_copy(e0, 512, 4 + c).start()
        return tuple(y)

    y = list(lax.fori_loop(0, 3, epi_body, (jnp.zeros((16, 512), F32), jnp.zeros((16, 512), F32))))
    idx1 = idx_s[0]
    idx2 = idx_s[1]

    def patch_row(t, yrow):
        xr, w = load_row(t)
        bits = pltpu.bitcast(_rbf(xr + yrow), U32)
        w = jnp.where(t % 2 == 0,
                      (w & jnp.uint32(0xFFFF0000)) | (bits >> 16),
                      (w & jnp.uint32(0xFFFF)) | bits)
        for k in range(KT):
            xn_t[k, pl.ds(t // 2, 1), :] = w[:, 128 * k:128 * (k + 1)]

    def patch():
        gate = _rbf(jax.nn.sigmoid(gate_s[:, 0:1]))
        yy = _rbf(_rbf(jnp.concatenate(y, axis=1)) * gate)
        patch_row(idx1, yy[0:1])
        patch_row(idx2, yy[1:2])

    last = S - 128
    epi_chunk(last, ffn_groups(3 * FPER, 1, y, patch), None, False)
    out_copy(last, 128, 3).start()
    for c in range(3):
        out_copy(early + 128 * c, 128, c).wait()
        out_copy(512 * c, 512, 4 + c).wait()
    blk1 = jnp.minimum(idx1 // 16, last // 16 - 1)
    blk2 = jnp.minimum(idx2 // 16, last // 16 - 1)
    blk2 = jnp.where(blk2 == blk1, jnp.where(blk1 == 0, 1, blk1 - 1), blk2)
    fix = []
    for j, blk in enumerate((blk1, blk2)):
        r0 = pl.multiple_of(blk * 16, 16)
        combine_stored(r0, 16)
        fix.append(out_copy(r0, 16, 7 + j))
    for cp in fix:
        cp.start()
    out_copy(last, 128, 3).wait()
    for cp in fix:
        cp.wait()


@jax.jit
def pallas_parallel_sum__memory_aug_recurrent_mem_tr__moe_arch_mod__prompt_kernel(
    A_x: jax.Array,
    A_mem0: jax.Array,
    A_Wq: jax.Array,
    A_Wk: jax.Array,
    A_Wv: jax.Array,
    A_Wo: jax.Array,
    A_seg_len: jax.Array,
    B_x: jax.Array,
    B_w_r: jax.Array,
    B_w_gate: jax.Array,
    B_w_up: jax.Array,
    B_w_down: jax.Array,
):
    del A_seg_len, B_x
    assert A_x.shape == (1, S, D) and A_mem0.shape == (1, MEM, D)
    assert A_Wq.shape == (D, H, DH) and A_Wo.shape == (H, DH, D)
    assert B_w_gate.shape == (D, FF) and B_w_down.shape == (FF, D)
    any_spec = pl.BlockSpec(memory_space=pl.ANY)
    out = pl.pallas_call(
        _kernel,
        out_shape=jax.ShapeDtypeStruct((S, D), BF),
        in_specs=[any_spec] * 10,
        out_specs=any_spec,
        scratch_shapes=[
            pltpu.VMEM((S, D), BF),
            pltpu.VMEM((KT, S // 2, 128), U32),
            pltpu.VMEM((KT, PRE // 2, 128), U32),
            pltpu.VMEM((KT, 16 * NSEG, 128), U32),
            pltpu.VMEM((3 * H + 2, D // 2, 128), U32),
            pltpu.VMEM((KT, H * DH // 2, 128), U32),
            pltpu.VMEM((3 * H, RING32, 128), U32),
            pltpu.VMEM((H, RING32, 128), U32),
            pltpu.VMEM((KT, S // 2, 128), U32),
            pltpu.VMEM((S, D), BF),
            pltpu.VMEM((NCH, D // 2, 8, 128), U32),
            pltpu.VMEM((FT, D // 2, 128), U32),
            pltpu.VMEM((FT, D // 2, 128), U32),
            pltpu.VMEM((KT, FF // 2, 128), U32),
            pltpu.VMEM((MEM, D), BF),
            pltpu.VMEM((D,), BF),
            pltpu.VMEM((8, D), F32),
            pltpu.VMEM((16, 128), F32),
            pltpu.VMEM((8, D), U32),
            pltpu.VMEM((16, 128), F32),
            pltpu.SMEM((1,), jnp.int32),
            pltpu.SMEM((2,), jnp.int32),
            pltpu.SemaphoreType.DMA((NSEM,)),
        ],
        compiler_params=pltpu.CompilerParams(vmem_limit_bytes=126 * 1024 * 1024),
    )(A_x.reshape(S, D), A_mem0.reshape(MEM, D), A_Wq.reshape(D // 2, 2, H, DH), A_Wk.reshape(D // 2, 2, H, DH),
      A_Wv.reshape(D // 2, 2, H, DH), A_Wo.reshape(H * DH, D),
      B_w_r, B_w_gate, B_w_up, B_w_down)
    return out.reshape(1, S, D)
```

```python
import jax
import jax.numpy as jnp
from jax import lax
import jax.experimental.pallas as pl
import jax.experimental.pallas.tpu as pltpu

BF = jnp.bfloat16
U32 = jnp.uint32
F32 = jnp.float32

S = 2048
D = 1024
H = 32
DH = 128
MEM = 8
SEG = 32
NSEG = S // SEG
FF = 3584
KT = D // 128
FT = FF // 128
XS = 24
PRE = S - NSEG * XS
RING = 576
RING32 = RING // 2
NPAIR = H // 2
NCH = 12
NPRE = 16
SEM_SMALL, SEM_X, SEM_W = 0, 2, 3 + NPRE
SEM_WO, SEM_FFN, SEM_OUT = SEM_W + NCH, SEM_W + NCH + 1, SEM_W + NCH + 2
NSEM = SEM_OUT + 9

LAG_QK = 1
LAG_PV = 4
N_PART = 4
H_SPLIT = 26
REL_SCHED = {0: [(0, 0), (0, 1)], 1: [(0, 2), (0, 3)], 2: [(0, 4)], 3: [(0, 5)], 4: [(0, 6)], 5: [(0, 7)]}
REL_SCHED.update({6 + k: [(1, k)] for k in range(8)})
REL_SCHED.update({14 + k: [(2, k)] for k in range(8)})
K_SPLIT = 1
EPI_SCHED = [8 * n + g for n in range(8) for g in range(2)]
EPI_LAG = 0
EPI_NB = False
EPI_ALIAS = False
LN_LAG = 5
REL_NB = True
REL_LAG = 2
UNROLL = 4


def _b2u(x):
    return pltpu.bitcast(x, U32)


def _u2b(x):
    return pltpu.bitcast(x, BF)


def _dot(a, b):
    return jnp.dot(a, b, preferred_element_type=F32)


def _dot_nt(a, b):
    return lax.dot_general(a, b, (((1,), (1,)), ((), ())), preferred_element_type=F32)


def _after(w, dep, zero):
    if not dep:
        return w
    d = dep[0]
    for e in dep[1:]:
        d = d | e
    return jnp.concatenate([w[0:8] | (d & zero), w[8:]], axis=0)


def _rbf(x):
    return x.astype(BF).astype(F32)


def _kernel(x_hbm, mem0_hbm, wq_hbm, wk_hbm, wv_hbm, wo_hbm, wr_hbm, wg_hbm, wu_hbm, wd_hbm,
            out_hbm,
            x_s, xn_t, xn_pre, hbuf, wqkv, wo_s, ring, oring, abuf, out_s, raw,
            wg_s, wu_s, wd_s, mem0_s, wr_s, wrf_s, r_s, xsel_s, gate_s, zero_s, idx_s,
            sems):
    w32 = [w.bitcast(U32) for w in (wq_hbm, wk_hbm, wv_hbm)]
    wo32 = wo_hbm.bitcast(U32)
    wg32 = wg_hbm.bitcast(U32)
    wu32 = wu_hbm.bitcast(U32)
    wd32 = wd_hbm.bitcast(U32)

    x_first = pltpu.make_async_copy(x_hbm.at[pl.ds(0, PRE), :], x_s.at[pl.ds(0, PRE), :], sems.at[SEM_X])

    def x_piece(c):
        r0 = PRE + 96 * c if isinstance(c, int) else pl.multiple_of(PRE + 96 * c, 32)
        return pltpu.make_async_copy(x_hbm.at[pl.ds(r0, 96), :], x_s.at[pl.ds(r0, 96), :],
                                     sems.at[SEM_X + 1 + c])

    def w_start(c):
        for par in range(2):
            pltpu.make_async_copy(w32[c // 4].at[:, par, pl.ds(4 * (c % 4), 4), :],
                                  raw.at[c, :, pl.ds(4 * par, 4), :], sems.at[SEM_W + c]).start()

    def w_wait(c):
        pltpu.make_async_copy(raw.at[c], raw.at[c], sems.at[SEM_W + c]).wait()

    def wo_copy(n):
        return pltpu.make_async_copy(wo32.at[:, pl.ds(128 * n, 128)], wo_s.at[n], sems.at[SEM_WO])

    small_copies = [pltpu.make_async_copy(mem0_hbm, mem0_s, sems.at[SEM_SMALL]),
                    pltpu.make_async_copy(wr_hbm, wr_s, sems.at[SEM_SMALL + 1])]
    ffn_copies = (
        [pltpu.make_async_copy(wg32.at[:, pl.ds(128 * j, 128)], wg_s.at[j], sems.at[SEM_FFN]) for j in range(FT)]
        + [pltpu.make_async_copy(wu32.at[:, pl.ds(128 * j, 128)], wu_s.at[j], sems.at[SEM_FFN]) for j in range(FT)]
        + [pltpu.make_async_copy(wd32.at[:, pl.ds(128 * n, 128)], wd_s.at[n], sems.at[SEM_FFN]) for n in range(KT)])

    zero_s[0] = 0
    x_first.start()
    for c in small_copies:
        c.start()
    for c in range(NCH):
        w_start(c)
        for t in range(NPRE):
            if min(3 * t + 3, 4 * NCH - 1) // 4 == c + 1 or (c == 0 and t == 0):
                x_piece(t).start()
    for n in range(KT):
        wo_copy(n).start()
    eps_bf = 1.0013580322265625e-05

    def layernorm16(rq, dst_ref, dst_row, not_before=None):
        rq = pl.multiple_of(rq, 16)
        xf = x_s[pl.ds(rq, 16), :].astype(F32)
        if not_before is not None:
            x0 = _after(pltpu.bitcast(xf[:, 0:128], U32), [not_before], zero_box[0])
            xf = jnp.concatenate([pltpu.bitcast(x0, F32), xf[:, 128:]], axis=1)
        mean = jnp.sum(xf, axis=1, keepdims=True) * (1.0 / D)
        cen = xf - mean
        var = jnp.sum(cen * cen, axis=1, keepdims=True) * (1.0 / D)
        sd = _rbf(jnp.sqrt(_rbf(_rbf(var) + eps_bf)))
        xn = (_rbf(xf - _rbf(mean)) * (1.0 / sd)).astype(BF)
        wr = jnp.concatenate([wrf_s[...], wrf_s[...]], axis=0)
        score = _rbf(jnp.sum(xn.astype(F32) * wr, axis=1, keepdims=True))
        r_s[...] = jnp.where(lane16 == rq // 16, score, r_s[...])
        xp = _b2u(xn)
        hq = pl.multiple_of(rq // 2, 8)
        dst_row = pl.multiple_of(dst_row, 8)
        for k in range(KT):
            xn_t[k, pl.ds(hq, 8), :] = xp[:, 128 * k:128 * (k + 1)]
            dst_ref[k, pl.ds(dst_row, 8), :] = xp[:, 128 * k:128 * (k + 1)]

    zero_box = [None]

    def fresh_zero():
        zero_box[0] = jnp.full((8, 128), zero_s[0], jnp.int32).astype(U32)

    r_s[...] = jnp.full(r_s.shape, -jnp.inf, F32)
    lane16 = lax.broadcasted_iota(jnp.int32, (16, 128), 1)
    x_first.wait()
    for c in small_copies:
        c.wait()
    wrf_s[...] = jnp.broadcast_to(wr_s[...].astype(F32).reshape(1, D), (8, D))

    def ln_body(c, carry):
        for q in range(8):
            layernorm16(128 * c + 16 * q, xn_pre, 64 * c + 8 * q)
        return carry

    lax.fori_loop(0, PRE // 128, ln_body, 0)

    raw2 = raw.reshape(NCH * 4096, 128)

    def raw_view(p):
        return raw2.at[pl.ds((p >> 2) * 4096 + (p & 3), 4093), :]

    def relayout(src, dst, j, k, not_before=None):
        a = src[pl.ds(512 * k, 64, stride=8), :]
        if not_before is not None:
            a = a | jnp.concatenate([not_before & zero_box[0]] * 8, axis=0)
        b = src[pl.ds(512 * k + 4, 64, stride=8), :]
        rows = pl.ds(64 * k, 64)
        dst[2 * j, rows, :] = (a & jnp.uint32(0xFFFF)) | (b << 16)
        dst[2 * j + 1, rows, :] = (a >> 16) | (b & jnp.uint32(0xFFFF0000))

    def pre_dot(w_view, ring_view, j, k, dep=None):
        i, q = k // 4, k % 4
        lhs = jnp.concatenate([_u2b(xn_pre[kk, pl.ds(64 * q, 64), :]) for kk in range(KT)], axis=1)
        y = _dot(lhs, _u2b(_after(w_view[2 * j + i], dep, zero_box[0])))
        yp = _b2u(y.astype(BF))
        ring_view[2 * j + i, pl.ds(32 + 64 * q, 64), :] = yp
        return yp[0:8]

    w_wait(0)
    for k in range(8):
        relayout(raw_view(0), wqkv, 0, k)

    def pre_body(t, carry):
        x_piece(t).wait()

        @pl.when(((t & 3) != 0) & (t < NPRE - 1))
        def _():
            w_wait((3 * t + 3) >> 2)

        fresh_zero()
        deps = {}
        w_view = wqkv.at[pl.ds(6 * t, 8)]
        ring_view = ring.at[pl.ds(6 * t, 6)]
        srcs = [raw_view(jnp.minimum(3 * t + 1 + j, 4 * NCH - 1)) for j in range(3)]
        done = None
        for v in range(24):
            j, k = v // 8, v % 8
            prev = done
            done = pre_dot(w_view, ring_view, j, k, deps.get(v))
            for jr, kr in REL_SCHED.get(v, ()):
                relayout(srcs[jr], w_view, jr + 1, kr, prev if REL_NB else None)
                deps.setdefault(v + REL_LAG, []).append(w_view[2 * jr + 3, pl.ds(64 * kr + 56, 8), :])
            if v % 3 == 0 and v < 18:
                q = v // 3
                hrow = pl.multiple_of(64 * t, 64) + 32 * (q // 3) + 8 * (q % 3)
                layernorm16(PRE + 96 * t + 16 * q, hbuf, hrow, done if v else None)
                deps.setdefault(v + LN_LAG, []).append(hbuf[KT - 1, pl.ds(hrow, 8), :])
        return carry

    lax.fori_loop(0, NPRE, pre_body, 0)
    for c in ffn_copies:
        c.start()

    row = lax.broadcasted_iota(jnp.int32, (80, 80), 0)
    col = lax.broadcasted_iota(jnp.int32, (80, 80), 1)
    same_head = (jnp.where(row < 64, row >> 5, (row - 64) >> 3)
                 == jnp.where(col < 64, col >> 5, (col - 64) >> 3))
    allowed = same_head & ((col >= 64) | (row >= 64) | (col <= row))
    fill = jnp.where(same_head, -1e9, -jnp.inf).astype(F32)
    low_half = lax.broadcasted_iota(jnp.int32, (8, 128), 0) < 4
    high_half = jnp.logical_not(low_half)
    scale = DH ** -0.5

    def load_row(t):
        w = jnp.concatenate([xn_t[k, pl.ds(t // 2, 1), :] for k in range(KT)], axis=1)
        bits = jnp.where(t % 2 == 0, w << 16, w & jnp.uint32(0xFFFF0000))
        return pltpu.bitcast(bits, F32), w

    def select_tokens():
        r = r_s[...]
        tok = lane16 * 16 + lax.broadcasted_iota(jnp.int32, (16, 128), 0)
        top1 = jnp.max(r)
        idx1 = jnp.min(jnp.where(r == top1, tok, S - 1))
        r2 = jnp.where(tok == idx1, -jnp.inf, r)
        top2 = jnp.max(r2)
        idx2 = jnp.min(jnp.where((r2 == top2) & (tok != idx1), tok, S - 1))
        idx_s[0] = idx1
        idx_s[1] = idx2
        gate_s[...] = jnp.where(lax.broadcasted_iota(jnp.int32, (16, 128), 0) == 0, top1, top2)
        sel_row = lax.broadcasted_iota(jnp.int32, (16, D), 0)
        xs1, _ = load_row(idx1)
        xs2, _ = load_row(idx2)
        xsel_s[...] = _b2u(jnp.where(sel_row == 0, xs1, jnp.where(sel_row == 1, xs2, 0.0)).astype(BF))

    def one_step(i, u, mem):
        odd = u % 2
        s2 = i * (UNROLL // 2) + u // 2
        h_ld = pl.multiple_of(32 * s2, 32)
        r24 = pl.multiple_of((XS * s2) % RING32, 8)
        a24 = pl.multiple_of(XS * s2, 8)
        qkv_ld = pl.multiple_of((SEG * s2 + 32) % RING32, 32) + 16 * odd
        o_st = pl.multiple_of((SEG * s2) % RING32, 32) + 16 * odd
        m0 = 0 if odd else XS

        def with_mem(ref, idx, base, m):
            lo = ref[idx, pl.ds(base + 8 * odd, 8), :]
            hi = ref[idx, pl.ds(base + 8 + 8 * odd, 8), :]
            if odd:
                lo = jnp.where(low_half, m, lo)
            else:
                hi = jnp.where(low_half, hi, m)
            return _u2b(jnp.concatenate([lo, hi], axis=0))

        def store_tokens(ref, idx, base, yp):
            if odd:
                pltpu.store(ref.at[idx, pl.ds(base + 8, 8), :], yp[0:8], mask=high_half)
                ref[idx, pl.ds(base + 16, 8), :] = yp[8:16]
            else:
                ref[idx, pl.ds(base, 8), :] = yp[0:8]
                pltpu.store(ref.at[idx, pl.ds(base + 8, 8), :], yp[8:16], mask=low_half)

        lk = [with_mem(hbuf, k, h_ld, mem[k]) for k in range(KT)]
        lhs = jnp.concatenate(lk, axis=1)

        ymem = {}
        xs = {}
        probs = {}
        parts = {}

        def proj(h):
            split = h < K_SPLIT and u > 0
            if split:
                lhs7 = jnp.concatenate(lk[:KT - 1], axis=1)
                head = [_dot(lhs7, _u2b(wqkv[m * H + h, pl.ds(0, 448), :])) for m in range(3)]
            for m in range(3):
                if split:
                    y = _dot(lk[KT - 1], _u2b(wqkv[m * H + h, pl.ds(448, 64), :])) + head[m]
                else:
                    y = _dot(lhs, _u2b(wqkv[m * H + h]))
                store_tokens(ring, m * H + h, r24, _b2u(y.astype(BF)))
                ymem[(h, m)] = y[m0:m0 + MEM]
                xs[(h, m)] = ring[m * H + h, pl.ds(qkv_ld, SEG // 2), :]

        def pair(p, m):
            a, b = 2 * p, 2 * p + 1
            mm = jnp.concatenate([ymem[(a, m)], ymem[(b, m)]], axis=0).astype(BF)
            return jnp.concatenate([_u2b(xs[(a, m)]), _u2b(xs[(b, m)]), mm], axis=0)

        def qk(p):
            sc = _dot_nt(pair(p, 0), pair(p, 1))
            sc = jnp.where(allowed, sc * scale, fill)
            e = jnp.exp(sc - jnp.max(sc, axis=1, keepdims=True))
            l = jnp.sum(e, axis=1, keepdims=True)
            r = pl.reciprocal(l, approx=True)
            r = r * (2.0 - l * r)
            probs[p] = (e * r).astype(BF)

        def pv(p):
            op = _b2u(_dot(probs[p], pair(p, 2)).astype(BF))
            om = op[32:40]
            om_sw = pltpu.roll(om, 4, axis=0)
            for j, h in enumerate((2 * p, 2 * p + 1)):
                oring[h, pl.ds(o_st, SEG // 2), :] = op[16 * j:16 * j + 16]
                parts[h] = with_mem(oring, h, r24, om if j != odd else om_sw)

        def after(t):
            for lag, fn in ((LAG_QK, qk), (LAG_PV, pv)):
                if (t - 1 - lag) % 2 == 0 and 0 <= (t - 1 - lag) // 2 < NPAIR:
                    fn((t - 1 - lag) // 2)

        for t in range(H):
            proj(t)
            after(t)
            if u == 0 and t == 8:
                select_tokens()
        t = H
        lhs_a = jnp.concatenate([parts[j] for j in range(H_SPLIT)], axis=1)
        acc = []
        for n in range(N_PART):
            acc.append(_dot(lhs_a, _u2b(wo_s[n, pl.ds(0, H_SPLIT * 64), :])))
            after(t)
            t += 1
        while t - 1 - LAG_PV <= 2 * (NPAIR - 1):
            after(t)
            t += 1
        lhs_b = jnp.concatenate([parts[j] for j in range(H_SPLIT, H)], axis=1)
        lhs_o = jnp.concatenate([lhs_a, lhs_b], axis=1)
        new_mem = [None] * KT

        def finish(n, y):
            store_tokens(abuf, n, a24, _b2u(y.astype(BF)))
            ym = y[m0:m0 + MEM]
            new_mem[n] = _b2u(jnp.concatenate([ym, ym], axis=0).astype(BF))

        for n in range(N_PART, KT):
            finish(n, _dot(lhs_o, _u2b(wo_s[n])))
            if n == N_PART:
                for n2 in range(N_PART):
                    tail = _u2b(wo_s[n2, pl.ds(H_SPLIT * 64, (H - H_SPLIT) * 64), :])
                    finish(n2, _dot(lhs_b, tail) + acc[n2])
        return new_mem

    def body(i, mem):
        mem = list(mem)
        for u in range(UNROLL):
            mem = one_step(i, u, mem)
        return tuple(mem)

    for n in range(KT):
        wo_copy(n).wait()
    mi = mem0_s[...].astype(F32)
    mip = _b2u(jnp.concatenate([mi, mi], axis=0).astype(BF))
    lax.fori_loop(0, NSEG // UNROLL, body,
                  tuple(mip[:, 128 * k:128 * (k + 1)] for k in range(KT)))

    early = S - PRE
    zrow = pl.multiple_of(zero_s[0], 16)
    FPER = 9

    def half_rows(r0):
        return r0 // 2 if isinstance(r0, int) else pl.multiple_of(r0 // 2, 8)

    def combine(r0, nrows, n, a):
        xf = x_s[pl.ds(r0, nrows), pl.ds(128 * n, 128)].astype(F32)
        b = _u2b(xn_t[n, pl.ds(half_rows(r0), nrows // 2), :]).astype(F32)
        out_s[pl.ds(r0, nrows), pl.ds(128 * n, 128)] = (_rbf(xf + a) + b).astype(BF)

    def combine_stored(r0, nrows, not_before=None):
        for n in range(KT):
            a = abuf[n, pl.ds(half_rows(r0), nrows // 2), :]
            if not_before is not None:
                a = a | jnp.concatenate([not_before & zero_box[0]] * (nrows // 16), axis=0)
            combine(r0, nrows, n, _u2b(a).astype(F32))

    def out_copy(r0, nrows, j):
        return pltpu.make_async_copy(out_s.at[pl.ds(r0, nrows), :], out_hbm.at[pl.ds(r0, nrows), :],
                                     sems.at[SEM_OUT + j])

    def ffn_groups(j0, count, y, done):
        x_sel = _u2b(xsel_s[...])
        hid = {}

        def up(w_ref, j, key):
            part = _dot(x_sel[:, 0:512], _u2b(w_ref[j, pl.ds(0, 256), :]))
            yield
            hid[key] = _rbf(_dot(x_sel[:, 512:1024], _u2b(w_ref[j, pl.ds(256, 256), :])) + part)
            yield

        def down(jj):
            g = hid[("g", jj)]
            hb = (_rbf(g * _rbf(jax.nn.sigmoid(g))) * hid[("u", jj)]).astype(BF)
            rows = pl.ds(pl.multiple_of(64 * (j0 + jj), 64), 64)
            for half in range(2):
                w = jnp.concatenate([_u2b(wd_s[4 * half + n, rows, :]) for n in range(4)], axis=1)
                y[half] = _dot(hb, w) + y[half]
                yield

        for jj in range(count + 1):
            if jj < count:
                yield from up(wg_s, j0 + jj, ("g", jj))
                yield from up(wu_s, j0 + jj, ("u", jj))
            elif count == 1:
                yield
                yield
            if jj >= 1:
                yield from down(jj - 1)
        done()

    def epi_chunk(r0, side, pieces, keep):
        p0 = (r0 % RING) // 2
        p1 = ((r0 + 64) % RING) // 2
        if not isinstance(r0, int):
            p0, p1 = pl.multiple_of(p0, 32), pl.multiple_of(p1, 32)
        fresh_zero()
        deps = {}
        for n in range(KT):
            acc = None
            for g in range(8):
                lhs = jnp.concatenate(
                    [_u2b(jnp.concatenate([oring[h, pl.ds(p0, 32), :], oring[h, pl.ds(p1, 32), :]], axis=0))
                     for h in range(4 * g, 4 * g + 4)], axis=1)
                w = _after(wo_s[n, pl.ds(256 * g, 256), :], deps.get(8 * n + g), zero_box[0])
                y = _dot(lhs, _u2b(w))
                acc = y if acc is None else y + acc
                next(side, None)
                v = 8 * n + g
                if pieces is not None and v in EPI_SCHED:
                    r1 = pieces + 32 * EPI_SCHED.index(v)
                    combine_stored(r1, 32, pltpu.bitcast(acc[0:8], U32) if EPI_NB else None)
                    if EPI_LAG:
                        deps[v + EPI_LAG] = [_b2u(out_s[pl.ds(r1 + (zrow if EPI_ALIAS else 0), 16), pl.ds(D - 128, 128)])]
            ab = acc.astype(BF)
            if keep:
                abuf[n, pl.ds(half_rows(r0), 64), :] = _b2u(ab)
            combine(r0, 128, n, ab.astype(F32))

    for c in ffn_copies:
        c.wait()

    def epi_body(c, y):
        y = list(y)
        r0 = pl.multiple_of(early + 128 * c, 128)
        e0 = pl.multiple_of(512 * c, 512)
        epi_chunk(r0, ffn_groups(FPER * c, FPER, y, lambda: None), e0, True)
        out_copy(r0, 128, c).start()
        out_copy(e0, 512, 4 + c).start()
        return tuple(y)

    y = list(lax.fori_loop(0, 3, epi_body, (jnp.zeros((16, 512), F32), jnp.zeros((16, 512), F32))))
    idx1 = idx_s[0]
    idx2 = idx_s[1]

    def patch_row(t, yrow):
        xr, w = load_row(t)
        bits = pltpu.bitcast(_rbf(xr + yrow), U32)
        w = jnp.where(t % 2 == 0,
                      (w & jnp.uint32(0xFFFF0000)) | (bits >> 16),
                      (w & jnp.uint32(0xFFFF)) | bits)
        for k in range(KT):
            xn_t[k, pl.ds(t // 2, 1), :] = w[:, 128 * k:128 * (k + 1)]

    def patch():
        gate = _rbf(jax.nn.sigmoid(gate_s[:, 0:1]))
        yy = _rbf(_rbf(jnp.concatenate(y, axis=1)) * gate)
        patch_row(idx1, yy[0:1])
        patch_row(idx2, yy[1:2])

    last = S - 128
    epi_chunk(last, ffn_groups(3 * FPER, 1, y, patch), None, False)
    out_copy(last, 128, 3).start()
    for c in range(3):
        out_copy(early + 128 * c, 128, c).wait()
        out_copy(512 * c, 512, 4 + c).wait()
    blk1 = jnp.minimum(idx1 // 16, last // 16 - 1)
    blk2 = jnp.minimum(idx2 // 16, last // 16 - 1)
    blk2 = jnp.where(blk2 == blk1, jnp.where(blk1 == 0, 1, blk1 - 1), blk2)
    fix = []
    for j, blk in enumerate((blk1, blk2)):
        r0 = pl.multiple_of(blk * 16, 16)
        combine_stored(r0, 16)
        fix.append(out_copy(r0, 16, 7 + j))
    for cp in fix:
        cp.start()
    out_copy(last, 128, 3).wait()
    for cp in fix:
        cp.wait()


@jax.jit
def pallas_parallel_sum__memory_aug_recurrent_mem_tr__moe_arch_mod__prompt_kernel(
    A_x: jax.Array,
    A_mem0: jax.Array,
    A_Wq: jax.Array,
    A_Wk: jax.Array,
    A_Wv: jax.Array,
    A_Wo: jax.Array,
    A_seg_len: jax.Array,
    B_x: jax.Array,
    B_w_r: jax.Array,
    B_w_gate: jax.Array,
    B_w_up: jax.Array,
    B_w_down: jax.Array,
):
    del A_seg_len, B_x
    assert A_x.shape == (1, S, D) and A_mem0.shape == (1, MEM, D)
    assert A_Wq.shape == (D, H, DH) and A_Wo.shape == (H, DH, D)
    assert B_w_gate.shape == (D, FF) and B_w_down.shape == (FF, D)
    any_spec = pl.BlockSpec(memory_space=pl.ANY)
    out = pl.pallas_call(
        _kernel,
        out_shape=jax.ShapeDtypeStruct((S, D), BF),
        in_specs=[any_spec] * 10,
        out_specs=any_spec,
        scratch_shapes=[
            pltpu.VMEM((S, D), BF),
            pltpu.VMEM((KT, S // 2, 128), U32),
            pltpu.VMEM((KT, PRE // 2, 128), U32),
            pltpu.VMEM((KT, 16 * NSEG, 128), U32),
            pltpu.VMEM((3 * H + 2, D // 2, 128), U32),
            pltpu.VMEM((KT, H * DH // 2, 128), U32),
            pltpu.VMEM((3 * H, RING32, 128), U32),
            pltpu.VMEM((H, RING32, 128), U32),
            pltpu.VMEM((KT, S // 2, 128), U32),
            pltpu.VMEM((S, D), BF),
            pltpu.VMEM((NCH, D // 2, 8, 128), U32),
            pltpu.VMEM((FT, D // 2, 128), U32),
            pltpu.VMEM((FT, D // 2, 128), U32),
            pltpu.VMEM((KT, FF // 2, 128), U32),
            pltpu.VMEM((MEM, D), BF),
            pltpu.VMEM((D,), BF),
            pltpu.VMEM((8, D), F32),
            pltpu.VMEM((16, 128), F32),
            pltpu.VMEM((8, D), U32),
            pltpu.VMEM((16, 128), F32),
            pltpu.SMEM((1,), jnp.int32),
            pltpu.SMEM((2,), jnp.int32),
            pltpu.SemaphoreType.DMA((NSEM,)),
        ],
        compiler_params=pltpu.CompilerParams(vmem_limit_bytes=126 * 1024 * 1024),
    )(A_x.reshape(S, D), A_mem0.reshape(MEM, D), A_Wq.reshape(D // 2, 2, H, DH), A_Wk.reshape(D // 2, 2, H, DH),
      A_Wv.reshape(D // 2, 2, H, DH), A_Wo.reshape(H * DH, D),
      B_w_r, B_w_gate, B_w_up, B_w_down)
    return out.reshape(1, S, D)
```

```python
import jax
import jax.numpy as jnp
from jax import lax
import jax.experimental.pallas as pl
import jax.experimental.pallas.tpu as pltpu

BF = jnp.bfloat16
U32 = jnp.uint32
F32 = jnp.float32

S = 2048
D = 1024
H = 32
DH = 128
MEM = 8
SEG = 32
NSEG = S // SEG
FF = 3584
KT = D // 128
FT = FF // 128
XS = 24
PRE = S - NSEG * XS
RING = 576
RING32 = RING // 2
NPAIR = H // 2
NCH = 12
NPRE = 16
SEM_SMALL, SEM_X, SEM_W = 0, 2, 3 + NPRE
SEM_WO, SEM_FFN, SEM_OUT = SEM_W + NCH, SEM_W + NCH + 1, SEM_W + NCH + 2
NSEM = SEM_OUT + 9

LAG_QK = 1
LAG_PV = 4
N_PART = 4
H_SPLIT = 26
REL_SCHED = {0: [(0, 0), (0, 1)], 1: [(0, 2), (0, 3)], 2: [(0, 4)], 3: [(0, 5)], 4: [(0, 6)], 5: [(0, 7)]}
REL_SCHED.update({6 + k: [(1, k)] for k in range(8)})
REL_SCHED.update({14 + k: [(2, k)] for k in range(8)})
K_SPLIT = 2
EPI_SCHED = [8 * n + g for n in range(8) for g in range(2)]
EPI_LAG = 0
EPI_NB = False
EPI_ALIAS = False
LN_LAG = 5
REL_NB = True
REL_LAG = 2
UNROLL = 4


def _b2u(x):
    return pltpu.bitcast(x, U32)


def _u2b(x):
    return pltpu.bitcast(x, BF)


def _dot(a, b):
    return jnp.dot(a, b, preferred_element_type=F32)


def _dot_nt(a, b):
    return lax.dot_general(a, b, (((1,), (1,)), ((), ())), preferred_element_type=F32)


def _after(w, dep, zero):
    if not dep:
        return w
    d = dep[0]
    for e in dep[1:]:
        d = d | e
    return jnp.concatenate([w[0:8] | (d & zero), w[8:]], axis=0)


def _rbf(x):
    return x.astype(BF).astype(F32)


def _kernel(x_hbm, mem0_hbm, wq_hbm, wk_hbm, wv_hbm, wo_hbm, wr_hbm, wg_hbm, wu_hbm, wd_hbm,
            out_hbm,
            x_s, xn_t, xn_pre, hbuf, wqkv, wo_s, ring, oring, abuf, out_s, raw,
            wg_s, wu_s, wd_s, mem0_s, wr_s, wrf_s, r_s, xsel_s, gate_s, zero_s, idx_s,
            sems):
    w32 = [w.bitcast(U32) for w in (wq_hbm, wk_hbm, wv_hbm)]
    wo32 = wo_hbm.bitcast(U32)
    wg32 = wg_hbm.bitcast(U32)
    wu32 = wu_hbm.bitcast(U32)
    wd32 = wd_hbm.bitcast(U32)

    x_first = pltpu.make_async_copy(x_hbm.at[pl.ds(0, PRE), :], x_s.at[pl.ds(0, PRE), :], sems.at[SEM_X])

    def x_piece(c):
        r0 = PRE + 96 * c if isinstance(c, int) else pl.multiple_of(PRE + 96 * c, 32)
        return pltpu.make_async_copy(x_hbm.at[pl.ds(r0, 96), :], x_s.at[pl.ds(r0, 96), :],
                                     sems.at[SEM_X + 1 + c])

    def w_start(c):
        for par in range(2):
            pltpu.make_async_copy(w32[c // 4].at[:, par, pl.ds(4 * (c % 4), 4), :],
                                  raw.at[c, :, pl.ds(4 * par, 4), :], sems.at[SEM_W + c]).start()

    def w_wait(c):
        pltpu.make_async_copy(raw.at[c], raw.at[c], sems.at[SEM_W + c]).wait()

    def wo_copy(n):
        return pltpu.make_async_copy(wo32.at[:, pl.ds(128 * n, 128)], wo_s.at[n], sems.at[SEM_WO])

    small_copies = [pltpu.make_async_copy(mem0_hbm, mem0_s, sems.at[SEM_SMALL]),
                    pltpu.make_async_copy(wr_hbm, wr_s, sems.at[SEM_SMALL + 1])]
    ffn_copies = (
        [pltpu.make_async_copy(wg32.at[:, pl.ds(128 * j, 128)], wg_s.at[j], sems.at[SEM_FFN]) for j in range(FT)]
        + [pltpu.make_async_copy(wu32.at[:, pl.ds(128 * j, 128)], wu_s.at[j], sems.at[SEM_FFN]) for j in range(FT)]
        + [pltpu.make_async_copy(wd32.at[:, pl.ds(128 * n, 128)], wd_s.at[n], sems.at[SEM_FFN]) for n in range(KT)])

    zero_s[0] = 0
    x_first.start()
    for c in small_copies:
        c.start()
    for c in range(NCH):
        w_start(c)
        for t in range(NPRE):
            if min(3 * t + 3, 4 * NCH - 1) // 4 == c + 1 or (c == 0 and t == 0):
                x_piece(t).start()
    for n in range(KT):
        wo_copy(n).start()
    eps_bf = 1.0013580322265625e-05

    def layernorm16(rq, dst_ref, dst_row, not_before=None):
        rq = pl.multiple_of(rq, 16)
        xf = x_s[pl.ds(rq, 16), :].astype(F32)
        if not_before is not None:
            x0 = _after(pltpu.bitcast(xf[:, 0:128], U32), [not_before], zero_box[0])
            xf = jnp.concatenate([pltpu.bitcast(x0, F32), xf[:, 128:]], axis=1)
        mean = jnp.sum(xf, axis=1, keepdims=True) * (1.0 / D)
        cen = xf - mean
        var = jnp.sum(cen * cen, axis=1, keepdims=True) * (1.0 / D)
        sd = _rbf(jnp.sqrt(_rbf(_rbf(var) + eps_bf)))
        xn = (_rbf(xf - _rbf(mean)) * (1.0 / sd)).astype(BF)
        wr = jnp.concatenate([wrf_s[...], wrf_s[...]], axis=0)
        score = _rbf(jnp.sum(xn.astype(F32) * wr, axis=1, keepdims=True))
        r_s[...] = jnp.where(lane16 == rq // 16, score, r_s[...])
        xp = _b2u(xn)
        hq = pl.multiple_of(rq // 2, 8)
        dst_row = pl.multiple_of(dst_row, 8)
        for k in range(KT):
            xn_t[k, pl.ds(hq, 8), :] = xp[:, 128 * k:128 * (k + 1)]
            dst_ref[k, pl.ds(dst_row, 8), :] = xp[:, 128 * k:128 * (k + 1)]

    zero_box = [None]

    def fresh_zero():
        zero_box[0] = jnp.full((8, 128), zero_s[0], jnp.int32).astype(U32)

    r_s[...] = jnp.full(r_s.shape, -jnp.inf, F32)
    lane16 = lax.broadcasted_iota(jnp.int32, (16, 128), 1)
    x_first.wait()
    for c in small_copies:
        c.wait()
    wrf_s[...] = jnp.broadcast_to(wr_s[...].astype(F32).reshape(1, D), (8, D))

    def ln_body(c, carry):
        for q in range(8):
            layernorm16(128 * c + 16 * q, xn_pre, 64 * c + 8 * q)
        return carry

    lax.fori_loop(0, PRE // 128, ln_body, 0)

    raw2 = raw.reshape(NCH * 4096, 128)

    def raw_view(p):
        return raw2.at[pl.ds((p >> 2) * 4096 + (p & 3), 4093), :]

    def relayout(src, dst, j, k, not_before=None):
        a = src[pl.ds(512 * k, 64, stride=8), :]
        if not_before is not None:
            a = a | jnp.concatenate([not_before & zero_box[0]] * 8, axis=0)
        b = src[pl.ds(512 * k + 4, 64, stride=8), :]
        rows = pl.ds(64 * k, 64)
        dst[2 * j, rows, :] = (a & jnp.uint32(0xFFFF)) | (b << 16)
        dst[2 * j + 1, rows, :] = (a >> 16) | (b & jnp.uint32(0xFFFF0000))

    def pre_dot(w_view, ring_view, j, k, dep=None):
        i, q = k // 4, k % 4
        lhs = jnp.concatenate([_u2b(xn_pre[kk, pl.ds(64 * q, 64), :]) for kk in range(KT)], axis=1)
        y = _dot(lhs, _u2b(_after(w_view[2 * j + i], dep, zero_box[0])))
        yp = _b2u(y.astype(BF))
        ring_view[2 * j + i, pl.ds(32 + 64 * q, 64), :] = yp
        return yp[0:8]

    w_wait(0)
    for k in range(8):
        relayout(raw_view(0), wqkv, 0, k)

    def pre_body(t, carry):
        x_piece(t).wait()

        @pl.when(((t & 3) != 0) & (t < NPRE - 1))
        def _():
            w_wait((3 * t + 3) >> 2)

        fresh_zero()
        deps = {}
        w_view = wqkv.at[pl.ds(6 * t, 8)]
        ring_view = ring.at[pl.ds(6 * t, 6)]
        srcs = [raw_view(jnp.minimum(3 * t + 1 + j, 4 * NCH - 1)) for j in range(3)]
        done = None
        for v in range(24):
            j, k = v // 8, v % 8
            prev = done
            done = pre_dot(w_view, ring_view, j, k, deps.get(v))
            for jr, kr in REL_SCHED.get(v, ()):
                relayout(srcs[jr], w_view, jr + 1, kr, prev if REL_NB else None)
                deps.setdefault(v + REL_LAG, []).append(w_view[2 * jr + 3, pl.ds(64 * kr + 56, 8), :])
            if v % 3 == 0 and v < 18:
                q = v // 3
                hrow = pl.multiple_of(64 * t, 64) + 32 * (q // 3) + 8 * (q % 3)
                layernorm16(PRE + 96 * t + 16 * q, hbuf, hrow, done if v else None)
                deps.setdefault(v + LN_LAG, []).append(hbuf[KT - 1, pl.ds(hrow, 8), :])
        return carry

    lax.fori_loop(0, NPRE, pre_body, 0)
    for c in ffn_copies:
        c.start()

    row = lax.broadcasted_iota(jnp.int32, (80, 80), 0)
    col = lax.broadcasted_iota(jnp.int32, (80, 80), 1)
    same_head = (jnp.where(row < 64, row >> 5, (row - 64) >> 3)
                 == jnp.where(col < 64, col >> 5, (col - 64) >> 3))
    allowed = same_head & ((col >= 64) | (row >= 64) | (col <= row))
    fill = jnp.where(same_head, -1e9, -jnp.inf).astype(F32)
    low_half = lax.broadcasted_iota(jnp.int32, (8, 128), 0) < 4
    high_half = jnp.logical_not(low_half)
    scale = DH ** -0.5

    def load_row(t):
        w = jnp.concatenate([xn_t[k, pl.ds(t // 2, 1), :] for k in range(KT)], axis=1)
        bits = jnp.where(t % 2 == 0, w << 16, w & jnp.uint32(0xFFFF0000))
        return pltpu.bitcast(bits, F32), w

    def select_tokens():
        r = r_s[...]
        tok = lane16 * 16 + lax.broadcasted_iota(jnp.int32, (16, 128), 0)
        top1 = jnp.max(r)
        idx1 = jnp.min(jnp.where(r == top1, tok, S - 1))
        r2 = jnp.where(tok == idx1, -jnp.inf, r)
        top2 = jnp.max(r2)
        idx2 = jnp.min(jnp.where((r2 == top2) & (tok != idx1), tok, S - 1))
        idx_s[0] = idx1
        idx_s[1] = idx2
        gate_s[...] = jnp.where(lax.broadcasted_iota(jnp.int32, (16, 128), 0) == 0, top1, top2)
        sel_row = lax.broadcasted_iota(jnp.int32, (16, D), 0)
        xs1, _ = load_row(idx1)
        xs2, _ = load_row(idx2)
        xsel_s[...] = _b2u(jnp.where(sel_row == 0, xs1, jnp.where(sel_row == 1, xs2, 0.0)).astype(BF))

    def one_step(i, u, mem):
        odd = u % 2
        s2 = i * (UNROLL // 2) + u // 2
        h_ld = pl.multiple_of(16 * UNROLL * i, 32) + 32 * (u // 2)
        a24 = pl.multiple_of(12 * UNROLL * i, 8)
        r24 = pl.multiple_of(a24 % RING32, 8) + XS * (u // 2)
        a24 = a24 + XS * (u // 2)
        qkv_ld = pl.multiple_of((SEG * s2 + 32) % RING32, 32) + 16 * odd
        o_st = pl.multiple_of((SEG * s2) % RING32, 32) + 16 * odd
        m0 = 0 if odd else XS

        def with_mem(ref, idx, base, m):
            lo = ref[idx, pl.ds(base + 8 * odd, 8), :]
            hi = ref[idx, pl.ds(base + 8 + 8 * odd, 8), :]
            if odd:
                lo = jnp.where(low_half, m, lo)
            else:
                hi = jnp.where(low_half, hi, m)
            return _u2b(jnp.concatenate([lo, hi], axis=0))

        def store_tokens(ref, idx, base, yp):
            if odd:
                pltpu.store(ref.at[idx, pl.ds(base + 8, 8), :], yp[0:8], mask=high_half)
                ref[idx, pl.ds(base + 16, 8), :] = yp[8:16]
            else:
                ref[idx, pl.ds(base, 8), :] = yp[0:8]
                pltpu.store(ref.at[idx, pl.ds(base + 8, 8), :], yp[8:16], mask=low_half)

        lk = [with_mem(hbuf, k, h_ld, mem[k]) for k in range(KT)]
        lhs = jnp.concatenate(lk, axis=1)

        ymem = {}
        xs = {}
        probs = {}
        parts = {}

        def proj(h):
            split = h < K_SPLIT and u > 0
            if split:
                lhs7 = jnp.concatenate(lk[:KT - 1], axis=1)
                head = [_dot(lhs7, _u2b(wqkv[m * H + h, pl.ds(0, 448), :])) for m in range(3)]
            for m in range(3):
                if split:
                    y = _dot(lk[KT - 1], _u2b(wqkv[m * H + h, pl.ds(448, 64), :])) + head[m]
                else:
                    y = _dot(lhs, _u2b(wqkv[m * H + h]))
                store_tokens(ring, m * H + h, r24, _b2u(y.astype(BF)))
                ymem[(h, m)] = y[m0:m0 + MEM]
                xs[(h, m)] = ring[m * H + h, pl.ds(qkv_ld, SEG // 2), :]

        def pair(p, m):
            a, b = 2 * p, 2 * p + 1
            mm = jnp.concatenate([ymem[(a, m)], ymem[(b, m)]], axis=0).astype(BF)
            return jnp.concatenate([_u2b(xs[(a, m)]), _u2b(xs[(b, m)]), mm], axis=0)

        def qk(p):
            sc = _dot_nt(pair(p, 0), pair(p, 1))
            sc = jnp.where(allowed, sc * scale, fill)
            e = jnp.exp(sc - jnp.max(sc, axis=1, keepdims=True))
            l = jnp.sum(e, axis=1, keepdims=True)
            r = pl.reciprocal(l, approx=True)
            r = r * (2.0 - l * r)
            probs[p] = (e * r).astype(BF)

        def pv(p):
            op = _b2u(_dot(probs[p], pair(p, 2)).astype(BF))
            om = op[32:40]
            om_sw = pltpu.roll(om, 4, axis=0)
            for j, h in enumerate((2 * p, 2 * p + 1)):
                oring[h, pl.ds(o_st, SEG // 2), :] = op[16 * j:16 * j + 16]
                parts[h] = with_mem(oring, h, r24, om if j != odd else om_sw)

        def after(t):
            for lag, fn in ((LAG_QK, qk), (LAG_PV, pv)):
                if (t - 1 - lag) % 2 == 0 and 0 <= (t - 1 - lag) // 2 < NPAIR:
                    fn((t - 1 - lag) // 2)

        for t in range(H):
            proj(t)
            after(t)
            if u == 0 and t == 8:
                select_tokens()
        t = H
        lhs_a = jnp.concatenate([parts[j] for j in range(H_SPLIT)], axis=1)
        acc = []
        for n in range(N_PART):
            acc.append(_dot(lhs_a, _u2b(wo_s[n, pl.ds(0, H_SPLIT * 64), :])))
            after(t)
            t += 1
        while t - 1 - LAG_PV <= 2 * (NPAIR - 1):
            after(t)
            t += 1
        lhs_b = jnp.concatenate([parts[j] for j in range(H_SPLIT, H)], axis=1)
        lhs_o = jnp.concatenate([lhs_a, lhs_b], axis=1)
        new_mem = [None] * KT

        def finish(n, y):
            store_tokens(abuf, n, a24, _b2u(y.astype(BF)))
            ym = y[m0:m0 + MEM]
            new_mem[n] = _b2u(jnp.concatenate([ym, ym], axis=0).astype(BF))

        for n in range(N_PART, KT):
            finish(n, _dot(lhs_o, _u2b(wo_s[n])))
            if n == N_PART:
                for n2 in range(N_PART):
                    tail = _u2b(wo_s[n2, pl.ds(H_SPLIT * 64, (H - H_SPLIT) * 64), :])
                    finish(n2, _dot(lhs_b, tail) + acc[n2])
        return new_mem

    def body(i, mem):
        mem = list(mem)
        for u in range(UNROLL):
            mem = one_step(i, u, mem)
        return tuple(mem)

    for n in range(KT):
        wo_copy(n).wait()
    mi = mem0_s[...].astype(F32)
    mip = _b2u(jnp.concatenate([mi, mi], axis=0).astype(BF))
    lax.fori_loop(0, NSEG // UNROLL, body,
                  tuple(mip[:, 128 * k:128 * (k + 1)] for k in range(KT)))

    early = S - PRE
    zrow = pl.multiple_of(zero_s[0], 16)
    FPER = 9

    def half_rows(r0):
        return r0 // 2 if isinstance(r0, int) else pl.multiple_of(r0 // 2, 8)

    def combine(r0, nrows, n, a):
        xf = x_s[pl.ds(r0, nrows), pl.ds(128 * n, 128)].astype(F32)
        b = _u2b(xn_t[n, pl.ds(half_rows(r0), nrows // 2), :]).astype(F32)
        out_s[pl.ds(r0, nrows), pl.ds(128 * n, 128)] = (_rbf(xf + a) + b).astype(BF)

    def combine_stored(r0, nrows, not_before=None):
        for n in range(KT):
            a = abuf[n, pl.ds(half_rows(r0), nrows // 2), :]
            if not_before is not None:
                a = a | jnp.concatenate([not_before & zero_box[0]] * (nrows // 16), axis=0)
            combine(r0, nrows, n, _u2b(a).astype(F32))

    def out_copy(r0, nrows, j):
        return pltpu.make_async_copy(out_s.at[pl.ds(r0, nrows), :], out_hbm.at[pl.ds(r0, nrows), :],
                                     sems.at[SEM_OUT + j])

    def ffn_groups(j0, count, y, done):
        x_sel = _u2b(xsel_s[...])
        hid = {}

        def up(w_ref, j, key):
            part = _dot(x_sel[:, 0:512], _u2b(w_ref[j, pl.ds(0, 256), :]))
            yield
            hid[key] = _rbf(_dot(x_sel[:, 512:1024], _u2b(w_ref[j, pl.ds(256, 256), :])) + part)
            yield

        def down(jj):
            g = hid[("g", jj)]
            hb = (_rbf(g * _rbf(jax.nn.sigmoid(g))) * hid[("u", jj)]).astype(BF)
            rows = pl.ds(pl.multiple_of(64 * (j0 + jj), 64), 64)
            for half in range(2):
                w = jnp.concatenate([_u2b(wd_s[4 * half + n, rows, :]) for n in range(4)], axis=1)
                y[half] = _dot(hb, w) + y[half]
                yield

        for jj in range(count + 1):
            if jj < count:
                yield from up(wg_s, j0 + jj, ("g", jj))
                yield from up(wu_s, j0 + jj, ("u", jj))
            elif count == 1:
                yield
                yield
            if jj >= 1:
                yield from down(jj - 1)
        done()

    def epi_chunk(r0, side, pieces, keep):
        p0 = (r0 % RING) // 2
        p1 = ((r0 + 64) % RING) // 2
        if not isinstance(r0, int):
            p0, p1 = pl.multiple_of(p0, 32), pl.multiple_of(p1, 32)
        fresh_zero()
        deps = {}
        for n in range(KT):
            acc = None
            for g in range(8):
                lhs = jnp.concatenate(
                    [_u2b(jnp.concatenate([oring[h, pl.ds(p0, 32), :], oring[h, pl.ds(p1, 32), :]], axis=0))
                     for h in range(4 * g, 4 * g + 4)], axis=1)
                w = _after(wo_s[n, pl.ds(256 * g, 256), :], deps.get(8 * n + g), zero_box[0])
                y = _dot(lhs, _u2b(w))
                acc = y if acc is None else y + acc
                next(side, None)
                v = 8 * n + g
                if pieces is not None and v in EPI_SCHED:
                    r1 = pieces + 32 * EPI_SCHED.index(v)
                    combine_stored(r1, 32, pltpu.bitcast(acc[0:8], U32) if EPI_NB else None)
                    if EPI_LAG:
                        deps[v + EPI_LAG] = [_b2u(out_s[pl.ds(r1 + (zrow if EPI_ALIAS else 0), 16), pl.ds(D - 128, 128)])]
            ab = acc.astype(BF)
            if keep:
                abuf[n, pl.ds(half_rows(r0), 64), :] = _b2u(ab)
            combine(r0, 128, n, ab.astype(F32))

    for c in ffn_copies:
        c.wait()

    def epi_body(c, y):
        y = list(y)
        r0 = pl.multiple_of(early + 128 * c, 128)
        e0 = pl.multiple_of(512 * c, 512)
        epi_chunk(r0, ffn_groups(FPER * c, FPER, y, lambda: None), e0, True)
        out_copy(r0, 128, c).start()
        out_copy(e0, 512, 4 + c).start()
        return tuple(y)

    y = list(lax.fori_loop(0, 3, epi_body, (jnp.zeros((16, 512), F32), jnp.zeros((16, 512), F32))))
    idx1 = idx_s[0]
    idx2 = idx_s[1]

    def patch_row(t, yrow):
        xr, w = load_row(t)
        bits = pltpu.bitcast(_rbf(xr + yrow), U32)
        w = jnp.where(t % 2 == 0,
                      (w & jnp.uint32(0xFFFF0000)) | (bits >> 16),
                      (w & jnp.uint32(0xFFFF)) | bits)
        for k in range(KT):
            xn_t[k, pl.ds(t // 2, 1), :] = w[:, 128 * k:128 * (k + 1)]

    def patch():
        gate = _rbf(jax.nn.sigmoid(gate_s[:, 0:1]))
        yy = _rbf(_rbf(jnp.concatenate(y, axis=1)) * gate)
        patch_row(idx1, yy[0:1])
        patch_row(idx2, yy[1:2])

    last = S - 128
    epi_chunk(last, ffn_groups(3 * FPER, 1, y, patch), None, False)
    out_copy(last, 128, 3).start()
    for c in range(3):
        out_copy(early + 128 * c, 128, c).wait()
        out_copy(512 * c, 512, 4 + c).wait()
    blk1 = jnp.minimum(idx1 // 16, last // 16 - 1)
    blk2 = jnp.minimum(idx2 // 16, last // 16 - 1)
    blk2 = jnp.where(blk2 == blk1, jnp.where(blk1 == 0, 1, blk1 - 1), blk2)
    fix = []
    for j, blk in enumerate((blk1, blk2)):
        r0 = pl.multiple_of(blk * 16, 16)
        combine_stored(r0, 16)
        fix.append(out_copy(r0, 16, 7 + j))
    for cp in fix:
        cp.start()
    out_copy(last, 128, 3).wait()
    for cp in fix:
        cp.wait()


@jax.jit
def pallas_parallel_sum__memory_aug_recurrent_mem_tr__moe_arch_mod__prompt_kernel(
    A_x: jax.Array,
    A_mem0: jax.Array,
    A_Wq: jax.Array,
    A_Wk: jax.Array,
    A_Wv: jax.Array,
    A_Wo: jax.Array,
    A_seg_len: jax.Array,
    B_x: jax.Array,
    B_w_r: jax.Array,
    B_w_gate: jax.Array,
    B_w_up: jax.Array,
    B_w_down: jax.Array,
):
    del A_seg_len, B_x
    assert A_x.shape == (1, S, D) and A_mem0.shape == (1, MEM, D)
    assert A_Wq.shape == (D, H, DH) and A_Wo.shape == (H, DH, D)
    assert B_w_gate.shape == (D, FF) and B_w_down.shape == (FF, D)
    any_spec = pl.BlockSpec(memory_space=pl.ANY)
    out = pl.pallas_call(
        _kernel,
        out_shape=jax.ShapeDtypeStruct((S, D), BF),
        in_specs=[any_spec] * 10,
        out_specs=any_spec,
        scratch_shapes=[
            pltpu.VMEM((S, D), BF),
            pltpu.VMEM((KT, S // 2, 128), U32),
            pltpu.VMEM((KT, PRE // 2, 128), U32),
            pltpu.VMEM((KT, 16 * NSEG, 128), U32),
            pltpu.VMEM((3 * H + 2, D // 2, 128), U32),
            pltpu.VMEM((KT, H * DH // 2, 128), U32),
            pltpu.VMEM((3 * H, RING32, 128), U32),
            pltpu.VMEM((H, RING32, 128), U32),
            pltpu.VMEM((KT, S // 2, 128), U32),
            pltpu.VMEM((S, D), BF),
            pltpu.VMEM((NCH, D // 2, 8, 128), U32),
            pltpu.VMEM((FT, D // 2, 128), U32),
            pltpu.VMEM((FT, D // 2, 128), U32),
            pltpu.VMEM((KT, FF // 2, 128), U32),
            pltpu.VMEM((MEM, D), BF),
            pltpu.VMEM((D,), BF),
            pltpu.VMEM((8, D), F32),
            pltpu.VMEM((16, 128), F32),
            pltpu.VMEM((8, D), U32),
            pltpu.VMEM((16, 128), F32),
            pltpu.SMEM((1,), jnp.int32),
            pltpu.SMEM((2,), jnp.int32),
            pltpu.SemaphoreType.DMA((NSEM,)),
        ],
        compiler_params=pltpu.CompilerParams(vmem_limit_bytes=126 * 1024 * 1024),
    )(A_x.reshape(S, D), A_mem0.reshape(MEM, D), A_Wq.reshape(D // 2, 2, H, DH), A_Wk.reshape(D // 2, 2, H, DH),
      A_Wv.reshape(D // 2, 2, H, DH), A_Wo.reshape(H * DH, D),
      B_w_r, B_w_gate, B_w_up, B_w_down)
    return out.reshape(1, S, D)
```

```python
import jax
import jax.numpy as jnp
from jax import lax
import jax.experimental.pallas as pl
import jax.experimental.pallas.tpu as pltpu

BF = jnp.bfloat16
U32 = jnp.uint32
F32 = jnp.float32

S = 2048
D = 1024
H = 32
DH = 128
MEM = 8
SEG = 32
NSEG = S // SEG
FF = 3584
KT = D // 128
FT = FF // 128
XS = 24
PRE = S - NSEG * XS
RING = 576
RING32 = RING // 2
NPAIR = H // 2
NCH = 12
NPRE = 16
SEM_SMALL, SEM_X, SEM_W = 0, 2, 3 + NPRE
SEM_WO, SEM_FFN, SEM_OUT = SEM_W + NCH, SEM_W + NCH + 1, SEM_W + NCH + 2
NSEM = SEM_OUT + 9

LAG_QK = 1
LAG_PV = 4
N_PART = 4
H_SPLIT = 26
REL_SCHED = {0: [(0, 0), (0, 1)], 1: [(0, 2), (0, 3)], 2: [(0, 4)], 3: [(0, 5)], 4: [(0, 6)], 5: [(0, 7)]}
REL_SCHED.update({6 + k: [(1, k)] for k in range(8)})
REL_SCHED.update({14 + k: [(2, k)] for k in range(8)})
K_SPLIT = 2
EPI_SCHED = [v * 5 // 2 for v in range(24)]
EPI_LAG = 4
ECH = 160
EPI_NB = False
EPI_ALIAS = False
LN_LAG = 5
REL_NB = True
REL_LAG = 2
UNROLL = 4


def _b2u(x):
    return pltpu.bitcast(x, U32)


def _u2b(x):
    return pltpu.bitcast(x, BF)


def _dot(a, b):
    return jnp.dot(a, b, preferred_element_type=F32)


def _dot_nt(a, b):
    return lax.dot_general(a, b, (((1,), (1,)), ((), ())), preferred_element_type=F32)


def _after(w, dep, zero):
    if not dep:
        return w
    d = dep[0]
    for e in dep[1:]:
        d = d | e
    return jnp.concatenate([w[0:8] | (d & zero), w[8:]], axis=0)


def _rbf(x):
    return x.astype(BF).astype(F32)


def _kernel(x_hbm, mem0_hbm, wq_hbm, wk_hbm, wv_hbm, wo_hbm, wr_hbm, wg_hbm, wu_hbm, wd_hbm,
            out_hbm,
            x_s, xn_t, xn_pre, hbuf, wqkv, wo_s, ring, oring, abuf, out_s, raw,
            wg_s, wu_s, wd_s, mem0_s, wr_s, wrf_s, r_s, xsel_s, gate_s, zero_s, idx_s,
            sems):
    w32 = [w.bitcast(U32) for w in (wq_hbm, wk_hbm, wv_hbm)]
    wo32 = wo_hbm.bitcast(U32)
    wg32 = wg_hbm.bitcast(U32)
    wu32 = wu_hbm.bitcast(U32)
    wd32 = wd_hbm.bitcast(U32)

    x_first = pltpu.make_async_copy(x_hbm.at[pl.ds(0, PRE), :], x_s.at[pl.ds(0, PRE), :], sems.at[SEM_X])

    def x_piece(c):
        r0 = PRE + 96 * c if isinstance(c, int) else pl.multiple_of(PRE + 96 * c, 32)
        return pltpu.make_async_copy(x_hbm.at[pl.ds(r0, 96), :], x_s.at[pl.ds(r0, 96), :],
                                     sems.at[SEM_X + 1 + c])

    def w_start(c):
        for par in range(2):
            pltpu.make_async_copy(w32[c // 4].at[:, par, pl.ds(4 * (c % 4), 4), :],
                                  raw.at[c, :, pl.ds(4 * par, 4), :], sems.at[SEM_W + c]).start()

    def w_wait(c):
        pltpu.make_async_copy(raw.at[c], raw.at[c], sems.at[SEM_W + c]).wait()

    def wo_copy(n):
        return pltpu.make_async_copy(wo32.at[:, pl.ds(128 * n, 128)], wo_s.at[n], sems.at[SEM_WO])

    small_copies = [pltpu.make_async_copy(mem0_hbm, mem0_s, sems.at[SEM_SMALL]),
                    pltpu.make_async_copy(wr_hbm, wr_s, sems.at[SEM_SMALL + 1])]
    ffn_copies = (
        [pltpu.make_async_copy(wg32.at[:, pl.ds(128 * j, 128)], wg_s.at[j], sems.at[SEM_FFN]) for j in range(FT)]
        + [pltpu.make_async_copy(wu32.at[:, pl.ds(128 * j, 128)], wu_s.at[j], sems.at[SEM_FFN]) for j in range(FT)]
        + [pltpu.make_async_copy(wd32.at[:, pl.ds(128 * n, 128)], wd_s.at[n], sems.at[SEM_FFN]) for n in range(KT)])

    zero_s[0] = 0
    x_first.start()
    for c in small_copies:
        c.start()
    for c in range(NCH):
        w_start(c)
        for t in range(NPRE):
            if min(3 * t + 3, 4 * NCH - 1) // 4 == c + 1 or (c == 0 and t == 0):
                x_piece(t).start()
    for n in range(KT):
        wo_copy(n).start()
    eps_bf = 1.0013580322265625e-05

    def layernorm16(rq, dst_ref, dst_row, not_before=None):
        rq = pl.multiple_of(rq, 16)
        xf = x_s[pl.ds(rq, 16), :].astype(F32)
        if not_before is not None:
            x0 = _after(pltpu.bitcast(xf[:, 0:128], U32), [not_before], zero_box[0])
            xf = jnp.concatenate([pltpu.bitcast(x0, F32), xf[:, 128:]], axis=1)
        mean = jnp.sum(xf, axis=1, keepdims=True) * (1.0 / D)
        cen = xf - mean
        var = jnp.sum(cen * cen, axis=1, keepdims=True) * (1.0 / D)
        sd = _rbf(jnp.sqrt(_rbf(_rbf(var) + eps_bf)))
        xn = (_rbf(xf - _rbf(mean)) * (1.0 / sd)).astype(BF)
        wr = jnp.concatenate([wrf_s[...], wrf_s[...]], axis=0)
        score = _rbf(jnp.sum(xn.astype(F32) * wr, axis=1, keepdims=True))
        r_s[...] = jnp.where(lane16 == rq // 16, score, r_s[...])
        xp = _b2u(xn)
        hq = pl.multiple_of(rq // 2, 8)
        dst_row = pl.multiple_of(dst_row, 8)
        for k in range(KT):
            xn_t[k, pl.ds(hq, 8), :] = xp[:, 128 * k:128 * (k + 1)]
            dst_ref[k, pl.ds(dst_row, 8), :] = xp[:, 128 * k:128 * (k + 1)]

    zero_box = [None]

    def fresh_zero():
        zero_box[0] = jnp.full((8, 128), zero_s[0], jnp.int32).astype(U32)

    r_s[...] = jnp.full(r_s.shape, -jnp.inf, F32)
    lane16 = lax.broadcasted_iota(jnp.int32, (16, 128), 1)
    x_first.wait()
    for c in small_copies:
        c.wait()
    wrf_s[...] = jnp.broadcast_to(wr_s[...].astype(F32).reshape(1, D), (8, D))

    def ln_body(c, carry):
        for q in range(8):
            layernorm16(128 * c + 16 * q, xn_pre, 64 * c + 8 * q)
        return carry

    lax.fori_loop(0, PRE // 128, ln_body, 0)

    raw2 = raw.reshape(NCH * 4096, 128)

    def raw_view(p):
        return raw2.at[pl.ds((p >> 2) * 4096 + (p & 3), 4093), :]

    def relayout(src, dst, j, k, not_before=None):
        a = src[pl.ds(512 * k, 64, stride=8), :]
        if not_before is not None:
            a = a | jnp.concatenate([not_before & zero_box[0]] * 8, axis=0)
        b = src[pl.ds(512 * k + 4, 64, stride=8), :]
        rows = pl.ds(64 * k, 64)
        dst[2 * j, rows, :] = (a & jnp.uint32(0xFFFF)) | (b << 16)
        dst[2 * j + 1, rows, :] = (a >> 16) | (b & jnp.uint32(0xFFFF0000))

    def pre_dot(w_view, ring_view, j, k, dep=None):
        i, q = k // 4, k % 4
        lhs = jnp.concatenate([_u2b(xn_pre[kk, pl.ds(64 * q, 64), :]) for kk in range(KT)], axis=1)
        y = _dot(lhs, _u2b(_after(w_view[2 * j + i], dep, zero_box[0])))
        yp = _b2u(y.astype(BF))
        ring_view[2 * j + i, pl.ds(32 + 64 * q, 64), :] = yp
        return yp[0:8]

    w_wait(0)
    for k in range(8):
        relayout(raw_view(0), wqkv, 0, k)

    def pre_body(t, carry):
        x_piece(t).wait()

        @pl.when(((t & 3) != 0) & (t < NPRE - 1))
        def _():
            w_wait((3 * t + 3) >> 2)

        fresh_zero()
        deps = {}
        w_view = wqkv.at[pl.ds(6 * t, 8)]
        ring_view = ring.at[pl.ds(6 * t, 6)]
        srcs = [raw_view(jnp.minimum(3 * t + 1 + j, 4 * NCH - 1)) for j in range(3)]
        done = None
        for v in range(24):
            j, k = v // 8, v % 8
            prev = done
            done = pre_dot(w_view, ring_view, j, k, deps.get(v))
            for jr, kr in REL_SCHED.get(v, ()):
                relayout(srcs[jr], w_view, jr + 1, kr, prev if REL_NB else None)
                deps.setdefault(v + REL_LAG, []).append(w_view[2 * jr + 3, pl.ds(64 * kr + 56, 8), :])
            if v % 3 == 0 and v < 18:
                q = v // 3
                hrow = pl.multiple_of(64 * t, 64) + 32 * (q // 3) + 8 * (q % 3)
                layernorm16(PRE + 96 * t + 16 * q, hbuf, hrow, done if v else None)
                deps.setdefault(v + LN_LAG, []).append(hbuf[KT - 1, pl.ds(hrow, 8), :])
        return carry

    lax.fori_loop(0, NPRE, pre_body, 0)
    for c in ffn_copies:
        c.start()

    row = lax.broadcasted_iota(jnp.int32, (80, 80), 0)
    col = lax.broadcasted_iota(jnp.int32, (80, 80), 1)
    same_head = (jnp.where(row < 64, row >> 5, (row - 64) >> 3)
                 == jnp.where(col < 64, col >> 5, (col - 64) >> 3))
    allowed = same_head & ((col >= 64) | (row >= 64) | (col <= row))
    fill = jnp.where(same_head, -1e9, -jnp.inf).astype(F32)
    low_half = lax.broadcasted_iota(jnp.int32, (8, 128), 0) < 4
    high_half = jnp.logical_not(low_half)
    scale = DH ** -0.5

    def load_row(t):
        w = jnp.concatenate([xn_t[k, pl.ds(t // 2, 1), :] for k in range(KT)], axis=1)
        bits = jnp.where(t % 2 == 0, w << 16, w & jnp.uint32(0xFFFF0000))
        return pltpu.bitcast(bits, F32), w

    def select_tokens():
        r = r_s[...]
        tok = lane16 * 16 + lax.broadcasted_iota(jnp.int32, (16, 128), 0)
        top1 = jnp.max(r)
        idx1 = jnp.min(jnp.where(r == top1, tok, S - 1))
        r2 = jnp.where(tok == idx1, -jnp.inf, r)
        top2 = jnp.max(r2)
        idx2 = jnp.min(jnp.where((r2 == top2) & (tok != idx1), tok, S - 1))
        idx_s[0] = idx1
        idx_s[1] = idx2
        gate_s[...] = jnp.where(lax.broadcasted_iota(jnp.int32, (16, 128), 0) == 0, top1, top2)
        sel_row = lax.broadcasted_iota(jnp.int32, (16, D), 0)
        xs1, _ = load_row(idx1)
        xs2, _ = load_row(idx2)
        xsel_s[...] = _b2u(jnp.where(sel_row == 0, xs1, jnp.where(sel_row == 1, xs2, 0.0)).astype(BF))

    def one_step(i, u, mem):
        odd = u % 2
        s2 = i * (UNROLL // 2) + u // 2
        h_ld = pl.multiple_of(16 * UNROLL * i, 32) + 32 * (u // 2)
        a24 = pl.multiple_of(12 * UNROLL * i, 8)
        r24 = pl.multiple_of(a24 % RING32, 8) + XS * (u // 2)
        a24 = a24 + XS * (u // 2)
        qkv_ld = pl.multiple_of((SEG * s2 + 32) % RING32, 32) + 16 * odd
        o_st = pl.multiple_of((SEG * s2) % RING32, 32) + 16 * odd
        m0 = 0 if odd else XS

        def with_mem(ref, idx, base, m):
            lo = ref[idx, pl.ds(base + 8 * odd, 8), :]
            hi = ref[idx, pl.ds(base + 8 + 8 * odd, 8), :]
            if odd:
                lo = jnp.where(low_half, m, lo)
            else:
                hi = jnp.where(low_half, hi, m)
            return _u2b(jnp.concatenate([lo, hi], axis=0))

        def store_tokens(ref, idx, base, yp):
            if odd:
                pltpu.store(ref.at[idx, pl.ds(base + 8, 8), :], yp[0:8], mask=high_half)
                ref[idx, pl.ds(base + 16, 8), :] = yp[8:16]
            else:
                ref[idx, pl.ds(base, 8), :] = yp[0:8]
                pltpu.store(ref.at[idx, pl.ds(base + 8, 8), :], yp[8:16], mask=low_half)

        lk = [with_mem(hbuf, k, h_ld, mem[k]) for k in range(KT)]
        lhs = jnp.concatenate(lk, axis=1)

        ymem = {}
        xs = {}
        probs = {}
        parts = {}

        def proj(h):
            split = h < K_SPLIT and u > 0
            if split:
                lhs7 = jnp.concatenate(lk[:KT - 1], axis=1)
                head = [_dot(lhs7, _u2b(wqkv[m * H + h, pl.ds(0, 448), :])) for m in range(3)]
            for m in range(3):
                if split:
                    y = _dot(lk[KT - 1], _u2b(wqkv[m * H + h, pl.ds(448, 64), :])) + head[m]
                else:
                    y = _dot(lhs, _u2b(wqkv[m * H + h]))
                store_tokens(ring, m * H + h, r24, _b2u(y.astype(BF)))
                ymem[(h, m)] = y[m0:m0 + MEM]
                xs[(h, m)] = ring[m * H + h, pl.ds(qkv_ld, SEG // 2), :]

        def pair(p, m):
            a, b = 2 * p, 2 * p + 1
            mm = jnp.concatenate([ymem[(a, m)], ymem[(b, m)]], axis=0).astype(BF)
            return jnp.concatenate([_u2b(xs[(a, m)]), _u2b(xs[(b, m)]), mm], axis=0)

        def qk(p):
            sc = _dot_nt(pair(p, 0), pair(p, 1))
            sc = jnp.where(allowed, sc * scale, fill)
            e = jnp.exp(sc - jnp.max(sc, axis=1, keepdims=True))
            l = jnp.sum(e, axis=1, keepdims=True)
            r = pl.reciprocal(l, approx=True)
            r = r * (2.0 - l * r)
            probs[p] = (e * r).astype(BF)

        def pv(p):
            op = _b2u(_dot(probs[p], pair(p, 2)).astype(BF))
            om = op[32:40]
            om_sw = pltpu.roll(om, 4, axis=0)
            for j, h in enumerate((2 * p, 2 * p + 1)):
                oring[h, pl.ds(o_st, SEG // 2), :] = op[16 * j:16 * j + 16]
                parts[h] = with_mem(oring, h, r24, om if j != odd else om_sw)

        def after(t):
            for lag, fn in ((LAG_QK, qk), (LAG_PV, pv)):
                if (t - 1 - lag) % 2 == 0 and 0 <= (t - 1 - lag) // 2 < NPAIR:
                    fn((t - 1 - lag) // 2)

        for t in range(H):
            proj(t)
            after(t)
            if u == 0 and t == 8:
                select_tokens()
        t = H
        lhs_a = jnp.concatenate([parts[j] for j in range(H_SPLIT)], axis=1)
        acc = []
        for n in range(N_PART):
            acc.append(_dot(lhs_a, _u2b(wo_s[n, pl.ds(0, H_SPLIT * 64), :])))
            after(t)
            t += 1
        while t - 1 - LAG_PV <= 2 * (NPAIR - 1):
            after(t)
            t += 1
        lhs_b = jnp.concatenate([parts[j] for j in range(H_SPLIT, H)], axis=1)
        lhs_o = jnp.concatenate([lhs_a, lhs_b], axis=1)
        new_mem = [None] * KT

        def finish(n, y):
            store_tokens(abuf, n, a24, _b2u(y.astype(BF)))
            ym = y[m0:m0 + MEM]
            new_mem[n] = _b2u(jnp.concatenate([ym, ym], axis=0).astype(BF))

        for n in range(N_PART, KT):
            finish(n, _dot(lhs_o, _u2b(wo_s[n])))
            if n == N_PART:
                for n2 in range(N_PART):
                    tail = _u2b(wo_s[n2, pl.ds(H_SPLIT * 64, (H - H_SPLIT) * 64), :])
                    finish(n2, _dot(lhs_b, tail) + acc[n2])
        return new_mem

    def body(i, mem):
        mem = list(mem)
        for u in range(UNROLL):
            mem = one_step(i, u, mem)
        return tuple(mem)

    for n in range(KT):
        wo_copy(n).wait()
    mi = mem0_s[...].astype(F32)
    mip = _b2u(jnp.concatenate([mi, mi], axis=0).astype(BF))
    lax.fori_loop(0, NSEG // UNROLL, body,
                  tuple(mip[:, 128 * k:128 * (k + 1)] for k in range(KT)))

    early = S - PRE
    zrow = pl.multiple_of(zero_s[0], 16)
    FPER = 9

    def half_rows(r0):
        return r0 // 2 if isinstance(r0, int) else pl.multiple_of(r0 // 2, 8)

    def combine(r0, nrows, n, a):
        xf = x_s[pl.ds(r0, nrows), pl.ds(128 * n, 128)].astype(F32)
        b = _u2b(xn_t[n, pl.ds(half_rows(r0), nrows // 2), :]).astype(F32)
        out_s[pl.ds(r0, nrows), pl.ds(128 * n, 128)] = (_rbf(xf + a) + b).astype(BF)

    def combine_stored(r0, nrows, not_before=None):
        for n in range(KT):
            a = abuf[n, pl.ds(half_rows(r0), nrows // 2), :]
            if not_before is not None:
                a = a | jnp.concatenate([not_before & zero_box[0]] * (nrows // 16), axis=0)
            combine(r0, nrows, n, _u2b(a).astype(F32))

    def out_copy(r0, nrows, j):
        return pltpu.make_async_copy(out_s.at[pl.ds(r0, nrows), :], out_hbm.at[pl.ds(r0, nrows), :],
                                     sems.at[SEM_OUT + j])

    def ffn_groups(j0, count, y, done):
        x_sel = _u2b(xsel_s[...])
        hid = {}

        def up(w_ref, j, key):
            part = _dot(x_sel[:, 0:512], _u2b(w_ref[j, pl.ds(0, 256), :]))
            yield
            hid[key] = _rbf(_dot(x_sel[:, 512:1024], _u2b(w_ref[j, pl.ds(256, 256), :])) + part)
            yield

        def down(jj):
            g = hid[("g", jj)]
            hb = (_rbf(g * _rbf(jax.nn.sigmoid(g))) * hid[("u", jj)]).astype(BF)
            rows = pl.ds(pl.multiple_of(64 * (j0 + jj), 64), 64)
            for half in range(2):
                w = jnp.concatenate([_u2b(wd_s[4 * half + n, rows, :]) for n in range(4)], axis=1)
                y[half] = _dot(hb, w) + y[half]
                yield

        for jj in range(count + 1):
            if jj < count:
                yield from up(wg_s, j0 + jj, ("g", jj))
                yield from up(wu_s, j0 + jj, ("u", jj))
            elif count == 1:
                yield
                yield
            if jj >= 1:
                yield from down(jj - 1)
        done()

    def epi_chunk(r0, nrows, side, pieces, keep):
        pos = [((r0 + 32 * j) % RING) // 2 for j in range(nrows // 32)]
        if not isinstance(r0, int):
            pos = [pl.multiple_of(p, 16) for p in pos]
        fresh_zero()
        deps = {}
        for n in range(KT):
            acc = None
            for g in range(8):
                lhs = jnp.concatenate(
                    [_u2b(jnp.concatenate([oring[h, pl.ds(p, 16), :] for p in pos], axis=0))
                     for h in range(4 * g, 4 * g + 4)], axis=1)
                w = _after(wo_s[n, pl.ds(256 * g, 256), :], deps.get(8 * n + g), zero_box[0])
                y = _dot(lhs, _u2b(w))
                acc = y if acc is None else y + acc
                next(side, None)
                v = 8 * n + g
                if pieces is not None and v in EPI_SCHED:
                    r1 = pieces + 32 * EPI_SCHED.index(v)
                    combine_stored(r1, 32, pltpu.bitcast(acc[0:8], U32) if EPI_NB else None)
                    if EPI_LAG:
                        deps[v + EPI_LAG] = [_b2u(out_s[pl.ds(r1 + (zrow if EPI_ALIAS else 0), 16), pl.ds(D - 128, 128)])]
            ab = acc.astype(BF)
            if keep:
                abuf[n, pl.ds(half_rows(r0), nrows // 2), :] = _b2u(ab)
            combine(r0, nrows, n, ab.astype(F32))

    for c in ffn_copies:
        c.wait()

    def epi_body(c, y):
        y = list(y)
        r0 = pl.multiple_of(early + ECH * c, 32)
        e0 = pl.multiple_of((early // 2) * (c & 1), 256)

        @pl.when(c == 2)
        def _():
            out_copy(0, early // 2, 4).wait()

        epi_chunk(r0, ECH, ffn_groups(FPER * c, FPER, y, lambda: None), e0, True)
        out_copy(r0, ECH, c).start()

        @pl.when(c < 2)
        def _():
            out_copy(e0, early // 2, 4 + c).start()

        return tuple(y)

    y = list(lax.fori_loop(0, 3, epi_body, (jnp.zeros((16, 512), F32), jnp.zeros((16, 512), F32))))
    idx1 = idx_s[0]
    idx2 = idx_s[1]

    def patch_row(t, yrow):
        xr, w = load_row(t)
        bits = pltpu.bitcast(_rbf(xr + yrow), U32)
        w = jnp.where(t % 2 == 0,
                      (w & jnp.uint32(0xFFFF0000)) | (bits >> 16),
                      (w & jnp.uint32(0xFFFF)) | bits)
        for k in range(KT):
            xn_t[k, pl.ds(t // 2, 1), :] = w[:, 128 * k:128 * (k + 1)]

    def patch():
        gate = _rbf(jax.nn.sigmoid(gate_s[:, 0:1]))
        yy = _rbf(_rbf(jnp.concatenate(y, axis=1)) * gate)
        patch_row(idx1, yy[0:1])
        patch_row(idx2, yy[1:2])

    last = early + 3 * ECH
    epi_chunk(last, S - last, ffn_groups(3 * FPER, 1, y, patch), None, False)
    out_copy(last, S - last, 3).start()
    for c in range(3):
        out_copy(early + ECH * c, ECH, c).wait()
    out_copy(early // 2, early // 2, 5).wait()
    blk1 = jnp.minimum(idx1 // 16, last // 16 - 1)
    blk2 = jnp.minimum(idx2 // 16, last // 16 - 1)
    blk2 = jnp.where(blk2 == blk1, jnp.where(blk1 == 0, 1, blk1 - 1), blk2)
    fix = []
    for j, blk in enumerate((blk1, blk2)):
        r0 = pl.multiple_of(blk * 16, 16)
        combine_stored(r0, 16)
        fix.append(out_copy(r0, 16, 7 + j))
    for cp in fix:
        cp.start()
    out_copy(last, S - last, 3).wait()
    for cp in fix:
        cp.wait()


@jax.jit
def pallas_parallel_sum__memory_aug_recurrent_mem_tr__moe_arch_mod__prompt_kernel(
    A_x: jax.Array,
    A_mem0: jax.Array,
    A_Wq: jax.Array,
    A_Wk: jax.Array,
    A_Wv: jax.Array,
    A_Wo: jax.Array,
    A_seg_len: jax.Array,
    B_x: jax.Array,
    B_w_r: jax.Array,
    B_w_gate: jax.Array,
    B_w_up: jax.Array,
    B_w_down: jax.Array,
):
    del A_seg_len, B_x
    assert A_x.shape == (1, S, D) and A_mem0.shape == (1, MEM, D)
    assert A_Wq.shape == (D, H, DH) and A_Wo.shape == (H, DH, D)
    assert B_w_gate.shape == (D, FF) and B_w_down.shape == (FF, D)
    any_spec = pl.BlockSpec(memory_space=pl.ANY)
    out = pl.pallas_call(
        _kernel,
        out_shape=jax.ShapeDtypeStruct((S, D), BF),
        in_specs=[any_spec] * 10,
        out_specs=any_spec,
        scratch_shapes=[
            pltpu.VMEM((S, D), BF),
            pltpu.VMEM((KT, S // 2, 128), U32),
            pltpu.VMEM((KT, PRE // 2, 128), U32),
            pltpu.VMEM((KT, 16 * NSEG, 128), U32),
            pltpu.VMEM((3 * H + 2, D // 2, 128), U32),
            pltpu.VMEM((KT, H * DH // 2, 128), U32),
            pltpu.VMEM((3 * H, RING32, 128), U32),
            pltpu.VMEM((H, RING32, 128), U32),
            pltpu.VMEM((KT, S // 2, 128), U32),
            pltpu.VMEM((S, D), BF),
            pltpu.VMEM((NCH, D // 2, 8, 128), U32),
            pltpu.VMEM((FT, D // 2, 128), U32),
            pltpu.VMEM((FT, D // 2, 128), U32),
            pltpu.VMEM((KT, FF // 2, 128), U32),
            pltpu.VMEM((MEM, D), BF),
            pltpu.VMEM((D,), BF),
            pltpu.VMEM((8, D), F32),
            pltpu.VMEM((16, 128), F32),
            pltpu.VMEM((8, D), U32),
            pltpu.VMEM((16, 128), F32),
            pltpu.SMEM((1,), jnp.int32),
            pltpu.SMEM((2,), jnp.int32),
            pltpu.SemaphoreType.DMA((NSEM,)),
        ],
        compiler_params=pltpu.CompilerParams(vmem_limit_bytes=126 * 1024 * 1024),
    )(A_x.reshape(S, D), A_mem0.reshape(MEM, D), A_Wq.reshape(D // 2, 2, H, DH), A_Wk.reshape(D // 2, 2, H, DH),
      A_Wv.reshape(D // 2, 2, H, DH), A_Wo.reshape(H * DH, D),
      B_w_r, B_w_gate, B_w_up, B_w_down)
    return out.reshape(1, S, D)
```

```python
import jax
import jax.numpy as jnp
from jax import lax
import jax.experimental.pallas as pl
import jax.experimental.pallas.tpu as pltpu

BF = jnp.bfloat16
U32 = jnp.uint32
F32 = jnp.float32

S = 2048
D = 1024
H = 32
DH = 128
MEM = 8
SEG = 32
NSEG = S // SEG
FF = 3584
KT = D // 128
FT = FF // 128
XS = 24
PRE = S - NSEG * XS
RING = 576
RING32 = RING // 2
NPAIR = H // 2
NPQ = 3 * NPAIR
NPRE = 16
SEM_SMALL, SEM_X0, SEM_X = 0, 2, 6
SEM_W0 = SEM_X + NPRE
SEM_W = SEM_W0 + 3
SEM_WO = SEM_W + NPRE
SEM_FFN, SEM_OUT = SEM_WO + 1, SEM_WO + 2
NSEM = SEM_OUT + 9

LAG_QK = 1
LAG_PV = 4
N_PART = 4
H_SPLIT = 26
REL_SCHED = {0: [(0, 0), (0, 1)], 1: [(0, 2), (0, 3)], 2: [(0, 4)], 3: [(0, 5)], 4: [(0, 6)], 5: [(0, 7)]}
REL_SCHED.update({6 + k: [(1, k)] for k in range(8)})
REL_SCHED.update({14 + k: [(2, k)] for k in range(8)})
K_SPLIT = 2
EPI_SCHED = [v * 5 // 2 for v in range(24)]
EPI_LAG = 4
ECH = 160
EPI_NB = False
EPI_ALIAS = False
REL_SCHED0 = {8 * j + k: [(j, kk) for kk in range(8) if kk * 6 // 8 == k] for j in range(3) for k in range(6)}
LN_SCHED = {3 * q: [q] for q in range(6)}
LN_SCHED0 = {16: [0, 1], 17: [2, 3], 18: [4, 5]}
FIRST_BATCH = 12
LN_LAG = 5
REL_LAG = 2
UNROLL = 4


def _b2u(x):
    return pltpu.bitcast(x, U32)


def _u2b(x):
    return pltpu.bitcast(x, BF)


def _dot(a, b):
    return jnp.dot(a, b, preferred_element_type=F32)


def _dot_nt(a, b):
    return lax.dot_general(a, b, (((1,), (1,)), ((), ())), preferred_element_type=F32)


def _after(w, dep, zero):
    if not dep:
        return w
    d = dep[0]
    for e in dep[1:]:
        d = d | e
    return jnp.concatenate([w[0:8] | (d & zero), w[8:]], axis=0)


def _rbf(x):
    return x.astype(BF).astype(F32)


def _kernel(x_hbm, mem0_hbm, wq_hbm, wk_hbm, wv_hbm, wo_hbm, wr_hbm, wg_hbm, wu_hbm, wd_hbm,
            out_hbm,
            x_s, xn_t, xn_pre, hbuf, wqkv, wo_s, ring, oring, abuf, out_s, raw,
            wg_s, wu_s, wd_s, mem0_s, wr_s, wrf_s, r_s, xsel_s, gate_s, zero_s, idx_s,
            sems):
    w32 = [w.bitcast(U32) for w in (wq_hbm, wk_hbm, wv_hbm)]
    wo32 = wo_hbm.bitcast(U32)
    wg32 = wg_hbm.bitcast(U32)
    wu32 = wu_hbm.bitcast(U32)
    wd32 = wd_hbm.bitcast(U32)

    def rows_copy(r0, n, sem):
        return pltpu.make_async_copy(x_hbm.at[pl.ds(r0, n), :], x_s.at[pl.ds(r0, n), :], sems.at[sem])

    def x_first(c):
        return rows_copy(128 * c if isinstance(c, int) else pl.multiple_of(128 * c, 128), 128, SEM_X0 + c)

    def x_piece(c):
        r0 = PRE + 96 * c if isinstance(c, int) else pl.multiple_of(PRE + 96 * c, 32)
        return rows_copy(r0, 96, SEM_X + c)

    def pair_copy(p):
        q = min(p, NPQ - 1)
        sem = SEM_W0 + p if p < 4 else SEM_W + (p - 1) // 3
        return pltpu.make_async_copy(w32[q // NPAIR].at[:, q % NPAIR, :], raw.at[p], sems.at[sem])

    def pairs_wait(t):
        dst = raw.at[pl.ds(3 * t + 1, 3)]
        pltpu.make_async_copy(dst, dst, sems.at[SEM_W + t]).wait()

    def wo_copy(n):
        return pltpu.make_async_copy(wo32.at[:, pl.ds(128 * n, 128)], wo_s.at[n], sems.at[SEM_WO])

    small_copies = [pltpu.make_async_copy(mem0_hbm, mem0_s, sems.at[SEM_SMALL]),
                    pltpu.make_async_copy(wr_hbm, wr_s, sems.at[SEM_SMALL + 1])]
    ffn_copies = (
        [pltpu.make_async_copy(wg32.at[:, pl.ds(128 * j, 128)], wg_s.at[j], sems.at[SEM_FFN]) for j in range(FT)]
        + [pltpu.make_async_copy(wu32.at[:, pl.ds(128 * j, 128)], wu_s.at[j], sems.at[SEM_FFN]) for j in range(FT)]
        + [pltpu.make_async_copy(wd32.at[:, pl.ds(128 * n, 128)], wd_s.at[n], sems.at[SEM_FFN]) for n in range(KT)])

    zero_s[0] = 0
    for c in range(4):
        x_first(c).start()
        if c == 0:
            for cp in small_copies:
                cp.start()

    def queue(t0, t1):
        for t in range(t0, t1):
            for p in range(3 * t + 1, 3 * t + 4):
                pair_copy(p).start()
            x_piece(t).start()

    pair_copy(0).start()
    queue(0, FIRST_BATCH)
    eps_bf = 1.0013580322265625e-05

    def layernorm16(rq, dst_ref, dst_row, not_before=None):
        rq = rq if isinstance(rq, int) else pl.multiple_of(rq, 16)
        xf = x_s[pl.ds(rq, 16), :].astype(F32)
        if not_before is not None:
            x0 = _after(pltpu.bitcast(xf[:, 0:128], U32), [not_before], zero_box[0])
            xf = jnp.concatenate([pltpu.bitcast(x0, F32), xf[:, 128:]], axis=1)
        mean = jnp.sum(xf, axis=1, keepdims=True) * (1.0 / D)
        cen = xf - mean
        var = jnp.sum(cen * cen, axis=1, keepdims=True) * (1.0 / D)
        sd = _rbf(jnp.sqrt(_rbf(_rbf(var) + eps_bf)))
        xn = (_rbf(xf - _rbf(mean)) * (1.0 / sd)).astype(BF)
        wr = jnp.concatenate([wrf_s[...], wrf_s[...]], axis=0)
        score = _rbf(jnp.sum(xn.astype(F32) * wr, axis=1, keepdims=True))
        r_s[...] = jnp.where(lane16 == rq // 16, score, r_s[...])
        xp = _b2u(xn)
        hq = rq // 2 if isinstance(rq, int) else pl.multiple_of(rq // 2, 8)
        dst_row = dst_row if isinstance(dst_row, int) else pl.multiple_of(dst_row, 8)
        for k in range(KT):
            xn_t[k, pl.ds(hq, 8), :] = xp[:, 128 * k:128 * (k + 1)]
            dst_ref[k, pl.ds(dst_row, 8), :] = xp[:, 128 * k:128 * (k + 1)]

    zero_box = [None]

    def fresh_zero():
        zero_box[0] = jnp.full((8, 128), zero_s[0], jnp.int32).astype(U32)

    r_s[...] = jnp.full(r_s.shape, -jnp.inf, F32)
    lane16 = lax.broadcasted_iota(jnp.int32, (16, 128), 1)
    for c in small_copies:
        c.wait()
    wrf_s[...] = jnp.broadcast_to(wr_s[...].astype(F32).reshape(1, D), (8, D))

    def ln_body(c, carry):
        x_first(c).wait()
        for q in range(8):
            layernorm16(128 * c + 16 * q, xn_pre, 64 * c + 8 * q)
        return carry

    lax.fori_loop(0, PRE // 128, ln_body, 0)


    def relayout(src, dst, j, k, not_before=None):
        a = src[j, pl.ds(128 * k, 64, stride=2), :]
        if not_before is not None:
            a = a | jnp.concatenate([not_before & zero_box[0]] * 8, axis=0)
        b = src[j, pl.ds(128 * k + 1, 64, stride=2), :]
        rows = pl.ds(64 * k, 64)
        dst[2 * j, rows, :] = (a & jnp.uint32(0xFFFF)) | (b << 16)
        dst[2 * j + 1, rows, :] = (a >> 16) | (b & jnp.uint32(0xFFFF0000))

    def pre_dot(w_view, ring_view, j, k, dep=None):
        i, q = k // 4, k % 4
        lhs = jnp.concatenate([_u2b(xn_pre[kk, pl.ds(64 * q, 64), :]) for kk in range(KT)], axis=1)
        y = _dot(lhs, _u2b(_after(w_view[2 * j + i], dep, zero_box[0])))
        yp = _b2u(y.astype(BF))
        ring_view[2 * j + i, pl.ds(32 + 64 * q, 64), :] = yp
        return yp[0:8]

    pair_copy(0).wait()
    for k in range(8):
        relayout(raw, wqkv, 0, k)

    def pre_iter(t, barriers):
        deps = {}
        raw_view = raw.at[pl.ds(3 * t, 4)]
        w_view = wqkv.at[pl.ds(6 * t, 8)]
        ring_view = ring.at[pl.ds(6 * t, 6)]
        rel_sched, ln_sched = (REL_SCHED0, LN_SCHED0) if barriers else (REL_SCHED, LN_SCHED)
        done = None
        for v in range(24):
            j, k = v // 8, v % 8
            if v == 0 or v in barriers:
                for wait in barriers.get(v, ()):
                    wait()
                fresh_zero()
                done = None
            prev = done
            done = pre_dot(w_view, ring_view, j, k, deps.get(v))
            for jr, kr in rel_sched.get(v, ()):
                relayout(raw_view, w_view, jr + 1, kr, prev)
                deps.setdefault(v + REL_LAG, []).append(w_view[2 * jr + 3, pl.ds(64 * kr + 56, 8), :])
            for q in ln_sched.get(v, ()):
                hrow = 32 * (q // 3) + 8 * (q % 3)
                hrow += 64 * t if isinstance(t, int) else pl.multiple_of(64 * t, 64)
                layernorm16(PRE + 96 * t + 16 * q, hbuf, hrow, done if prev is not None else None)
                deps.setdefault(v + LN_LAG, []).append(hbuf[KT - 1, pl.ds(hrow, 8), :])

    def second_batch():
        queue(FIRST_BATCH, NPRE)
        for n in range(KT):
            wo_copy(n).start()

    pre_iter(0, {0: [pair_copy(1).wait], 8: [pair_copy(2).wait],
                 16: [pair_copy(3).wait, x_piece(0).wait, second_batch]})

    def pre_body(t, carry):
        x_piece(t).wait()
        pairs_wait(t)
        pre_iter(t, {})
        return carry

    lax.fori_loop(1, NPRE, pre_body, 0)
    for c in ffn_copies:
        c.start()

    row = lax.broadcasted_iota(jnp.int32, (80, 80), 0)
    col = lax.broadcasted_iota(jnp.int32, (80, 80), 1)
    same_head = (jnp.where(row < 64, row >> 5, (row - 64) >> 3)
                 == jnp.where(col < 64, col >> 5, (col - 64) >> 3))
    allowed = same_head & ((col >= 64) | (row >= 64) | (col <= row))
    fill = jnp.where(same_head, -1e9, -jnp.inf).astype(F32)
    low_half = lax.broadcasted_iota(jnp.int32, (8, 128), 0) < 4
    high_half = jnp.logical_not(low_half)
    scale = DH ** -0.5

    def load_row(t):
        w = jnp.concatenate([xn_t[k, pl.ds(t // 2, 1), :] for k in range(KT)], axis=1)
        bits = jnp.where(t % 2 == 0, w << 16, w & jnp.uint32(0xFFFF0000))
        return pltpu.bitcast(bits, F32), w

    def select_tokens():
        r = r_s[...]
        tok = lane16 * 16 + lax.broadcasted_iota(jnp.int32, (16, 128), 0)
        top1 = jnp.max(r)
        idx1 = jnp.min(jnp.where(r == top1, tok, S - 1))
        r2 = jnp.where(tok == idx1, -jnp.inf, r)
        top2 = jnp.max(r2)
        idx2 = jnp.min(jnp.where((r2 == top2) & (tok != idx1), tok, S - 1))
        idx_s[0] = idx1
        idx_s[1] = idx2
        gate_s[...] = jnp.where(lax.broadcasted_iota(jnp.int32, (16, 128), 0) == 0, top1, top2)
        sel_row = lax.broadcasted_iota(jnp.int32, (16, D), 0)
        xs1, _ = load_row(idx1)
        xs2, _ = load_row(idx2)
        xsel_s[...] = _b2u(jnp.where(sel_row == 0, xs1, jnp.where(sel_row == 1, xs2, 0.0)).astype(BF))

    def one_step(i, u, mem):
        odd = u % 2
        s2 = i * (UNROLL // 2) + u // 2
        h_ld = pl.multiple_of(16 * UNROLL * i, 32) + 32 * (u // 2)
        a24 = pl.multiple_of(12 * UNROLL * i, 8)
        r24 = pl.multiple_of(a24 % RING32, 8) + XS * (u // 2)
        a24 = a24 + XS * (u // 2)
        qkv_ld = pl.multiple_of((SEG * s2 + 32) % RING32, 32) + 16 * odd
        o_st = pl.multiple_of((SEG * s2) % RING32, 32) + 16 * odd
        m0 = 0 if odd else XS

        def with_mem(ref, idx, base, m):
            lo = ref[idx, pl.ds(base + 8 * odd, 8), :]
            hi = ref[idx, pl.ds(base + 8 + 8 * odd, 8), :]
            if odd:
                lo = jnp.where(low_half, m, lo)
            else:
                hi = jnp.where(low_half, hi, m)
            return _u2b(jnp.concatenate([lo, hi], axis=0))

        def store_tokens(ref, idx, base, yp):
            if odd:
                pltpu.store(ref.at[idx, pl.ds(base + 8, 8), :], yp[0:8], mask=high_half)
                ref[idx, pl.ds(base + 16, 8), :] = yp[8:16]
            else:
                ref[idx, pl.ds(base, 8), :] = yp[0:8]
                pltpu.store(ref.at[idx, pl.ds(base + 8, 8), :], yp[8:16], mask=low_half)

        lk = [with_mem(hbuf, k, h_ld, mem[k]) for k in range(KT)]
        lhs = jnp.concatenate(lk, axis=1)

        ymem = {}
        xs = {}
        probs = {}
        parts = {}

        def proj(h):
            split = h < K_SPLIT and u > 0
            if split:
                lhs7 = jnp.concatenate(lk[:KT - 1], axis=1)
                head = [_dot(lhs7, _u2b(wqkv[m * H + h, pl.ds(0, 448), :])) for m in range(3)]
            for m in range(3):
                if split:
                    y = _dot(lk[KT - 1], _u2b(wqkv[m * H + h, pl.ds(448, 64), :])) + head[m]
                else:
                    y = _dot(lhs, _u2b(wqkv[m * H + h]))
                store_tokens(ring, m * H + h, r24, _b2u(y.astype(BF)))
                ymem[(h, m)] = y[m0:m0 + MEM]
                xs[(h, m)] = ring[m * H + h, pl.ds(qkv_ld, SEG // 2), :]

        def pair(p, m):
            a, b = 2 * p, 2 * p + 1
            mm = jnp.concatenate([ymem[(a, m)], ymem[(b, m)]], axis=0).astype(BF)
            return jnp.concatenate([_u2b(xs[(a, m)]), _u2b(xs[(b, m)]), mm], axis=0)

        def qk(p):
            sc = _dot_nt(pair(p, 0), pair(p, 1))
            sc = jnp.where(allowed, sc * scale, fill)
            e = jnp.exp(sc - jnp.max(sc, axis=1, keepdims=True))
            l = jnp.sum(e, axis=1, keepdims=True)
            r = pl.reciprocal(l, approx=True)
            r = r * (2.0 - l * r)
            probs[p] = (e * r).astype(BF)

        def pv(p):
            op = _b2u(_dot(probs[p], pair(p, 2)).astype(BF))
            om = op[32:40]
            om_sw = pltpu.roll(om, 4, axis=0)
            for j, h in enumerate((2 * p, 2 * p + 1)):
                oring[h, pl.ds(o_st, SEG // 2), :] = op[16 * j:16 * j + 16]
                parts[h] = with_mem(oring, h, r24, om if j != odd else om_sw)

        def after(t):
            for lag, fn in ((LAG_QK, qk), (LAG_PV, pv)):
                if (t - 1 - lag) % 2 == 0 and 0 <= (t - 1 - lag) // 2 < NPAIR:
                    fn((t - 1 - lag) // 2)

        for t in range(H):
            proj(t)
            after(t)
            if u == 0 and t == 8:
                select_tokens()
        t = H
        lhs_a = jnp.concatenate([parts[j] for j in range(H_SPLIT)], axis=1)
        acc = []
        for n in range(N_PART):
            acc.append(_dot(lhs_a, _u2b(wo_s[n, pl.ds(0, H_SPLIT * 64), :])))
            after(t)
            t += 1
        while t - 1 - LAG_PV <= 2 * (NPAIR - 1):
            after(t)
            t += 1
        lhs_b = jnp.concatenate([parts[j] for j in range(H_SPLIT, H)], axis=1)
        lhs_o = jnp.concatenate([lhs_a, lhs_b], axis=1)
        new_mem = [None] * KT

        def finish(n, y):
            store_tokens(abuf, n, a24, _b2u(y.astype(BF)))
            ym = y[m0:m0 + MEM]
            new_mem[n] = _b2u(jnp.concatenate([ym, ym], axis=0).astype(BF))

        for n in range(N_PART, KT):
            finish(n, _dot(lhs_o, _u2b(wo_s[n])))
            if n == N_PART:
                for n2 in range(N_PART):
                    tail = _u2b(wo_s[n2, pl.ds(H_SPLIT * 64, (H - H_SPLIT) * 64), :])
                    finish(n2, _dot(lhs_b, tail) + acc[n2])
        return new_mem

    def body(i, mem):
        mem = list(mem)
        for u in range(UNROLL):
            mem = one_step(i, u, mem)
        return tuple(mem)

    for n in range(KT):
        wo_copy(n).wait()
    mi = mem0_s[...].astype(F32)
    mip = _b2u(jnp.concatenate([mi, mi], axis=0).astype(BF))
    lax.fori_loop(0, NSEG // UNROLL, body,
                  tuple(mip[:, 128 * k:128 * (k + 1)] for k in range(KT)))

    early = S - PRE
    zrow = pl.multiple_of(zero_s[0], 16)
    FPER = 9

    def half_rows(r0):
        return r0 // 2 if isinstance(r0, int) else pl.multiple_of(r0 // 2, 8)

    def combine(r0, nrows, n, a):
        xf = x_s[pl.ds(r0, nrows), pl.ds(128 * n, 128)].astype(F32)
        b = _u2b(xn_t[n, pl.ds(half_rows(r0), nrows // 2), :]).astype(F32)
        out_s[pl.ds(r0, nrows), pl.ds(128 * n, 128)] = (_rbf(xf + a) + b).astype(BF)

    def combine_stored(r0, nrows, not_before=None):
        for n in range(KT):
            a = abuf[n, pl.ds(half_rows(r0), nrows // 2), :]
            if not_before is not None:
                a = a | jnp.concatenate([not_before & zero_box[0]] * (nrows // 16), axis=0)
            combine(r0, nrows, n, _u2b(a).astype(F32))

    def out_copy(r0, nrows, j):
        return pltpu.make_async_copy(out_s.at[pl.ds(r0, nrows), :], out_hbm.at[pl.ds(r0, nrows), :],
                                     sems.at[SEM_OUT + j])

    def ffn_groups(j0, count, y, done):
        x_sel = _u2b(xsel_s[...])
        hid = {}

        def up(w_ref, j, key):
            part = _dot(x_sel[:, 0:512], _u2b(w_ref[j, pl.ds(0, 256), :]))
            yield
            hid[key] = _rbf(_dot(x_sel[:, 512:1024], _u2b(w_ref[j, pl.ds(256, 256), :])) + part)
            yield

        def down(jj):
            g = hid[("g", jj)]
            hb = (_rbf(g * _rbf(jax.nn.sigmoid(g))) * hid[("u", jj)]).astype(BF)
            rows = pl.ds(pl.multiple_of(64 * (j0 + jj), 64), 64)
            for half in range(2):
                w = jnp.concatenate([_u2b(wd_s[4 * half + n, rows, :]) for n in range(4)], axis=1)
                y[half] = _dot(hb, w) + y[half]
                yield

        for jj in range(count + 1):
            if jj < count:
                yield from up(wg_s, j0 + jj, ("g", jj))
                yield from up(wu_s, j0 + jj, ("u", jj))
            elif count == 1:
                yield
                yield
            if jj >= 1:
                yield from down(jj - 1)
        done()

    def epi_chunk(r0, nrows, side, pieces, keep):
        pos = [((r0 + 32 * j) % RING) // 2 for j in range(nrows // 32)]
        if not isinstance(r0, int):
            pos = [pl.multiple_of(p, 16) for p in pos]
        fresh_zero()
        deps = {}
        for n in range(KT):
            acc = None
            for g in range(8):
                lhs = jnp.concatenate(
                    [_u2b(jnp.concatenate([oring[h, pl.ds(p, 16), :] for p in pos], axis=0))
                     for h in range(4 * g, 4 * g + 4)], axis=1)
                w = _after(wo_s[n, pl.ds(256 * g, 256), :], deps.get(8 * n + g), zero_box[0])
                y = _dot(lhs, _u2b(w))
                acc = y if acc is None else y + acc
                next(side, None)
                v = 8 * n + g
                if pieces is not None and v in EPI_SCHED:
                    r1 = pieces + 32 * EPI_SCHED.index(v)
                    combine_stored(r1, 32, pltpu.bitcast(acc[0:8], U32) if EPI_NB else None)
                    if EPI_LAG:
                        deps[v + EPI_LAG] = [_b2u(out_s[pl.ds(r1 + (zrow if EPI_ALIAS else 0), 16), pl.ds(D - 128, 128)])]
            ab = acc.astype(BF)
            if keep:
                abuf[n, pl.ds(half_rows(r0), nrows // 2), :] = _b2u(ab)
            combine(r0, nrows, n, ab.astype(F32))

    for c in ffn_copies:
        c.wait()

    def epi_body(c, y):
        y = list(y)
        r0 = pl.multiple_of(early + ECH * c, 32)
        e0 = pl.multiple_of((early // 2) * (c & 1), 256)

        @pl.when(c == 2)
        def _():
            out_copy(0, early // 2, 4).wait()

        epi_chunk(r0, ECH, ffn_groups(FPER * c, FPER, y, lambda: None), e0, True)
        out_copy(r0, ECH, c).start()

        @pl.when(c < 2)
        def _():
            out_copy(e0, early // 2, 4 + c).start()

        return tuple(y)

    y = list(lax.fori_loop(0, 3, epi_body, (jnp.zeros((16, 512), F32), jnp.zeros((16, 512), F32))))
    idx1 = idx_s[0]
    idx2 = idx_s[1]

    def patch_row(t, yrow):
        xr, w = load_row(t)
        bits = pltpu.bitcast(_rbf(xr + yrow), U32)
        w = jnp.where(t % 2 == 0,
                      (w & jnp.uint32(0xFFFF0000)) | (bits >> 16),
                      (w & jnp.uint32(0xFFFF)) | bits)
        for k in range(KT):
            xn_t[k, pl.ds(t // 2, 1), :] = w[:, 128 * k:128 * (k + 1)]

    def patch():
        gate = _rbf(jax.nn.sigmoid(gate_s[:, 0:1]))
        yy = _rbf(_rbf(jnp.concatenate(y, axis=1)) * gate)
        patch_row(idx1, yy[0:1])
        patch_row(idx2, yy[1:2])

    last = early + 3 * ECH
    epi_chunk(last, S - last, ffn_groups(3 * FPER, 1, y, patch), None, False)
    out_copy(last, S - last, 3).start()
    for c in range(3):
        out_copy(early + ECH * c, ECH, c).wait()
    out_copy(early // 2, early // 2, 5).wait()
    blk1 = jnp.minimum(idx1 // 16, last // 16 - 1)
    blk2 = jnp.minimum(idx2 // 16, last // 16 - 1)
    blk2 = jnp.where(blk2 == blk1, jnp.where(blk1 == 0, 1, blk1 - 1), blk2)
    fix = []
    for j, blk in enumerate((blk1, blk2)):
        r0 = pl.multiple_of(blk * 16, 16)
        combine_stored(r0, 16)
        fix.append(out_copy(r0, 16, 7 + j))
    for cp in fix:
        cp.start()
    out_copy(last, S - last, 3).wait()
    for cp in fix:
        cp.wait()


@jax.jit
def pallas_parallel_sum__memory_aug_recurrent_mem_tr__moe_arch_mod__prompt_kernel(
    A_x: jax.Array,
    A_mem0: jax.Array,
    A_Wq: jax.Array,
    A_Wk: jax.Array,
    A_Wv: jax.Array,
    A_Wo: jax.Array,
    A_seg_len: jax.Array,
    B_x: jax.Array,
    B_w_r: jax.Array,
    B_w_gate: jax.Array,
    B_w_up: jax.Array,
    B_w_down: jax.Array,
):
    del A_seg_len, B_x
    assert A_x.shape == (1, S, D) and A_mem0.shape == (1, MEM, D)
    assert A_Wq.shape == (D, H, DH) and A_Wo.shape == (H, DH, D)
    assert B_w_gate.shape == (D, FF) and B_w_down.shape == (FF, D)
    any_spec = pl.BlockSpec(memory_space=pl.ANY)
    out = pl.pallas_call(
        _kernel,
        out_shape=jax.ShapeDtypeStruct((S, D), BF),
        in_specs=[any_spec] * 10,
        out_specs=any_spec,
        scratch_shapes=[
            pltpu.VMEM((S, D), BF),
            pltpu.VMEM((KT, S // 2, 128), U32),
            pltpu.VMEM((KT, PRE // 2, 128), U32),
            pltpu.VMEM((KT, 16 * NSEG, 128), U32),
            pltpu.VMEM((3 * H + 2, D // 2, 128), U32),
            pltpu.VMEM((KT, H * DH // 2, 128), U32),
            pltpu.VMEM((3 * H, RING32, 128), U32),
            pltpu.VMEM((H, RING32, 128), U32),
            pltpu.VMEM((KT, S // 2, 128), U32),
            pltpu.VMEM((S, D), BF),
            pltpu.VMEM((NPQ + 1, D, 128), U32),
            pltpu.VMEM((FT, D // 2, 128), U32),
            pltpu.VMEM((FT, D // 2, 128), U32),
            pltpu.VMEM((KT, FF // 2, 128), U32),
            pltpu.VMEM((MEM, D), BF),
            pltpu.VMEM((D,), BF),
            pltpu.VMEM((8, D), F32),
            pltpu.VMEM((16, 128), F32),
            pltpu.VMEM((8, D), U32),
            pltpu.VMEM((16, 128), F32),
            pltpu.SMEM((1,), jnp.int32),
            pltpu.SMEM((2,), jnp.int32),
            pltpu.SemaphoreType.DMA((NSEM,)),
        ],
        compiler_params=pltpu.CompilerParams(vmem_limit_bytes=126 * 1024 * 1024),
    )(A_x.reshape(S, D), A_mem0.reshape(MEM, D), A_Wq, A_Wk, A_Wv, A_Wo.reshape(H * DH, D),
      B_w_r, B_w_gate, B_w_up, B_w_down)
    return out.reshape(1, S, D)
```

```python
import jax
import jax.numpy as jnp
from jax import lax
import jax.experimental.pallas as pl
import jax.experimental.pallas.tpu as pltpu

BF = jnp.bfloat16
U32 = jnp.uint32
F32 = jnp.float32

S = 2048
D = 1024
H = 32
DH = 128
MEM = 8
SEG = 32
NSEG = S // SEG
FF = 3584
KT = D // 128
FT = FF // 128
XS = 24
PRE = S - NSEG * XS
RING = 576
RING32 = RING // 2
NPAIR = H // 2
NPQ = 3 * NPAIR
NPRE = 16
SEM_SMALL, SEM_X0, SEM_X = 0, 2, 6
SEM_W0 = SEM_X + NPRE
SEM_W = SEM_W0 + 3
SEM_WO = SEM_W + NPRE
SEM_FFN, SEM_OUT = SEM_WO + 1, SEM_WO + 2
NSEM = SEM_OUT + 9

LAG_QK = 1
LAG_PV = 4
N_PART = 4
H_SPLIT = 26
REL_SCHED = {0: [(0, 0), (0, 1)], 1: [(0, 2), (0, 3)], 2: [(0, 4)], 3: [(0, 5)], 4: [(0, 6)], 5: [(0, 7)]}
REL_SCHED.update({6 + k: [(1, k)] for k in range(8)})
REL_SCHED.update({14 + k: [(2, k)] for k in range(8)})
K_SPLIT = 2
EPI_SCHED = [v * 5 // 2 for v in range(24)]
EPI_LAG = 4
ECH = 160
EPI_NB = False
EPI_ALIAS = False
REL_SCHED0 = {4: [(0, k) for k in range(4)], 5: [(0, k) for k in range(4, 8)],
              12: [(1, k) for k in range(4)], 13: [(1, k) for k in range(4, 8)]}
REL_SCHED0.update({14 + k: [(2, k)] for k in range(8)})
SCORE_SCHED = [1, 7, 13]
LN_SCHED = {3 * q: [q] for q in range(6)}
LN_SCHED0 = {13 + q: [q] for q in range(6)}
FIRST_BATCH = 12
LN_LAG = 5
REL_LAG = 2
UNROLL = 4


def _b2u(x):
    return pltpu.bitcast(x, U32)


def _u2b(x):
    return pltpu.bitcast(x, BF)


def _dot(a, b):
    return jnp.dot(a, b, preferred_element_type=F32)


def _dot_nt(a, b):
    return lax.dot_general(a, b, (((1,), (1,)), ((), ())), preferred_element_type=F32)


def _after(w, dep, zero):
    if not dep:
        return w
    d = dep[0]
    for e in dep[1:]:
        d = d | e
    return jnp.concatenate([w[0:8] | (d & zero), w[8:]], axis=0)


def _rbf(x):
    return x.astype(BF).astype(F32)


def _kernel(x_hbm, mem0_hbm, wq_hbm, wk_hbm, wv_hbm, wo_hbm, wr_hbm, wg_hbm, wu_hbm, wd_hbm,
            out_hbm,
            x_s, xn_t, xn_pre, hbuf, wqkv, wo_s, ring, oring, abuf, out_s, raw,
            wg_s, wu_s, wd_s, mem0_s, wr_s, wrf_s, r_s, xsel_s, gate_s, zero_s, idx_s,
            sems):
    w32 = [w.bitcast(U32) for w in (wq_hbm, wk_hbm, wv_hbm)]
    wo32 = wo_hbm.bitcast(U32)
    wg32 = wg_hbm.bitcast(U32)
    wu32 = wu_hbm.bitcast(U32)
    wd32 = wd_hbm.bitcast(U32)

    def rows_copy(r0, n, sem):
        return pltpu.make_async_copy(x_hbm.at[pl.ds(r0, n), :], x_s.at[pl.ds(r0, n), :], sems.at[sem])

    def x_first(c):
        return rows_copy(128 * c if isinstance(c, int) else pl.multiple_of(128 * c, 128), 128, SEM_X0 + c)

    def x_piece(c):
        r0 = PRE + 96 * c if isinstance(c, int) else pl.multiple_of(PRE + 96 * c, 32)
        return rows_copy(r0, 96, SEM_X + c)

    def pair_copy(p):
        q = min(p, NPQ - 1)
        sem = SEM_W0 + p if p < 4 else SEM_W + (p - 1) // 3
        return pltpu.make_async_copy(w32[q // NPAIR].at[:, q % NPAIR, :], raw.at[p], sems.at[sem])

    def pairs_wait(t):
        dst = raw.at[pl.ds(3 * t + 1, 3)]
        pltpu.make_async_copy(dst, dst, sems.at[SEM_W + t]).wait()

    def wo_copy(n):
        return pltpu.make_async_copy(wo32.at[:, pl.ds(128 * n, 128)], wo_s.at[n], sems.at[SEM_WO])

    small_copies = [pltpu.make_async_copy(mem0_hbm, mem0_s, sems.at[SEM_SMALL]),
                    pltpu.make_async_copy(wr_hbm, wr_s, sems.at[SEM_SMALL + 1])]
    ffn_copies = (
        [pltpu.make_async_copy(wg32.at[:, pl.ds(128 * j, 128)], wg_s.at[j], sems.at[SEM_FFN]) for j in range(FT)]
        + [pltpu.make_async_copy(wu32.at[:, pl.ds(128 * j, 128)], wu_s.at[j], sems.at[SEM_FFN]) for j in range(FT)]
        + [pltpu.make_async_copy(wd32.at[:, pl.ds(128 * n, 128)], wd_s.at[n], sems.at[SEM_FFN]) for n in range(KT)])

    zero_s[0] = 0
    for c in range(4):
        x_first(c).start()
        if c == 0:
            for cp in small_copies:
                cp.start()

    def queue(t0, t1):
        for t in range(t0, t1):
            for p in range(3 * t + 1, 3 * t + 4):
                pair_copy(p).start()
            x_piece(t).start()

    pair_copy(0).start()
    queue(0, FIRST_BATCH)
    eps_bf = 1.0013580322265625e-05

    def score16(g, xn):
        wr = jnp.concatenate([wrf_s[...], wrf_s[...]], axis=0)
        score = _rbf(jnp.sum(xn.astype(F32) * wr, axis=1, keepdims=True))
        r_s[...] = jnp.where(lane16 == g, score, r_s[...])

    def layernorm16(rq, dst_ref, dst_row, not_before=None):
        rq = rq if isinstance(rq, int) else pl.multiple_of(rq, 16)
        xf = x_s[pl.ds(rq, 16), :].astype(F32)
        if not_before is not None:
            x0 = _after(pltpu.bitcast(xf[:, 0:128], U32), [not_before], zero_box[0])
            xf = jnp.concatenate([pltpu.bitcast(x0, F32), xf[:, 128:]], axis=1)
        mean = jnp.sum(xf, axis=1, keepdims=True) * (1.0 / D)
        cen = xf - mean
        var = jnp.sum(cen * cen, axis=1, keepdims=True) * (1.0 / D)
        sd = _rbf(jnp.sqrt(_rbf(_rbf(var) + eps_bf)))
        xn = (_rbf(xf - _rbf(mean)) * (1.0 / sd)).astype(BF)
        if dst_ref is hbuf:
            score16(rq // 16, xn)
        xp = _b2u(xn)
        hq = rq // 2 if isinstance(rq, int) else pl.multiple_of(rq // 2, 8)
        dst_row = dst_row if isinstance(dst_row, int) else pl.multiple_of(dst_row, 8)
        for k in range(KT):
            xn_t[k, pl.ds(hq, 8), :] = xp[:, 128 * k:128 * (k + 1)]
            dst_ref[k, pl.ds(dst_row, 8), :] = xp[:, 128 * k:128 * (k + 1)]

    zero_box = [None]

    def fresh_zero():
        zero_box[0] = jnp.full((8, 128), zero_s[0], jnp.int32).astype(U32)

    r_s[...] = jnp.full(r_s.shape, -jnp.inf, F32)
    lane16 = lax.broadcasted_iota(jnp.int32, (16, 128), 1)

    def ln_body(c, carry):
        x_first(c).wait()
        for q in range(8):
            layernorm16(128 * c + 16 * q, xn_pre, 64 * c + 8 * q)
        return carry

    lax.fori_loop(0, PRE // 128, ln_body, 0)


    def relayout(src, dst, j, k, not_before=None):
        a = src[j, pl.ds(128 * k, 64, stride=2), :]
        if not_before is not None:
            a = a | jnp.concatenate([not_before & zero_box[0]] * 8, axis=0)
        b = src[j, pl.ds(128 * k + 1, 64, stride=2), :]
        rows = pl.ds(64 * k, 64)
        dst[2 * j, rows, :] = (a & jnp.uint32(0xFFFF)) | (b << 16)
        dst[2 * j + 1, rows, :] = (a >> 16) | (b & jnp.uint32(0xFFFF0000))

    def pre_dot(w_view, ring_view, j, k, dep=None):
        i, q = k // 4, k % 4
        lhs = jnp.concatenate([_u2b(xn_pre[kk, pl.ds(64 * q, 64), :]) for kk in range(KT)], axis=1)
        y = _dot(lhs, _u2b(_after(w_view[2 * j + i], dep, zero_box[0])))
        yp = _b2u(y.astype(BF))
        ring_view[2 * j + i, pl.ds(32 + 64 * q, 64), :] = yp
        return yp[0:8]

    for c in small_copies:
        c.wait()
    pair_copy(0).wait()
    for k in range(8):
        relayout(raw, wqkv, 0, k)
    wrf_s[...] = jnp.broadcast_to(wr_s[...].astype(F32).reshape(1, D), (8, D))

    def pre_iter(t, barriers):
        deps = {}
        raw_view = raw.at[pl.ds(3 * t, 4)]
        w_view = wqkv.at[pl.ds(6 * t, 8)]
        ring_view = ring.at[pl.ds(6 * t, 6)]
        rel_sched, ln_sched = (REL_SCHED0, LN_SCHED0) if barriers else (REL_SCHED, LN_SCHED)
        done = None
        for v in range(24):
            j, k = v // 8, v % 8
            if v == 0 or v in barriers:
                for wait in barriers.get(v, ()):
                    wait()
                fresh_zero()
                done = None
            prev = done
            done = pre_dot(w_view, ring_view, j, k, deps.get(v))
            for jr, kr in rel_sched.get(v, ()):
                relayout(raw_view, w_view, jr + 1, kr, prev)
                deps.setdefault(v + REL_LAG, []).append(w_view[2 * jr + 3, pl.ds(64 * kr + 56, 8), :])
            for q in ln_sched.get(v, ()):
                hrow = 32 * (q // 3) + 8 * (q % 3)
                hrow += 64 * t if isinstance(t, int) else pl.multiple_of(64 * t, 64)
                layernorm16(PRE + 96 * t + 16 * q, hbuf, hrow, done if prev is not None else None)
                deps.setdefault(v + LN_LAG, []).append(hbuf[KT - 1, pl.ds(hrow, 8), :])
            if not barriers and v in SCORE_SCHED:
                g = jnp.minimum(3 * (t - 1) + SCORE_SCHED.index(v), PRE // 16 - 1)
                rows = pl.ds(pl.multiple_of(8 * g, 8), 8)
                xp = [xn_pre[kk, rows, :] for kk in range(KT)]
                xp[0] = xp[0] | (done & zero_box[0])
                score16(g, _u2b(jnp.concatenate(xp, axis=1)))

    def second_batch():
        queue(FIRST_BATCH, NPRE)
        for n in range(KT):
            wo_copy(n).start()

    pre_iter(0, {4: [pair_copy(1).wait],
                 12: [pair_copy(2).wait, pair_copy(3).wait, x_piece(0).wait, second_batch]})

    def pre_body(t, carry):
        x_piece(t).wait()
        pairs_wait(t)
        pre_iter(t, {})
        return carry

    lax.fori_loop(1, NPRE, pre_body, 0)
    for c in ffn_copies:
        c.start()

    row = lax.broadcasted_iota(jnp.int32, (80, 80), 0)
    col = lax.broadcasted_iota(jnp.int32, (80, 80), 1)
    same_head = (jnp.where(row < 64, row >> 5, (row - 64) >> 3)
                 == jnp.where(col < 64, col >> 5, (col - 64) >> 3))
    allowed = same_head & ((col >= 64) | (row >= 64) | (col <= row))
    fill = jnp.where(same_head, -1e9, -jnp.inf).astype(F32)
    low_half = lax.broadcasted_iota(jnp.int32, (8, 128), 0) < 4
    high_half = jnp.logical_not(low_half)
    scale = DH ** -0.5

    def load_row(t):
        w = jnp.concatenate([xn_t[k, pl.ds(t // 2, 1), :] for k in range(KT)], axis=1)
        bits = jnp.where(t % 2 == 0, w << 16, w & jnp.uint32(0xFFFF0000))
        return pltpu.bitcast(bits, F32), w

    def select_tokens():
        r = r_s[...]
        tok = lane16 * 16 + lax.broadcasted_iota(jnp.int32, (16, 128), 0)
        top1 = jnp.max(r)
        idx1 = jnp.min(jnp.where(r == top1, tok, S - 1))
        r2 = jnp.where(tok == idx1, -jnp.inf, r)
        top2 = jnp.max(r2)
        idx2 = jnp.min(jnp.where((r2 == top2) & (tok != idx1), tok, S - 1))
        idx_s[0] = idx1
        idx_s[1] = idx2
        gate_s[...] = jnp.where(lax.broadcasted_iota(jnp.int32, (16, 128), 0) == 0, top1, top2)
        sel_row = lax.broadcasted_iota(jnp.int32, (16, D), 0)
        xs1, _ = load_row(idx1)
        xs2, _ = load_row(idx2)
        xsel_s[...] = _b2u(jnp.where(sel_row == 0, xs1, jnp.where(sel_row == 1, xs2, 0.0)).astype(BF))

    def one_step(i, u, mem):
        odd = u % 2
        s2 = i * (UNROLL // 2) + u // 2
        h_ld = pl.multiple_of(16 * UNROLL * i, 32) + 32 * (u // 2)
        a24 = pl.multiple_of(12 * UNROLL * i, 8)
        r24 = pl.multiple_of(a24 % RING32, 8) + XS * (u // 2)
        a24 = a24 + XS * (u // 2)
        qkv_ld = pl.multiple_of((SEG * s2 + 32) % RING32, 32) + 16 * odd
        o_st = pl.multiple_of((SEG * s2) % RING32, 32) + 16 * odd
        m0 = 0 if odd else XS

        def with_mem(ref, idx, base, m):
            lo = ref[idx, pl.ds(base + 8 * odd, 8), :]
            hi = ref[idx, pl.ds(base + 8 + 8 * odd, 8), :]
            if odd:
                lo = jnp.where(low_half, m, lo)
            else:
                hi = jnp.where(low_half, hi, m)
            return _u2b(jnp.concatenate([lo, hi], axis=0))

        def store_tokens(ref, idx, base, yp):
            if odd:
                pltpu.store(ref.at[idx, pl.ds(base + 8, 8), :], yp[0:8], mask=high_half)
                ref[idx, pl.ds(base + 16, 8), :] = yp[8:16]
            else:
                ref[idx, pl.ds(base, 8), :] = yp[0:8]
                pltpu.store(ref.at[idx, pl.ds(base + 8, 8), :], yp[8:16], mask=low_half)

        lk = [with_mem(hbuf, k, h_ld, mem[k]) for k in range(KT)]
        lhs = jnp.concatenate(lk, axis=1)

        ymem = {}
        xs = {}
        probs = {}
        parts = {}

        def proj(h):
            split = h < K_SPLIT and u > 0
            if split:
                lhs7 = jnp.concatenate(lk[:KT - 1], axis=1)
                head = [_dot(lhs7, _u2b(wqkv[m * H + h, pl.ds(0, 448), :])) for m in range(3)]
            for m in range(3):
                if split:
                    y = _dot(lk[KT - 1], _u2b(wqkv[m * H + h, pl.ds(448, 64), :])) + head[m]
                else:
                    y = _dot(lhs, _u2b(wqkv[m * H + h]))
                store_tokens(ring, m * H + h, r24, _b2u(y.astype(BF)))
                ymem[(h, m)] = y[m0:m0 + MEM]
                xs[(h, m)] = ring[m * H + h, pl.ds(qkv_ld, SEG // 2), :]

        def pair(p, m):
            a, b = 2 * p, 2 * p + 1
            mm = jnp.concatenate([ymem[(a, m)], ymem[(b, m)]], axis=0).astype(BF)
            return jnp.concatenate([_u2b(xs[(a, m)]), _u2b(xs[(b, m)]), mm], axis=0)

        def qk(p):
            sc = _dot_nt(pair(p, 0), pair(p, 1))
            sc = jnp.where(allowed, sc * scale, fill)
            e = jnp.exp(sc - jnp.max(sc, axis=1, keepdims=True))
            l = jnp.sum(e, axis=1, keepdims=True)
            r = pl.reciprocal(l, approx=True)
            r = r * (2.0 - l * r)
            probs[p] = (e * r).astype(BF)

        def pv(p):
            op = _b2u(_dot(probs[p], pair(p, 2)).astype(BF))
            om = op[32:40]
            om_sw = pltpu.roll(om, 4, axis=0)
            for j, h in enumerate((2 * p, 2 * p + 1)):
                oring[h, pl.ds(o_st, SEG // 2), :] = op[16 * j:16 * j + 16]
                parts[h] = with_mem(oring, h, r24, om if j != odd else om_sw)

        def after(t):
            for lag, fn in ((LAG_QK, qk), (LAG_PV, pv)):
                if (t - 1 - lag) % 2 == 0 and 0 <= (t - 1 - lag) // 2 < NPAIR:
                    fn((t - 1 - lag) // 2)

        for t in range(H):
            proj(t)
            after(t)
            if u == 0 and t == 8:
                select_tokens()
        t = H
        lhs_a = jnp.concatenate([parts[j] for j in range(H_SPLIT)], axis=1)
        acc = []
        for n in range(N_PART):
            acc.append(_dot(lhs_a, _u2b(wo_s[n, pl.ds(0, H_SPLIT * 64), :])))
            after(t)
            t += 1
        while t - 1 - LAG_PV <= 2 * (NPAIR - 1):
            after(t)
            t += 1
        lhs_b = jnp.concatenate([parts[j] for j in range(H_SPLIT, H)], axis=1)
        lhs_o = jnp.concatenate([lhs_a, lhs_b], axis=1)
        new_mem = [None] * KT

        def finish(n, y):
            store_tokens(abuf, n, a24, _b2u(y.astype(BF)))
            ym = y[m0:m0 + MEM]
            new_mem[n] = _b2u(jnp.concatenate([ym, ym], axis=0).astype(BF))

        for n in range(N_PART, KT):
            finish(n, _dot(lhs_o, _u2b(wo_s[n])))
            if n == N_PART:
                for n2 in range(N_PART):
                    tail = _u2b(wo_s[n2, pl.ds(H_SPLIT * 64, (H - H_SPLIT) * 64), :])
                    finish(n2, _dot(lhs_b, tail) + acc[n2])
        return new_mem

    def body(i, mem):
        mem = list(mem)
        for u in range(UNROLL):
            mem = one_step(i, u, mem)
        return tuple(mem)

    for n in range(KT):
        wo_copy(n).wait()
    mi = mem0_s[...].astype(F32)
    mip = _b2u(jnp.concatenate([mi, mi], axis=0).astype(BF))
    lax.fori_loop(0, NSEG // UNROLL, body,
                  tuple(mip[:, 128 * k:128 * (k + 1)] for k in range(KT)))

    early = S - PRE
    zrow = pl.multiple_of(zero_s[0], 16)
    FPER = 9

    def half_rows(r0):
        return r0 // 2 if isinstance(r0, int) else pl.multiple_of(r0 // 2, 8)

    def combine(r0, nrows, n, a):
        xf = x_s[pl.ds(r0, nrows), pl.ds(128 * n, 128)].astype(F32)
        b = _u2b(xn_t[n, pl.ds(half_rows(r0), nrows // 2), :]).astype(F32)
        out_s[pl.ds(r0, nrows), pl.ds(128 * n, 128)] = (_rbf(xf + a) + b).astype(BF)

    def combine_stored(r0, nrows, not_before=None):
        for n in range(KT):
            a = abuf[n, pl.ds(half_rows(r0), nrows // 2), :]
            if not_before is not None:
                a = a | jnp.concatenate([not_before & zero_box[0]] * (nrows // 16), axis=0)
            combine(r0, nrows, n, _u2b(a).astype(F32))

    def out_copy(r0, nrows, j):
        return pltpu.make_async_copy(out_s.at[pl.ds(r0, nrows), :], out_hbm.at[pl.ds(r0, nrows), :],
                                     sems.at[SEM_OUT + j])

    def ffn_groups(j0, count, y, done):
        x_sel = _u2b(xsel_s[...])
        hid = {}

        def up(w_ref, j, key):
            part = _dot(x_sel[:, 0:512], _u2b(w_ref[j, pl.ds(0, 256), :]))
            yield
            hid[key] = _rbf(_dot(x_sel[:, 512:1024], _u2b(w_ref[j, pl.ds(256, 256), :])) + part)
            yield

        def down(jj):
            g = hid[("g", jj)]
            hb = (_rbf(g * _rbf(jax.nn.sigmoid(g))) * hid[("u", jj)]).astype(BF)
            rows = pl.ds(pl.multiple_of(64 * (j0 + jj), 64), 64)
            for half in range(2):
                w = jnp.concatenate([_u2b(wd_s[4 * half + n, rows, :]) for n in range(4)], axis=1)
                y[half] = _dot(hb, w) + y[half]
                yield

        for jj in range(count + 1):
            if jj < count:
                yield from up(wg_s, j0 + jj, ("g", jj))
                yield from up(wu_s, j0 + jj, ("u", jj))
            elif count == 1:
                yield
                yield
            if jj >= 1:
                yield from down(jj - 1)
        done()

    def epi_chunk(r0, nrows, side, pieces, keep):
        pos = [((r0 + 32 * j) % RING) // 2 for j in range(nrows // 32)]
        if not isinstance(r0, int):
            pos = [pl.multiple_of(p, 16) for p in pos]
        fresh_zero()
        deps = {}
        for n in range(KT):
            acc = None
            for g in range(8):
                lhs = jnp.concatenate(
                    [_u2b(jnp.concatenate([oring[h, pl.ds(p, 16), :] for p in pos], axis=0))
                     for h in range(4 * g, 4 * g + 4)], axis=1)
                w = _after(wo_s[n, pl.ds(256 * g, 256), :], deps.get(8 * n + g), zero_box[0])
                y = _dot(lhs, _u2b(w))
                acc = y if acc is None else y + acc
                next(side, None)
                v = 8 * n + g
                if pieces is not None and v in EPI_SCHED:
                    r1 = pieces + 32 * EPI_SCHED.index(v)
                    combine_stored(r1, 32, pltpu.bitcast(acc[0:8], U32) if EPI_NB else None)
                    if EPI_LAG:
                        deps[v + EPI_LAG] = [_b2u(out_s[pl.ds(r1 + (zrow if EPI_ALIAS else 0), 16), pl.ds(D - 128, 128)])]
            ab = acc.astype(BF)
            if keep:
                abuf[n, pl.ds(half_rows(r0), nrows // 2), :] = _b2u(ab)
            combine(r0, nrows, n, ab.astype(F32))

    for c in ffn_copies:
        c.wait()

    def epi_body(c, y):
        y = list(y)
        r0 = pl.multiple_of(early + ECH * c, 32)
        e0 = pl.multiple_of((early // 2) * (c & 1), 256)

        @pl.when(c == 2)
        def _():
            out_copy(0, early // 2, 4).wait()

        epi_chunk(r0, ECH, ffn_groups(FPER * c, FPER, y, lambda: None), e0, True)
        out_copy(r0, ECH, c).start()

        @pl.when(c < 2)
        def _():
            out_copy(e0, early // 2, 4 + c).start()

        return tuple(y)

    y = list(lax.fori_loop(0, 3, epi_body, (jnp.zeros((16, 512), F32), jnp.zeros((16, 512), F32))))
    idx1 = idx_s[0]
    idx2 = idx_s[1]

    def patch_row(t, yrow):
        xr, w = load_row(t)
        bits = pltpu.bitcast(_rbf(xr + yrow), U32)
        w = jnp.where(t % 2 == 0,
                      (w & jnp.uint32(0xFFFF0000)) | (bits >> 16),
                      (w & jnp.uint32(0xFFFF)) | bits)
        for k in range(KT):
            xn_t[k, pl.ds(t // 2, 1), :] = w[:, 128 * k:128 * (k + 1)]

    def patch():
        gate = _rbf(jax.nn.sigmoid(gate_s[:, 0:1]))
        yy = _rbf(_rbf(jnp.concatenate(y, axis=1)) * gate)
        patch_row(idx1, yy[0:1])
        patch_row(idx2, yy[1:2])

    last = early + 3 * ECH
    epi_chunk(last, S - last, ffn_groups(3 * FPER, 1, y, patch), None, False)
    out_copy(last, S - last, 3).start()
    for c in range(3):
        out_copy(early + ECH * c, ECH, c).wait()
    out_copy(early // 2, early // 2, 5).wait()
    blk1 = jnp.minimum(idx1 // 16, last // 16 - 1)
    blk2 = jnp.minimum(idx2 // 16, last // 16 - 1)
    blk2 = jnp.where(blk2 == blk1, jnp.where(blk1 == 0, 1, blk1 - 1), blk2)
    fix = []
    for j, blk in enumerate((blk1, blk2)):
        r0 = pl.multiple_of(blk * 16, 16)
        combine_stored(r0, 16)
        fix.append(out_copy(r0, 16, 7 + j))
    for cp in fix:
        cp.start()
    out_copy(last, S - last, 3).wait()
    for cp in fix:
        cp.wait()


@jax.jit
def pallas_parallel_sum__memory_aug_recurrent_mem_tr__moe_arch_mod__prompt_kernel(
    A_x: jax.Array,
    A_mem0: jax.Array,
    A_Wq: jax.Array,
    A_Wk: jax.Array,
    A_Wv: jax.Array,
    A_Wo: jax.Array,
    A_seg_len: jax.Array,
    B_x: jax.Array,
    B_w_r: jax.Array,
    B_w_gate: jax.Array,
    B_w_up: jax.Array,
    B_w_down: jax.Array,
):
    del A_seg_len, B_x
    assert A_x.shape == (1, S, D) and A_mem0.shape == (1, MEM, D)
    assert A_Wq.shape == (D, H, DH) and A_Wo.shape == (H, DH, D)
    assert B_w_gate.shape == (D, FF) and B_w_down.shape == (FF, D)
    any_spec = pl.BlockSpec(memory_space=pl.ANY)
    out = pl.pallas_call(
        _kernel,
        out_shape=jax.ShapeDtypeStruct((S, D), BF),
        in_specs=[any_spec] * 10,
        out_specs=any_spec,
        scratch_shapes=[
            pltpu.VMEM((S, D), BF),
            pltpu.VMEM((KT, S // 2, 128), U32),
            pltpu.VMEM((KT, PRE // 2, 128), U32),
            pltpu.VMEM((KT, 16 * NSEG, 128), U32),
            pltpu.VMEM((3 * H + 2, D // 2, 128), U32),
            pltpu.VMEM((KT, H * DH // 2, 128), U32),
            pltpu.VMEM((3 * H, RING32, 128), U32),
            pltpu.VMEM((H, RING32, 128), U32),
            pltpu.VMEM((KT, S // 2, 128), U32),
            pltpu.VMEM((S, D), BF),
            pltpu.VMEM((NPQ + 1, D, 128), U32),
            pltpu.VMEM((FT, D // 2, 128), U32),
            pltpu.VMEM((FT, D // 2, 128), U32),
            pltpu.VMEM((KT, FF // 2, 128), U32),
            pltpu.VMEM((MEM, D), BF),
            pltpu.VMEM((D,), BF),
            pltpu.VMEM((8, D), F32),
            pltpu.VMEM((16, 128), F32),
            pltpu.VMEM((8, D), U32),
            pltpu.VMEM((16, 128), F32),
            pltpu.SMEM((1,), jnp.int32),
            pltpu.SMEM((2,), jnp.int32),
            pltpu.SemaphoreType.DMA((NSEM,)),
        ],
        compiler_params=pltpu.CompilerParams(vmem_limit_bytes=126 * 1024 * 1024),
    )(A_x.reshape(S, D), A_mem0.reshape(MEM, D), A_Wq, A_Wk, A_Wv, A_Wo.reshape(H * DH, D),
      B_w_r, B_w_gate, B_w_up, B_w_down)
    return out.reshape(1, S, D)
```

```python
import jax
import jax.numpy as jnp
from jax import lax
import jax.experimental.pallas as pl
import jax.experimental.pallas.tpu as pltpu

BF = jnp.bfloat16
U32 = jnp.uint32
F32 = jnp.float32

S = 2048
D = 1024
H = 32
DH = 128
MEM = 8
SEG = 32
NSEG = S // SEG
FF = 3584
KT = D // 128
FT = FF // 128
XS = 24
PRE = S - NSEG * XS
RING = 576
RING32 = RING // 2
NPAIR = H // 2
NPQ = 3 * NPAIR
NPRE = 16
SEM_SMALL, SEM_X0, SEM_X = 0, 2, 6
SEM_W0 = SEM_X + NPRE
SEM_W = SEM_W0 + 3
SEM_WO = SEM_W + NPRE
SEM_FFN, SEM_OUT = SEM_WO + 1, SEM_WO + 2
NSEM = SEM_OUT + 9

LAG_QK = 1
LAG_PV = 4
N_PART = 4
H_SPLIT = 26
REL_SCHED = {0: [(0, 0), (0, 1)], 1: [(0, 2), (0, 3)], 2: [(0, 4)], 3: [(0, 5)], 4: [(0, 6)], 5: [(0, 7)]}
REL_SCHED.update({6 + k: [(1, k)] for k in range(8)})
REL_SCHED.update({14 + k: [(2, k)] for k in range(8)})
K_SPLIT = 2
EPI_SCHED = [v * 5 // 2 for v in range(24)]
EPI_LAG = 4
ECH = 160
EPI_NB = False
EPI_ALIAS = False
REL_SCHED0 = {4: [(0, k) for k in range(4)], 5: [(0, k) for k in range(4, 8)],
              12: [(1, k) for k in range(4)], 13: [(1, k) for k in range(4, 8)]}
REL_SCHED0.update({14 + k: [(2, k)] for k in range(8)})
SCORE_SCHED = [1, 7, 13]
LN_SCHED = {3 * q: [q] for q in range(6)}
LN_SCHED0 = {13 + q: [q] for q in range(6)}
FIRST_BATCH = 12
LN_LAG = 5
REL_LAG = 2
UNROLL = 4


def _b2u(x):
    return pltpu.bitcast(x, U32)


def _u2b(x):
    return pltpu.bitcast(x, BF)


def _dot(a, b):
    return jnp.dot(a, b, preferred_element_type=F32)


def _dot_nt(a, b):
    return lax.dot_general(a, b, (((1,), (1,)), ((), ())), preferred_element_type=F32)


def _after(w, dep, zero):
    if not dep:
        return w
    d = dep[0]
    for e in dep[1:]:
        d = d | e
    return jnp.concatenate([w[0:8] | (d & zero), w[8:]], axis=0)


def _rbf(x):
    return x.astype(BF).astype(F32)


def _kernel(x_hbm, mem0_hbm, wq_hbm, wk_hbm, wv_hbm, wo_hbm, wr_hbm, wg_hbm, wu_hbm, wd_hbm,
            out_hbm,
            x_s, xn_t, xn_pre, hbuf, wqkv, wo_s, ring, oring, abuf, out_s, raw,
            wg_s, wu_s, wd_s, mem0_s, wr_s, wrf_s, r_s, xsel_s, gate_s, zero_s, idx_s,
            sems):
    w32 = [w.bitcast(U32) for w in (wq_hbm, wk_hbm, wv_hbm)]
    wo32 = wo_hbm.bitcast(U32)
    wg32 = wg_hbm.bitcast(U32)
    wu32 = wu_hbm.bitcast(U32)
    wd32 = wd_hbm.bitcast(U32)

    def rows_copy(r0, n, sem):
        return pltpu.make_async_copy(x_hbm.at[pl.ds(r0, n), :], x_s.at[pl.ds(r0, n), :], sems.at[sem])

    def x_first(c):
        return rows_copy(128 * c if isinstance(c, int) else pl.multiple_of(128 * c, 128), 128, SEM_X0 + c)

    def x_piece(c):
        r0 = PRE + 96 * c if isinstance(c, int) else pl.multiple_of(PRE + 96 * c, 32)
        return rows_copy(r0, 96, SEM_X + c)

    def pair_copy(p):
        q = min(p, NPQ - 1)
        sem = SEM_W0 + p if p < 4 else SEM_W + (p - 1) // 3
        return pltpu.make_async_copy(w32[q // NPAIR].at[:, q % NPAIR, :], raw.at[p], sems.at[sem])

    def pairs_wait(t):
        dst = raw.at[pl.ds(3 * t + 1, 3)]
        pltpu.make_async_copy(dst, dst, sems.at[SEM_W + t]).wait()

    def wo_copy(n):
        return pltpu.make_async_copy(wo32.at[:, pl.ds(128 * n, 128)], wo_s.at[n], sems.at[SEM_WO])

    small_copies = [pltpu.make_async_copy(mem0_hbm, mem0_s, sems.at[SEM_SMALL]),
                    pltpu.make_async_copy(wr_hbm, wr_s, sems.at[SEM_SMALL + 1])]
    ffn_copies = [pltpu.make_async_copy(s_, d_, sems.at[SEM_FFN])
                  for s_, d_ in ((wg32, wg_s), (wu32, wu_s), (wd32, wd_s))]

    zero_s[0] = 0
    for c in range(4):
        x_first(c).start()
        if c == 0:
            for cp in small_copies:
                cp.start()

    def queue(t0, t1):
        for t in range(t0, t1):
            for p in range(3 * t + 1, 3 * t + 4):
                pair_copy(p).start()
            x_piece(t).start()

    pair_copy(0).start()
    queue(0, FIRST_BATCH)
    eps_bf = 1.0013580322265625e-05

    def score16(g, xn):
        wr = jnp.concatenate([wrf_s[...], wrf_s[...]], axis=0)
        score = _rbf(jnp.sum(xn.astype(F32) * wr, axis=1, keepdims=True))
        r_s[...] = jnp.where(lane16 == g, score, r_s[...])

    def layernorm16(rq, dst_ref, dst_row, not_before=None):
        rq = rq if isinstance(rq, int) else pl.multiple_of(rq, 16)
        xf = x_s[pl.ds(rq, 16), :].astype(F32)
        if not_before is not None:
            x0 = _after(pltpu.bitcast(xf[:, 0:128], U32), [not_before], zero_box[0])
            xf = jnp.concatenate([pltpu.bitcast(x0, F32), xf[:, 128:]], axis=1)
        mean = jnp.sum(xf, axis=1, keepdims=True) * (1.0 / D)
        cen = xf - mean
        var = jnp.sum(cen * cen, axis=1, keepdims=True) * (1.0 / D)
        sd = _rbf(jnp.sqrt(_rbf(_rbf(var) + eps_bf)))
        xn = (_rbf(xf - _rbf(mean)) * (1.0 / sd)).astype(BF)
        if dst_ref is hbuf:
            score16(rq // 16, xn)
        xp = _b2u(xn)
        hq = rq // 2 if isinstance(rq, int) else pl.multiple_of(rq // 2, 8)
        dst_row = dst_row if isinstance(dst_row, int) else pl.multiple_of(dst_row, 8)
        for k in range(KT):
            xn_t[k, pl.ds(hq, 8), :] = xp[:, 128 * k:128 * (k + 1)]
            dst_ref[k, pl.ds(dst_row, 8), :] = xp[:, 128 * k:128 * (k + 1)]

    zero_box = [None]

    def fresh_zero():
        zero_box[0] = jnp.full((8, 128), zero_s[0], jnp.int32).astype(U32)

    r_s[...] = jnp.full(r_s.shape, -jnp.inf, F32)
    lane16 = lax.broadcasted_iota(jnp.int32, (16, 128), 1)

    def ln_body(c, carry):
        x_first(c).wait()
        for q in range(8):
            layernorm16(128 * c + 16 * q, xn_pre, 64 * c + 8 * q)
        return carry

    lax.fori_loop(0, PRE // 128, ln_body, 0)


    def relayout(src, dst, j, k, not_before=None):
        a = src[j, pl.ds(128 * k, 64, stride=2), :]
        if not_before is not None:
            a = a | jnp.concatenate([not_before & zero_box[0]] * 8, axis=0)
        b = src[j, pl.ds(128 * k + 1, 64, stride=2), :]
        rows = pl.ds(64 * k, 64)
        dst[2 * j, rows, :] = (a & jnp.uint32(0xFFFF)) | (b << 16)
        dst[2 * j + 1, rows, :] = (a >> 16) | (b & jnp.uint32(0xFFFF0000))

    def pre_dot(w_view, ring_view, j, k, dep=None):
        i, q = k // 4, k % 4
        lhs = jnp.concatenate([_u2b(xn_pre[kk, pl.ds(64 * q, 64), :]) for kk in range(KT)], axis=1)
        y = _dot(lhs, _u2b(_after(w_view[2 * j + i], dep, zero_box[0])))
        yp = _b2u(y.astype(BF))
        ring_view[2 * j + i, pl.ds(32 + 64 * q, 64), :] = yp
        return yp[0:8]

    for c in small_copies:
        c.wait()
    pair_copy(0).wait()
    for k in range(8):
        relayout(raw, wqkv, 0, k)
    wrf_s[...] = jnp.broadcast_to(wr_s[...].astype(F32).reshape(1, D), (8, D))

    def pre_iter(t, barriers):
        deps = {}
        raw_view = raw.at[pl.ds(3 * t, 4)]
        w_view = wqkv.at[pl.ds(6 * t, 8)]
        ring_view = ring.at[pl.ds(6 * t, 6)]
        rel_sched, ln_sched = (REL_SCHED0, LN_SCHED0) if barriers else (REL_SCHED, LN_SCHED)
        done = None
        for v in range(24):
            j, k = v // 8, v % 8
            if v == 0 or v in barriers:
                for wait in barriers.get(v, ()):
                    wait()
                fresh_zero()
                done = None
            prev = done
            done = pre_dot(w_view, ring_view, j, k, deps.get(v))
            for jr, kr in rel_sched.get(v, ()):
                relayout(raw_view, w_view, jr + 1, kr, prev)
                deps.setdefault(v + REL_LAG, []).append(w_view[2 * jr + 3, pl.ds(64 * kr + 56, 8), :])
            for q in ln_sched.get(v, ()):
                hrow = 32 * (q // 3) + 8 * (q % 3)
                hrow += 64 * t if isinstance(t, int) else pl.multiple_of(64 * t, 64)
                layernorm16(PRE + 96 * t + 16 * q, hbuf, hrow, done if prev is not None else None)
                deps.setdefault(v + LN_LAG, []).append(hbuf[KT - 1, pl.ds(hrow, 8), :])
            if not barriers and v in SCORE_SCHED:
                g = jnp.minimum(3 * (t - 1) + SCORE_SCHED.index(v), PRE // 16 - 1)
                rows = pl.ds(pl.multiple_of(8 * g, 8), 8)
                xp = [xn_pre[kk, rows, :] for kk in range(KT)]
                xp[0] = xp[0] | (done & zero_box[0])
                score16(g, _u2b(jnp.concatenate(xp, axis=1)))

    def second_batch():
        queue(FIRST_BATCH, NPRE)
        for n in range(KT):
            wo_copy(n).start()
        for cp in ffn_copies:
            cp.start()

    pre_iter(0, {4: [pair_copy(1).wait],
                 12: [pair_copy(2).wait, pair_copy(3).wait, x_piece(0).wait, second_batch]})

    def pre_body(t, carry):
        x_piece(t).wait()
        pairs_wait(t)
        pre_iter(t, {})
        return carry

    lax.fori_loop(1, NPRE, pre_body, 0)
    row = lax.broadcasted_iota(jnp.int32, (80, 80), 0)
    col = lax.broadcasted_iota(jnp.int32, (80, 80), 1)
    same_head = (jnp.where(row < 64, row >> 5, (row - 64) >> 3)
                 == jnp.where(col < 64, col >> 5, (col - 64) >> 3))
    allowed = same_head & ((col >= 64) | (row >= 64) | (col <= row))
    fill = jnp.where(same_head, -1e9, -jnp.inf).astype(F32)
    low_half = lax.broadcasted_iota(jnp.int32, (8, 128), 0) < 4
    high_half = jnp.logical_not(low_half)
    scale = DH ** -0.5

    def load_row(t):
        w = jnp.concatenate([xn_t[k, pl.ds(t // 2, 1), :] for k in range(KT)], axis=1)
        bits = jnp.where(t % 2 == 0, w << 16, w & jnp.uint32(0xFFFF0000))
        return pltpu.bitcast(bits, F32), w

    def select_tokens():
        r = r_s[...]
        tok = lane16 * 16 + lax.broadcasted_iota(jnp.int32, (16, 128), 0)
        top1 = jnp.max(r)
        idx1 = jnp.min(jnp.where(r == top1, tok, S - 1))
        r2 = jnp.where(tok == idx1, -jnp.inf, r)
        top2 = jnp.max(r2)
        idx2 = jnp.min(jnp.where((r2 == top2) & (tok != idx1), tok, S - 1))
        idx_s[0] = idx1
        idx_s[1] = idx2
        gate_s[...] = jnp.where(lax.broadcasted_iota(jnp.int32, (16, 128), 0) == 0, top1, top2)
        sel_row = lax.broadcasted_iota(jnp.int32, (16, D), 0)
        xs1, _ = load_row(idx1)
        xs2, _ = load_row(idx2)
        xsel_s[...] = _b2u(jnp.where(sel_row == 0, xs1, jnp.where(sel_row == 1, xs2, 0.0)).astype(BF))

    def one_step(i, u, mem):
        odd = u % 2
        s2 = i * (UNROLL // 2) + u // 2
        h_ld = pl.multiple_of(16 * UNROLL * i, 32) + 32 * (u // 2)
        a24 = pl.multiple_of(12 * UNROLL * i, 8)
        r24 = pl.multiple_of(a24 % RING32, 8) + XS * (u // 2)
        a24 = a24 + XS * (u // 2)
        qkv_ld = pl.multiple_of((SEG * s2 + 32) % RING32, 32) + 16 * odd
        o_st = pl.multiple_of((SEG * s2) % RING32, 32) + 16 * odd
        m0 = 0 if odd else XS

        def with_mem(ref, idx, base, m):
            lo = ref[idx, pl.ds(base + 8 * odd, 8), :]
            hi = ref[idx, pl.ds(base + 8 + 8 * odd, 8), :]
            if odd:
                lo = jnp.where(low_half, m, lo)
            else:
                hi = jnp.where(low_half, hi, m)
            return _u2b(jnp.concatenate([lo, hi], axis=0))

        def store_tokens(ref, idx, base, yp):
            if odd:
                pltpu.store(ref.at[idx, pl.ds(base + 8, 8), :], yp[0:8], mask=high_half)
                ref[idx, pl.ds(base + 16, 8), :] = yp[8:16]
            else:
                ref[idx, pl.ds(base, 8), :] = yp[0:8]
                pltpu.store(ref.at[idx, pl.ds(base + 8, 8), :], yp[8:16], mask=low_half)

        lk = [with_mem(hbuf, k, h_ld, mem[k]) for k in range(KT)]
        lhs = jnp.concatenate(lk, axis=1)

        ymem = {}
        xs = {}
        probs = {}
        parts = {}

        def proj(h):
            split = h < K_SPLIT and u > 0
            if split:
                lhs7 = jnp.concatenate(lk[:KT - 1], axis=1)
                head = [_dot(lhs7, _u2b(wqkv[m * H + h, pl.ds(0, 448), :])) for m in range(3)]
            for m in range(3):
                if split:
                    y = _dot(lk[KT - 1], _u2b(wqkv[m * H + h, pl.ds(448, 64), :])) + head[m]
                else:
                    y = _dot(lhs, _u2b(wqkv[m * H + h]))
                store_tokens(ring, m * H + h, r24, _b2u(y.astype(BF)))
                ymem[(h, m)] = y[m0:m0 + MEM]
                xs[(h, m)] = ring[m * H + h, pl.ds(qkv_ld, SEG // 2), :]

        def pair(p, m):
            a, b = 2 * p, 2 * p + 1
            mm = jnp.concatenate([ymem[(a, m)], ymem[(b, m)]], axis=0).astype(BF)
            return jnp.concatenate([_u2b(xs[(a, m)]), _u2b(xs[(b, m)]), mm], axis=0)

        def qk(p):
            sc = _dot_nt(pair(p, 0), pair(p, 1))
            sc = jnp.where(allowed, sc * scale, fill)
            e = jnp.exp(sc - jnp.max(sc, axis=1, keepdims=True))
            l = jnp.sum(e, axis=1, keepdims=True)
            r = pl.reciprocal(l, approx=True)
            r = r * (2.0 - l * r)
            probs[p] = (e * r).astype(BF)

        def pv(p):
            op = _b2u(_dot(probs[p], pair(p, 2)).astype(BF))
            om = op[32:40]
            om_sw = pltpu.roll(om, 4, axis=0)
            for j, h in enumerate((2 * p, 2 * p + 1)):
                oring[h, pl.ds(o_st, SEG // 2), :] = op[16 * j:16 * j + 16]
                parts[h] = with_mem(oring, h, r24, om if j != odd else om_sw)

        def after(t):
            for lag, fn in ((LAG_QK, qk), (LAG_PV, pv)):
                if (t - 1 - lag) % 2 == 0 and 0 <= (t - 1 - lag) // 2 < NPAIR:
                    fn((t - 1 - lag) // 2)

        for t in range(H):
            proj(t)
            after(t)
            if u == 0 and t == 8:
                select_tokens()
        t = H
        lhs_a = jnp.concatenate([parts[j] for j in range(H_SPLIT)], axis=1)
        acc = []
        for n in range(N_PART):
            acc.append(_dot(lhs_a, _u2b(wo_s[n, pl.ds(0, H_SPLIT * 64), :])))
            after(t)
            t += 1
        while t - 1 - LAG_PV <= 2 * (NPAIR - 1):
            after(t)
            t += 1
        lhs_b = jnp.concatenate([parts[j] for j in range(H_SPLIT, H)], axis=1)
        lhs_o = jnp.concatenate([lhs_a, lhs_b], axis=1)
        new_mem = [None] * KT

        def finish(n, y):
            store_tokens(abuf, n, a24, _b2u(y.astype(BF)))
            ym = y[m0:m0 + MEM]
            new_mem[n] = _b2u(jnp.concatenate([ym, ym], axis=0).astype(BF))

        for n in range(N_PART, KT):
            finish(n, _dot(lhs_o, _u2b(wo_s[n])))
            if n == N_PART:
                for n2 in range(N_PART):
                    tail = _u2b(wo_s[n2, pl.ds(H_SPLIT * 64, (H - H_SPLIT) * 64), :])
                    finish(n2, _dot(lhs_b, tail) + acc[n2])
        return new_mem

    def body(i, mem):
        mem = list(mem)
        for u in range(UNROLL):
            mem = one_step(i, u, mem)
        return tuple(mem)

    for n in range(KT):
        wo_copy(n).wait()
    mi = mem0_s[...].astype(F32)
    mip = _b2u(jnp.concatenate([mi, mi], axis=0).astype(BF))
    lax.fori_loop(0, NSEG // UNROLL, body,
                  tuple(mip[:, 128 * k:128 * (k + 1)] for k in range(KT)))

    early = S - PRE
    zrow = pl.multiple_of(zero_s[0], 16)
    FPER = 9

    def half_rows(r0):
        return r0 // 2 if isinstance(r0, int) else pl.multiple_of(r0 // 2, 8)

    def combine(r0, nrows, n, a):
        xf = x_s[pl.ds(r0, nrows), pl.ds(128 * n, 128)].astype(F32)
        b = _u2b(xn_t[n, pl.ds(half_rows(r0), nrows // 2), :]).astype(F32)
        out_s[pl.ds(r0, nrows), pl.ds(128 * n, 128)] = (_rbf(xf + a) + b).astype(BF)

    def combine_stored(r0, nrows, not_before=None):
        for n in range(KT):
            a = abuf[n, pl.ds(half_rows(r0), nrows // 2), :]
            if not_before is not None:
                a = a | jnp.concatenate([not_before & zero_box[0]] * (nrows // 16), axis=0)
            combine(r0, nrows, n, _u2b(a).astype(F32))

    def out_copy(r0, nrows, j):
        return pltpu.make_async_copy(out_s.at[pl.ds(r0, nrows), :], out_hbm.at[pl.ds(r0, nrows), :],
                                     sems.at[SEM_OUT + j])

    def ffn_groups(j0, count, y, done):
        x_sel = _u2b(xsel_s[...])
        hid = {}

        def up(w_ref, j, key):
            cols = pl.ds(128 * j if isinstance(j, int) else pl.multiple_of(128 * j, 128), 128)
            part = _dot(x_sel[:, 0:512], _u2b(w_ref[pl.ds(0, 256), cols]))
            yield
            hid[key] = _rbf(_dot(x_sel[:, 512:1024], _u2b(w_ref[pl.ds(256, 256), cols])) + part)
            yield

        def down(jj):
            g = hid[("g", jj)]
            hb = (_rbf(g * _rbf(jax.nn.sigmoid(g))) * hid[("u", jj)]).astype(BF)
            rows = pl.ds(pl.multiple_of(64 * (j0 + jj), 64), 64)
            for half in range(2):
                y[half] = _dot(hb, _u2b(wd_s[rows, pl.ds(512 * half, 512)])) + y[half]
                yield

        for jj in range(count + 1):
            if jj < count:
                yield from up(wg_s, j0 + jj, ("g", jj))
                yield from up(wu_s, j0 + jj, ("u", jj))
            elif count == 1:
                yield
                yield
            if jj >= 1:
                yield from down(jj - 1)
        done()

    def epi_chunk(r0, nrows, side, pieces, keep):
        pos = [((r0 + 32 * j) % RING) // 2 for j in range(nrows // 32)]
        if not isinstance(r0, int):
            pos = [pl.multiple_of(p, 16) for p in pos]
        fresh_zero()
        deps = {}
        for n in range(KT):
            acc = None
            for g in range(8):
                lhs = jnp.concatenate(
                    [_u2b(jnp.concatenate([oring[h, pl.ds(p, 16), :] for p in pos], axis=0))
                     for h in range(4 * g, 4 * g + 4)], axis=1)
                w = _after(wo_s[n, pl.ds(256 * g, 256), :], deps.get(8 * n + g), zero_box[0])
                y = _dot(lhs, _u2b(w))
                acc = y if acc is None else y + acc
                next(side, None)
                v = 8 * n + g
                if pieces is not None and v in EPI_SCHED:
                    r1 = pieces + 32 * EPI_SCHED.index(v)
                    combine_stored(r1, 32, pltpu.bitcast(acc[0:8], U32) if EPI_NB else None)
                    if EPI_LAG:
                        deps[v + EPI_LAG] = [_b2u(out_s[pl.ds(r1 + (zrow if EPI_ALIAS else 0), 16), pl.ds(D - 128, 128)])]
            ab = acc.astype(BF)
            if keep:
                abuf[n, pl.ds(half_rows(r0), nrows // 2), :] = _b2u(ab)
            combine(r0, nrows, n, ab.astype(F32))

    for c in ffn_copies:
        c.wait()

    def epi_body(c, y):
        y = list(y)
        r0 = pl.multiple_of(early + ECH * c, 32)
        e0 = pl.multiple_of((early // 2) * (c & 1), 256)

        @pl.when(c == 2)
        def _():
            out_copy(0, early // 2, 4).wait()

        epi_chunk(r0, ECH, ffn_groups(FPER * c, FPER, y, lambda: None), e0, True)
        out_copy(r0, ECH, c).start()

        @pl.when(c < 2)
        def _():
            out_copy(e0, early // 2, 4 + c).start()

        return tuple(y)

    y = list(lax.fori_loop(0, 3, epi_body, (jnp.zeros((16, 512), F32), jnp.zeros((16, 512), F32))))
    idx1 = idx_s[0]
    idx2 = idx_s[1]

    def patch_row(t, yrow):
        xr, w = load_row(t)
        bits = pltpu.bitcast(_rbf(xr + yrow), U32)
        w = jnp.where(t % 2 == 0,
                      (w & jnp.uint32(0xFFFF0000)) | (bits >> 16),
                      (w & jnp.uint32(0xFFFF)) | bits)
        for k in range(KT):
            xn_t[k, pl.ds(t // 2, 1), :] = w[:, 128 * k:128 * (k + 1)]

    def patch():
        gate = _rbf(jax.nn.sigmoid(gate_s[:, 0:1]))
        yy = _rbf(_rbf(jnp.concatenate(y, axis=1)) * gate)
        patch_row(idx1, yy[0:1])
        patch_row(idx2, yy[1:2])

    last = early + 3 * ECH
    epi_chunk(last, S - last, ffn_groups(3 * FPER, 1, y, patch), None, False)
    out_copy(last, S - last, 3).start()
    for c in range(3):
        out_copy(early + ECH * c, ECH, c).wait()
    out_copy(early // 2, early // 2, 5).wait()
    blk1 = jnp.minimum(idx1 // 16, last // 16 - 1)
    blk2 = jnp.minimum(idx2 // 16, last // 16 - 1)
    blk2 = jnp.where(blk2 == blk1, jnp.where(blk1 == 0, 1, blk1 - 1), blk2)
    fix = []
    for j, blk in enumerate((blk1, blk2)):
        r0 = pl.multiple_of(blk * 16, 16)
        combine_stored(r0, 16)
        fix.append(out_copy(r0, 16, 7 + j))
    for cp in fix:
        cp.start()
    out_copy(last, S - last, 3).wait()
    for cp in fix:
        cp.wait()


@jax.jit
def pallas_parallel_sum__memory_aug_recurrent_mem_tr__moe_arch_mod__prompt_kernel(
    A_x: jax.Array,
    A_mem0: jax.Array,
    A_Wq: jax.Array,
    A_Wk: jax.Array,
    A_Wv: jax.Array,
    A_Wo: jax.Array,
    A_seg_len: jax.Array,
    B_x: jax.Array,
    B_w_r: jax.Array,
    B_w_gate: jax.Array,
    B_w_up: jax.Array,
    B_w_down: jax.Array,
):
    del A_seg_len, B_x
    assert A_x.shape == (1, S, D) and A_mem0.shape == (1, MEM, D)
    assert A_Wq.shape == (D, H, DH) and A_Wo.shape == (H, DH, D)
    assert B_w_gate.shape == (D, FF) and B_w_down.shape == (FF, D)
    any_spec = pl.BlockSpec(memory_space=pl.ANY)
    out = pl.pallas_call(
        _kernel,
        out_shape=jax.ShapeDtypeStruct((S, D), BF),
        in_specs=[any_spec] * 10,
        out_specs=any_spec,
        scratch_shapes=[
            pltpu.VMEM((S, D), BF),
            pltpu.VMEM((KT, S // 2, 128), U32),
            pltpu.VMEM((KT, PRE // 2, 128), U32),
            pltpu.VMEM((KT, 16 * NSEG, 128), U32),
            pltpu.VMEM((3 * H + 2, D // 2, 128), U32),
            pltpu.VMEM((KT, H * DH // 2, 128), U32),
            pltpu.VMEM((3 * H, RING32, 128), U32),
            pltpu.VMEM((H, RING32, 128), U32),
            pltpu.VMEM((KT, S // 2, 128), U32),
            pltpu.VMEM((S, D), BF),
            pltpu.VMEM((NPQ + 1, D, 128), U32),
            pltpu.VMEM((D // 2, FF), U32),
            pltpu.VMEM((D // 2, FF), U32),
            pltpu.VMEM((FF // 2, D), U32),
            pltpu.VMEM((MEM, D), BF),
            pltpu.VMEM((D,), BF),
            pltpu.VMEM((8, D), F32),
            pltpu.VMEM((16, 128), F32),
            pltpu.VMEM((8, D), U32),
            pltpu.VMEM((16, 128), F32),
            pltpu.SMEM((1,), jnp.int32),
            pltpu.SMEM((2,), jnp.int32),
            pltpu.SemaphoreType.DMA((NSEM,)),
        ],
        compiler_params=pltpu.CompilerParams(vmem_limit_bytes=126 * 1024 * 1024),
    )(A_x.reshape(S, D), A_mem0.reshape(MEM, D), A_Wq, A_Wk, A_Wv, A_Wo.reshape(H * DH, D),
      B_w_r, B_w_gate, B_w_up, B_w_down)
    return out.reshape(1, S, D)
```

```python
import jax
import jax.numpy as jnp
from jax import lax
import jax.experimental.pallas as pl
import jax.experimental.pallas.tpu as pltpu

BF = jnp.bfloat16
U32 = jnp.uint32
F32 = jnp.float32

S = 2048
D = 1024
H = 32
DH = 128
MEM = 8
SEG = 32
NSEG = S // SEG
FF = 3584
KT = D // 128
FT = FF // 128
XS = 24
PRE = S - NSEG * XS
RING = 576
RING32 = RING // 2
NPAIR = H // 2
NPQ = 3 * NPAIR
NPRE = 16
SEM_SMALL, SEM_X0, SEM_X = 0, 2, 6
SEM_W0 = SEM_X + NPRE
SEM_W = SEM_W0 + 3
SEM_WO = SEM_W + NPRE
SEM_FFN, SEM_OUT = SEM_WO + 1, SEM_WO + 2
NSEM = SEM_OUT + 9

LAG_QK = 1
LAG_PV = 4
N_PART = 4
H_SPLIT = 26
REL_SCHED = {0: [(0, 0), (0, 1)], 1: [(0, 2), (0, 3)], 2: [(0, 4)], 3: [(0, 5)], 4: [(0, 6)], 5: [(0, 7)]}
REL_SCHED.update({6 + k: [(1, k)] for k in range(8)})
REL_SCHED.update({14 + k: [(2, k)] for k in range(8)})
K_SPLIT = 2
EPI_SCHED = [v * 5 // 2 for v in range(24)]
EPI_LAG = 4
ECH = 160
EPI_NB = False
EPI_ALIAS = False
REL_SCHED0 = {4: [(0, k) for k in range(4)], 5: [(0, k) for k in range(4, 8)],
              12: [(1, k) for k in range(4)], 13: [(1, k) for k in range(4, 8)]}
REL_SCHED0.update({14 + k: [(2, k)] for k in range(8)})
SCORE_SCHED = [1, 7, 13]
LN_SCHED = {3 * q: [q] for q in range(6)}
LN_SCHED0 = {13 + q: [q] for q in range(6)}
FIRST_BATCH = 12
LN_LAG = 5
REL_LAG = 2
UNROLL = 4


def _b2u(x):
    return pltpu.bitcast(x, U32)


def _u2b(x):
    return pltpu.bitcast(x, BF)


def _dot(a, b):
    return jnp.dot(a, b, preferred_element_type=F32)


def _dot_nt(a, b):
    return lax.dot_general(a, b, (((1,), (1,)), ((), ())), preferred_element_type=F32)


def _after(w, dep, zero):
    if not dep:
        return w
    d = dep[0]
    for e in dep[1:]:
        d = d | e
    return jnp.concatenate([w[0:8] | (d & zero), w[8:]], axis=0)


def _rbf(x):
    return x.astype(BF).astype(F32)


def _kernel(x_hbm, mem0_hbm, wq_hbm, wk_hbm, wv_hbm, wo_hbm, wr_hbm, wg_hbm, wu_hbm, wd_hbm,
            out_hbm,
            x_s, xn_t, xn_pre, hbuf, wqkv, wo_s, ring, oring, abuf, out_s, raw,
            wg_s, wu_s, wd_s, mem0_s, wr_s, wrf_s, r_s, xsel_s, gate_s, zero_s, idx_s,
            sems):
    w32 = [w.bitcast(U32) for w in (wq_hbm, wk_hbm, wv_hbm)]
    wo32 = wo_hbm.bitcast(U32)
    wg32 = wg_hbm.bitcast(U32)
    wu32 = wu_hbm.bitcast(U32)
    wd32 = wd_hbm.bitcast(U32)

    def rows_copy(r0, n, sem):
        return pltpu.make_async_copy(x_hbm.at[pl.ds(r0, n), :], x_s.at[pl.ds(r0, n), :], sems.at[sem])

    def x_first(c):
        return rows_copy(128 * c if isinstance(c, int) else pl.multiple_of(128 * c, 128), 128, SEM_X0 + c)

    def x_piece(c):
        r0 = PRE + 96 * c if isinstance(c, int) else pl.multiple_of(PRE + 96 * c, 32)
        return rows_copy(r0, 96, SEM_X + c)

    def pair_copy(p):
        q = min(p, NPQ - 1)
        sem = SEM_W0 + p if p < 4 else SEM_W + (p - 1) // 3
        return pltpu.make_async_copy(w32[q // NPAIR].at[:, q % NPAIR, :], raw.at[p], sems.at[sem])

    def pairs_wait(t):
        dst = raw.at[pl.ds(3 * t + 1, 3)]
        pltpu.make_async_copy(dst, dst, sems.at[SEM_W + t]).wait()

    def wo_copy(n):
        return pltpu.make_async_copy(wo32.at[:, pl.ds(128 * n, 128)], wo_s.at[n], sems.at[SEM_WO])

    small_copies = [pltpu.make_async_copy(mem0_hbm, mem0_s, sems.at[SEM_SMALL]),
                    pltpu.make_async_copy(wr_hbm, wr_s, sems.at[SEM_SMALL + 1])]
    ffn_copies = [pltpu.make_async_copy(s_, d_, sems.at[SEM_FFN])
                  for s_, d_ in ((wg32, wg_s), (wu32, wu_s), (wd32, wd_s))]

    zero_s[0] = 0
    for c in range(4):
        x_first(c).start()
        if c == 0:
            for cp in small_copies:
                cp.start()

    def queue(t0, t1):
        for t in range(t0, t1):
            for p in range(3 * t + 1, 3 * t + 4):
                pair_copy(p).start()
            x_piece(t).start()

    pair_copy(0).start()
    queue(0, FIRST_BATCH)
    eps_bf = 1.0013580322265625e-05

    def score16(g, xn):
        wr = jnp.concatenate([wrf_s[...], wrf_s[...]], axis=0)
        score = _rbf(jnp.sum(xn.astype(F32) * wr, axis=1, keepdims=True))
        r_s[...] = jnp.where(lane16 == g, score, r_s[...])

    def layernorm16(rq, dst_ref, dst_row, not_before=None):
        rq = rq if isinstance(rq, int) else pl.multiple_of(rq, 16)
        xf = x_s[pl.ds(rq, 16), :].astype(F32)
        if not_before is not None:
            x0 = _after(pltpu.bitcast(xf[:, 0:128], U32), [not_before], zero_box[0])
            xf = jnp.concatenate([pltpu.bitcast(x0, F32), xf[:, 128:]], axis=1)
        mean = jnp.sum(xf, axis=1, keepdims=True) * (1.0 / D)
        cen = xf - mean
        var = jnp.sum(cen * cen, axis=1, keepdims=True) * (1.0 / D)
        sd = _rbf(jnp.sqrt(_rbf(_rbf(var) + eps_bf)))
        xn = (_rbf(xf - _rbf(mean)) * (1.0 / sd)).astype(BF)
        if dst_ref is hbuf:
            score16(rq // 16, xn)
        xp = _b2u(xn)
        hq = rq // 2 if isinstance(rq, int) else pl.multiple_of(rq // 2, 8)
        dst_row = dst_row if isinstance(dst_row, int) else pl.multiple_of(dst_row, 8)
        for k in range(KT):
            xn_t[k, pl.ds(hq, 8), :] = xp[:, 128 * k:128 * (k + 1)]
            dst_ref[k, pl.ds(dst_row, 8), :] = xp[:, 128 * k:128 * (k + 1)]

    zero_box = [None]

    def fresh_zero():
        zero_box[0] = jnp.full((8, 128), zero_s[0], jnp.int32).astype(U32)

    r_s[...] = jnp.full(r_s.shape, -jnp.inf, F32)
    lane16 = lax.broadcasted_iota(jnp.int32, (16, 128), 1)

    def ln_body(c, carry):
        x_first(c).wait()
        for q in range(8):
            layernorm16(128 * c + 16 * q, xn_pre, 64 * c + 8 * q)
        return carry

    lax.fori_loop(0, PRE // 128, ln_body, 0)


    def relayout(src, dst, j, k, not_before=None):
        a = src[j, pl.ds(128 * k, 64, stride=2), :]
        if not_before is not None:
            a = a | jnp.concatenate([not_before & zero_box[0]] * 8, axis=0)
        b = src[j, pl.ds(128 * k + 1, 64, stride=2), :]
        rows = pl.ds(64 * k, 64)
        dst[2 * j, rows, :] = (a & jnp.uint32(0xFFFF)) | (b << 16)
        dst[2 * j + 1, rows, :] = (a >> 16) | (b & jnp.uint32(0xFFFF0000))

    def pre_dot(w_view, ring_view, j, k, dep=None):
        i, q = k // 4, k % 4
        lhs = jnp.concatenate([_u2b(xn_pre[kk, pl.ds(64 * q, 64), :]) for kk in range(KT)], axis=1)
        y = _dot(lhs, _u2b(_after(w_view[2 * j + i], dep, zero_box[0])))
        yp = _b2u(y.astype(BF))
        ring_view[2 * j + i, pl.ds(32 + 64 * q, 64), :] = yp
        return yp[0:8]

    for c in small_copies:
        c.wait()
    pair_copy(0).wait()
    for k in range(8):
        relayout(raw, wqkv, 0, k)
    wrf_s[...] = jnp.broadcast_to(wr_s[...].astype(F32).reshape(1, D), (8, D))

    def pre_iter(t, barriers):
        deps = {}
        raw_view = raw.at[pl.ds(3 * t, 4)]
        w_view = wqkv.at[pl.ds(6 * t, 8)]
        ring_view = ring.at[pl.ds(6 * t, 6)]
        rel_sched, ln_sched = (REL_SCHED0, LN_SCHED0) if barriers else (REL_SCHED, LN_SCHED)
        done = None
        for v in range(24):
            j, k = v // 8, v % 8
            if v == 0 or v in barriers:
                for wait in barriers.get(v, ()):
                    wait()
                fresh_zero()
                done = None
            prev = done
            done = pre_dot(w_view, ring_view, j, k, deps.get(v))
            for jr, kr in rel_sched.get(v, ()):
                relayout(raw_view, w_view, jr + 1, kr, prev)
                deps.setdefault(v + REL_LAG, []).append(w_view[2 * jr + 3, pl.ds(64 * kr + 56, 8), :])
            for q in ln_sched.get(v, ()):
                hrow = 32 * (q // 3) + 8 * (q % 3)
                hrow += 64 * t if isinstance(t, int) else pl.multiple_of(64 * t, 64)
                layernorm16(PRE + 96 * t + 16 * q, hbuf, hrow, done if prev is not None else None)
                deps.setdefault(v + LN_LAG, []).append(hbuf[KT - 1, pl.ds(hrow, 8), :])
            if not barriers and v in SCORE_SCHED:
                g = jnp.minimum(3 * (t - 1) + SCORE_SCHED.index(v), PRE // 16 - 1)
                rows = pl.ds(pl.multiple_of(8 * g, 8), 8)
                xp = [xn_pre[kk, rows, :] for kk in range(KT)]
                xp[0] = xp[0] | (done & zero_box[0])
                score16(g, _u2b(jnp.concatenate(xp, axis=1)))

    def second_batch():
        queue(FIRST_BATCH, NPRE)
        for n in range(KT):
            wo_copy(n).start()
        for cp in ffn_copies:
            cp.start()

    pre_iter(0, {4: [pair_copy(1).wait],
                 12: [pair_copy(2).wait, pair_copy(3).wait, x_piece(0).wait, second_batch]})

    def pre_body(t, carry):
        x_piece(t).wait()
        pairs_wait(t)
        pre_iter(t, {})
        return carry

    lax.fori_loop(1, NPRE, pre_body, 0)
    row = lax.broadcasted_iota(jnp.int32, (80, 80), 0)
    col = lax.broadcasted_iota(jnp.int32, (80, 80), 1)
    same_head = (jnp.where(row < 64, row >> 5, (row - 64) >> 3)
                 == jnp.where(col < 64, col >> 5, (col - 64) >> 3))
    allowed = same_head & ((col >= 64) | (row >= 64) | (col <= row))
    fill = jnp.where(same_head, -1e9, -jnp.inf).astype(F32)
    low_half = lax.broadcasted_iota(jnp.int32, (8, 128), 0) < 4
    high_half = jnp.logical_not(low_half)
    scale = DH ** -0.5

    def load_row(t):
        w = jnp.concatenate([xn_t[k, pl.ds(t // 2, 1), :] for k in range(KT)], axis=1)
        bits = jnp.where(t % 2 == 0, w << 16, w & jnp.uint32(0xFFFF0000))
        return pltpu.bitcast(bits, F32), w

    def select_tokens():
        r = r_s[...]
        tok = lane16 * 16 + lax.broadcasted_iota(jnp.int32, (16, 128), 0)
        top1 = jnp.max(r)
        idx1 = jnp.min(jnp.where(r == top1, tok, S - 1))
        r2 = jnp.where(tok == idx1, -jnp.inf, r)
        top2 = jnp.max(r2)
        idx2 = jnp.min(jnp.where((r2 == top2) & (tok != idx1), tok, S - 1))
        idx_s[0] = idx1
        idx_s[1] = idx2
        gate_s[...] = jnp.where(lax.broadcasted_iota(jnp.int32, (16, 128), 0) == 0, top1, top2)
        sel_row = lax.broadcasted_iota(jnp.int32, (8, D), 0)
        xs1, _ = load_row(idx1)
        xs2, _ = load_row(idx2)
        xsel_s[...] = jnp.where(sel_row == 0, xs1, jnp.where(sel_row == 1, xs2, 0.0))

    def one_step(i, u, mem):
        odd = u % 2
        s2 = i * (UNROLL // 2) + u // 2
        h_ld = pl.multiple_of(16 * UNROLL * i, 32) + 32 * (u // 2)
        a24 = pl.multiple_of(12 * UNROLL * i, 8)
        r24 = pl.multiple_of(a24 % RING32, 8) + XS * (u // 2)
        a24 = a24 + XS * (u // 2)
        qkv_ld = pl.multiple_of((SEG * s2 + 32) % RING32, 32) + 16 * odd
        o_st = pl.multiple_of((SEG * s2) % RING32, 32) + 16 * odd
        m0 = 0 if odd else XS

        def with_mem(ref, idx, base, m):
            lo = ref[idx, pl.ds(base + 8 * odd, 8), :]
            hi = ref[idx, pl.ds(base + 8 + 8 * odd, 8), :]
            if odd:
                lo = jnp.where(low_half, m, lo)
            else:
                hi = jnp.where(low_half, hi, m)
            return _u2b(jnp.concatenate([lo, hi], axis=0))

        def store_tokens(ref, idx, base, yp):
            if odd:
                pltpu.store(ref.at[idx, pl.ds(base + 8, 8), :], yp[0:8], mask=high_half)
                ref[idx, pl.ds(base + 16, 8), :] = yp[8:16]
            else:
                ref[idx, pl.ds(base, 8), :] = yp[0:8]
                pltpu.store(ref.at[idx, pl.ds(base + 8, 8), :], yp[8:16], mask=low_half)

        lk = [with_mem(hbuf, k, h_ld, mem[k]) for k in range(KT)]
        lhs = jnp.concatenate(lk, axis=1)

        ymem = {}
        xs = {}
        probs = {}
        parts = {}

        def proj(h):
            split = h < K_SPLIT and u > 0
            if split:
                lhs7 = jnp.concatenate(lk[:KT - 1], axis=1)
                head = [_dot(lhs7, _u2b(wqkv[m * H + h, pl.ds(0, 448), :])) for m in range(3)]
            for m in range(3):
                if split:
                    y = _dot(lk[KT - 1], _u2b(wqkv[m * H + h, pl.ds(448, 64), :])) + head[m]
                else:
                    y = _dot(lhs, _u2b(wqkv[m * H + h]))
                store_tokens(ring, m * H + h, r24, _b2u(y.astype(BF)))
                ymem[(h, m)] = y[m0:m0 + MEM]
                xs[(h, m)] = ring[m * H + h, pl.ds(qkv_ld, SEG // 2), :]

        def pair(p, m):
            a, b = 2 * p, 2 * p + 1
            mm = jnp.concatenate([ymem[(a, m)], ymem[(b, m)]], axis=0).astype(BF)
            return jnp.concatenate([_u2b(xs[(a, m)]), _u2b(xs[(b, m)]), mm], axis=0)

        def qk(p):
            sc = _dot_nt(pair(p, 0), pair(p, 1))
            sc = jnp.where(allowed, sc * scale, fill)
            e = jnp.exp(sc - jnp.max(sc, axis=1, keepdims=True))
            l = jnp.sum(e, axis=1, keepdims=True)
            r = pl.reciprocal(l, approx=True)
            r = r * (2.0 - l * r)
            probs[p] = (e * r).astype(BF)

        def pv(p):
            op = _b2u(_dot(probs[p], pair(p, 2)).astype(BF))
            om = op[32:40]
            om_sw = pltpu.roll(om, 4, axis=0)
            for j, h in enumerate((2 * p, 2 * p + 1)):
                oring[h, pl.ds(o_st, SEG // 2), :] = op[16 * j:16 * j + 16]
                parts[h] = with_mem(oring, h, r24, om if j != odd else om_sw)

        def after(t):
            for lag, fn in ((LAG_QK, qk), (LAG_PV, pv)):
                if (t - 1 - lag) % 2 == 0 and 0 <= (t - 1 - lag) // 2 < NPAIR:
                    fn((t - 1 - lag) // 2)

        for t in range(H):
            proj(t)
            after(t)
            if u == 0 and t == 8:
                select_tokens()
        t = H
        lhs_a = jnp.concatenate([parts[j] for j in range(H_SPLIT)], axis=1)
        acc = []
        for n in range(N_PART):
            acc.append(_dot(lhs_a, _u2b(wo_s[n, pl.ds(0, H_SPLIT * 64), :])))
            after(t)
            t += 1
        while t - 1 - LAG_PV <= 2 * (NPAIR - 1):
            after(t)
            t += 1
        lhs_b = jnp.concatenate([parts[j] for j in range(H_SPLIT, H)], axis=1)
        lhs_o = jnp.concatenate([lhs_a, lhs_b], axis=1)
        new_mem = [None] * KT

        def finish(n, y):
            store_tokens(abuf, n, a24, _b2u(y.astype(BF)))
            ym = y[m0:m0 + MEM]
            new_mem[n] = _b2u(jnp.concatenate([ym, ym], axis=0).astype(BF))

        for n in range(N_PART, KT):
            finish(n, _dot(lhs_o, _u2b(wo_s[n])))
            if n == N_PART:
                for n2 in range(N_PART):
                    tail = _u2b(wo_s[n2, pl.ds(H_SPLIT * 64, (H - H_SPLIT) * 64), :])
                    finish(n2, _dot(lhs_b, tail) + acc[n2])
        return new_mem

    def body(i, mem):
        mem = list(mem)
        for u in range(UNROLL):
            mem = one_step(i, u, mem)
        return tuple(mem)

    for n in range(KT):
        wo_copy(n).wait()
    mi = mem0_s[...].astype(F32)
    mip = _b2u(jnp.concatenate([mi, mi], axis=0).astype(BF))
    lax.fori_loop(0, NSEG // UNROLL, body,
                  tuple(mip[:, 128 * k:128 * (k + 1)] for k in range(KT)))

    early = S - PRE
    zrow = pl.multiple_of(zero_s[0], 16)
    FPER = 9

    def half_rows(r0):
        return r0 // 2 if isinstance(r0, int) else pl.multiple_of(r0 // 2, 8)

    def combine(r0, nrows, n, a):
        xf = x_s[pl.ds(r0, nrows), pl.ds(128 * n, 128)].astype(F32)
        b = _u2b(xn_t[n, pl.ds(half_rows(r0), nrows // 2), :]).astype(F32)
        out_s[pl.ds(r0, nrows), pl.ds(128 * n, 128)] = (_rbf(xf + a) + b).astype(BF)

    def combine_stored(r0, nrows, not_before=None):
        for n in range(KT):
            a = abuf[n, pl.ds(half_rows(r0), nrows // 2), :]
            if not_before is not None:
                a = a | jnp.concatenate([not_before & zero_box[0]] * (nrows // 16), axis=0)
            combine(r0, nrows, n, _u2b(a).astype(F32))

    def out_copy(r0, nrows, j):
        return pltpu.make_async_copy(out_s.at[pl.ds(r0, nrows), :], out_hbm.at[pl.ds(r0, nrows), :],
                                     sems.at[SEM_OUT + j])

    def ffn_groups(j0, count, y, done):
        x_sel = xsel_s[...]
        hid = {}

        def up(w_ref, j, key):
            cols = pl.ds(128 * j if isinstance(j, int) else pl.multiple_of(128 * j, 128), 128)
            part = _dot(x_sel[:, 0:512], _u2b(w_ref[pl.ds(0, 256), cols]).astype(F32))
            yield
            hid[key] = _rbf(_dot(x_sel[:, 512:1024], _u2b(w_ref[pl.ds(256, 256), cols]).astype(F32)) + part)
            yield

        def down(jj):
            g = hid[("g", jj)]
            hb = _rbf(_rbf(g * _rbf(jax.nn.sigmoid(g))) * hid[("u", jj)])
            rows = pl.ds(pl.multiple_of(64 * (j0 + jj), 64), 64)
            for half in range(2):
                y[half] = _dot(hb, _u2b(wd_s[rows, pl.ds(512 * half, 512)]).astype(F32)) + y[half]
                yield

        for jj in range(count + 1):
            if jj < count:
                yield from up(wg_s, j0 + jj, ("g", jj))
                yield from up(wu_s, j0 + jj, ("u", jj))
            elif count == 1:
                yield
                yield
            if jj >= 1:
                yield from down(jj - 1)
        done()

    def epi_chunk(r0, nrows, side, pieces, keep):
        pos = [((r0 + 32 * j) % RING) // 2 for j in range(nrows // 32)]
        if not isinstance(r0, int):
            pos = [pl.multiple_of(p, 16) for p in pos]
        fresh_zero()
        deps = {}
        for n in range(KT):
            acc = None
            for g in range(8):
                lhs = jnp.concatenate(
                    [_u2b(jnp.concatenate([oring[h, pl.ds(p, 16), :] for p in pos], axis=0))
                     for h in range(4 * g, 4 * g + 4)], axis=1)
                w = _after(wo_s[n, pl.ds(256 * g, 256), :], deps.get(8 * n + g), zero_box[0])
                y = _dot(lhs, _u2b(w))
                acc = y if acc is None else y + acc
                next(side, None)
                v = 8 * n + g
                if pieces is not None and v in EPI_SCHED:
                    r1 = pieces + 32 * EPI_SCHED.index(v)
                    combine_stored(r1, 32, pltpu.bitcast(acc[0:8], U32) if EPI_NB else None)
                    if EPI_LAG:
                        deps[v + EPI_LAG] = [_b2u(out_s[pl.ds(r1 + (zrow if EPI_ALIAS else 0), 16), pl.ds(D - 128, 128)])]
            ab = acc.astype(BF)
            if keep:
                abuf[n, pl.ds(half_rows(r0), nrows // 2), :] = _b2u(ab)
            combine(r0, nrows, n, ab.astype(F32))

    for c in ffn_copies:
        c.wait()

    def epi_body(c, y):
        y = list(y)
        r0 = pl.multiple_of(early + ECH * c, 32)
        e0 = pl.multiple_of((early // 2) * (c & 1), 256)

        @pl.when(c == 2)
        def _():
            out_copy(0, early // 2, 4).wait()

        epi_chunk(r0, ECH, ffn_groups(FPER * c, FPER, y, lambda: None), e0, True)
        out_copy(r0, ECH, c).start()

        @pl.when(c < 2)
        def _():
            out_copy(e0, early // 2, 4 + c).start()

        return tuple(y)

    y = list(lax.fori_loop(0, 3, epi_body, (jnp.zeros((8, 512), F32), jnp.zeros((8, 512), F32))))
    idx1 = idx_s[0]
    idx2 = idx_s[1]

    def patch_row(t, yrow):
        xr, w = load_row(t)
        bits = pltpu.bitcast(_rbf(xr + yrow), U32)
        w = jnp.where(t % 2 == 0,
                      (w & jnp.uint32(0xFFFF0000)) | (bits >> 16),
                      (w & jnp.uint32(0xFFFF)) | bits)
        for k in range(KT):
            xn_t[k, pl.ds(t // 2, 1), :] = w[:, 128 * k:128 * (k + 1)]

    def patch():
        gate = _rbf(jax.nn.sigmoid(gate_s[0:8, 0:1]))
        yy = _rbf(_rbf(jnp.concatenate(y, axis=1)) * gate)
        patch_row(idx1, yy[0:1])
        patch_row(idx2, yy[1:2])

    last = early + 3 * ECH
    epi_chunk(last, S - last, ffn_groups(3 * FPER, 1, y, patch), None, False)
    out_copy(last, S - last, 3).start()
    for c in range(3):
        out_copy(early + ECH * c, ECH, c).wait()
    out_copy(early // 2, early // 2, 5).wait()
    blk1 = jnp.minimum(idx1 // 16, last // 16 - 1)
    blk2 = jnp.minimum(idx2 // 16, last // 16 - 1)
    blk2 = jnp.where(blk2 == blk1, jnp.where(blk1 == 0, 1, blk1 - 1), blk2)
    fix = []
    for j, blk in enumerate((blk1, blk2)):
        r0 = pl.multiple_of(blk * 16, 16)
        combine_stored(r0, 16)
        fix.append(out_copy(r0, 16, 7 + j))
    for cp in fix:
        cp.start()
    out_copy(last, S - last, 3).wait()
    for cp in fix:
        cp.wait()


@jax.jit
def pallas_parallel_sum__memory_aug_recurrent_mem_tr__moe_arch_mod__prompt_kernel(
    A_x: jax.Array,
    A_mem0: jax.Array,
    A_Wq: jax.Array,
    A_Wk: jax.Array,
    A_Wv: jax.Array,
    A_Wo: jax.Array,
    A_seg_len: jax.Array,
    B_x: jax.Array,
    B_w_r: jax.Array,
    B_w_gate: jax.Array,
    B_w_up: jax.Array,
    B_w_down: jax.Array,
):
    del A_seg_len, B_x
    assert A_x.shape == (1, S, D) and A_mem0.shape == (1, MEM, D)
    assert A_Wq.shape == (D, H, DH) and A_Wo.shape == (H, DH, D)
    assert B_w_gate.shape == (D, FF) and B_w_down.shape == (FF, D)
    any_spec = pl.BlockSpec(memory_space=pl.ANY)
    out = pl.pallas_call(
        _kernel,
        out_shape=jax.ShapeDtypeStruct((S, D), BF),
        in_specs=[any_spec] * 10,
        out_specs=any_spec,
        scratch_shapes=[
            pltpu.VMEM((S, D), BF),
            pltpu.VMEM((KT, S // 2, 128), U32),
            pltpu.VMEM((KT, PRE // 2, 128), U32),
            pltpu.VMEM((KT, 16 * NSEG, 128), U32),
            pltpu.VMEM((3 * H + 2, D // 2, 128), U32),
            pltpu.VMEM((KT, H * DH // 2, 128), U32),
            pltpu.VMEM((3 * H, RING32, 128), U32),
            pltpu.VMEM((H, RING32, 128), U32),
            pltpu.VMEM((KT, S // 2, 128), U32),
            pltpu.VMEM((S, D), BF),
            pltpu.VMEM((NPQ + 1, D, 128), U32),
            pltpu.VMEM((D // 2, FF), U32),
            pltpu.VMEM((D // 2, FF), U32),
            pltpu.VMEM((FF // 2, D), U32),
            pltpu.VMEM((MEM, D), BF),
            pltpu.VMEM((D,), BF),
            pltpu.VMEM((8, D), F32),
            pltpu.VMEM((16, 128), F32),
            pltpu.VMEM((8, D), F32),
            pltpu.VMEM((16, 128), F32),
            pltpu.SMEM((1,), jnp.int32),
            pltpu.SMEM((2,), jnp.int32),
            pltpu.SemaphoreType.DMA((NSEM,)),
        ],
        compiler_params=pltpu.CompilerParams(vmem_limit_bytes=126 * 1024 * 1024),
    )(A_x.reshape(S, D), A_mem0.reshape(MEM, D), A_Wq, A_Wk, A_Wv, A_Wo.reshape(H * DH, D),
      B_w_r, B_w_gate, B_w_up, B_w_down)
    return out.reshape(1, S, D)
```

```python
import jax
import jax.numpy as jnp
from jax import lax
import jax.experimental.pallas as pl
import jax.experimental.pallas.tpu as pltpu

BF = jnp.bfloat16
U32 = jnp.uint32
F32 = jnp.float32

S = 2048
D = 1024
H = 32
DH = 128
MEM = 8
SEG = 32
NSEG = S // SEG
FF = 3584
KT = D // 128
FT = FF // 128
XS = 24
PRE = S - NSEG * XS
RING = 576
RING32 = RING // 2
NPAIR = H // 2
NPQ = 3 * NPAIR
NPRE = 16
SEM_SMALL, SEM_X0, SEM_X = 0, 2, 6
SEM_W0 = SEM_X + NPRE
SEM_W = SEM_W0 + 3
SEM_WO = SEM_W + NPRE
SEM_FFN, SEM_OUT = SEM_WO + 1, SEM_WO + 2
NSEM = SEM_OUT + 9

LAG_QK = 1
LAG_PV = 4
N_PART = 4
H_SPLIT = 26
REL_SCHED = {0: [(0, 0), (0, 1)], 1: [(0, 2), (0, 3)], 2: [(0, 4)], 3: [(0, 5)], 4: [(0, 6)], 5: [(0, 7)]}
REL_SCHED.update({6 + k: [(1, k)] for k in range(8)})
REL_SCHED.update({14 + k: [(2, k)] for k in range(8)})
K_SPLIT = 2
EPI_SCHED = [v * 5 // 2 for v in range(24)]
EPI_LAG = 4
ECH = 160
REL_SCHED0 = {4: [(0, k) for k in range(4)], 5: [(0, k) for k in range(4, 8)],
              12: [(1, k) for k in range(4)], 13: [(1, k) for k in range(4, 8)]}
REL_SCHED0.update({14 + k: [(2, k)] for k in range(8)})
SCORE_SCHED = [1, 7, 13]
LN_SCHED = {3 * q: [q] for q in range(6)}
LN_SCHED0 = {13 + q: [q] for q in range(6)}
FIRST_BATCH = 12
LN_LAG = 5
REL_LAG = 2
UNROLL = 4


def _b2u(x):
    return pltpu.bitcast(x, U32)


def _u2b(x):
    return pltpu.bitcast(x, BF)


def _dot(a, b):
    return jnp.dot(a, b, preferred_element_type=F32)


def _dot_nt(a, b):
    return lax.dot_general(a, b, (((1,), (1,)), ((), ())), preferred_element_type=F32)


def _after(w, dep, zero):
    if not dep:
        return w
    d = dep[0]
    for e in dep[1:]:
        d = d | e
    return jnp.concatenate([w[0:8] | (d & zero), w[8:]], axis=0)


def _rbf(x):
    return x.astype(BF).astype(F32)


def _kernel(x_hbm, mem0_hbm, wq_hbm, wk_hbm, wv_hbm, wo_hbm, wr_hbm, wg_hbm, wu_hbm, wd_hbm,
            out_hbm,
            x_s, xn_t, xn_pre, hbuf, wqkv, wo_s, ring, oring, abuf, out_s, raw,
            wg_s, wu_s, wd_s, mem0_s, wr_s, wrf_s, r_s, xsel_s, gate_s, fix_s, zero_s, idx_s,
            sems):
    w32 = [w.bitcast(U32) for w in (wq_hbm, wk_hbm, wv_hbm)]
    wo32 = wo_hbm.bitcast(U32)
    wg32 = wg_hbm.bitcast(U32)
    wu32 = wu_hbm.bitcast(U32)
    wd32 = wd_hbm.bitcast(U32)

    def rows_copy(r0, n, sem):
        return pltpu.make_async_copy(x_hbm.at[pl.ds(r0, n), :], x_s.at[pl.ds(r0, n), :], sems.at[sem])

    def x_first(c):
        return rows_copy(128 * c if isinstance(c, int) else pl.multiple_of(128 * c, 128), 128, SEM_X0 + c)

    def x_piece(c):
        r0 = PRE + 96 * c if isinstance(c, int) else pl.multiple_of(PRE + 96 * c, 32)
        return rows_copy(r0, 96, SEM_X + c)

    def pair_copy(p):
        q = min(p, NPQ - 1)
        sem = SEM_W0 + p if p < 4 else SEM_W + (p - 1) // 3
        return pltpu.make_async_copy(w32[q // NPAIR].at[:, q % NPAIR, :], raw.at[p], sems.at[sem])

    def pairs_wait(t):
        dst = raw.at[pl.ds(3 * t + 1, 3)]
        pltpu.make_async_copy(dst, dst, sems.at[SEM_W + t]).wait()

    def wo_copy(n):
        return pltpu.make_async_copy(wo32.at[:, pl.ds(128 * n, 128)], wo_s.at[n], sems.at[SEM_WO])

    small_copies = [pltpu.make_async_copy(mem0_hbm, mem0_s, sems.at[SEM_SMALL]),
                    pltpu.make_async_copy(wr_hbm, wr_s, sems.at[SEM_SMALL + 1])]
    ffn_copies = [pltpu.make_async_copy(s_, d_, sems.at[SEM_FFN])
                  for s_, d_ in ((wg32, wg_s), (wu32, wu_s), (wd32, wd_s))]

    zero_s[0] = 0
    for c in range(4):
        x_first(c).start()
        if c == 0:
            for cp in small_copies:
                cp.start()

    def queue(t0, t1):
        for t in range(t0, t1):
            for p in range(3 * t + 1, 3 * t + 4):
                pair_copy(p).start()
            x_piece(t).start()

    pair_copy(0).start()
    queue(0, FIRST_BATCH)
    eps_bf = 1.0013580322265625e-05

    def score16(g, xn):
        wr = jnp.concatenate([wrf_s[...], wrf_s[...]], axis=0)
        score = _rbf(jnp.sum(xn.astype(F32) * wr, axis=1, keepdims=True))
        r_s[...] = jnp.where(lane16 == g, score, r_s[...])

    def layernorm16(rq, dst_ref, dst_row, not_before=None):
        rq = rq if isinstance(rq, int) else pl.multiple_of(rq, 16)
        xf = x_s[pl.ds(rq, 16), :].astype(F32)
        if not_before is not None:
            x0 = _after(pltpu.bitcast(xf[:, 0:128], U32), [not_before], zero_box[0])
            xf = jnp.concatenate([pltpu.bitcast(x0, F32), xf[:, 128:]], axis=1)
        mean = jnp.sum(xf, axis=1, keepdims=True) * (1.0 / D)
        cen = xf - mean
        var = jnp.sum(cen * cen, axis=1, keepdims=True) * (1.0 / D)
        sd = _rbf(jnp.sqrt(_rbf(_rbf(var) + eps_bf)))
        xn = (_rbf(xf - _rbf(mean)) * (1.0 / sd)).astype(BF)
        if dst_ref is hbuf:
            score16(rq // 16, xn)
        xp = _b2u(xn)
        hq = rq // 2 if isinstance(rq, int) else pl.multiple_of(rq // 2, 8)
        dst_row = dst_row if isinstance(dst_row, int) else pl.multiple_of(dst_row, 8)
        for k in range(KT):
            xn_t[k, pl.ds(hq, 8), :] = xp[:, 128 * k:128 * (k + 1)]
            dst_ref[k, pl.ds(dst_row, 8), :] = xp[:, 128 * k:128 * (k + 1)]

    zero_box = [None]

    def fresh_zero():
        zero_box[0] = jnp.full((8, 128), zero_s[0], jnp.int32).astype(U32)

    r_s[...] = jnp.full(r_s.shape, -jnp.inf, F32)
    lane16 = lax.broadcasted_iota(jnp.int32, (16, 128), 1)

    def ln_body(c, carry):
        x_first(c).wait()
        for q in range(8):
            layernorm16(128 * c + 16 * q, xn_pre, 64 * c + 8 * q)
        return carry

    lax.fori_loop(0, PRE // 128, ln_body, 0)


    def relayout(src, dst, j, k, not_before=None):
        a = src[j, pl.ds(128 * k, 64, stride=2), :]
        if not_before is not None:
            a = a | jnp.concatenate([not_before & zero_box[0]] * 8, axis=0)
        b = src[j, pl.ds(128 * k + 1, 64, stride=2), :]
        rows = pl.ds(64 * k, 64)
        dst[2 * j, rows, :] = (a & jnp.uint32(0xFFFF)) | (b << 16)
        dst[2 * j + 1, rows, :] = (a >> 16) | (b & jnp.uint32(0xFFFF0000))

    def pre_dot(w_view, ring_view, j, k, dep=None):
        i, q = k // 4, k % 4
        lhs = jnp.concatenate([_u2b(xn_pre[kk, pl.ds(64 * q, 64), :]) for kk in range(KT)], axis=1)
        y = _dot(lhs, _u2b(_after(w_view[2 * j + i], dep, zero_box[0])))
        yp = _b2u(y.astype(BF))
        ring_view[2 * j + i, pl.ds(32 + 64 * q, 64), :] = yp
        return yp[0:8]

    for c in small_copies:
        c.wait()
    pair_copy(0).wait()
    for k in range(8):
        relayout(raw, wqkv, 0, k)
    wrf_s[...] = jnp.broadcast_to(wr_s[...].astype(F32).reshape(1, D), (8, D))

    def pre_iter(t, barriers):
        deps = {}
        raw_view = raw.at[pl.ds(3 * t, 4)]
        w_view = wqkv.at[pl.ds(6 * t, 8)]
        ring_view = ring.at[pl.ds(6 * t, 6)]
        rel_sched, ln_sched = (REL_SCHED0, LN_SCHED0) if barriers else (REL_SCHED, LN_SCHED)
        done = None
        for v in range(24):
            j, k = v // 8, v % 8
            if v == 0 or v in barriers:
                for wait in barriers.get(v, ()):
                    wait()
                fresh_zero()
                done = None
            prev = done
            done = pre_dot(w_view, ring_view, j, k, deps.get(v))
            for jr, kr in rel_sched.get(v, ()):
                relayout(raw_view, w_view, jr + 1, kr, prev)
                deps.setdefault(v + REL_LAG, []).append(w_view[2 * jr + 3, pl.ds(64 * kr + 56, 8), :])
            for q in ln_sched.get(v, ()):
                hrow = 32 * (q // 3) + 8 * (q % 3)
                hrow += 64 * t if isinstance(t, int) else pl.multiple_of(64 * t, 64)
                layernorm16(PRE + 96 * t + 16 * q, hbuf, hrow, done if prev is not None else None)
                deps.setdefault(v + LN_LAG, []).append(hbuf[KT - 1, pl.ds(hrow, 8), :])
            if not barriers and v in SCORE_SCHED:
                g = jnp.minimum(3 * (t - 1) + SCORE_SCHED.index(v), PRE // 16 - 1)
                rows = pl.ds(pl.multiple_of(8 * g, 8), 8)
                xp = [xn_pre[kk, rows, :] for kk in range(KT)]
                xp[0] = xp[0] | (done & zero_box[0])
                score16(g, _u2b(jnp.concatenate(xp, axis=1)))

    def second_batch():
        queue(FIRST_BATCH, NPRE)
        for n in range(KT):
            wo_copy(n).start()
        for cp in ffn_copies:
            cp.start()

    pre_iter(0, {4: [pair_copy(1).wait],
                 12: [pair_copy(2).wait, pair_copy(3).wait, x_piece(0).wait, second_batch]})

    def pre_body(t, carry):
        x_piece(t).wait()
        pairs_wait(t)
        pre_iter(t, {})
        return carry

    lax.fori_loop(1, NPRE, pre_body, 0)
    row = lax.broadcasted_iota(jnp.int32, (80, 80), 0)
    col = lax.broadcasted_iota(jnp.int32, (80, 80), 1)
    same_head = (jnp.where(row < 64, row >> 5, (row - 64) >> 3)
                 == jnp.where(col < 64, col >> 5, (col - 64) >> 3))
    allowed = same_head & ((col >= 64) | (row >= 64) | (col <= row))
    fill = jnp.where(same_head, -1e9, -jnp.inf).astype(F32)
    low_half = lax.broadcasted_iota(jnp.int32, (8, 128), 0) < 4
    high_half = jnp.logical_not(low_half)
    scale = DH ** -0.5

    def load_row(t):
        w = jnp.concatenate([xn_t[k, pl.ds(t // 2, 1), :] for k in range(KT)], axis=1)
        bits = jnp.where(t % 2 == 0, w << 16, w & jnp.uint32(0xFFFF0000))
        return pltpu.bitcast(bits, F32), w

    def select_tokens():
        r = r_s[...]
        tok = lane16 * 16 + lax.broadcasted_iota(jnp.int32, (16, 128), 0)
        top1 = jnp.max(r)
        idx1 = jnp.min(jnp.where(r == top1, tok, S - 1))
        r2 = jnp.where(tok == idx1, -jnp.inf, r)
        top2 = jnp.max(r2)
        idx2 = jnp.min(jnp.where((r2 == top2) & (tok != idx1), tok, S - 1))
        idx_s[0] = idx1
        idx_s[1] = idx2
        gate_s[...] = jnp.where(lax.broadcasted_iota(jnp.int32, (16, 128), 0) == 0, top1, top2)
        sel_row = lax.broadcasted_iota(jnp.int32, (8, D), 0)
        xs1, _ = load_row(idx1)
        xs2, _ = load_row(idx2)
        xsel_s[...] = jnp.where(sel_row == 0, xs1, jnp.where(sel_row == 1, xs2, 0.0))

    def one_step(i, u, mem):
        odd = u % 2
        s2 = i * (UNROLL // 2) + u // 2
        h_ld = pl.multiple_of(16 * UNROLL * i, 32) + 32 * (u // 2)
        a24 = pl.multiple_of(12 * UNROLL * i, 8)
        r24 = pl.multiple_of(a24 % RING32, 8) + XS * (u // 2)
        a24 = a24 + XS * (u // 2)
        qkv_ld = pl.multiple_of((SEG * s2 + 32) % RING32, 32) + 16 * odd
        o_st = pl.multiple_of((SEG * s2) % RING32, 32) + 16 * odd
        m0 = 0 if odd else XS

        def with_mem(ref, idx, base, m):
            lo = ref[idx, pl.ds(base + 8 * odd, 8), :]
            hi = ref[idx, pl.ds(base + 8 + 8 * odd, 8), :]
            if odd:
                lo = jnp.where(low_half, m, lo)
            else:
                hi = jnp.where(low_half, hi, m)
            return _u2b(jnp.concatenate([lo, hi], axis=0))

        def store_tokens(ref, idx, base, yp):
            if odd:
                pltpu.store(ref.at[idx, pl.ds(base + 8, 8), :], yp[0:8], mask=high_half)
                ref[idx, pl.ds(base + 16, 8), :] = yp[8:16]
            else:
                ref[idx, pl.ds(base, 8), :] = yp[0:8]
                pltpu.store(ref.at[idx, pl.ds(base + 8, 8), :], yp[8:16], mask=low_half)

        lk = [with_mem(hbuf, k, h_ld, mem[k]) for k in range(KT)]
        lhs = jnp.concatenate(lk, axis=1)

        ymem = {}
        xs = {}
        probs = {}
        parts = {}

        def proj(h):
            split = h < K_SPLIT and u > 0
            if split:
                lhs7 = jnp.concatenate(lk[:KT - 1], axis=1)
                head = [_dot(lhs7, _u2b(wqkv[m * H + h, pl.ds(0, 448), :])) for m in range(3)]
            for m in range(3):
                if split:
                    y = _dot(lk[KT - 1], _u2b(wqkv[m * H + h, pl.ds(448, 64), :])) + head[m]
                else:
                    y = _dot(lhs, _u2b(wqkv[m * H + h]))
                store_tokens(ring, m * H + h, r24, _b2u(y.astype(BF)))
                ymem[(h, m)] = y[m0:m0 + MEM]
                xs[(h, m)] = ring[m * H + h, pl.ds(qkv_ld, SEG // 2), :]

        def pair(p, m):
            a, b = 2 * p, 2 * p + 1
            mm = jnp.concatenate([ymem[(a, m)], ymem[(b, m)]], axis=0).astype(BF)
            return jnp.concatenate([_u2b(xs[(a, m)]), _u2b(xs[(b, m)]), mm], axis=0)

        def qk(p):
            sc = _dot_nt(pair(p, 0), pair(p, 1))
            sc = jnp.where(allowed, sc * scale, fill)
            e = jnp.exp(sc - jnp.max(sc, axis=1, keepdims=True))
            l = jnp.sum(e, axis=1, keepdims=True)
            r = pl.reciprocal(l, approx=True)
            r = r * (2.0 - l * r)
            probs[p] = (e * r).astype(BF)

        def pv(p):
            op = _b2u(_dot(probs[p], pair(p, 2)).astype(BF))
            om = op[32:40]
            om_sw = pltpu.roll(om, 4, axis=0)
            for j, h in enumerate((2 * p, 2 * p + 1)):
                oring[h, pl.ds(o_st, SEG // 2), :] = op[16 * j:16 * j + 16]
                parts[h] = with_mem(oring, h, r24, om if j != odd else om_sw)

        def after(t):
            for lag, fn in ((LAG_QK, qk), (LAG_PV, pv)):
                if (t - 1 - lag) % 2 == 0 and 0 <= (t - 1 - lag) // 2 < NPAIR:
                    fn((t - 1 - lag) // 2)

        for t in range(H):
            proj(t)
            after(t)
            if u == 0 and t == 8:
                select_tokens()
        t = H
        lhs_a = jnp.concatenate([parts[j] for j in range(H_SPLIT)], axis=1)
        acc = []
        for n in range(N_PART):
            acc.append(_dot(lhs_a, _u2b(wo_s[n, pl.ds(0, H_SPLIT * 64), :])))
            after(t)
            t += 1
        while t - 1 - LAG_PV <= 2 * (NPAIR - 1):
            after(t)
            t += 1
        lhs_b = jnp.concatenate([parts[j] for j in range(H_SPLIT, H)], axis=1)
        lhs_o = jnp.concatenate([lhs_a, lhs_b], axis=1)
        new_mem = [None] * KT

        def finish(n, y):
            store_tokens(abuf, n, a24, _b2u(y.astype(BF)))
            ym = y[m0:m0 + MEM]
            new_mem[n] = _b2u(jnp.concatenate([ym, ym], axis=0).astype(BF))

        for n in range(N_PART, KT):
            finish(n, _dot(lhs_o, _u2b(wo_s[n])))
            if n == N_PART:
                for n2 in range(N_PART):
                    tail = _u2b(wo_s[n2, pl.ds(H_SPLIT * 64, (H - H_SPLIT) * 64), :])
                    finish(n2, _dot(lhs_b, tail) + acc[n2])
        return new_mem

    def body(i, mem):
        mem = list(mem)
        for u in range(UNROLL):
            mem = one_step(i, u, mem)
        return tuple(mem)

    for n in range(KT):
        wo_copy(n).wait()
    mi = mem0_s[...].astype(F32)
    mip = _b2u(jnp.concatenate([mi, mi], axis=0).astype(BF))
    lax.fori_loop(0, NSEG // UNROLL, body,
                  tuple(mip[:, 128 * k:128 * (k + 1)] for k in range(KT)))

    early = S - PRE
    FPER = 10

    def half_rows(r0):
        return r0 // 2 if isinstance(r0, int) else pl.multiple_of(r0 // 2, 8)

    def combine(r0, nrows, n, a, dst=None):
        xf = x_s[pl.ds(r0, nrows), pl.ds(128 * n, 128)].astype(F32)
        b = _u2b(xn_t[n, pl.ds(half_rows(r0), nrows // 2), :]).astype(F32)
        res = (_rbf(xf + a) + b).astype(BF)
        if dst is None:
            out_s[pl.ds(r0, nrows), pl.ds(128 * n, 128)] = res
        else:
            dst[:, pl.ds(128 * n, 128)] = res

    def combine_stored(r0, nrows, dst=None):
        for n in range(KT):
            combine(r0, nrows, n, _u2b(abuf[n, pl.ds(half_rows(r0), nrows // 2), :]).astype(F32), dst)

    def out_copy(r0, nrows, j):
        return pltpu.make_async_copy(out_s.at[pl.ds(r0, nrows), :], out_hbm.at[pl.ds(r0, nrows), :],
                                     sems.at[SEM_OUT + j])

    def ffn_groups(j0, y):
        x_sel = xsel_s[...]
        hid = {}

        def up(w_ref, j, key):
            cols = pl.ds(pl.multiple_of(128 * j, 128), 128)
            part = _dot(x_sel[:, 0:512], _u2b(w_ref[pl.ds(0, 256), cols]).astype(F32))
            yield
            hid[key] = _rbf(_dot(x_sel[:, 512:1024], _u2b(w_ref[pl.ds(256, 256), cols]).astype(F32)) + part)
            yield

        def down(jj, j):
            g = hid[("g", jj)]
            hb = _rbf(_rbf(g * _rbf(jax.nn.sigmoid(g))) * hid[("u", jj)])
            if 2 * FPER + jj >= FT:
                hb = jnp.where(j0 + jj < FT, hb, 0.0)
            rows = pl.ds(pl.multiple_of(64 * j, 64), 64)
            for half in range(2):
                y[half] = _dot(hb, _u2b(wd_s[rows, pl.ds(512 * half, 512)]).astype(F32)) + y[half]
                yield

        tile = [jnp.minimum(j0 + jj, FT - 1) for jj in range(FPER)]
        for jj in range(FPER + 1):
            if jj < FPER:
                yield from up(wg_s, tile[jj], ("g", jj))
                yield from up(wu_s, tile[jj], ("u", jj))
            if jj >= 1:
                yield from down(jj - 1, tile[jj - 1])

    def epi_chunk(r0, nrows, side, pieces, keep):
        pos = [((r0 + 32 * j) % RING) // 2 for j in range(nrows // 32)]
        if not isinstance(r0, int):
            pos = [pl.multiple_of(p, 16) for p in pos]
        fresh_zero()
        deps = {}
        for n in range(KT):
            acc = None
            for g in range(8):
                lhs = jnp.concatenate(
                    [_u2b(jnp.concatenate([oring[h, pl.ds(p, 16), :] for p in pos], axis=0))
                     for h in range(4 * g, 4 * g + 4)], axis=1)
                w = _after(wo_s[n, pl.ds(256 * g, 256), :], deps.get(8 * n + g), zero_box[0])
                y = _dot(lhs, _u2b(w))
                acc = y if acc is None else y + acc
                next(side, None)
                v = 8 * n + g
                if pieces is not None and v in EPI_SCHED:
                    r1 = pieces + 32 * EPI_SCHED.index(v)
                    combine_stored(r1, 32)
                    deps[v + EPI_LAG] = [_b2u(out_s[pl.ds(r1, 16), pl.ds(D - 128, 128)])]
            ab = acc.astype(BF)
            if keep:
                abuf[n, pl.ds(half_rows(r0), nrows // 2), :] = _b2u(ab)
            combine(r0, nrows, n, ab.astype(F32))

    for c in ffn_copies:
        c.wait()

    def epi_body(c, y):
        y = list(y)
        r0 = pl.multiple_of(early + ECH * c, 32)
        e0 = pl.multiple_of((early // 2) * (c & 1), 256)

        @pl.when(c == 2)
        def _():
            out_copy(0, early // 2, 4).wait()

        epi_chunk(r0, ECH, ffn_groups(FPER * c, y), e0, True)
        out_copy(r0, ECH, c).start()

        @pl.when(c < 2)
        def _():
            out_copy(e0, early // 2, 4 + c).start()

        return tuple(y)

    y = list(lax.fori_loop(0, 3, epi_body, (jnp.zeros((8, 512), F32), jnp.zeros((8, 512), F32))))
    idx1 = idx_s[0]
    idx2 = idx_s[1]

    def patch_row(t, yrow):
        xr, w = load_row(t)
        bits = pltpu.bitcast(_rbf(xr + yrow), U32)
        w = jnp.where(t % 2 == 0,
                      (w & jnp.uint32(0xFFFF0000)) | (bits >> 16),
                      (w & jnp.uint32(0xFFFF)) | bits)
        for k in range(KT):
            xn_t[k, pl.ds(t // 2, 1), :] = w[:, 128 * k:128 * (k + 1)]

    gate = _rbf(jax.nn.sigmoid(gate_s[0:8, 0:1]))
    yy = _rbf(_rbf(jnp.concatenate(y, axis=1)) * gate)
    patch_row(idx1, yy[0:1])
    patch_row(idx2, yy[1:2])

    last = early + 3 * ECH
    blk1 = jnp.minimum(idx1 // 16, last // 16 - 1)
    blk2 = jnp.minimum(idx2 // 16, last // 16 - 1)
    blk2 = jnp.where(blk2 == blk1, jnp.where(blk1 == 0, 1, blk1 - 1), blk2)
    fix = []
    for j, blk in enumerate((blk1, blk2)):
        r0 = pl.multiple_of(blk * 16, 16)
        combine_stored(r0, 16, fix_s.at[j])
        fix.append(pltpu.make_async_copy(fix_s.at[j], out_hbm.at[pl.ds(r0, 16), :], sems.at[SEM_OUT + 7 + j]))

    epi_chunk(last, S - last, iter(()), None, False)
    out_copy(last, S - last, 3).start()
    for c in range(3):
        out_copy(early + ECH * c, ECH, c).wait()
    out_copy(early // 2, early // 2, 5).wait()
    for cp in fix:
        cp.start()
    out_copy(last, S - last, 3).wait()
    for cp in fix:
        cp.wait()


@jax.jit
def pallas_parallel_sum__memory_aug_recurrent_mem_tr__moe_arch_mod__prompt_kernel(
    A_x: jax.Array,
    A_mem0: jax.Array,
    A_Wq: jax.Array,
    A_Wk: jax.Array,
    A_Wv: jax.Array,
    A_Wo: jax.Array,
    A_seg_len: jax.Array,
    B_x: jax.Array,
    B_w_r: jax.Array,
    B_w_gate: jax.Array,
    B_w_up: jax.Array,
    B_w_down: jax.Array,
):
    del A_seg_len, B_x
    assert A_x.shape == (1, S, D) and A_mem0.shape == (1, MEM, D)
    assert A_Wq.shape == (D, H, DH) and A_Wo.shape == (H, DH, D)
    assert B_w_gate.shape == (D, FF) and B_w_down.shape == (FF, D)
    any_spec = pl.BlockSpec(memory_space=pl.ANY)
    out = pl.pallas_call(
        _kernel,
        out_shape=jax.ShapeDtypeStruct((S, D), BF),
        in_specs=[any_spec] * 10,
        out_specs=any_spec,
        scratch_shapes=[
            pltpu.VMEM((S, D), BF),
            pltpu.VMEM((KT, S // 2, 128), U32),
            pltpu.VMEM((KT, PRE // 2, 128), U32),
            pltpu.VMEM((KT, 16 * NSEG, 128), U32),
            pltpu.VMEM((3 * H + 2, D // 2, 128), U32),
            pltpu.VMEM((KT, H * DH // 2, 128), U32),
            pltpu.VMEM((3 * H, RING32, 128), U32),
            pltpu.VMEM((H, RING32, 128), U32),
            pltpu.VMEM((KT, S // 2, 128), U32),
            pltpu.VMEM((S, D), BF),
            pltpu.VMEM((NPQ + 1, D, 128), U32),
            pltpu.VMEM((D // 2, FF), U32),
            pltpu.VMEM((D // 2, FF), U32),
            pltpu.VMEM((FF // 2, D), U32),
            pltpu.VMEM((MEM, D), BF),
            pltpu.VMEM((D,), BF),
            pltpu.VMEM((8, D), F32),
            pltpu.VMEM((16, 128), F32),
            pltpu.VMEM((8, D), F32),
            pltpu.VMEM((16, 128), F32),
            pltpu.VMEM((2, 16, D), BF),
            pltpu.SMEM((1,), jnp.int32),
            pltpu.SMEM((2,), jnp.int32),
            pltpu.SemaphoreType.DMA((NSEM,)),
        ],
        compiler_params=pltpu.CompilerParams(vmem_limit_bytes=126 * 1024 * 1024),
    )(A_x.reshape(S, D), A_mem0.reshape(MEM, D), A_Wq, A_Wk, A_Wv, A_Wo.reshape(H * DH, D),
      B_w_r, B_w_gate, B_w_up, B_w_down)
    return out.reshape(1, S, D)
```

```python
import jax
import jax.numpy as jnp
from jax import lax
import jax.experimental.pallas as pl
import jax.experimental.pallas.tpu as pltpu

BF = jnp.bfloat16
U32 = jnp.uint32
F32 = jnp.float32

S = 2048
D = 1024
H = 32
DH = 128
MEM = 8
SEG = 32
NSEG = S // SEG
FF = 3584
KT = D // 128
FT = FF // 128
XS = 24
PRE = S - NSEG * XS
RING = 576
RING32 = RING // 2
NPAIR = H // 2
NPQ = 3 * NPAIR
NPRE = 16
SEM_SMALL, SEM_X0, SEM_X = 0, 2, 6
SEM_W0 = SEM_X + NPRE
SEM_W = SEM_W0 + 3
SEM_WO = SEM_W + NPRE
SEM_FFN, SEM_OUT = SEM_WO + 1, SEM_WO + 2
NSEM = SEM_OUT + 9

LAG_QK = 1
LAG_PV = 4
N_PART = 4
H_SPLIT = 26
REL_SCHED = {0: [(0, 0), (0, 1)], 1: [(0, 2), (0, 3)], 2: [(0, 4)], 3: [(0, 5)], 4: [(0, 6)], 5: [(0, 7)]}
REL_SCHED.update({6 + k: [(1, k)] for k in range(8)})
REL_SCHED.update({14 + k: [(2, k)] for k in range(8)})
K_SPLIT = 2
EPI_SCHED = [v * 5 // 2 for v in range(24)]
EPI_LAG = 4
ECH = 160
REL_SCHED0 = {4: [(0, k) for k in range(4)], 5: [(0, k) for k in range(4, 8)],
              12: [(1, k) for k in range(4)], 13: [(1, k) for k in range(4, 8)]}
REL_SCHED0.update({14 + k: [(2, k)] for k in range(8)})
SCORE_SCHED = [1, 7, 13]
LN_SCHED = {3 * q: [q] for q in range(6)}
LN_SCHED0 = {13 + q: [q] for q in range(6)}
FIRST_BATCH = 12
LN_LAG = 5
FFN_DELAY = 2
REL_LAG = 2
UNROLL = 4


def _b2u(x):
    return pltpu.bitcast(x, U32)


def _u2b(x):
    return pltpu.bitcast(x, BF)


def _dot(a, b):
    return jnp.dot(a, b, preferred_element_type=F32)


def _dot_nt(a, b):
    return lax.dot_general(a, b, (((1,), (1,)), ((), ())), preferred_element_type=F32)


def _after(w, dep, zero):
    if not dep:
        return w
    d = dep[0]
    for e in dep[1:]:
        d = d | e
    return jnp.concatenate([w[0:8] | (d & zero), w[8:]], axis=0)


def _rbf(x):
    return x.astype(BF).astype(F32)


def _kernel(x_hbm, mem0_hbm, wq_hbm, wk_hbm, wv_hbm, wo_hbm, wr_hbm, wg_hbm, wu_hbm, wd_hbm,
            out_hbm,
            x_s, xn_t, xn_pre, hbuf, wqkv, wo_s, ring, oring, abuf, out_s, raw,
            wg_s, wu_s, wd_s, mem0_s, wr_s, wrf_s, r_s, sel_s, gate_s, fix_s, zero_s,
            sems):
    w32 = [w.bitcast(U32) for w in (wq_hbm, wk_hbm, wv_hbm)]
    wo32 = wo_hbm.bitcast(U32)
    wg32 = wg_hbm.bitcast(U32)
    wu32 = wu_hbm.bitcast(U32)
    wd32 = wd_hbm.bitcast(U32)

    def rows_copy(r0, n, sem):
        return pltpu.make_async_copy(x_hbm.at[pl.ds(r0, n), :], x_s.at[pl.ds(r0, n), :], sems.at[sem])

    def x_first(c):
        return rows_copy(128 * c if isinstance(c, int) else pl.multiple_of(128 * c, 128), 128, SEM_X0 + c)

    def x_piece(c):
        r0 = PRE + 96 * c if isinstance(c, int) else pl.multiple_of(PRE + 96 * c, 32)
        return rows_copy(r0, 96, SEM_X + c)

    def pair_copy(p):
        q = min(p, NPQ - 1)
        sem = SEM_W0 + p if p < 4 else SEM_W + (p - 1) // 3
        return pltpu.make_async_copy(w32[q // NPAIR].at[:, q % NPAIR, :], raw.at[p], sems.at[sem])

    def pairs_wait(t):
        dst = raw.at[pl.ds(3 * t + 1, 3)]
        pltpu.make_async_copy(dst, dst, sems.at[SEM_W + t]).wait()

    def wo_copy(n):
        return pltpu.make_async_copy(wo32.at[:, pl.ds(128 * n, 128)], wo_s.at[n], sems.at[SEM_WO])

    small_copies = [pltpu.make_async_copy(mem0_hbm, mem0_s, sems.at[SEM_SMALL]),
                    pltpu.make_async_copy(wr_hbm, wr_s, sems.at[SEM_SMALL + 1])]
    ffn_copies = [pltpu.make_async_copy(s_, d_, sems.at[SEM_FFN])
                  for s_, d_ in ((wg32, wg_s), (wu32, wu_s), (wd32, wd_s))]

    zero_s[0] = 0
    for c in range(4):
        x_first(c).start()
        if c == 0:
            for cp in small_copies:
                cp.start()

    def queue(t0, t1):
        for t in range(t0, t1):
            for p in range(3 * t + 1, 3 * t + 4):
                pair_copy(p).start()
            x_piece(t).start()

    pair_copy(0).start()
    queue(0, FIRST_BATCH)
    eps_bf = 1.0013580322265625e-05

    def score16(g, xn):
        wr = jnp.concatenate([wrf_s[...], wrf_s[...]], axis=0)
        score = _rbf(jnp.sum(xn.astype(F32) * wr, axis=1, keepdims=True))
        r_s[...] = jnp.where(lane16 == g, score, r_s[...])

    def layernorm16(rq, dst_ref, dst_row, not_before=None):
        rq = rq if isinstance(rq, int) else pl.multiple_of(rq, 16)
        xf = x_s[pl.ds(rq, 16), :].astype(F32)
        if not_before is not None:
            x0 = _after(pltpu.bitcast(xf[:, 0:128], U32), [not_before], zero_box[0])
            xf = jnp.concatenate([pltpu.bitcast(x0, F32), xf[:, 128:]], axis=1)
        mean = jnp.sum(xf, axis=1, keepdims=True) * (1.0 / D)
        cen = xf - mean
        var = jnp.sum(cen * cen, axis=1, keepdims=True) * (1.0 / D)
        sd = _rbf(jnp.sqrt(_rbf(_rbf(var) + eps_bf)))
        xn = (_rbf(xf - _rbf(mean)) * (1.0 / sd)).astype(BF)
        if dst_ref is hbuf:
            score16(rq // 16, xn)
        xp = _b2u(xn)
        hq = rq // 2 if isinstance(rq, int) else pl.multiple_of(rq // 2, 8)
        dst_row = dst_row if isinstance(dst_row, int) else pl.multiple_of(dst_row, 8)
        for k in range(KT):
            xn_t[k, pl.ds(hq, 8), :] = xp[:, 128 * k:128 * (k + 1)]
            dst_ref[k, pl.ds(dst_row, 8), :] = xp[:, 128 * k:128 * (k + 1)]

    zero_box = [None]

    def fresh_zero():
        zero_box[0] = jnp.full((8, 128), zero_s[0], jnp.int32).astype(U32)

    r_s[...] = jnp.full(r_s.shape, -jnp.inf, F32)
    lane16 = lax.broadcasted_iota(jnp.int32, (16, 128), 1)

    def ln_body(c, carry):
        x_first(c).wait()
        for q in range(8):
            layernorm16(128 * c + 16 * q, xn_pre, 64 * c + 8 * q)
        return carry

    lax.fori_loop(0, PRE // 128, ln_body, 0)


    def relayout(src, dst, j, k, not_before=None):
        a = src[j, pl.ds(128 * k, 64, stride=2), :]
        if not_before is not None:
            a = a | jnp.concatenate([not_before & zero_box[0]] * 8, axis=0)
        b = src[j, pl.ds(128 * k + 1, 64, stride=2), :]
        rows = pl.ds(64 * k, 64)
        dst[2 * j, rows, :] = (a & jnp.uint32(0xFFFF)) | (b << 16)
        dst[2 * j + 1, rows, :] = (a >> 16) | (b & jnp.uint32(0xFFFF0000))

    def pre_dot(w_view, ring_view, j, k, dep=None):
        i, q = k // 4, k % 4
        lhs = jnp.concatenate([_u2b(xn_pre[kk, pl.ds(64 * q, 64), :]) for kk in range(KT)], axis=1)
        y = _dot(lhs, _u2b(_after(w_view[2 * j + i], dep, zero_box[0])))
        yp = _b2u(y.astype(BF))
        ring_view[2 * j + i, pl.ds(32 + 64 * q, 64), :] = yp
        return yp[0:8]

    for c in small_copies:
        c.wait()
    pair_copy(0).wait()
    for k in range(8):
        relayout(raw, wqkv, 0, k)
    wrf_s[...] = jnp.broadcast_to(wr_s[...].astype(F32).reshape(1, D), (8, D))

    def pre_iter(t, barriers):
        deps = {}
        raw_view = raw.at[pl.ds(3 * t, 4)]
        w_view = wqkv.at[pl.ds(6 * t, 8)]
        ring_view = ring.at[pl.ds(6 * t, 6)]
        rel_sched, ln_sched = (REL_SCHED0, LN_SCHED0) if barriers else (REL_SCHED, LN_SCHED)
        done = None
        for v in range(24):
            j, k = v // 8, v % 8
            if v == 0 or v in barriers:
                for wait in barriers.get(v, ()):
                    wait()
                fresh_zero()
                done = None
            prev = done
            done = pre_dot(w_view, ring_view, j, k, deps.get(v))
            for jr, kr in rel_sched.get(v, ()):
                relayout(raw_view, w_view, jr + 1, kr, prev)
                deps.setdefault(v + REL_LAG, []).append(w_view[2 * jr + 3, pl.ds(64 * kr + 56, 8), :])
            for q in ln_sched.get(v, ()):
                hrow = 32 * (q // 3) + 8 * (q % 3)
                hrow += 64 * t if isinstance(t, int) else pl.multiple_of(64 * t, 64)
                layernorm16(PRE + 96 * t + 16 * q, hbuf, hrow, done if prev is not None else None)
                deps.setdefault(v + LN_LAG, []).append(hbuf[KT - 1, pl.ds(hrow, 8), :])
            if not barriers and v in SCORE_SCHED:
                g = jnp.minimum(3 * (t - 1) + SCORE_SCHED.index(v), PRE // 16 - 1)
                rows = pl.ds(pl.multiple_of(8 * g, 8), 8)
                xp = [xn_pre[kk, rows, :] for kk in range(KT)]
                xp[0] = xp[0] | (done & zero_box[0])
                score16(g, _u2b(jnp.concatenate(xp, axis=1)))

    def second_batch():
        queue(FIRST_BATCH, NPRE)
        for n in range(KT):
            wo_copy(n).start()
        for cp in ffn_copies:
            cp.start()

    pre_iter(0, {4: [pair_copy(1).wait],
                 12: [pair_copy(2).wait, pair_copy(3).wait, x_piece(0).wait, second_batch]})

    def pre_body(t, carry):
        x_piece(t).wait()
        pairs_wait(t)
        pre_iter(t, {})
        return carry

    lax.fori_loop(1, NPRE, pre_body, 0)
    row = lax.broadcasted_iota(jnp.int32, (80, 80), 0)
    col = lax.broadcasted_iota(jnp.int32, (80, 80), 1)
    same_head = (jnp.where(row < 64, row >> 5, (row - 64) >> 3)
                 == jnp.where(col < 64, col >> 5, (col - 64) >> 3))
    allowed = same_head & ((col >= 64) | (row >= 64) | (col <= row))
    fill = jnp.where(same_head, -1e9, -jnp.inf).astype(F32)
    low_half = lax.broadcasted_iota(jnp.int32, (8, 128), 0) < 4
    high_half = jnp.logical_not(low_half)
    scale = DH ** -0.5

    def load_row(t):
        w = jnp.concatenate([xn_t[k, pl.ds(t // 2, 1), :] for k in range(KT)], axis=1)
        bits = jnp.where(t % 2 == 0, w << 16, w & jnp.uint32(0xFFFF0000))
        return pltpu.bitcast(bits, F32), w

    def select_tokens():
        r = r_s[...]
        tok = lane16 * 16 + lax.broadcasted_iota(jnp.int32, (16, 128), 0)

        def full(op, v):
            return op(op(v, axis=0, keepdims=True), axis=1, keepdims=True)

        top1 = full(jnp.max, r)
        idx1 = full(jnp.min, jnp.where(r == top1, tok, S - 1))
        r2 = jnp.where(tok == idx1, -jnp.inf, r)
        top2 = full(jnp.max, r2)
        idx2 = full(jnp.min, jnp.where((r2 == top2) & (tok != idx1), tok, S - 1))
        first = lax.broadcasted_iota(jnp.int32, (8, 128), 0) == 0
        gate_s[...] = jnp.where(first, top1, top2)
        sel_s[...] = jnp.where(first, idx1, idx2)

    def one_step(i, u, mem):
        odd = u % 2
        s2 = i * (UNROLL // 2) + u // 2
        h_ld = pl.multiple_of(16 * UNROLL * i, 32) + 32 * (u // 2)
        a24 = pl.multiple_of(12 * UNROLL * i, 8)
        r24 = pl.multiple_of(a24 % RING32, 8) + XS * (u // 2)
        a24 = a24 + XS * (u // 2)
        qkv_ld = pl.multiple_of((SEG * s2 + 32) % RING32, 32) + 16 * odd
        o_st = pl.multiple_of((SEG * s2) % RING32, 32) + 16 * odd
        m0 = 0 if odd else XS

        def with_mem(ref, idx, base, m):
            lo = ref[idx, pl.ds(base + 8 * odd, 8), :]
            hi = ref[idx, pl.ds(base + 8 + 8 * odd, 8), :]
            if odd:
                lo = jnp.where(low_half, m, lo)
            else:
                hi = jnp.where(low_half, hi, m)
            return _u2b(jnp.concatenate([lo, hi], axis=0))

        def store_tokens(ref, idx, base, yp):
            if odd:
                pltpu.store(ref.at[idx, pl.ds(base + 8, 8), :], yp[0:8], mask=high_half)
                ref[idx, pl.ds(base + 16, 8), :] = yp[8:16]
            else:
                ref[idx, pl.ds(base, 8), :] = yp[0:8]
                pltpu.store(ref.at[idx, pl.ds(base + 8, 8), :], yp[8:16], mask=low_half)

        lk = [with_mem(hbuf, k, h_ld, mem[k]) for k in range(KT)]
        lhs = jnp.concatenate(lk, axis=1)

        ymem = {}
        xs = {}
        probs = {}
        parts = {}

        def proj(h):
            split = h < K_SPLIT and u > 0
            if split:
                lhs7 = jnp.concatenate(lk[:KT - 1], axis=1)
                head = [_dot(lhs7, _u2b(wqkv[m * H + h, pl.ds(0, 448), :])) for m in range(3)]
            for m in range(3):
                if split:
                    y = _dot(lk[KT - 1], _u2b(wqkv[m * H + h, pl.ds(448, 64), :])) + head[m]
                else:
                    y = _dot(lhs, _u2b(wqkv[m * H + h]))
                store_tokens(ring, m * H + h, r24, _b2u(y.astype(BF)))
                ymem[(h, m)] = y[m0:m0 + MEM]
                xs[(h, m)] = ring[m * H + h, pl.ds(qkv_ld, SEG // 2), :]

        def pair(p, m):
            a, b = 2 * p, 2 * p + 1
            mm = jnp.concatenate([ymem[(a, m)], ymem[(b, m)]], axis=0).astype(BF)
            return jnp.concatenate([_u2b(xs[(a, m)]), _u2b(xs[(b, m)]), mm], axis=0)

        def qk(p):
            sc = _dot_nt(pair(p, 0), pair(p, 1))
            sc = jnp.where(allowed, sc * scale, fill)
            e = jnp.exp(sc - jnp.max(sc, axis=1, keepdims=True))
            l = jnp.sum(e, axis=1, keepdims=True)
            r = pl.reciprocal(l, approx=True)
            r = r * (2.0 - l * r)
            probs[p] = (e * r).astype(BF)

        def pv(p):
            op = _b2u(_dot(probs[p], pair(p, 2)).astype(BF))
            om = op[32:40]
            om_sw = pltpu.roll(om, 4, axis=0)
            for j, h in enumerate((2 * p, 2 * p + 1)):
                oring[h, pl.ds(o_st, SEG // 2), :] = op[16 * j:16 * j + 16]
                parts[h] = with_mem(oring, h, r24, om if j != odd else om_sw)

        def after(t):
            for lag, fn in ((LAG_QK, qk), (LAG_PV, pv)):
                if (t - 1 - lag) % 2 == 0 and 0 <= (t - 1 - lag) // 2 < NPAIR:
                    fn((t - 1 - lag) // 2)

        for t in range(H):
            proj(t)
            after(t)
            if u == 0 and t == 8:
                select_tokens()
        t = H
        lhs_a = jnp.concatenate([parts[j] for j in range(H_SPLIT)], axis=1)
        acc = []
        for n in range(N_PART):
            acc.append(_dot(lhs_a, _u2b(wo_s[n, pl.ds(0, H_SPLIT * 64), :])))
            after(t)
            t += 1
        while t - 1 - LAG_PV <= 2 * (NPAIR - 1):
            after(t)
            t += 1
        lhs_b = jnp.concatenate([parts[j] for j in range(H_SPLIT, H)], axis=1)
        lhs_o = jnp.concatenate([lhs_a, lhs_b], axis=1)
        new_mem = [None] * KT

        def finish(n, y):
            store_tokens(abuf, n, a24, _b2u(y.astype(BF)))
            ym = y[m0:m0 + MEM]
            new_mem[n] = _b2u(jnp.concatenate([ym, ym], axis=0).astype(BF))

        for n in range(N_PART, KT):
            finish(n, _dot(lhs_o, _u2b(wo_s[n])))
            if n == N_PART:
                for n2 in range(N_PART):
                    tail = _u2b(wo_s[n2, pl.ds(H_SPLIT * 64, (H - H_SPLIT) * 64), :])
                    finish(n2, _dot(lhs_b, tail) + acc[n2])
        return new_mem

    def body(i, mem):
        mem = list(mem)
        for u in range(UNROLL):
            mem = one_step(i, u, mem)
        return tuple(mem)

    for n in range(KT):
        wo_copy(n).wait()
    mi = mem0_s[...].astype(F32)
    mip = _b2u(jnp.concatenate([mi, mi], axis=0).astype(BF))
    lax.fori_loop(0, NSEG // UNROLL, body,
                  tuple(mip[:, 128 * k:128 * (k + 1)] for k in range(KT)))

    early = S - PRE
    FPER = 10

    def half_rows(r0):
        return r0 // 2 if isinstance(r0, int) else pl.multiple_of(r0 // 2, 8)

    def combine(r0, nrows, n, a, dst=None):
        xf = x_s[pl.ds(r0, nrows), pl.ds(128 * n, 128)].astype(F32)
        b = _u2b(xn_t[n, pl.ds(half_rows(r0), nrows // 2), :]).astype(F32)
        res = (_rbf(xf + a) + b).astype(BF)
        if dst is None:
            out_s[pl.ds(r0, nrows), pl.ds(128 * n, 128)] = res
        else:
            dst[:, pl.ds(128 * n, 128)] = res

    def combine_stored(r0, nrows, dst=None):
        for n in range(KT):
            combine(r0, nrows, n, _u2b(abuf[n, pl.ds(half_rows(r0), nrows // 2), :]).astype(F32), dst)

    def out_copy(r0, nrows, j):
        return pltpu.make_async_copy(out_s.at[pl.ds(r0, nrows), :], out_hbm.at[pl.ds(r0, nrows), :],
                                     sems.at[SEM_OUT + j])

    def ffn_groups(j0, y):
        sel_row = lax.broadcasted_iota(jnp.int32, (8, D), 0)
        xs1, _ = load_row(sel_s[0, 0])
        xs2, _ = load_row(sel_s[1, 0])
        x_sel = jnp.where(sel_row == 0, xs1, jnp.where(sel_row == 1, xs2, 0.0))
        hid = {}
        for _ in range(FFN_DELAY):
            yield

        def up(w_ref, j, key):
            cols = pl.ds(pl.multiple_of(128 * j, 128), 128)
            part = _dot(x_sel[:, 0:512], _u2b(w_ref[pl.ds(0, 256), cols]).astype(F32))
            yield
            hid[key] = _rbf(_dot(x_sel[:, 512:1024], _u2b(w_ref[pl.ds(256, 256), cols]).astype(F32)) + part)
            yield

        def down(jj, j):
            g = hid[("g", jj)]
            hb = _rbf(_rbf(g * _rbf(jax.nn.sigmoid(g))) * hid[("u", jj)])
            if 2 * FPER + jj >= FT:
                hb = jnp.where(j0 + jj < FT, hb, 0.0)
            rows = pl.ds(pl.multiple_of(64 * j, 64), 64)
            for half in range(2):
                y[half] = _dot(hb, _u2b(wd_s[rows, pl.ds(512 * half, 512)]).astype(F32)) + y[half]
                yield

        tile = [jnp.minimum(j0 + jj, FT - 1) for jj in range(FPER)]
        for jj in range(FPER + 1):
            if jj < FPER:
                yield from up(wg_s, tile[jj], ("g", jj))
                yield from up(wu_s, tile[jj], ("u", jj))
            if jj >= 1:
                yield from down(jj - 1, tile[jj - 1])

    def epi_chunk(r0, nrows, side, pieces, keep):
        pos = [((r0 + 32 * j) % RING) // 2 for j in range(nrows // 32)]
        if not isinstance(r0, int):
            pos = [pl.multiple_of(p, 16) for p in pos]
        fresh_zero()
        deps = {}
        for n in range(KT):
            acc = None
            for g in range(8):
                lhs = jnp.concatenate(
                    [_u2b(jnp.concatenate([oring[h, pl.ds(p, 16), :] for p in pos], axis=0))
                     for h in range(4 * g, 4 * g + 4)], axis=1)
                w = _after(wo_s[n, pl.ds(256 * g, 256), :], deps.get(8 * n + g), zero_box[0])
                y = _dot(lhs, _u2b(w))
                acc = y if acc is None else y + acc
                next(side, None)
                v = 8 * n + g
                if pieces is not None and v in EPI_SCHED:
                    r1 = pieces + 32 * EPI_SCHED.index(v)
                    combine_stored(r1, 32)
                    deps[v + EPI_LAG] = [_b2u(out_s[pl.ds(r1, 16), pl.ds(D - 128, 128)])]
            ab = acc.astype(BF)
            if keep:
                abuf[n, pl.ds(half_rows(r0), nrows // 2), :] = _b2u(ab)
            combine(r0, nrows, n, ab.astype(F32))

    for c in ffn_copies:
        c.wait()

    def epi_body(c, y):
        y = list(y)
        r0 = pl.multiple_of(early + ECH * c, 32)
        e0 = pl.multiple_of((early // 2) * (c & 1), 256)

        @pl.when(c == 2)
        def _():
            out_copy(0, early // 2, 4).wait()

        epi_chunk(r0, ECH, ffn_groups(FPER * c, y), e0, True)
        out_copy(r0, ECH, c).start()

        @pl.when(c < 2)
        def _():
            out_copy(e0, early // 2, 4 + c).start()

        return tuple(y)

    y = list(lax.fori_loop(0, 3, epi_body, (jnp.zeros((8, 512), F32), jnp.zeros((8, 512), F32))))
    idx1 = sel_s[0, 0]
    idx2 = sel_s[1, 0]

    def patch_row(t, yrow):
        xr, w = load_row(t)
        bits = pltpu.bitcast(_rbf(xr + yrow), U32)
        w = jnp.where(t % 2 == 0,
                      (w & jnp.uint32(0xFFFF0000)) | (bits >> 16),
                      (w & jnp.uint32(0xFFFF)) | bits)
        for k in range(KT):
            xn_t[k, pl.ds(t // 2, 1), :] = w[:, 128 * k:128 * (k + 1)]

    gate = _rbf(jax.nn.sigmoid(gate_s[:, 0:1]))
    yy = _rbf(_rbf(jnp.concatenate(y, axis=1)) * gate)
    patch_row(idx1, yy[0:1])
    patch_row(idx2, yy[1:2])

    last = early + 3 * ECH
    blk1 = jnp.minimum(idx1 // 16, last // 16 - 1)
    blk2 = jnp.minimum(idx2 // 16, last // 16 - 1)
    blk2 = jnp.where(blk2 == blk1, jnp.where(blk1 == 0, 1, blk1 - 1), blk2)
    fix = []
    for j, blk in enumerate((blk1, blk2)):
        r0 = pl.multiple_of(blk * 16, 16)
        combine_stored(r0, 16, fix_s.at[j])
        fix.append(pltpu.make_async_copy(fix_s.at[j], out_hbm.at[pl.ds(r0, 16), :], sems.at[SEM_OUT + 7 + j]))

    epi_chunk(last, S - last, iter(()), None, False)
    out_copy(last, S - last, 3).start()
    for c in range(3):
        out_copy(early + ECH * c, ECH, c).wait()
    out_copy(early // 2, early // 2, 5).wait()
    for cp in fix:
        cp.start()
    out_copy(last, S - last, 3).wait()
    for cp in fix:
        cp.wait()


@jax.jit
def pallas_parallel_sum__memory_aug_recurrent_mem_tr__moe_arch_mod__prompt_kernel(
    A_x: jax.Array,
    A_mem0: jax.Array,
    A_Wq: jax.Array,
    A_Wk: jax.Array,
    A_Wv: jax.Array,
    A_Wo: jax.Array,
    A_seg_len: jax.Array,
    B_x: jax.Array,
    B_w_r: jax.Array,
    B_w_gate: jax.Array,
    B_w_up: jax.Array,
    B_w_down: jax.Array,
):
    del A_seg_len, B_x
    assert A_x.shape == (1, S, D) and A_mem0.shape == (1, MEM, D)
    assert A_Wq.shape == (D, H, DH) and A_Wo.shape == (H, DH, D)
    assert B_w_gate.shape == (D, FF) and B_w_down.shape == (FF, D)
    any_spec = pl.BlockSpec(memory_space=pl.ANY)
    out = pl.pallas_call(
        _kernel,
        out_shape=jax.ShapeDtypeStruct((S, D), BF),
        in_specs=[any_spec] * 10,
        out_specs=any_spec,
        scratch_shapes=[
            pltpu.VMEM((S, D), BF),
            pltpu.VMEM((KT, S // 2, 128), U32),
            pltpu.VMEM((KT, PRE // 2, 128), U32),
            pltpu.VMEM((KT, 16 * NSEG, 128), U32),
            pltpu.VMEM((3 * H + 2, D // 2, 128), U32),
            pltpu.VMEM((KT, H * DH // 2, 128), U32),
            pltpu.VMEM((3 * H, RING32, 128), U32),
            pltpu.VMEM((H, RING32, 128), U32),
            pltpu.VMEM((KT, S // 2, 128), U32),
            pltpu.VMEM((S, D), BF),
            pltpu.VMEM((NPQ + 1, D, 128), U32),
            pltpu.VMEM((D // 2, FF), U32),
            pltpu.VMEM((D // 2, FF), U32),
            pltpu.VMEM((FF // 2, D), U32),
            pltpu.VMEM((MEM, D), BF),
            pltpu.VMEM((D,), BF),
            pltpu.VMEM((8, D), F32),
            pltpu.VMEM((16, 128), F32),
            pltpu.VMEM((8, 128), jnp.int32),
            pltpu.VMEM((8, 128), F32),
            pltpu.VMEM((2, 16, D), BF),
            pltpu.SMEM((1,), jnp.int32),
            pltpu.SemaphoreType.DMA((NSEM,)),
        ],
        compiler_params=pltpu.CompilerParams(vmem_limit_bytes=126 * 1024 * 1024),
    )(A_x.reshape(S, D), A_mem0.reshape(MEM, D), A_Wq, A_Wk, A_Wv, A_Wo.reshape(H * DH, D),
      B_w_r, B_w_gate, B_w_up, B_w_down)
    return out.reshape(1, S, D)
```

```python
import jax
import jax.numpy as jnp
from jax import lax
import jax.experimental.pallas as pl
import jax.experimental.pallas.tpu as pltpu

BF = jnp.bfloat16
U32 = jnp.uint32
F32 = jnp.float32

S = 2048
D = 1024
H = 32
DH = 128
MEM = 8
SEG = 32
NSEG = S // SEG
FF = 3584
KT = D // 128
FT = FF // 128
XS = 24
PRE = S - NSEG * XS
RING = 576
RING32 = RING // 2
NPAIR = H // 2
NPQ = 3 * NPAIR
PP = 6
NPRE = NPQ // PP
LNP = 14
NLN = (S - PRE) // 16
SEM_SMALL, SEM_X0, SEM_X = 0, 2, 6
SEM_W0 = SEM_X + NPRE
SEM_W = SEM_W0 + PP
SEM_WO = SEM_W + NPRE
SEM_FFN0, SEM_FFN, SEM_FIX, SEM_OUT = SEM_WO + 1, SEM_WO + 2, SEM_WO + 3, SEM_WO + 5
NSEM = SEM_OUT + 16

LAG_QK = 1
LAG_PV = 4
N_PART = 4
H_SPLIT = 26
REL_SCHED = {0: [(0, 0), (0, 1)], 1: [(0, 2), (0, 3)], 2: [(0, 4)], 3: [(0, 5)], 4: [(0, 6)], 5: [(0, 7)]}
REL_SCHED.update({8 * j - 2 + k: [(j, k)] for j in range(1, PP) for k in range(8)})
N_PART_ODD = 4
H_SPLIT_ODD = 24
K_SPLIT = 2
EPI_SCHED = [v * 5 // 2 for v in range(24)]
EPI_LAG = 4
ECH = 160
REL_SCHED0 = {4: [(0, k) for k in range(4)], 5: [(0, k) for k in range(4, 8)],
              12: [(1, k) for k in range(4)], 13: [(1, k) for k in range(4, 8)],
              24: [(3, 0), (3, 1)], 25: [(3, 2), (3, 3)], 26: [(3, 4)], 27: [(3, 5)], 28: [(3, 6)], 29: [(3, 7)]}
REL_SCHED0.update({8 * j - 2 + k: [(j, k)] for j in (2, 4, 5) for k in range(8)})
BARRIERS0 = {4: [1], 12: [2, 3], 24: [4, 5, 6]}
SCORE_SCHED = [1, 10, 19, 28, 37]
LN_SCHED = [3 * q for q in range(LNP)]
FIRST_BATCH = 6
LN_LAG = 5
FFN_DELAY = 2
REL_LAG = 2
UNROLL = 4


def _b2u(x):
    return pltpu.bitcast(x, U32)


def _u2b(x):
    return pltpu.bitcast(x, BF)


def _dot(a, b):
    return jnp.dot(a, b, preferred_element_type=F32)


def _dot_nt(a, b):
    return lax.dot_general(a, b, (((1,), (1,)), ((), ())), preferred_element_type=F32)


def _after(w, dep, zero):
    if not dep:
        return w
    d = dep[0]
    for e in dep[1:]:
        d = d | e
    return jnp.concatenate([w[0:8] | (d & zero), w[8:]], axis=0)


def _rbf(x):
    return x.astype(BF).astype(F32)


def _kernel(x_hbm, mem0_hbm, wq_hbm, wk_hbm, wv_hbm, wo_hbm, wr_hbm, wg_hbm, wu_hbm, wd_hbm,
            out_hbm,
            x_s, xn_t, xn_pre, hbuf, wqkv, wo_s, ring, abuf, out_s, raw,
            wg_s, wu_s, wd_s, mem0_s, wr_s, wrf_s, r_s, sel_s, gate_s, xsel_s, fix_s, zero_s,
            sems):
    w32 = [w.bitcast(U32) for w in (wq_hbm, wk_hbm, wv_hbm)]
    wo32 = wo_hbm.bitcast(U32)
    wg32 = wg_hbm.bitcast(U32)
    wu32 = wu_hbm.bitcast(U32)
    wd32 = wd_hbm.bitcast(U32)

    def rows_copy(r0, n, sem):
        return pltpu.make_async_copy(x_hbm.at[pl.ds(r0, n), :], x_s.at[pl.ds(r0, n), :], sems.at[sem])

    def x_first(c):
        return rows_copy(128 * c if isinstance(c, int) else pl.multiple_of(128 * c, 128), 128, SEM_X0 + c)

    def x_piece(t, last):
        r0 = PRE + 16 * LNP * (t - 1)
        n = S - PRE - 16 * LNP * (NPRE - 2) if last else 16 * LNP
        return rows_copy(r0 if isinstance(t, int) else pl.multiple_of(r0, 32), n, SEM_X + t)

    def pair_copy(p):
        q = min(p, NPQ - 1)
        sem = SEM_W0 + p if p <= PP else SEM_W + (p - 1) // PP
        return pltpu.make_async_copy(w32[q // NPAIR].at[:, q % NPAIR, :], raw.at[p], sems.at[sem])

    def pairs_wait(t):
        dst = raw.at[pl.ds(PP * t + 1, PP)]
        pltpu.make_async_copy(dst, dst, sems.at[SEM_W + t]).wait()

    def wo_copy(n):
        return pltpu.make_async_copy(wo32.at[:, pl.ds(128 * n, 128)], wo_s.at[n], sems.at[SEM_WO])

    small_copies = [pltpu.make_async_copy(mem0_hbm, mem0_s, sems.at[SEM_SMALL]),
                    pltpu.make_async_copy(wr_hbm, wr_s, sems.at[SEM_SMALL + 1])]
    ffn0_copies = [
        pltpu.make_async_copy(wg32.at[:, pl.ds(0, 128)], wg_s.at[:, pl.ds(0, 128)], sems.at[SEM_FFN0]),
        pltpu.make_async_copy(wu32.at[:, pl.ds(0, 128)], wu_s.at[:, pl.ds(0, 128)], sems.at[SEM_FFN0]),
        pltpu.make_async_copy(wd32.at[pl.ds(0, 64), :], wd_s.at[pl.ds(0, 64), :], sems.at[SEM_FFN0])]
    ffn_copies = [
        pltpu.make_async_copy(wg32.at[:, pl.ds(128, FF - 128)], wg_s.at[:, pl.ds(128, FF - 128)], sems.at[SEM_FFN]),
        pltpu.make_async_copy(wu32.at[:, pl.ds(128, FF - 128)], wu_s.at[:, pl.ds(128, FF - 128)], sems.at[SEM_FFN]),
        pltpu.make_async_copy(wd32.at[pl.ds(64, FF // 2 - 64), :], wd_s.at[pl.ds(64, FF // 2 - 64), :],
                              sems.at[SEM_FFN])]

    zero_s[0] = 0
    for c in range(4):
        x_first(c).start()
        if c == 0:
            for cp in small_copies:
                cp.start()

    def queue(t0, t1):
        for t in range(t0, t1):
            for p in range(PP * t + 1, PP * t + PP + 1):
                pair_copy(p).start()
            if t >= 1:
                x_piece(t, t == NPRE - 1).start()

    pair_copy(0).start()
    queue(0, FIRST_BATCH)
    eps_bf = 1.0013580322265625e-05

    def score16(g, xn):
        wr = jnp.concatenate([wrf_s[...], wrf_s[...]], axis=0)
        score = _rbf(jnp.sum(xn.astype(F32) * wr, axis=1, keepdims=True))
        r_s[...] = jnp.where(lane16 == g, score, r_s[...])

    def layernorm16(rq, dst_ref, dst_row, not_before=None):
        rq = rq if isinstance(rq, int) else pl.multiple_of(rq, 16)
        xf = x_s[pl.ds(rq, 16), :].astype(F32)
        if not_before is not None:
            x0 = _after(pltpu.bitcast(xf[:, 0:128], U32), [not_before], zero_box[0])
            xf = jnp.concatenate([pltpu.bitcast(x0, F32), xf[:, 128:]], axis=1)
        mean = jnp.sum(xf, axis=1, keepdims=True) * (1.0 / D)
        cen = xf - mean
        var = jnp.sum(cen * cen, axis=1, keepdims=True) * (1.0 / D)
        sd = _rbf(jnp.sqrt(_rbf(_rbf(var) + eps_bf)))
        xn = (_rbf(xf - _rbf(mean)) * (1.0 / sd)).astype(BF)
        if dst_ref is hbuf:
            score16(rq // 16, xn)
        xp = _b2u(xn)
        hq = rq // 2 if isinstance(rq, int) else pl.multiple_of(rq // 2, 8)
        dst_row = dst_row if isinstance(dst_row, int) else pl.multiple_of(dst_row, 8)
        for k in range(KT):
            xn_t[k, pl.ds(hq, 8), :] = xp[:, 128 * k:128 * (k + 1)]
            dst_ref[k, pl.ds(dst_row, 8), :] = xp[:, 128 * k:128 * (k + 1)]

    zero_box = [None]

    def fresh_zero():
        zero_box[0] = jnp.full((8, 128), zero_s[0], jnp.int32).astype(U32)

    r_s[...] = jnp.full(r_s.shape, -jnp.inf, F32)
    lane16 = lax.broadcasted_iota(jnp.int32, (16, 128), 1)

    def ln_body(c, carry):
        x_first(c).wait()
        for q in range(8):
            layernorm16(128 * c + 16 * q, xn_pre, 64 * c + 8 * q)
        return carry

    lax.fori_loop(0, PRE // 128, ln_body, 0)


    def relayout(src, dst, j, k, not_before=None):
        a = src[j, pl.ds(128 * k, 64, stride=2), :]
        if not_before is not None:
            a = a | jnp.concatenate([not_before & zero_box[0]] * 8, axis=0)
        b = src[j, pl.ds(128 * k + 1, 64, stride=2), :]
        rows = pl.ds(64 * k, 64)
        dst[2 * j, rows, :] = (a & jnp.uint32(0xFFFF)) | (b << 16)
        dst[2 * j + 1, rows, :] = (a >> 16) | (b & jnp.uint32(0xFFFF0000))

    def pre_dot(w_view, ring_view, j, k, dep=None):
        i, q = k // 4, k % 4
        lhs = jnp.concatenate([_u2b(xn_pre[kk, pl.ds(64 * q, 64), :]) for kk in range(KT)], axis=1)
        y = _dot(lhs, _u2b(_after(w_view[2 * j + i], dep, zero_box[0])))
        yp = _b2u(y.astype(BF))
        ring_view[2 * j + i, pl.ds(32 + 64 * q, 64), :] = yp
        return yp[0:8]

    for c in small_copies:
        c.wait()
    pair_copy(0).wait()
    for k in range(8):
        relayout(raw, wqkv, 0, k)
    wrf_s[...] = jnp.broadcast_to(wr_s[...].astype(F32).reshape(1, D), (8, D))

    def second_batch():
        queue(FIRST_BATCH, NPRE)
        for n in range(KT):
            wo_copy(n).start()
        for cp in ffn0_copies + ffn_copies:
            cp.start()

    def pre_iter(t, first):
        deps = {}
        raw_view = raw.at[pl.ds(PP * t, PP + 1)]
        w_view = wqkv.at[pl.ds(2 * PP * t, 2 * PP + 2)]
        ring_view = ring.at[pl.ds(2 * PP * t, 2 * PP)]
        done = None
        for v in range(8 * PP):
            j, k = v // 8, v % 8
            if v == 0 or (first and v in BARRIERS0):
                if v:
                    for p in BARRIERS0[v]:
                        pair_copy(p).wait()
                    if v == max(BARRIERS0):
                        second_batch()
                fresh_zero()
                done = None
            prev = done
            done = pre_dot(w_view, ring_view, j, k, deps.get(v))
            for jr, kr in (REL_SCHED0 if first else REL_SCHED).get(v, ()):
                relayout(raw_view, w_view, jr + 1, kr, prev)
                deps.setdefault(v + REL_LAG, []).append(w_view[2 * jr + 3, pl.ds(64 * kr + 56, 8), :])
            if first:
                continue
            if v in LN_SCHED:
                q = jnp.minimum(LNP * (t - 1) + LN_SCHED.index(v), NLN - 1)
                hrow = pl.multiple_of(32 * (q // 3) + 8 * (q % 3), 8)
                layernorm16(PRE + 16 * q, hbuf, hrow, done if prev is not None else None)
                deps.setdefault(v + LN_LAG, []).append(hbuf[KT - 1, pl.ds(hrow, 8), :])
            if v in SCORE_SCHED:
                g = jnp.minimum(len(SCORE_SCHED) * (t - 1) + SCORE_SCHED.index(v), PRE // 16 - 1)
                rows = pl.ds(pl.multiple_of(8 * g, 8), 8)
                xp = [xn_pre[kk, rows, :] for kk in range(KT)]
                xp[0] = xp[0] | (done & zero_box[0])
                score16(g, _u2b(jnp.concatenate(xp, axis=1)))

    pre_iter(0, True)

    def pre_body(t, carry):
        pairs_wait(t)

        @pl.when(t < NPRE - 1)
        def _():
            x_piece(t, False).wait()

        @pl.when(t == NPRE - 1)
        def _():
            x_piece(NPRE - 1, True).wait()
        pre_iter(t, False)
        return carry

    lax.fori_loop(1, NPRE, pre_body, 0)
    row = lax.broadcasted_iota(jnp.int32, (80, 80), 0)
    col = lax.broadcasted_iota(jnp.int32, (80, 80), 1)
    same_head = (jnp.where(row < 64, row >> 5, (row - 64) >> 3)
                 == jnp.where(col < 64, col >> 5, (col - 64) >> 3))
    allowed = same_head & ((col >= 64) | (row >= 64) | (col <= row))
    fill = jnp.where(same_head, -1e9, -jnp.inf).astype(F32)
    low_half = lax.broadcasted_iota(jnp.int32, (8, 128), 0) < 4
    high_half = jnp.logical_not(low_half)
    scale = DH ** -0.5

    def load_row(t):
        w = jnp.concatenate([xn_t[k, pl.ds(t // 2, 1), :] for k in range(KT)], axis=1)
        bits = jnp.where(t % 2 == 0, w << 16, w & jnp.uint32(0xFFFF0000))
        return pltpu.bitcast(bits, F32), w

    def select_tokens():
        r = r_s[...]
        tok = lane16 * 16 + lax.broadcasted_iota(jnp.int32, (16, 128), 0)

        def full(op, v):
            return op(op(v, axis=0, keepdims=True), axis=1, keepdims=True)

        top1 = full(jnp.max, r)
        idx1 = full(jnp.min, jnp.where(r == top1, tok, S - 1))
        r2 = jnp.where(tok == idx1, -jnp.inf, r)
        top2 = full(jnp.max, r2)
        idx2 = full(jnp.min, jnp.where((r2 == top2) & (tok != idx1), tok, S - 1))
        first = lax.broadcasted_iota(jnp.int32, (8, 128), 0) == 0
        gate_s[...] = jnp.where(first, top1, top2)
        sel_s[...] = jnp.where(first, idx1, idx2)

    NIT = NSEG // UNROLL
    ROWS = SEG * UNROLL

    def half_rows(r0):
        return pl.multiple_of(r0 // 2, 8)

    def residual(xf, a, b):
        return (_rbf(xf + a) + b).astype(BF)

    def out_copy(i):
        r0 = ROWS * i if isinstance(i, int) else pl.multiple_of(ROWS * i, ROWS)
        return pltpu.make_async_copy(out_s.at[pl.ds(r0, ROWS), :], out_hbm.at[pl.ds(r0, ROWS), :],
                                     sems.at[SEM_OUT + i])

    def ffn_groups(i, y):
        x_sel = xsel_s[...]
        live = (i >= 1) & (i < NIT - 1)
        hid = {}

        def up(w_ref, j, key):
            cols = pl.ds(pl.multiple_of(128 * j, 128), 128)
            part = _dot(x_sel[:, 0:512], _u2b(w_ref[pl.ds(0, 256), cols]).astype(F32))
            yield
            hid[key] = _rbf(_dot(x_sel[:, 512:1024], _u2b(w_ref[pl.ds(256, 256), cols]).astype(F32)) + part)
            yield

        for jj in range(2):
            j = jnp.clip(2 * (i - 1) + jj, 0, FT - 1)
            yield from up(wg_s, j, "g")
            yield from up(wu_s, j, "u")
            g = hid["g"]
            hb = jnp.where(live, _rbf(_rbf(g * _rbf(jax.nn.sigmoid(g))) * hid["u"]), 0.0)
            rows = pl.ds(pl.multiple_of(64 * j, 64), 64)
            yield
            for half in range(2):
                y[half] = _dot(hb, _u2b(wd_s[rows, pl.ds(512 * half, 512)]).astype(F32)) + y[half]
                yield

    def one_step(i, u, mem, held, side):
        odd = u % 2
        s2 = i * (UNROLL // 2) + u // 2
        h_ld = pl.multiple_of(16 * UNROLL * i, 32) + 32 * (u // 2)
        r24 = pl.multiple_of((12 * UNROLL * i) % RING32, 8) + XS * (u // 2)
        qkv_ld = pl.multiple_of((SEG * s2 + 32) % RING32, 32) + 16 * odd
        m0 = 0 if odd else XS

        def with_mem(lo, hi, m):
            if odd:
                return [jnp.where(low_half, m, lo), hi]
            return [lo, jnp.where(low_half, hi, m)]

        def store_tokens(ref, idx, base, yp):
            if odd:
                pltpu.store(ref.at[idx, pl.ds(base + 8, 8), :], yp[0:8], mask=high_half)
                ref[idx, pl.ds(base + 16, yp.shape[0] - 8), :] = yp[8:]
            else:
                ref[idx, pl.ds(base, 8), :] = yp[0:8]
                pltpu.store(ref.at[idx, pl.ds(base + 8, 8), :], yp[8:16], mask=low_half)

        lk = [_u2b(jnp.concatenate(with_mem(hbuf[k, pl.ds(h_ld + 8 * odd, 8), :],
                                            hbuf[k, pl.ds(h_ld + 8 + 8 * odd, 8), :], mem[k]), axis=0))
              for k in range(KT)]
        lhs = jnp.concatenate(lk, axis=1)

        ymem = {}
        xs = {}
        probs = {}
        parts = {}

        def proj(h):
            split = h < K_SPLIT and u > 0
            if split:
                lhs7 = jnp.concatenate(lk[:KT - 1], axis=1)
                head = [_dot(lhs7, _u2b(wqkv[m * H + h, pl.ds(0, 448), :])) for m in range(3)]
            for m in range(3):
                if split:
                    y = _dot(lk[KT - 1], _u2b(wqkv[m * H + h, pl.ds(448, 64), :])) + head[m]
                else:
                    y = _dot(lhs, _u2b(wqkv[m * H + h]))
                store_tokens(ring, m * H + h, r24, _b2u(y.astype(BF)))
                ymem[(h, m)] = y[m0:m0 + MEM]
                xs[(h, m)] = ring[m * H + h, pl.ds(qkv_ld, SEG // 2), :]

        def pair(p, m):
            a, b = 2 * p, 2 * p + 1
            mm = jnp.concatenate([ymem[(a, m)], ymem[(b, m)]], axis=0).astype(BF)
            return jnp.concatenate([_u2b(xs[(a, m)]), _u2b(xs[(b, m)]), mm], axis=0)

        def qk(p):
            sc = _dot_nt(pair(p, 0), pair(p, 1))
            sc = jnp.where(allowed, sc * scale, fill)
            e = jnp.exp(sc - jnp.max(sc, axis=1, keepdims=True))
            l = jnp.sum(e, axis=1, keepdims=True)
            r = pl.reciprocal(l, approx=True)
            r = r * (2.0 - l * r)
            probs[p] = (e * r).astype(BF)

        def pv(p):
            op = _b2u(_dot(probs[p], pair(p, 2)).astype(BF))
            om = op[32:40]
            om_sw = pltpu.roll(om, 4, axis=0)
            for j, h in enumerate((2 * p, 2 * p + 1)):
                x0, x1 = op[16 * j:16 * j + 8], op[16 * j + 8:16 * j + 16]
                m = om if j != odd else om_sw
                if odd:
                    rows = with_mem(held[h], x0, m) + [x1]
                else:
                    rows = with_mem(x0, x1, m)
                    held[h] = x1
                parts[h] = _u2b(jnp.concatenate(rows, axis=0))

        def after(t):
            for lag, fn in ((LAG_QK, qk), (LAG_PV, pv)):
                if (t - 1 - lag) % 2 == 0 and 0 <= (t - 1 - lag) // 2 < NPAIR:
                    fn((t - 1 - lag) // 2)

        def side_group():
            if odd:
                next(side, None)

        for t in range(H):
            proj(t)
            after(t)
            if u == 0 and t == 8:
                select_tokens()
        t = H
        n_part, h_split = (N_PART_ODD, H_SPLIT_ODD) if odd else (N_PART, H_SPLIT)
        lhs_a = jnp.concatenate([parts[j] for j in range(h_split)], axis=1)
        acc = []
        for n in range(n_part):
            acc.append(_dot(lhs_a, _u2b(wo_s[n, pl.ds(0, h_split * 64), :])))
            after(t)
            side_group()
            t += 1
        while t - 1 - LAG_PV <= 2 * (NPAIR - 1):
            after(t)
            t += 1
        lhs_b = jnp.concatenate([parts[j] for j in range(h_split, H)], axis=1)
        lhs_o = jnp.concatenate([lhs_a, lhs_b], axis=1)
        new_mem = [None] * KT
        pair_row = pl.multiple_of(ROWS * i, 64) + 64 * (u // 2)

        def finish(n, y):
            ym = y[m0:m0 + MEM]
            new_mem[n] = _b2u(jnp.concatenate([ym, ym], axis=0).astype(BF))
            yb = y.astype(BF)
            store_tokens(abuf, n, h_ld, _b2u(yb))
            cols = pl.ds(128 * n, 128)
            lo, cnt = (XS, 2 * SEG - XS) if odd else (0, XS)
            rows = pl.ds(pl.multiple_of(pair_row + lo, 8), cnt)
            a = yb.astype(F32)
            b = _u2b(xn_t[n, pl.ds(h_ld + 8 * odd, y.shape[0] // 2), :]).astype(F32)
            sl = slice(MEM, MEM + cnt) if odd else slice(0, cnt)
            out_s[rows, cols] = residual(x_s[rows, cols].astype(F32), a[sl], b[sl])

        order = list(range(n_part, KT))
        for n in order:
            finish(n, _dot(lhs_o, _u2b(wo_s[n])))
            if n < KT - 1:
                side_group()
            if n == n_part:
                for n2 in range(n_part):
                    tail = _u2b(wo_s[n2, pl.ds(h_split * 64, (H - h_split) * 64), :])
                    finish(n2, _dot(lhs_b, tail) + acc[n2])
        return new_mem

    def patch_row(t, yrow):
        xr, w = load_row(t)
        bits = pltpu.bitcast(_rbf(xr + yrow), U32)
        w = jnp.where(t % 2 == 0,
                      (w & jnp.uint32(0xFFFF0000)) | (bits >> 16),
                      (w & jnp.uint32(0xFFFF)) | bits)
        for k in range(KT):
            xn_t[k, pl.ds(t // 2, 1), :] = w[:, 128 * k:128 * (k + 1)]

    def fix_copy(j, r0):
        return pltpu.make_async_copy(fix_s.at[j], out_hbm.at[pl.ds(r0, 16), :], sems.at[SEM_FIX + j])

    def body(i, carry):
        mem, y = list(carry[:KT]), list(carry[KT:])

        @pl.when(i == 1)
        def _():
            for cp in ffn_copies:
                cp.wait()
            sel_row = lax.broadcasted_iota(jnp.int32, (8, D), 0)
            xs1, _ = load_row(sel_s[0, 0])
            xs2, _ = load_row(sel_s[1, 0])
            xsel_s[...] = jnp.where(sel_row == 0, xs1, jnp.where(sel_row == 1, xs2, 0.0))

        @pl.when(i == NIT - 1)
        def _():
            idx1 = sel_s[0, 0]
            idx2 = sel_s[1, 0]
            gate = _rbf(jax.nn.sigmoid(gate_s[:, 0:1]))
            yy = _rbf(_rbf(jnp.concatenate(y, axis=1)) * gate)
            patch_row(idx1, yy[0:1])
            patch_row(idx2, yy[1:2])
            top = (S - ROWS) // 16 - 1
            blk1 = jnp.minimum(idx1 // 16, top)
            blk2 = jnp.minimum(idx2 // 16, top)
            blk2 = jnp.where(blk2 == blk1, jnp.where(blk1 == 0, 1, blk1 - 1), blk2)
            r0s = [pl.multiple_of(blk * 16, 16) for blk in (blk1, blk2)]
            for j, r0 in enumerate(r0s):
                for n in range(KT):
                    cols = pl.ds(128 * n, 128)
                    fix_s[j, :, cols] = residual(x_s[pl.ds(r0, 16), cols].astype(F32),
                                                 _u2b(abuf[n, pl.ds(half_rows(r0), 8), :]).astype(F32),
                                                 _u2b(xn_t[n, pl.ds(half_rows(r0), 8), :]).astype(F32))
            for c in range(NIT - 1):
                out_copy(c).wait()
            for j, r0 in enumerate(r0s):
                fix_copy(j, r0).start()

        side = ffn_groups(i, y)
        held = {}
        for u in range(UNROLL):
            mem = one_step(i, u, mem, held, side)
        for _ in side:
            raise AssertionError("ffn groups left over")
        out_copy(i).start()
        return tuple(mem) + tuple(y)

    for n in range(KT):
        wo_copy(n).wait()
    for cp in ffn0_copies:
        cp.wait()
    xsel_s[...] = jnp.zeros(xsel_s.shape, F32)
    mi = mem0_s[...].astype(F32)
    mip = _b2u(jnp.concatenate([mi, mi], axis=0).astype(BF))
    lax.fori_loop(0, NIT, body,
                  tuple(mip[:, 128 * k:128 * (k + 1)] for k in range(KT))
                  + (jnp.zeros((8, 512), F32), jnp.zeros((8, 512), F32)))
    for j in range(2):
        fix_copy(j, 0).wait()
    out_copy(NIT - 1).wait()


@jax.jit
def pallas_parallel_sum__memory_aug_recurrent_mem_tr__moe_arch_mod__prompt_kernel(
    A_x: jax.Array,
    A_mem0: jax.Array,
    A_Wq: jax.Array,
    A_Wk: jax.Array,
    A_Wv: jax.Array,
    A_Wo: jax.Array,
    A_seg_len: jax.Array,
    B_x: jax.Array,
    B_w_r: jax.Array,
    B_w_gate: jax.Array,
    B_w_up: jax.Array,
    B_w_down: jax.Array,
):
    del A_seg_len, B_x
    assert A_x.shape == (1, S, D) and A_mem0.shape == (1, MEM, D)
    assert A_Wq.shape == (D, H, DH) and A_Wo.shape == (H, DH, D)
    assert B_w_gate.shape == (D, FF) and B_w_down.shape == (FF, D)
    any_spec = pl.BlockSpec(memory_space=pl.ANY)
    out = pl.pallas_call(
        _kernel,
        out_shape=jax.ShapeDtypeStruct((S, D), BF),
        in_specs=[any_spec] * 10,
        out_specs=any_spec,
        scratch_shapes=[
            pltpu.VMEM((S, D), BF),
            pltpu.VMEM((KT, S // 2, 128), U32),
            pltpu.VMEM((KT, PRE // 2, 128), U32),
            pltpu.VMEM((KT, 16 * NSEG, 128), U32),
            pltpu.VMEM((3 * H + 2, D // 2, 128), U32),
            pltpu.VMEM((KT, H * DH // 2, 128), U32),
            pltpu.VMEM((3 * H, RING32, 128), U32),
            pltpu.VMEM((KT, S // 2, 128), U32),
            pltpu.VMEM((S, D), BF),
            pltpu.VMEM((NPQ + 1, D, 128), U32),
            pltpu.VMEM((D // 2, FF), U32),
            pltpu.VMEM((D // 2, FF), U32),
            pltpu.VMEM((FF // 2, D), U32),
            pltpu.VMEM((MEM, D), BF),
            pltpu.VMEM((D,), BF),
            pltpu.VMEM((8, D), F32),
            pltpu.VMEM((16, 128), F32),
            pltpu.VMEM((8, 128), jnp.int32),
            pltpu.VMEM((8, 128), F32),
            pltpu.VMEM((8, D), F32),
            pltpu.VMEM((2, 16, D), BF),
            pltpu.SMEM((1,), jnp.int32),
            pltpu.SemaphoreType.DMA((NSEM,)),
        ],
        compiler_params=pltpu.CompilerParams(vmem_limit_bytes=126 * 1024 * 1024),
    )(A_x.reshape(S, D), A_mem0.reshape(MEM, D), A_Wq, A_Wk, A_Wv, A_Wo.reshape(H * DH, D),
      B_w_r, B_w_gate, B_w_up, B_w_down)
    return out.reshape(1, S, D)
```

```python
import jax
import jax.numpy as jnp
from jax import lax
import jax.experimental.pallas as pl
import jax.experimental.pallas.tpu as pltpu

BF = jnp.bfloat16
U32 = jnp.uint32
F32 = jnp.float32

S = 2048
D = 1024
H = 32
DH = 128
MEM = 8
SEG = 32
NSEG = S // SEG
FF = 3584
KT = D // 128
FT = FF // 128
XS = 24
PRE = S - NSEG * XS
RING = 576
RING32 = RING // 2
NPAIR = H // 2
NPQ = 3 * NPAIR
PP = 6
NPRE = NPQ // PP
LNP = 14
NLN = (S - PRE) // 16
SEM_SMALL, SEM_X0, SEM_X = 0, 2, 6
SEM_W0 = SEM_X + NPRE
SEM_W = SEM_W0 + PP
SEM_WO = SEM_W + NPRE
SEM_FFN0, SEM_FFN, SEM_FIX, SEM_OUT = SEM_WO + 1, SEM_WO + 2, SEM_WO + 3, SEM_WO + 5
NSEM = SEM_OUT + 3

LAG_QK = 1
LAG_PV = 4
N_PART = 4
H_SPLIT = 26
REL_SCHED = {0: [(0, 0), (0, 1)], 1: [(0, 2), (0, 3)], 2: [(0, 4)], 3: [(0, 5)], 4: [(0, 6)], 5: [(0, 7)]}
REL_SCHED.update({8 * j - 2 + k: [(j, k)] for j in range(1, PP) for k in range(8)})
N_PART_ODD = 4
H_SPLIT_ODD = 24
K_SPLIT = 2
EPI_SCHED = [v * 5 // 2 for v in range(24)]
EPI_LAG = 4
ECH = 160
REL_SCHED0 = {4: [(0, k) for k in range(4)], 5: [(0, k) for k in range(4, 8)],
              12: [(1, k) for k in range(4)], 13: [(1, k) for k in range(4, 8)],
              24: [(3, 0), (3, 1)], 25: [(3, 2), (3, 3)], 26: [(3, 4)], 27: [(3, 5)], 28: [(3, 6)], 29: [(3, 7)]}
REL_SCHED0.update({8 * j - 2 + k: [(j, k)] for j in (2, 4, 5) for k in range(8)})
BARRIERS0 = {4: [1], 12: [2, 3], 24: [4, 5, 6]}
SCORE_SCHED = [1, 10, 19, 28, 37]
LN_SCHED = [3 * q for q in range(LNP)]
FIRST_BATCH = 6
LN_LAG = 5
FFN_DELAY = 2
REL_LAG = 2
UNROLL = 4


def _b2u(x):
    return pltpu.bitcast(x, U32)


def _u2b(x):
    return pltpu.bitcast(x, BF)


def _dot(a, b):
    return jnp.dot(a, b, preferred_element_type=F32)


def _dot_nt(a, b):
    return lax.dot_general(a, b, (((1,), (1,)), ((), ())), preferred_element_type=F32)


def _after(w, dep, zero):
    if not dep:
        return w
    d = dep[0]
    for e in dep[1:]:
        d = d | e
    return jnp.concatenate([w[0:8] | (d & zero), w[8:]], axis=0)


def _rbf(x):
    return x.astype(BF).astype(F32)


def _kernel(x_hbm, mem0_hbm, wq_hbm, wk_hbm, wv_hbm, wo_hbm, wr_hbm, wg_hbm, wu_hbm, wd_hbm,
            out_hbm,
            x_s, xn_t, xn_pre, hbuf, wqkv, wo_s, ring, abuf, out_s, raw,
            wg_s, wu_s, wd_s, mem0_s, wr_s, wrf_s, r_s, sel_s, gate_s, xsel_s, yy_s, zero_s, idx_s,
            sems):
    w32 = [w.bitcast(U32) for w in (wq_hbm, wk_hbm, wv_hbm)]
    wo32 = wo_hbm.bitcast(U32)
    wg32 = wg_hbm.bitcast(U32)
    wu32 = wu_hbm.bitcast(U32)
    wd32 = wd_hbm.bitcast(U32)

    def rows_copy(r0, n, sem):
        return pltpu.make_async_copy(x_hbm.at[pl.ds(r0, n), :], x_s.at[pl.ds(r0, n), :], sems.at[sem])

    def x_first(c):
        return rows_copy(128 * c if isinstance(c, int) else pl.multiple_of(128 * c, 128), 128, SEM_X0 + c)

    def x_piece(t, last):
        r0 = PRE + 16 * LNP * (t - 1)
        n = S - PRE - 16 * LNP * (NPRE - 2) if last else 16 * LNP
        return rows_copy(r0 if isinstance(t, int) else pl.multiple_of(r0, 32), n, SEM_X + t)

    def pair_copy(p):
        q = min(p, NPQ - 1)
        sem = SEM_W0 + p if p <= PP else SEM_W + (p - 1) // PP
        return pltpu.make_async_copy(w32[q // NPAIR].at[:, q % NPAIR, :], raw.at[p], sems.at[sem])

    def pairs_wait(t):
        dst = raw.at[pl.ds(PP * t + 1, PP)]
        pltpu.make_async_copy(dst, dst, sems.at[SEM_W + t]).wait()

    def wo_copy(n):
        return pltpu.make_async_copy(wo32.at[:, pl.ds(128 * n, 128)], wo_s.at[n], sems.at[SEM_WO])

    small_copies = [pltpu.make_async_copy(mem0_hbm, mem0_s, sems.at[SEM_SMALL]),
                    pltpu.make_async_copy(wr_hbm, wr_s, sems.at[SEM_SMALL + 1])]
    ffn0_copies = [
        pltpu.make_async_copy(wg32.at[:, pl.ds(0, 128)], wg_s.at[:, pl.ds(0, 128)], sems.at[SEM_FFN0]),
        pltpu.make_async_copy(wu32.at[:, pl.ds(0, 128)], wu_s.at[:, pl.ds(0, 128)], sems.at[SEM_FFN0]),
        pltpu.make_async_copy(wd32.at[pl.ds(0, 64), :], wd_s.at[pl.ds(0, 64), :], sems.at[SEM_FFN0])]
    ffn_copies = [
        pltpu.make_async_copy(wg32.at[:, pl.ds(128, FF - 128)], wg_s.at[:, pl.ds(128, FF - 128)], sems.at[SEM_FFN]),
        pltpu.make_async_copy(wu32.at[:, pl.ds(128, FF - 128)], wu_s.at[:, pl.ds(128, FF - 128)], sems.at[SEM_FFN]),
        pltpu.make_async_copy(wd32.at[pl.ds(64, FF // 2 - 64), :], wd_s.at[pl.ds(64, FF // 2 - 64), :],
                              sems.at[SEM_FFN])]

    zero_s[0] = 0
    for c in range(4):
        x_first(c).start()
        if c == 0:
            for cp in small_copies:
                cp.start()

    def queue(t0, t1):
        for t in range(t0, t1):
            for p in range(PP * t + 1, PP * t + PP + 1):
                pair_copy(p).start()
            if t >= 1:
                x_piece(t, t == NPRE - 1).start()

    pair_copy(0).start()
    queue(0, FIRST_BATCH)
    eps_bf = 1.0013580322265625e-05

    def score16(g, xn):
        wr = jnp.concatenate([wrf_s[...], wrf_s[...]], axis=0)
        score = _rbf(jnp.sum(xn.astype(F32) * wr, axis=1, keepdims=True))
        r_s[...] = jnp.where(lane16 == g, score, r_s[...])

    def layernorm16(rq, dst_ref, dst_row, not_before=None):
        rq = rq if isinstance(rq, int) else pl.multiple_of(rq, 16)
        xf = x_s[pl.ds(rq, 16), :].astype(F32)
        if not_before is not None:
            x0 = _after(pltpu.bitcast(xf[:, 0:128], U32), [not_before], zero_box[0])
            xf = jnp.concatenate([pltpu.bitcast(x0, F32), xf[:, 128:]], axis=1)
        mean = jnp.sum(xf, axis=1, keepdims=True) * (1.0 / D)
        cen = xf - mean
        var = jnp.sum(cen * cen, axis=1, keepdims=True) * (1.0 / D)
        sd = _rbf(jnp.sqrt(_rbf(_rbf(var) + eps_bf)))
        xn = (_rbf(xf - _rbf(mean)) * (1.0 / sd)).astype(BF)
        if dst_ref is hbuf:
            score16(rq // 16, xn)
        xp = _b2u(xn)
        hq = rq // 2 if isinstance(rq, int) else pl.multiple_of(rq // 2, 8)
        dst_row = dst_row if isinstance(dst_row, int) else pl.multiple_of(dst_row, 8)
        for k in range(KT):
            xn_t[k, pl.ds(hq, 8), :] = xp[:, 128 * k:128 * (k + 1)]
            dst_ref[k, pl.ds(dst_row, 8), :] = xp[:, 128 * k:128 * (k + 1)]

    zero_box = [None]

    def fresh_zero():
        zero_box[0] = jnp.full((8, 128), zero_s[0], jnp.int32).astype(U32)

    r_s[...] = jnp.full(r_s.shape, -jnp.inf, F32)
    lane16 = lax.broadcasted_iota(jnp.int32, (16, 128), 1)

    def ln_body(c, carry):
        x_first(c).wait()
        for q in range(8):
            layernorm16(128 * c + 16 * q, xn_pre, 64 * c + 8 * q)
        return carry

    lax.fori_loop(0, PRE // 128, ln_body, 0)


    def relayout(src, dst, j, k, not_before=None):
        a = src[j, pl.ds(128 * k, 64, stride=2), :]
        if not_before is not None:
            a = a | jnp.concatenate([not_before & zero_box[0]] * 8, axis=0)
        b = src[j, pl.ds(128 * k + 1, 64, stride=2), :]
        rows = pl.ds(64 * k, 64)
        dst[2 * j, rows, :] = (a & jnp.uint32(0xFFFF)) | (b << 16)
        dst[2 * j + 1, rows, :] = (a >> 16) | (b & jnp.uint32(0xFFFF0000))

    def pre_dot(w_view, ring_view, j, k, dep=None):
        i, q = k // 4, k % 4
        lhs = jnp.concatenate([_u2b(xn_pre[kk, pl.ds(64 * q, 64), :]) for kk in range(KT)], axis=1)
        y = _dot(lhs, _u2b(_after(w_view[2 * j + i], dep, zero_box[0])))
        yp = _b2u(y.astype(BF))
        ring_view[2 * j + i, pl.ds(32 + 64 * q, 64), :] = yp
        return yp[0:8]

    for c in small_copies:
        c.wait()
    pair_copy(0).wait()
    for k in range(8):
        relayout(raw, wqkv, 0, k)
    wrf_s[...] = jnp.broadcast_to(wr_s[...].astype(F32).reshape(1, D), (8, D))

    def second_batch():
        queue(FIRST_BATCH, NPRE)
        for n in range(KT):
            wo_copy(n).start()
        for cp in ffn0_copies + ffn_copies:
            cp.start()

    def pre_iter(t, first):
        deps = {}
        raw_view = raw.at[pl.ds(PP * t, PP + 1)]
        w_view = wqkv.at[pl.ds(2 * PP * t, 2 * PP + 2)]
        ring_view = ring.at[pl.ds(2 * PP * t, 2 * PP)]
        done = None
        for v in range(8 * PP):
            j, k = v // 8, v % 8
            if v == 0 or (first and v in BARRIERS0):
                if v:
                    for p in BARRIERS0[v]:
                        pair_copy(p).wait()
                    if v == max(BARRIERS0):
                        second_batch()
                fresh_zero()
                done = None
            prev = done
            done = pre_dot(w_view, ring_view, j, k, deps.get(v))
            for jr, kr in (REL_SCHED0 if first else REL_SCHED).get(v, ()):
                relayout(raw_view, w_view, jr + 1, kr, prev)
                deps.setdefault(v + REL_LAG, []).append(w_view[2 * jr + 3, pl.ds(64 * kr + 56, 8), :])
            if first:
                continue
            if v in LN_SCHED:
                q = jnp.minimum(LNP * (t - 1) + LN_SCHED.index(v), NLN - 1)
                hrow = pl.multiple_of(32 * (q // 3) + 8 * (q % 3), 8)
                layernorm16(PRE + 16 * q, hbuf, hrow, done if prev is not None else None)
                deps.setdefault(v + LN_LAG, []).append(hbuf[KT - 1, pl.ds(hrow, 8), :])
            if v in SCORE_SCHED:
                g = jnp.minimum(len(SCORE_SCHED) * (t - 1) + SCORE_SCHED.index(v), PRE // 16 - 1)
                rows = pl.ds(pl.multiple_of(8 * g, 8), 8)
                xp = [xn_pre[kk, rows, :] for kk in range(KT)]
                xp[0] = xp[0] | (done & zero_box[0])
                score16(g, _u2b(jnp.concatenate(xp, axis=1)))

    pre_iter(0, True)

    def pre_body(t, carry):
        pairs_wait(t)

        @pl.when(t < NPRE - 1)
        def _():
            x_piece(t, False).wait()

        @pl.when(t == NPRE - 1)
        def _():
            x_piece(NPRE - 1, True).wait()
        pre_iter(t, False)
        return carry

    lax.fori_loop(1, NPRE, pre_body, 0)
    row = lax.broadcasted_iota(jnp.int32, (80, 80), 0)
    col = lax.broadcasted_iota(jnp.int32, (80, 80), 1)
    same_head = (jnp.where(row < 64, row >> 5, (row - 64) >> 3)
                 == jnp.where(col < 64, col >> 5, (col - 64) >> 3))
    allowed = same_head & ((col >= 64) | (row >= 64) | (col <= row))
    fill = jnp.where(same_head, -1e9, -jnp.inf).astype(F32)
    low_half = lax.broadcasted_iota(jnp.int32, (8, 128), 0) < 4
    high_half = jnp.logical_not(low_half)
    scale = DH ** -0.5

    def load_row(t):
        w = jnp.concatenate([xn_t[k, pl.ds(t // 2, 1), :] for k in range(KT)], axis=1)
        bits = jnp.where(t % 2 == 0, w << 16, w & jnp.uint32(0xFFFF0000))
        return pltpu.bitcast(bits, F32), w

    def select_tokens():
        r = r_s[...]
        tok = lane16 * 16 + lax.broadcasted_iota(jnp.int32, (16, 128), 0)

        def full(op, v):
            return op(op(v, axis=0, keepdims=True), axis=1, keepdims=True)

        top1 = full(jnp.max, r)
        idx1 = full(jnp.min, jnp.where(r == top1, tok, S - 1))
        r2 = jnp.where(tok == idx1, -jnp.inf, r)
        top2 = full(jnp.max, r2)
        idx2 = full(jnp.min, jnp.where((r2 == top2) & (tok != idx1), tok, S - 1))
        first = lax.broadcasted_iota(jnp.int32, (8, 128), 0) == 0
        gate_s[...] = jnp.where(first, top1, top2)
        sel_s[...] = jnp.where(first, idx1, idx2)

    NIT = NSEG // UNROLL
    ROWS = SEG * UNROLL

    def half_rows(r0):
        return pl.multiple_of(r0 // 2, 8)

    def residual(xf, a, b):
        return (_rbf(xf + a) + b).astype(BF)

    def out_copy(j):
        r0, n = (0, S - 2 * ROWS) if j == 0 else (S - (3 - j) * ROWS, ROWS)
        return pltpu.make_async_copy(out_s.at[pl.ds(r0, n), :], out_hbm.at[pl.ds(r0, n), :],
                                     sems.at[SEM_OUT + j])

    def ffn_groups(i, y):
        x_sel = xsel_s[...]
        live = (i >= 1) & (i < NIT - 1)
        hid = {}

        def up(w_ref, j, key):
            cols = pl.ds(pl.multiple_of(128 * j, 128), 128)
            part = _dot(x_sel[:, 0:512], _u2b(w_ref[pl.ds(0, 256), cols]).astype(F32))
            yield
            hid[key] = _rbf(_dot(x_sel[:, 512:1024], _u2b(w_ref[pl.ds(256, 256), cols]).astype(F32)) + part)
            yield

        for jj in range(2):
            j = jnp.clip(2 * (i - 1) + jj, 0, FT - 1)
            yield from up(wg_s, j, "g")
            yield from up(wu_s, j, "u")
            g = hid["g"]
            hb = jnp.where(live, _rbf(_rbf(g * _rbf(jax.nn.sigmoid(g))) * hid["u"]), 0.0)
            rows = pl.ds(pl.multiple_of(64 * j, 64), 64)
            yield
            for half in range(2):
                y[half] = _dot(hb, _u2b(wd_s[rows, pl.ds(512 * half, 512)]).astype(F32)) + y[half]
                yield

    def one_step(i, u, mem, held, side):
        odd = u % 2
        s2 = i * (UNROLL // 2) + u // 2
        h_ld = pl.multiple_of(16 * UNROLL * i, 32) + 32 * (u // 2)
        r24 = pl.multiple_of((12 * UNROLL * i) % RING32, 8) + XS * (u // 2)
        qkv_ld = pl.multiple_of((SEG * s2 + 32) % RING32, 32) + 16 * odd
        m0 = 0 if odd else XS

        def with_mem(lo, hi, m):
            if odd:
                return [jnp.where(low_half, m, lo), hi]
            return [lo, jnp.where(low_half, hi, m)]

        def store_tokens(ref, idx, base, yp):
            if odd:
                pltpu.store(ref.at[idx, pl.ds(base + 8, 8), :], yp[0:8], mask=high_half)
                ref[idx, pl.ds(base + 16, yp.shape[0] - 8), :] = yp[8:]
            else:
                ref[idx, pl.ds(base, 8), :] = yp[0:8]
                pltpu.store(ref.at[idx, pl.ds(base + 8, 8), :], yp[8:16], mask=low_half)

        lk = [_u2b(jnp.concatenate(with_mem(hbuf[k, pl.ds(h_ld + 8 * odd, 8), :],
                                            hbuf[k, pl.ds(h_ld + 8 + 8 * odd, 8), :], mem[k]), axis=0))
              for k in range(KT)]
        lhs = jnp.concatenate(lk, axis=1)

        ymem = {}
        xs = {}
        probs = {}
        parts = {}

        def proj(h):
            split = h < K_SPLIT and u > 0
            if split:
                lhs7 = jnp.concatenate(lk[:KT - 1], axis=1)
                head = [_dot(lhs7, _u2b(wqkv[m * H + h, pl.ds(0, 448), :])) for m in range(3)]
            for m in range(3):
                if split:
                    y = _dot(lk[KT - 1], _u2b(wqkv[m * H + h, pl.ds(448, 64), :])) + head[m]
                else:
                    y = _dot(lhs, _u2b(wqkv[m * H + h]))
                store_tokens(ring, m * H + h, r24, _b2u(y.astype(BF)))
                ymem[(h, m)] = y[m0:m0 + MEM]
                xs[(h, m)] = ring[m * H + h, pl.ds(qkv_ld, SEG // 2), :]

        def pair(p, m):
            a, b = 2 * p, 2 * p + 1
            mm = jnp.concatenate([ymem[(a, m)], ymem[(b, m)]], axis=0).astype(BF)
            return jnp.concatenate([_u2b(xs[(a, m)]), _u2b(xs[(b, m)]), mm], axis=0)

        def qk(p):
            sc = _dot_nt(pair(p, 0), pair(p, 1))
            sc = jnp.where(allowed, sc * scale, fill)
            e = jnp.exp(sc - jnp.max(sc, axis=1, keepdims=True))
            l = jnp.sum(e, axis=1, keepdims=True)
            r = pl.reciprocal(l, approx=True)
            r = r * (2.0 - l * r)
            probs[p] = (e * r).astype(BF)

        def pv(p):
            op = _b2u(_dot(probs[p], pair(p, 2)).astype(BF))
            om = op[32:40]
            om_sw = pltpu.roll(om, 4, axis=0)
            for j, h in enumerate((2 * p, 2 * p + 1)):
                x0, x1 = op[16 * j:16 * j + 8], op[16 * j + 8:16 * j + 16]
                m = om if j != odd else om_sw
                if odd:
                    rows = with_mem(held[h], x0, m) + [x1]
                else:
                    rows = with_mem(x0, x1, m)
                    held[h] = x1
                parts[h] = _u2b(jnp.concatenate(rows, axis=0))

        def after(t):
            for lag, fn in ((LAG_QK, qk), (LAG_PV, pv)):
                if (t - 1 - lag) % 2 == 0 and 0 <= (t - 1 - lag) // 2 < NPAIR:
                    fn((t - 1 - lag) // 2)

        def side_group():
            if odd:
                next(side, None)

        for t in range(H):
            proj(t)
            after(t)
            if u == 0 and t == 8:
                select_tokens()
        t = H
        n_part, h_split = (N_PART_ODD, H_SPLIT_ODD) if odd else (N_PART, H_SPLIT)
        lhs_a = jnp.concatenate([parts[j] for j in range(h_split)], axis=1)
        acc = []
        for n in range(n_part):
            acc.append(_dot(lhs_a, _u2b(wo_s[n, pl.ds(0, h_split * 64), :])))
            after(t)
            side_group()
            t += 1
        while t - 1 - LAG_PV <= 2 * (NPAIR - 1):
            after(t)
            t += 1
        lhs_b = jnp.concatenate([parts[j] for j in range(h_split, H)], axis=1)
        lhs_o = jnp.concatenate([lhs_a, lhs_b], axis=1)
        new_mem = [None] * KT
        pair_row = pl.multiple_of(ROWS * i, 64) + 64 * (u // 2)

        def finish(n, y):
            ym = y[m0:m0 + MEM]
            new_mem[n] = _b2u(jnp.concatenate([ym, ym], axis=0).astype(BF))
            yb = y.astype(BF)
            store_tokens(abuf, n, h_ld, _b2u(yb))
            cols = pl.ds(128 * n, 128)
            lo, cnt = (XS, 2 * SEG - XS) if odd else (0, XS)
            rows = pl.ds(pl.multiple_of(pair_row + lo, 8), cnt)
            a = yb.astype(F32)
            b = _u2b(xn_t[n, pl.ds(h_ld + 8 * odd, y.shape[0] // 2), :]).astype(F32)
            sl = slice(MEM, MEM + cnt) if odd else slice(0, cnt)
            out_s[rows, cols] = residual(x_s[rows, cols].astype(F32), a[sl], b[sl])

        order = list(range(n_part, KT))
        for n in order:
            finish(n, _dot(lhs_o, _u2b(wo_s[n])))
            if n < KT - 1:
                side_group()
            if n == n_part:
                for n2 in range(n_part):
                    tail = _u2b(wo_s[n2, pl.ds(h_split * 64, (H - h_split) * 64), :])
                    finish(n2, _dot(lhs_b, tail) + acc[n2])
        return new_mem

    def patch_row(t, yrow):
        xr, w = load_row(t)
        bits = pltpu.bitcast(_rbf(xr + yrow), U32)
        w = jnp.where(t % 2 == 0,
                      (w & jnp.uint32(0xFFFF0000)) | (bits >> 16),
                      (w & jnp.uint32(0xFFFF)) | bits)
        for k in range(KT):
            xn_t[k, pl.ds(t // 2, 1), :] = w[:, 128 * k:128 * (k + 1)]

    def fix_copy(j, r0):
        return pltpu.make_async_copy(out_s.at[pl.ds(r0, 16), :], out_hbm.at[pl.ds(r0, 16), :],
                                     sems.at[SEM_FIX + j])

    def gather_tokens():
        for cp in ffn_copies:
            cp.wait()
        idx_s[0] = sel_s[0, 0]
        idx_s[1] = sel_s[1, 0]
        sel_row = lax.broadcasted_iota(jnp.int32, (8, D), 0)
        xs1, _ = load_row(idx_s[0])
        xs2, _ = load_row(idx_s[1])
        xsel_s[...] = jnp.where(sel_row == 0, xs1, jnp.where(sel_row == 1, xs2, 0.0))

    def apply_ffn():
        out_copy(0).wait()
        patch_row(idx_s[0], yy_s[0:1, :])
        patch_row(idx_s[1], yy_s[1:2, :])
        blks = [idx_s[j] >> 4 for j in range(2)]
        for blk in blks:
            r0 = pl.multiple_of(jnp.minimum(blk, (S - ROWS) // 16 - 1) * 16, 16)
            for n in range(KT):
                cols = pl.ds(128 * n, 128)
                out_s[pl.ds(r0, 16), cols] = residual(
                    x_s[pl.ds(r0, 16), cols].astype(F32),
                    _u2b(abuf[n, pl.ds(half_rows(r0), 8), :]).astype(F32),
                    _u2b(xn_t[n, pl.ds(half_rows(r0), 8), :]).astype(F32))
        blk1, blk2 = [jnp.minimum(blk, (S - 2 * ROWS) // 16 - 1) for blk in blks]
        blk2 = jnp.where(blk2 == blk1, jnp.where(blk1 == 0, 1, blk1 - 1), blk2)
        for j, blk in enumerate((blk1, blk2)):
            fix_copy(j, pl.multiple_of(blk * 16, 16)).start()
        out_copy(1).start()

    def body(i, carry):
        mem, y = list(carry[:KT]), list(carry[KT:])

        @pl.when((i == 1) | (i >= NIT - 2))
        def _():
            pl.when(i == 1)(gather_tokens)
            pl.when(i == NIT - 2)(lambda: out_copy(0).start())
            pl.when(i == NIT - 1)(apply_ffn)

        side = ffn_groups(i, y)
        held = {}
        for u in range(UNROLL):
            mem = one_step(i, u, mem, held, side)
        for _ in side:
            raise AssertionError("ffn groups left over")
        gate = _rbf(jax.nn.sigmoid(gate_s[:, 0:1]))
        yy_s[...] = _rbf(_rbf(jnp.concatenate(y, axis=1)) * gate)
        return tuple(mem) + tuple(y)

    for n in range(KT):
        wo_copy(n).wait()
    for cp in ffn0_copies:
        cp.wait()
    xsel_s[...] = jnp.zeros(xsel_s.shape, F32)
    mi = mem0_s[...].astype(F32)
    mip = _b2u(jnp.concatenate([mi, mi], axis=0).astype(BF))
    lax.fori_loop(0, NIT, body,
                  tuple(mip[:, 128 * k:128 * (k + 1)] for k in range(KT))
                  + (jnp.zeros((8, 512), F32), jnp.zeros((8, 512), F32)))
    out_copy(2).start()
    for j in range(2):
        fix_copy(j, 0).wait()
    out_copy(1).wait()
    out_copy(2).wait()


@jax.jit
def pallas_parallel_sum__memory_aug_recurrent_mem_tr__moe_arch_mod__prompt_kernel(
    A_x: jax.Array,
    A_mem0: jax.Array,
    A_Wq: jax.Array,
    A_Wk: jax.Array,
    A_Wv: jax.Array,
    A_Wo: jax.Array,
    A_seg_len: jax.Array,
    B_x: jax.Array,
    B_w_r: jax.Array,
    B_w_gate: jax.Array,
    B_w_up: jax.Array,
    B_w_down: jax.Array,
):
    del A_seg_len, B_x
    assert A_x.shape == (1, S, D) and A_mem0.shape == (1, MEM, D)
    assert A_Wq.shape == (D, H, DH) and A_Wo.shape == (H, DH, D)
    assert B_w_gate.shape == (D, FF) and B_w_down.shape == (FF, D)
    any_spec = pl.BlockSpec(memory_space=pl.ANY)
    out = pl.pallas_call(
        _kernel,
        out_shape=jax.ShapeDtypeStruct((S, D), BF),
        in_specs=[any_spec] * 10,
        out_specs=any_spec,
        scratch_shapes=[
            pltpu.VMEM((S, D), BF),
            pltpu.VMEM((KT, S // 2, 128), U32),
            pltpu.VMEM((KT, PRE // 2, 128), U32),
            pltpu.VMEM((KT, 16 * NSEG, 128), U32),
            pltpu.VMEM((3 * H + 2, D // 2, 128), U32),
            pltpu.VMEM((KT, H * DH // 2, 128), U32),
            pltpu.VMEM((3 * H, RING32, 128), U32),
            pltpu.VMEM((KT, S // 2, 128), U32),
            pltpu.VMEM((S, D), BF),
            pltpu.VMEM((NPQ + 1, D, 128), U32),
            pltpu.VMEM((D // 2, FF), U32),
            pltpu.VMEM((D // 2, FF), U32),
            pltpu.VMEM((FF // 2, D), U32),
            pltpu.VMEM((MEM, D), BF),
            pltpu.VMEM((D,), BF),
            pltpu.VMEM((8, D), F32),
            pltpu.VMEM((16, 128), F32),
            pltpu.VMEM((8, 128), jnp.int32),
            pltpu.VMEM((8, 128), F32),
            pltpu.VMEM((8, D), F32),
            pltpu.VMEM((8, D), F32),
            pltpu.SMEM((1,), jnp.int32),
            pltpu.SMEM((2,), jnp.int32),
            pltpu.SemaphoreType.DMA((NSEM,)),
        ],
        compiler_params=pltpu.CompilerParams(vmem_limit_bytes=126 * 1024 * 1024,
                                             disable_bounds_checks=True, disable_semaphore_checks=True),
    )(A_x.reshape(S, D), A_mem0.reshape(MEM, D), A_Wq, A_Wk, A_Wv, A_Wo.reshape(H * DH, D),
      B_w_r, B_w_gate, B_w_up, B_w_down)
    return out.reshape(1, S, D)
```

```python
import jax
import jax.numpy as jnp
from jax import lax
import jax.experimental.pallas as pl
import jax.experimental.pallas.tpu as pltpu

BF = jnp.bfloat16
U32 = jnp.uint32
F32 = jnp.float32

S = 2048
D = 1024
H = 32
DH = 128
MEM = 8
SEG = 32
NSEG = S // SEG
FF = 3584
KT = D // 128
FT = FF // 128
XS = 24
PRE = S - NSEG * XS
RING = 576
RING32 = RING // 2
NPAIR = H // 2
NPQ = 3 * NPAIR
PP = 6
NPRE = NPQ // PP
LNP = 16
SEM_SMALL, SEM_X0, SEM_X = 0, 2, 6
SEM_W0 = SEM_X + NPRE
SEM_W = SEM_W0 + PP
SEM_WO = SEM_W + NPRE
SEM_FFN0, SEM_FFN, SEM_FIX, SEM_OUT = SEM_WO + 1, SEM_WO + 2, SEM_WO + 3, SEM_WO + 5
NSEM = SEM_OUT + 3

LAG_QK = 1
LAG_PV = 4
N_PART = 4
H_SPLIT = 26
REL_SCHED = {0: [(0, 0), (0, 1)], 1: [(0, 2), (0, 3)], 2: [(0, 4)], 3: [(0, 5)], 4: [(0, 6)], 5: [(0, 7)]}
REL_SCHED.update({8 * j - 2 + k: [(j, k)] for j in range(1, PP) for k in range(8)})
N_PART_ODD = 4
H_SPLIT_ODD = 24
K_SPLIT = 2
EPI_SCHED = [v * 5 // 2 for v in range(24)]
EPI_LAG = 4
ECH = 160
REL_SCHED0 = {4: [(0, k) for k in range(4)], 5: [(0, k) for k in range(4, 8)],
              12: [(1, k) for k in range(4)], 13: [(1, k) for k in range(4, 8)],
              24: [(3, 0), (3, 1)], 25: [(3, 2), (3, 3)], 26: [(3, 4)], 27: [(3, 5)], 28: [(3, 6)], 29: [(3, 7)]}
REL_SCHED0.update({8 * j - 2 + k: [(j, k)] for j in (2, 4, 5) for k in range(8)})
BARRIERS0 = {4: [1], 12: [2, 3], 24: [4, 5, 6]}
SCORE_SCHED = [1, 16, 31]
LN_SCHED = [11 * q // 4 for q in range(LNP)]
FIRST_BATCH = 6
LN_LAG = 5
FFN_DELAY = 2
REL_LAG = 2
UNROLL = 4


def _b2u(x):
    return pltpu.bitcast(x, U32)


def _u2b(x):
    return pltpu.bitcast(x, BF)


def _dot(a, b):
    return jnp.dot(a, b, preferred_element_type=F32)


def _dot_nt(a, b):
    return lax.dot_general(a, b, (((1,), (1,)), ((), ())), preferred_element_type=F32)


def _after(w, dep, zero):
    if not dep:
        return w
    d = dep[0]
    for e in dep[1:]:
        d = d | e
    return jnp.concatenate([w[0:8] | (d & zero), w[8:]], axis=0)


def _rbf(x):
    return x.astype(BF).astype(F32)


def _kernel(x_hbm, mem0_hbm, wq_hbm, wk_hbm, wv_hbm, wo_hbm, wr_hbm, wg_hbm, wu_hbm, wd_hbm,
            out_hbm,
            x_s, xn_t, xn_pre, hbuf, wqkv, wo_s, ring, abuf, out_s, raw,
            wg_s, wu_s, wd_s, mem0_s, wr_s, wrf_s, r_s, sel_s, gate_s, xsel_s, yy_s, zero_s, idx_s,
            sems):
    w32 = [w.bitcast(U32) for w in (wq_hbm, wk_hbm, wv_hbm)]
    wo32 = wo_hbm.bitcast(U32)
    wg32 = wg_hbm.bitcast(U32)
    wu32 = wu_hbm.bitcast(U32)
    wd32 = wd_hbm.bitcast(U32)

    def rows_copy(r0, n, sem):
        return pltpu.make_async_copy(x_hbm.at[pl.ds(r0, n), :], x_s.at[pl.ds(r0, n), :], sems.at[sem])

    def x_first(c):
        return rows_copy(128 * c if isinstance(c, int) else pl.multiple_of(128 * c, 128), 128, SEM_X0 + c)

    def x_piece(t):
        r0 = PRE + 16 * LNP * (t - 2)
        return rows_copy(r0 if isinstance(t, int) else pl.multiple_of(r0, 256), 16 * LNP, SEM_X + t)

    def pair_copy(p):
        q = min(p, NPQ - 1)
        sem = SEM_W0 + p if p <= PP else SEM_W + (p - 1) // PP
        return pltpu.make_async_copy(w32[q // NPAIR].at[:, q % NPAIR, :], raw.at[p], sems.at[sem])

    def pairs_wait(t):
        dst = raw.at[pl.ds(PP * t + 1, PP)]
        pltpu.make_async_copy(dst, dst, sems.at[SEM_W + t]).wait()

    def wo_copy(n):
        return pltpu.make_async_copy(wo32.at[:, pl.ds(128 * n, 128)], wo_s.at[n], sems.at[SEM_WO])

    small_copies = [pltpu.make_async_copy(mem0_hbm, mem0_s, sems.at[SEM_SMALL]),
                    pltpu.make_async_copy(wr_hbm, wr_s, sems.at[SEM_SMALL + 1])]
    ffn0_copies = [
        pltpu.make_async_copy(wg32.at[:, pl.ds(0, 128)], wg_s.at[:, pl.ds(0, 128)], sems.at[SEM_FFN0]),
        pltpu.make_async_copy(wu32.at[:, pl.ds(0, 128)], wu_s.at[:, pl.ds(0, 128)], sems.at[SEM_FFN0]),
        pltpu.make_async_copy(wd32.at[pl.ds(0, 64), :], wd_s.at[pl.ds(0, 64), :], sems.at[SEM_FFN0])]
    ffn_copies = [
        pltpu.make_async_copy(wg32.at[:, pl.ds(128, FF - 128)], wg_s.at[:, pl.ds(128, FF - 128)], sems.at[SEM_FFN]),
        pltpu.make_async_copy(wu32.at[:, pl.ds(128, FF - 128)], wu_s.at[:, pl.ds(128, FF - 128)], sems.at[SEM_FFN]),
        pltpu.make_async_copy(wd32.at[pl.ds(64, FF // 2 - 64), :], wd_s.at[pl.ds(64, FF // 2 - 64), :],
                              sems.at[SEM_FFN])]

    zero_s[0] = 0
    for c in range(4):
        x_first(c).start()
        if c == 0:
            for cp in small_copies:
                cp.start()

    def queue(t0, t1):
        for t in range(t0, t1):
            for p in range(PP * t + 1, PP * t + PP + 1):
                pair_copy(p).start()
            if t >= 2:
                x_piece(t).start()

    pair_copy(0).start()
    queue(0, FIRST_BATCH)
    eps_bf = 1.0013580322265625e-05

    def score16(g, xn):
        wr = jnp.concatenate([wrf_s[...], wrf_s[...]], axis=0)
        score = _rbf(jnp.sum(xn.astype(F32) * wr, axis=1, keepdims=True))
        r_s[...] = jnp.where(lane16 == g, score, r_s[...])

    def layernorm16(rq, dst_ref, dst_row, not_before=None):
        rq = rq if isinstance(rq, int) else pl.multiple_of(rq, 16)
        xf = x_s[pl.ds(rq, 16), :].astype(F32)
        if not_before is not None:
            x0 = _after(pltpu.bitcast(xf[:, 0:128], U32), [not_before], zero_box[0])
            xf = jnp.concatenate([pltpu.bitcast(x0, F32), xf[:, 128:]], axis=1)
        mean = jnp.sum(xf, axis=1, keepdims=True) * (1.0 / D)
        cen = xf - mean
        var = jnp.sum(cen * cen, axis=1, keepdims=True) * (1.0 / D)
        sd = _rbf(jnp.sqrt(_rbf(_rbf(var) + eps_bf)))
        xn = (_rbf(xf - _rbf(mean)) * (1.0 / sd)).astype(BF)
        if dst_ref is hbuf:
            score16(rq // 16, xn)
        xp = _b2u(xn)
        hq = rq // 2 if isinstance(rq, int) else pl.multiple_of(rq // 2, 8)
        dst_row = dst_row if isinstance(dst_row, int) else pl.multiple_of(dst_row, 8)
        for k in range(KT):
            xn_t[k, pl.ds(hq, 8), :] = xp[:, 128 * k:128 * (k + 1)]
            dst_ref[k, pl.ds(dst_row, 8), :] = xp[:, 128 * k:128 * (k + 1)]

    zero_box = [None]

    def fresh_zero():
        zero_box[0] = jnp.full((8, 128), zero_s[0], jnp.int32).astype(U32)

    r_s[...] = jnp.full(r_s.shape, -jnp.inf, F32)
    lane16 = lax.broadcasted_iota(jnp.int32, (16, 128), 1)

    def ln_body(c, carry):
        x_first(c).wait()
        for q in range(8):
            layernorm16(128 * c + 16 * q, xn_pre, 64 * c + 8 * q)
        return carry

    lax.fori_loop(0, PRE // 128, ln_body, 0)


    def relayout(src, dst, j, k, not_before=None):
        a = src[j, pl.ds(128 * k, 64, stride=2), :]
        if not_before is not None:
            a = a | jnp.concatenate([not_before & zero_box[0]] * 8, axis=0)
        b = src[j, pl.ds(128 * k + 1, 64, stride=2), :]
        rows = pl.ds(64 * k, 64)
        dst[2 * j, rows, :] = (a & jnp.uint32(0xFFFF)) | (b << 16)
        dst[2 * j + 1, rows, :] = (a >> 16) | (b & jnp.uint32(0xFFFF0000))

    def pre_dot(w_view, ring_view, j, k, dep=None):
        i, q = k // 4, k % 4
        lhs = jnp.concatenate([_u2b(xn_pre[kk, pl.ds(64 * q, 64), :]) for kk in range(KT)], axis=1)
        y = _dot(lhs, _u2b(_after(w_view[2 * j + i], dep, zero_box[0])))
        yp = _b2u(y.astype(BF))
        ring_view[2 * j + i, pl.ds(32 + 64 * q, 64), :] = yp
        return yp[0:8]

    for c in small_copies:
        c.wait()
    pair_copy(0).wait()
    for k in range(8):
        relayout(raw, wqkv, 0, k)
    wrf_s[...] = jnp.broadcast_to(wr_s[...].astype(F32).reshape(1, D), (8, D))

    def second_batch():
        queue(FIRST_BATCH, NPRE)
        for n in range(KT):
            wo_copy(n).start()
        for cp in ffn0_copies + ffn_copies:
            cp.start()

    def pre_iter(t, first):
        deps = {}
        raw_view = raw.at[pl.ds(PP * t, PP + 1)]
        w_view = wqkv.at[pl.ds(2 * PP * t, 2 * PP + 2)]
        ring_view = ring.at[pl.ds(2 * PP * t, 2 * PP)]
        done = None
        for v in range(8 * PP):
            j, k = v // 8, v % 8
            if v == 0 or (first and v in BARRIERS0):
                if v:
                    for p in BARRIERS0[v]:
                        pair_copy(p).wait()
                    if v == max(BARRIERS0):
                        second_batch()
                fresh_zero()
                done = None
            prev = done
            done = pre_dot(w_view, ring_view, j, k, deps.get(v))
            for jr, kr in (REL_SCHED0 if first else REL_SCHED).get(v, ()):
                relayout(raw_view, w_view, jr + 1, kr, prev)
                deps.setdefault(v + REL_LAG, []).append(w_view[2 * jr + 3, pl.ds(64 * kr + 56, 8), :])
            if first:
                continue
            if v in LN_SCHED:
                q = LNP * (t - 2) + LN_SCHED.index(v)
                hrow = pl.multiple_of(jnp.where(q < 0, XS, 32 * (q // 3) + 8 * (q % 3)), 8)
                layernorm16(PRE + 16 * q, hbuf, hrow, done if prev is not None else None)
                deps.setdefault(v + LN_LAG, []).append(hbuf[KT - 1, pl.ds(hrow, 8), :])
            if v in SCORE_SCHED:
                g = jnp.minimum(len(SCORE_SCHED) * (t - 1) + SCORE_SCHED.index(v), PRE // 16 - LNP - 1)
                rows = pl.ds(pl.multiple_of(8 * g, 8), 8)
                xp = [xn_pre[kk, rows, :] for kk in range(KT)]
                xp[0] = xp[0] | (done & zero_box[0])
                score16(g, _u2b(jnp.concatenate(xp, axis=1)))

    pre_iter(0, True)

    def pre_body(t, carry):
        pairs_wait(t)

        @pl.when(t >= 2)
        def _():
            x_piece(t).wait()
        pre_iter(t, False)
        return carry

    lax.fori_loop(1, NPRE, pre_body, 0)
    row = lax.broadcasted_iota(jnp.int32, (80, 80), 0)
    col = lax.broadcasted_iota(jnp.int32, (80, 80), 1)
    same_head = (jnp.where(row < 64, row >> 5, (row - 64) >> 3)
                 == jnp.where(col < 64, col >> 5, (col - 64) >> 3))
    allowed = same_head & ((col >= 64) | (row >= 64) | (col <= row))
    fill = jnp.where(same_head, -1e9, -jnp.inf).astype(F32)
    low_half = lax.broadcasted_iota(jnp.int32, (8, 128), 0) < 4
    high_half = jnp.logical_not(low_half)
    scale = DH ** -0.5

    def load_row(t):
        w = jnp.concatenate([xn_t[k, pl.ds(t // 2, 1), :] for k in range(KT)], axis=1)
        bits = jnp.where(t % 2 == 0, w << 16, w & jnp.uint32(0xFFFF0000))
        return pltpu.bitcast(bits, F32), w

    def select_tokens():
        r = r_s[...]
        tok = lane16 * 16 + lax.broadcasted_iota(jnp.int32, (16, 128), 0)

        def full(op, v):
            return op(op(v, axis=0, keepdims=True), axis=1, keepdims=True)

        top1 = full(jnp.max, r)
        idx1 = full(jnp.min, jnp.where(r == top1, tok, S - 1))
        r2 = jnp.where(tok == idx1, -jnp.inf, r)
        top2 = full(jnp.max, r2)
        idx2 = full(jnp.min, jnp.where((r2 == top2) & (tok != idx1), tok, S - 1))
        first = lax.broadcasted_iota(jnp.int32, (8, 128), 0) == 0
        gate_s[...] = jnp.where(first, top1, top2)
        sel_s[...] = jnp.where(first, idx1, idx2)

    NIT = NSEG // UNROLL
    ROWS = SEG * UNROLL

    def half_rows(r0):
        return pl.multiple_of(r0 // 2, 8)

    def residual(xf, a, b):
        return (_rbf(xf + a) + b).astype(BF)

    def out_copy(j):
        r0, n = (0, S - 2 * ROWS) if j == 0 else (S - (3 - j) * ROWS, ROWS)
        return pltpu.make_async_copy(out_s.at[pl.ds(r0, n), :], out_hbm.at[pl.ds(r0, n), :],
                                     sems.at[SEM_OUT + j])

    def ffn_groups(i, y):
        x_sel = xsel_s[...]
        live = (i >= 1) & (i < NIT - 1)
        hid = {}

        def up(w_ref, j, key):
            cols = pl.ds(pl.multiple_of(128 * j, 128), 128)
            part = _dot(x_sel[:, 0:512], _u2b(w_ref[pl.ds(0, 256), cols]).astype(F32))
            yield
            hid[key] = _rbf(_dot(x_sel[:, 512:1024], _u2b(w_ref[pl.ds(256, 256), cols]).astype(F32)) + part)
            yield

        for jj in range(2):
            j = jnp.clip(2 * (i - 1) + jj, 0, FT - 1)
            yield from up(wg_s, j, "g")
            yield from up(wu_s, j, "u")
            g = hid["g"]
            hb = jnp.where(live, _rbf(_rbf(g * _rbf(jax.nn.sigmoid(g))) * hid["u"]), 0.0)
            rows = pl.ds(pl.multiple_of(64 * j, 64), 64)
            yield
            for half in range(2):
                y[half] = _dot(hb, _u2b(wd_s[rows, pl.ds(512 * half, 512)]).astype(F32)) + y[half]
                yield

    def one_step(i, u, mem, held, side):
        odd = u % 2
        s2 = i * (UNROLL // 2) + u // 2
        h_ld = pl.multiple_of(16 * UNROLL * i, 32) + 32 * (u // 2)
        r24 = pl.multiple_of((12 * UNROLL * i) % RING32, 8) + XS * (u // 2)
        qkv_ld = pl.multiple_of((SEG * s2 + 32) % RING32, 32) + 16 * odd
        m0 = 0 if odd else XS

        def with_mem(lo, hi, m):
            if odd:
                return [jnp.where(low_half, m, lo), hi]
            return [lo, jnp.where(low_half, hi, m)]

        def store_tokens(ref, idx, base, yp):
            if odd:
                pltpu.store(ref.at[idx, pl.ds(base + 8, 8), :], yp[0:8], mask=high_half)
                ref[idx, pl.ds(base + 16, yp.shape[0] - 8), :] = yp[8:]
            else:
                ref[idx, pl.ds(base, 8), :] = yp[0:8]
                pltpu.store(ref.at[idx, pl.ds(base + 8, 8), :], yp[8:16], mask=low_half)

        lk = [_u2b(jnp.concatenate(with_mem(hbuf[k, pl.ds(h_ld + 8 * odd, 8), :],
                                            hbuf[k, pl.ds(h_ld + 8 + 8 * odd, 8), :], mem[k]), axis=0))
              for k in range(KT)]
        lhs = jnp.concatenate(lk, axis=1)

        ymem = {}
        xs = {}
        probs = {}
        parts = {}

        def proj(h):
            split = h < K_SPLIT and u > 0
            if split:
                lhs7 = jnp.concatenate(lk[:KT - 1], axis=1)
                head = [_dot(lhs7, _u2b(wqkv[m * H + h, pl.ds(0, 448), :])) for m in range(3)]
            for m in range(3):
                if split:
                    y = _dot(lk[KT - 1], _u2b(wqkv[m * H + h, pl.ds(448, 64), :])) + head[m]
                else:
                    y = _dot(lhs, _u2b(wqkv[m * H + h]))
                store_tokens(ring, m * H + h, r24, _b2u(y.astype(BF)))
                ymem[(h, m)] = y[m0:m0 + MEM]
                xs[(h, m)] = ring[m * H + h, pl.ds(qkv_ld, SEG // 2), :]

        def pair(p, m):
            a, b = 2 * p, 2 * p + 1
            mm = jnp.concatenate([ymem[(a, m)], ymem[(b, m)]], axis=0).astype(BF)
            return jnp.concatenate([_u2b(xs[(a, m)]), _u2b(xs[(b, m)]), mm], axis=0)

        def qk(p):
            sc = _dot_nt(pair(p, 0), pair(p, 1))
            sc = jnp.where(allowed, sc * scale, fill)
            e = jnp.exp(sc - jnp.max(sc, axis=1, keepdims=True))
            l = jnp.sum(e, axis=1, keepdims=True)
            r = pl.reciprocal(l, approx=True)
            r = r * (2.0 - l * r)
            probs[p] = (e * r).astype(BF)

        def pv(p):
            op = _b2u(_dot(probs[p], pair(p, 2)).astype(BF))
            om = op[32:40]
            om_sw = pltpu.roll(om, 4, axis=0)
            for j, h in enumerate((2 * p, 2 * p + 1)):
                x0, x1 = op[16 * j:16 * j + 8], op[16 * j + 8:16 * j + 16]
                m = om if j != odd else om_sw
                if odd:
                    rows = with_mem(held[h], x0, m) + [x1]
                else:
                    rows = with_mem(x0, x1, m)
                    held[h] = x1
                parts[h] = _u2b(jnp.concatenate(rows, axis=0))

        def after(t):
            for lag, fn in ((LAG_QK, qk), (LAG_PV, pv)):
                if (t - 1 - lag) % 2 == 0 and 0 <= (t - 1 - lag) // 2 < NPAIR:
                    fn((t - 1 - lag) // 2)

        def side_group():
            if odd:
                next(side, None)

        for t in range(H):
            proj(t)
            after(t)
            if u == 0 and t == 8:
                select_tokens()
        t = H
        n_part, h_split = (N_PART_ODD, H_SPLIT_ODD) if odd else (N_PART, H_SPLIT)
        lhs_a = jnp.concatenate([parts[j] for j in range(h_split)], axis=1)
        acc = []
        for n in range(n_part):
            acc.append(_dot(lhs_a, _u2b(wo_s[n, pl.ds(0, h_split * 64), :])))
            after(t)
            side_group()
            t += 1
        while t - 1 - LAG_PV <= 2 * (NPAIR - 1):
            after(t)
            t += 1
        lhs_b = jnp.concatenate([parts[j] for j in range(h_split, H)], axis=1)
        lhs_o = jnp.concatenate([lhs_a, lhs_b], axis=1)
        new_mem = [None] * KT
        pair_row = pl.multiple_of(ROWS * i, 64) + 64 * (u // 2)

        def finish(n, y):
            ym = y[m0:m0 + MEM]
            new_mem[n] = _b2u(jnp.concatenate([ym, ym], axis=0).astype(BF))
            yb = y.astype(BF)
            store_tokens(abuf, n, h_ld, _b2u(yb))
            cols = pl.ds(128 * n, 128)
            lo, cnt = (XS, 2 * SEG - XS) if odd else (0, XS)
            rows = pl.ds(pl.multiple_of(pair_row + lo, 8), cnt)
            a = yb.astype(F32)
            b = _u2b(xn_t[n, pl.ds(h_ld + 8 * odd, y.shape[0] // 2), :]).astype(F32)
            sl = slice(MEM, MEM + cnt) if odd else slice(0, cnt)
            out_s[rows, cols] = residual(x_s[rows, cols].astype(F32), a[sl], b[sl])

        order = list(range(n_part, KT))
        for n in order:
            finish(n, _dot(lhs_o, _u2b(wo_s[n])))
            if n < KT - 1:
                side_group()
            if n == n_part:
                for n2 in range(n_part):
                    tail = _u2b(wo_s[n2, pl.ds(h_split * 64, (H - h_split) * 64), :])
                    finish(n2, _dot(lhs_b, tail) + acc[n2])
        return new_mem

    def patch_row(t, yrow):
        xr, w = load_row(t)
        bits = pltpu.bitcast(_rbf(xr + yrow), U32)
        w = jnp.where(t % 2 == 0,
                      (w & jnp.uint32(0xFFFF0000)) | (bits >> 16),
                      (w & jnp.uint32(0xFFFF)) | bits)
        for k in range(KT):
            xn_t[k, pl.ds(t // 2, 1), :] = w[:, 128 * k:128 * (k + 1)]

    def fix_copy(j, r0):
        return pltpu.make_async_copy(out_s.at[pl.ds(r0, 16), :], out_hbm.at[pl.ds(r0, 16), :],
                                     sems.at[SEM_FIX + j])

    def gather_tokens():
        for cp in ffn_copies:
            cp.wait()
        idx_s[0] = sel_s[0, 0]
        idx_s[1] = sel_s[1, 0]
        sel_row = lax.broadcasted_iota(jnp.int32, (8, D), 0)
        xs1, _ = load_row(idx_s[0])
        xs2, _ = load_row(idx_s[1])
        xsel_s[...] = jnp.where(sel_row == 0, xs1, jnp.where(sel_row == 1, xs2, 0.0))

    def apply_ffn():
        out_copy(0).wait()
        patch_row(idx_s[0], yy_s[0:1, :])
        patch_row(idx_s[1], yy_s[1:2, :])
        blks = [idx_s[j] >> 4 for j in range(2)]
        for blk in blks:
            r0 = pl.multiple_of(jnp.minimum(blk, (S - ROWS) // 16 - 1) * 16, 16)
            for n in range(KT):
                cols = pl.ds(128 * n, 128)
                out_s[pl.ds(r0, 16), cols] = residual(
                    x_s[pl.ds(r0, 16), cols].astype(F32),
                    _u2b(abuf[n, pl.ds(half_rows(r0), 8), :]).astype(F32),
                    _u2b(xn_t[n, pl.ds(half_rows(r0), 8), :]).astype(F32))
        blk1, blk2 = [jnp.minimum(blk, (S - 2 * ROWS) // 16 - 1) for blk in blks]
        blk2 = jnp.where(blk2 == blk1, jnp.where(blk1 == 0, 1, blk1 - 1), blk2)
        for j, blk in enumerate((blk1, blk2)):
            fix_copy(j, pl.multiple_of(blk * 16, 16)).start()
        out_copy(1).start()

    def body(i, carry):
        mem, y = list(carry[:KT]), list(carry[KT:])

        @pl.when((i == 1) | (i >= NIT - 2))
        def _():
            pl.when(i == 1)(gather_tokens)
            pl.when(i == NIT - 2)(lambda: out_copy(0).start())
            pl.when(i == NIT - 1)(apply_ffn)

        side = ffn_groups(i, y)
        held = {}
        for u in range(UNROLL):
            mem = one_step(i, u, mem, held, side)
        for _ in side:
            raise AssertionError("ffn groups left over")
        gate = _rbf(jax.nn.sigmoid(gate_s[:, 0:1]))
        yy_s[...] = _rbf(_rbf(jnp.concatenate(y, axis=1)) * gate)
        return tuple(mem) + tuple(y)

    for n in range(KT):
        wo_copy(n).wait()
    for cp in ffn0_copies:
        cp.wait()
    xsel_s[...] = jnp.zeros(xsel_s.shape, F32)
    mi = mem0_s[...].astype(F32)
    mip = _b2u(jnp.concatenate([mi, mi], axis=0).astype(BF))
    lax.fori_loop(0, NIT, body,
                  tuple(mip[:, 128 * k:128 * (k + 1)] for k in range(KT))
                  + (jnp.zeros((8, 512), F32), jnp.zeros((8, 512), F32)))
    out_copy(2).start()
    for j in range(2):
        fix_copy(j, 0).wait()
    out_copy(1).wait()
    out_copy(2).wait()


@jax.jit
def pallas_parallel_sum__memory_aug_recurrent_mem_tr__moe_arch_mod__prompt_kernel(
    A_x: jax.Array,
    A_mem0: jax.Array,
    A_Wq: jax.Array,
    A_Wk: jax.Array,
    A_Wv: jax.Array,
    A_Wo: jax.Array,
    A_seg_len: jax.Array,
    B_x: jax.Array,
    B_w_r: jax.Array,
    B_w_gate: jax.Array,
    B_w_up: jax.Array,
    B_w_down: jax.Array,
):
    del A_seg_len, B_x
    assert A_x.shape == (1, S, D) and A_mem0.shape == (1, MEM, D)
    assert A_Wq.shape == (D, H, DH) and A_Wo.shape == (H, DH, D)
    assert B_w_gate.shape == (D, FF) and B_w_down.shape == (FF, D)
    any_spec = pl.BlockSpec(memory_space=pl.ANY)
    out = pl.pallas_call(
        _kernel,
        out_shape=jax.ShapeDtypeStruct((S, D), BF),
        in_specs=[any_spec] * 10,
        out_specs=any_spec,
        scratch_shapes=[
            pltpu.VMEM((S, D), BF),
            pltpu.VMEM((KT, S // 2, 128), U32),
            pltpu.VMEM((KT, PRE // 2, 128), U32),
            pltpu.VMEM((KT, 16 * NSEG, 128), U32),
            pltpu.VMEM((3 * H + 2, D // 2, 128), U32),
            pltpu.VMEM((KT, H * DH // 2, 128), U32),
            pltpu.VMEM((3 * H, RING32, 128), U32),
            pltpu.VMEM((KT, S // 2, 128), U32),
            pltpu.VMEM((S, D), BF),
            pltpu.VMEM((NPQ + 1, D, 128), U32),
            pltpu.VMEM((D // 2, FF), U32),
            pltpu.VMEM((D // 2, FF), U32),
            pltpu.VMEM((FF // 2, D), U32),
            pltpu.VMEM((MEM, D), BF),
            pltpu.VMEM((D,), BF),
            pltpu.VMEM((8, D), F32),
            pltpu.VMEM((16, 128), F32),
            pltpu.VMEM((8, 128), jnp.int32),
            pltpu.VMEM((8, 128), F32),
            pltpu.VMEM((8, D), F32),
            pltpu.VMEM((8, D), F32),
            pltpu.SMEM((1,), jnp.int32),
            pltpu.SMEM((2,), jnp.int32),
            pltpu.SemaphoreType.DMA((NSEM,)),
        ],
        compiler_params=pltpu.CompilerParams(vmem_limit_bytes=126 * 1024 * 1024,
                                             disable_bounds_checks=True, disable_semaphore_checks=True),
    )(A_x.reshape(S, D), A_mem0.reshape(MEM, D), A_Wq, A_Wk, A_Wv, A_Wo.reshape(H * DH, D),
      B_w_r, B_w_gate, B_w_up, B_w_down)
    return out.reshape(1, S, D)
```

```python
import jax
import jax.numpy as jnp
from jax import lax
import jax.experimental.pallas as pl
import jax.experimental.pallas.tpu as pltpu

BF = jnp.bfloat16
U32 = jnp.uint32
F32 = jnp.float32

S = 2048
D = 1024
H = 32
DH = 128
MEM = 8
SEG = 32
NSEG = S // SEG
FF = 3584
KT = D // 128
FT = FF // 128
XS = 24
PRE = S - NSEG * XS
RING = 576
RING32 = RING // 2
NPAIR = H // 2
NPQ = 3 * NPAIR
PP = 6
NPRE = NPQ // PP
LNP = 16
SEM_SMALL, SEM_X0, SEM_X = 0, 2, 6
SEM_W0 = SEM_X + NPRE
SEM_W = SEM_W0 + PP
SEM_WO = SEM_W + NPRE
SEM_FFN0, SEM_FFN, SEM_FIX, SEM_OUT = SEM_WO + 1, SEM_WO + 2, SEM_WO + 3, SEM_WO + 5
NSEM = SEM_OUT + 3

LAG_QK = 1
LAG_PV = 4
N_PART = 4
H_SPLIT = 26
REL_SCHED = {0: [(0, 0), (0, 1)], 1: [(0, 2), (0, 3)], 2: [(0, 4)], 3: [(0, 5)], 4: [(0, 6)], 5: [(0, 7)]}
REL_SCHED.update({8 * j - 2 + k: [(j, k)] for j in range(1, PP) for k in range(8)})
N_PART_ODD = 4
H_SPLIT_ODD = 24
K_SPLIT = 2
EPI_SCHED = [v * 5 // 2 for v in range(24)]
EPI_LAG = 4
ECH = 160
REL_SCHED0 = {6: [(0, k) for k in range(8)],
              13: [(1, k) for k in range(8)],
              26: [(3, k) for k in range(3)], 27: [(3, k) for k in range(3, 6)], 28: [(3, 6), (3, 7)]}
REL_SCHED0.update({8 * j - 2 + k: [(j, k)] for j in (2, 4, 5) for k in range(8)})
BARRIERS0 = {6: [1], 13: [2, 3], 26: [4, 5, 6]}
SCORE_SCHED = [1, 16, 31]
LN_SCHED = [11 * q // 4 for q in range(LNP)]
FIRST_BATCH = 6
LN_LAG = 5
FFN_DELAY = 2
REL_LAG = 2
UNROLL = 4


def _b2u(x):
    return pltpu.bitcast(x, U32)


def _u2b(x):
    return pltpu.bitcast(x, BF)


def _dot(a, b):
    return jnp.dot(a, b, preferred_element_type=F32)


def _dot_nt(a, b):
    return lax.dot_general(a, b, (((1,), (1,)), ((), ())), preferred_element_type=F32)


def _after(w, dep, zero):
    if not dep:
        return w
    d = dep[0]
    for e in dep[1:]:
        d = d | e
    return jnp.concatenate([w[0:8] | (d & zero), w[8:]], axis=0)


def _rbf(x):
    return x.astype(BF).astype(F32)


def _kernel(x_hbm, mem0_hbm, wq_hbm, wk_hbm, wv_hbm, wo_hbm, wr_hbm, wg_hbm, wu_hbm, wd_hbm,
            out_hbm,
            x_s, xn_t, xn_pre, hbuf, wqkv, wo_s, ring, abuf, out_s, raw,
            wg_s, wu_s, wd_s, mem0_s, wr_s, wrf_s, r_s, sel_s, gate_s, xsel_s, yy_s, zero_s, idx_s,
            sems):
    w32 = [w.bitcast(U32) for w in (wq_hbm, wk_hbm, wv_hbm)]
    wo32 = wo_hbm.bitcast(U32)
    wg32 = wg_hbm.bitcast(U32)
    wu32 = wu_hbm.bitcast(U32)
    wd32 = wd_hbm.bitcast(U32)

    def rows_copy(r0, n, sem):
        return pltpu.make_async_copy(x_hbm.at[pl.ds(r0, n), :], x_s.at[pl.ds(r0, n), :], sems.at[sem])

    def x_first(c):
        return rows_copy(128 * c if isinstance(c, int) else pl.multiple_of(128 * c, 128), 128, SEM_X0 + c)

    def x_piece(t):
        r0 = PRE + 16 * LNP * (t - 2)
        return rows_copy(r0 if isinstance(t, int) else pl.multiple_of(r0, 256), 16 * LNP, SEM_X + t)

    def pair_copy(p):
        q = min(p, NPQ - 1)
        sem = SEM_W0 + p if p <= PP else SEM_W + (p - 1) // PP
        return pltpu.make_async_copy(w32[q // NPAIR].at[:, q % NPAIR, :], raw.at[p], sems.at[sem])

    def pairs_wait(t):
        dst = raw.at[pl.ds(PP * t + 1, PP)]
        pltpu.make_async_copy(dst, dst, sems.at[SEM_W + t]).wait()

    def wo_copy(n):
        return pltpu.make_async_copy(wo32.at[:, pl.ds(128 * n, 128)], wo_s.at[n], sems.at[SEM_WO])

    small_copies = [pltpu.make_async_copy(mem0_hbm, mem0_s, sems.at[SEM_SMALL]),
                    pltpu.make_async_copy(wr_hbm, wr_s, sems.at[SEM_SMALL + 1])]
    ffn0_copies = [
        pltpu.make_async_copy(wg32.at[:, pl.ds(0, 128)], wg_s.at[:, pl.ds(0, 128)], sems.at[SEM_FFN0]),
        pltpu.make_async_copy(wu32.at[:, pl.ds(0, 128)], wu_s.at[:, pl.ds(0, 128)], sems.at[SEM_FFN0]),
        pltpu.make_async_copy(wd32.at[pl.ds(0, 64), :], wd_s.at[pl.ds(0, 64), :], sems.at[SEM_FFN0])]
    ffn_copies = [
        pltpu.make_async_copy(wg32.at[:, pl.ds(128, FF - 128)], wg_s.at[:, pl.ds(128, FF - 128)], sems.at[SEM_FFN]),
        pltpu.make_async_copy(wu32.at[:, pl.ds(128, FF - 128)], wu_s.at[:, pl.ds(128, FF - 128)], sems.at[SEM_FFN]),
        pltpu.make_async_copy(wd32.at[pl.ds(64, FF // 2 - 64), :], wd_s.at[pl.ds(64, FF // 2 - 64), :],
                              sems.at[SEM_FFN])]

    zero_s[0] = 0
    for c in range(4):
        x_first(c).start()
        if c == 0:
            for cp in small_copies:
                cp.start()
            pair_copy(0).start()

    def queue(t0, t1):
        for t in range(t0, t1):
            for p in range(PP * t + 1, PP * t + PP + 1):
                pair_copy(p).start()
            if t >= 2:
                x_piece(t).start()

    queue(0, FIRST_BATCH)
    eps_bf = 1.0013580322265625e-05

    def score16(g, xn):
        wr = jnp.concatenate([wrf_s[...], wrf_s[...]], axis=0)
        score = _rbf(jnp.sum(xn.astype(F32) * wr, axis=1, keepdims=True))
        r_s[...] = jnp.where(lane16 == g, score, r_s[...])

    def layernorm16(rq, dst_ref, dst_row, not_before=None):
        rq = rq if isinstance(rq, int) else pl.multiple_of(rq, 16)
        xf = x_s[pl.ds(rq, 16), :].astype(F32)
        if not_before is not None:
            x0 = _after(pltpu.bitcast(xf[:, 0:128], U32), [not_before], zero_box[0])
            xf = jnp.concatenate([pltpu.bitcast(x0, F32), xf[:, 128:]], axis=1)
        mean = jnp.sum(xf, axis=1, keepdims=True) * (1.0 / D)
        cen = xf - mean
        var = jnp.sum(cen * cen, axis=1, keepdims=True) * (1.0 / D)
        sd = _rbf(jnp.sqrt(_rbf(_rbf(var) + eps_bf)))
        xn = (_rbf(xf - _rbf(mean)) * (1.0 / sd)).astype(BF)
        if dst_ref is hbuf:
            score16(rq // 16, xn)
        xp = _b2u(xn)
        hq = rq // 2 if isinstance(rq, int) else pl.multiple_of(rq // 2, 8)
        dst_row = dst_row if isinstance(dst_row, int) else pl.multiple_of(dst_row, 8)
        for k in range(KT):
            xn_t[k, pl.ds(hq, 8), :] = xp[:, 128 * k:128 * (k + 1)]
            dst_ref[k, pl.ds(dst_row, 8), :] = xp[:, 128 * k:128 * (k + 1)]

    zero_box = [None]

    def fresh_zero():
        zero_box[0] = jnp.full((8, 128), zero_s[0], jnp.int32).astype(U32)

    r_s[...] = jnp.full(r_s.shape, -jnp.inf, F32)
    lane16 = lax.broadcasted_iota(jnp.int32, (16, 128), 1)

    x_first(0).wait()
    for q in range(8):
        layernorm16(16 * q, xn_pre, 8 * q)


    def relayout(src, dst, j, k, not_before=None):
        a = src[j, pl.ds(128 * k, 64, stride=2), :]
        if not_before is not None:
            a = a | jnp.concatenate([not_before & zero_box[0]] * 8, axis=0)
        b = src[j, pl.ds(128 * k + 1, 64, stride=2), :]
        rows = pl.ds(64 * k, 64)
        dst[2 * j, rows, :] = (a & jnp.uint32(0xFFFF)) | (b << 16)
        dst[2 * j + 1, rows, :] = (a >> 16) | (b & jnp.uint32(0xFFFF0000))

    def pre_dot(w_view, ring_view, h, row, dep=None):
        lhs = jnp.concatenate([_u2b(xn_pre[kk, pl.ds(row, 64), :]) for kk in range(KT)], axis=1)
        y = _dot(lhs, _u2b(_after(w_view[h], dep, zero_box[0])))
        yp = _b2u(y.astype(BF))
        ring_view[h, pl.ds(32 + row, 64), :] = yp
        return yp[0:8]

    for c in small_copies:
        c.wait()
    pair_copy(0).wait()
    for k in range(8):
        relayout(raw, wqkv, 0, k)
    wrf_s[...] = jnp.broadcast_to(wr_s[...].astype(F32).reshape(1, D), (8, D))

    def start_body(c, carry):
        x_first(c).wait()
        row = pl.multiple_of(64 * (c - 1), 64)
        for h in range(2):
            pre_dot(wqkv, ring, h, row)
        for q in range(8):
            layernorm16(2 * row + 128 + 16 * q, xn_pre, row + 64 + 8 * q)
        return carry

    lax.fori_loop(1, PRE // 128, start_body, 0)

    def second_batch():
        queue(FIRST_BATCH, NPRE)
        for n in range(KT):
            wo_copy(n).start()
        for cp in ffn0_copies + ffn_copies:
            cp.start()

    def pre_iter(t, first):
        deps = {}
        raw_view = raw.at[pl.ds(PP * t, PP + 1)]
        w_view = wqkv.at[pl.ds(2 * PP * t, 2 * PP + 2)]
        ring_view = ring.at[pl.ds(2 * PP * t, 2 * PP)]
        done = None
        for v in range(6 if first else 0, 8 * PP):
            h, row = v // 4, 64 * (v % 4)
            if first and v < 8:
                h, row = v - 6, 192
            if v == 0 or (first and v in BARRIERS0):
                if v:
                    for p in BARRIERS0[v]:
                        pair_copy(p).wait()
                    if v == max(BARRIERS0):
                        second_batch()
                fresh_zero()
                done = None
            prev = done
            done = pre_dot(w_view, ring_view, h, row, deps.get(v))
            for jr, kr in (REL_SCHED0 if first else REL_SCHED).get(v, ()):
                relayout(raw_view, w_view, jr + 1, kr, prev)
                deps.setdefault(v + REL_LAG, []).append(w_view[2 * jr + 3, pl.ds(64 * kr + 56, 8), :])
            if first:
                continue
            if v in LN_SCHED:
                q = LNP * (t - 2) + LN_SCHED.index(v)
                hrow = pl.multiple_of(jnp.where(q < 0, XS, 32 * (q // 3) + 8 * (q % 3)), 8)
                layernorm16(PRE + 16 * q, hbuf, hrow, done if prev is not None else None)
                deps.setdefault(v + LN_LAG, []).append(hbuf[KT - 1, pl.ds(hrow, 8), :])
            if v in SCORE_SCHED:
                g = jnp.minimum(len(SCORE_SCHED) * (t - 1) + SCORE_SCHED.index(v), PRE // 16 - LNP - 1)
                rows = pl.ds(pl.multiple_of(8 * g, 8), 8)
                xp = [xn_pre[kk, rows, :] for kk in range(KT)]
                xp[0] = xp[0] | (done & zero_box[0])
                score16(g, _u2b(jnp.concatenate(xp, axis=1)))

    pre_iter(0, True)

    def pre_body(t, carry):
        pairs_wait(t)

        @pl.when(t >= 2)
        def _():
            x_piece(t).wait()
        pre_iter(t, False)
        return carry

    lax.fori_loop(1, NPRE, pre_body, 0)
    row = lax.broadcasted_iota(jnp.int32, (80, 80), 0)
    col = lax.broadcasted_iota(jnp.int32, (80, 80), 1)
    same_head = (jnp.where(row < 64, row >> 5, (row - 64) >> 3)
                 == jnp.where(col < 64, col >> 5, (col - 64) >> 3))
    allowed = same_head & ((col >= 64) | (row >= 64) | (col <= row))
    fill = jnp.where(same_head, -1e9, -jnp.inf).astype(F32)
    low_half = lax.broadcasted_iota(jnp.int32, (8, 128), 0) < 4
    high_half = jnp.logical_not(low_half)
    scale = DH ** -0.5

    def load_row(t):
        w = jnp.concatenate([xn_t[k, pl.ds(t // 2, 1), :] for k in range(KT)], axis=1)
        bits = jnp.where(t % 2 == 0, w << 16, w & jnp.uint32(0xFFFF0000))
        return pltpu.bitcast(bits, F32), w

    def select_tokens():
        r = r_s[...]
        tok = lane16 * 16 + lax.broadcasted_iota(jnp.int32, (16, 128), 0)

        def full(op, v):
            return op(op(v, axis=0, keepdims=True), axis=1, keepdims=True)

        top1 = full(jnp.max, r)
        idx1 = full(jnp.min, jnp.where(r == top1, tok, S - 1))
        r2 = jnp.where(tok == idx1, -jnp.inf, r)
        top2 = full(jnp.max, r2)
        idx2 = full(jnp.min, jnp.where((r2 == top2) & (tok != idx1), tok, S - 1))
        first = lax.broadcasted_iota(jnp.int32, (8, 128), 0) == 0
        gate_s[...] = jnp.where(first, top1, top2)
        sel_s[...] = jnp.where(first, idx1, idx2)

    NIT = NSEG // UNROLL
    ROWS = SEG * UNROLL

    def half_rows(r0):
        return pl.multiple_of(r0 // 2, 8)

    def residual(xf, a, b):
        return (_rbf(xf + a) + b).astype(BF)

    def out_copy(j):
        r0, n = (0, S - 2 * ROWS) if j == 0 else (S - (3 - j) * ROWS, ROWS)
        return pltpu.make_async_copy(out_s.at[pl.ds(r0, n), :], out_hbm.at[pl.ds(r0, n), :],
                                     sems.at[SEM_OUT + j])

    def ffn_groups(i, y):
        x_sel = xsel_s[...]
        live = (i >= 1) & (i < NIT - 1)
        hid = {}

        def up(w_ref, j, key):
            cols = pl.ds(pl.multiple_of(128 * j, 128), 128)
            part = _dot(x_sel[:, 0:512], _u2b(w_ref[pl.ds(0, 256), cols]).astype(F32))
            yield
            hid[key] = _rbf(_dot(x_sel[:, 512:1024], _u2b(w_ref[pl.ds(256, 256), cols]).astype(F32)) + part)
            yield

        for jj in range(2):
            j = jnp.clip(2 * (i - 1) + jj, 0, FT - 1)
            yield from up(wg_s, j, "g")
            yield from up(wu_s, j, "u")
            g = hid["g"]
            hb = jnp.where(live, _rbf(_rbf(g * _rbf(jax.nn.sigmoid(g))) * hid["u"]), 0.0)
            rows = pl.ds(pl.multiple_of(64 * j, 64), 64)
            yield
            for half in range(2):
                y[half] = _dot(hb, _u2b(wd_s[rows, pl.ds(512 * half, 512)]).astype(F32)) + y[half]
                yield

    def one_step(i, u, mem, held, side):
        odd = u % 2
        s2 = i * (UNROLL // 2) + u // 2
        h_ld = pl.multiple_of(16 * UNROLL * i, 32) + 32 * (u // 2)
        r24 = pl.multiple_of((12 * UNROLL * i) % RING32, 8) + XS * (u // 2)
        qkv_ld = pl.multiple_of((SEG * s2 + 32) % RING32, 32) + 16 * odd
        m0 = 0 if odd else XS

        def with_mem(lo, hi, m):
            if odd:
                return [jnp.where(low_half, m, lo), hi]
            return [lo, jnp.where(low_half, hi, m)]

        def store_tokens(ref, idx, base, yp):
            if odd:
                pltpu.store(ref.at[idx, pl.ds(base + 8, 8), :], yp[0:8], mask=high_half)
                ref[idx, pl.ds(base + 16, yp.shape[0] - 8), :] = yp[8:]
            else:
                ref[idx, pl.ds(base, 8), :] = yp[0:8]
                pltpu.store(ref.at[idx, pl.ds(base + 8, 8), :], yp[8:16], mask=low_half)

        lk = [_u2b(jnp.concatenate(with_mem(hbuf[k, pl.ds(h_ld + 8 * odd, 8), :],
                                            hbuf[k, pl.ds(h_ld + 8 + 8 * odd, 8), :], mem[k]), axis=0))
              for k in range(KT)]
        lhs = jnp.concatenate(lk, axis=1)

        ymem = {}
        xs = {}
        probs = {}
        parts = {}

        def proj(h):
            split = h < K_SPLIT and u > 0
            if split:
                lhs7 = jnp.concatenate(lk[:KT - 1], axis=1)
                head = [_dot(lhs7, _u2b(wqkv[m * H + h, pl.ds(0, 448), :])) for m in range(3)]
            for m in range(3):
                if split:
                    y = _dot(lk[KT - 1], _u2b(wqkv[m * H + h, pl.ds(448, 64), :])) + head[m]
                else:
                    y = _dot(lhs, _u2b(wqkv[m * H + h]))
                store_tokens(ring, m * H + h, r24, _b2u(y.astype(BF)))
                ymem[(h, m)] = y[m0:m0 + MEM]
                xs[(h, m)] = ring[m * H + h, pl.ds(qkv_ld, SEG // 2), :]

        def pair(p, m):
            a, b = 2 * p, 2 * p + 1
            mm = jnp.concatenate([ymem[(a, m)], ymem[(b, m)]], axis=0).astype(BF)
            return jnp.concatenate([_u2b(xs[(a, m)]), _u2b(xs[(b, m)]), mm], axis=0)

        def qk(p):
            sc = _dot_nt(pair(p, 0), pair(p, 1))
            sc = jnp.where(allowed, sc * scale, fill)
            e = jnp.exp(sc - jnp.max(sc, axis=1, keepdims=True))
            l = jnp.sum(e, axis=1, keepdims=True)
            r = pl.reciprocal(l, approx=True)
            r = r * (2.0 - l * r)
            probs[p] = (e * r).astype(BF)

        def pv(p):
            op = _b2u(_dot(probs[p], pair(p, 2)).astype(BF))
            om = op[32:40]
            om_sw = pltpu.roll(om, 4, axis=0)
            for j, h in enumerate((2 * p, 2 * p + 1)):
                x0, x1 = op[16 * j:16 * j + 8], op[16 * j + 8:16 * j + 16]
                m = om if j != odd else om_sw
                if odd:
                    rows = with_mem(held[h], x0, m) + [x1]
                else:
                    rows = with_mem(x0, x1, m)
                    held[h] = x1
                parts[h] = _u2b(jnp.concatenate(rows, axis=0))

        def after(t):
            for lag, fn in ((LAG_QK, qk), (LAG_PV, pv)):
                if (t - 1 - lag) % 2 == 0 and 0 <= (t - 1 - lag) // 2 < NPAIR:
                    fn((t - 1 - lag) // 2)

        def side_group():
            if odd:
                next(side, None)

        for t in range(H):
            proj(t)
            after(t)
            if u == 0 and t == 8:
                select_tokens()
        t = H
        n_part, h_split = (N_PART_ODD, H_SPLIT_ODD) if odd else (N_PART, H_SPLIT)
        lhs_a = jnp.concatenate([parts[j] for j in range(h_split)], axis=1)
        acc = []
        for n in range(n_part):
            acc.append(_dot(lhs_a, _u2b(wo_s[n, pl.ds(0, h_split * 64), :])))
            after(t)
            side_group()
            t += 1
        while t - 1 - LAG_PV <= 2 * (NPAIR - 1):
            after(t)
            t += 1
        lhs_b = jnp.concatenate([parts[j] for j in range(h_split, H)], axis=1)
        lhs_o = jnp.concatenate([lhs_a, lhs_b], axis=1)
        new_mem = [None] * KT
        pair_row = pl.multiple_of(ROWS * i, 64) + 64 * (u // 2)

        def finish(n, y):
            ym = y[m0:m0 + MEM]
            new_mem[n] = _b2u(jnp.concatenate([ym, ym], axis=0).astype(BF))
            yb = y.astype(BF)
            store_tokens(abuf, n, h_ld, _b2u(yb))
            cols = pl.ds(128 * n, 128)
            lo, cnt = (XS, 2 * SEG - XS) if odd else (0, XS)
            rows = pl.ds(pl.multiple_of(pair_row + lo, 8), cnt)
            a = yb.astype(F32)
            b = _u2b(xn_t[n, pl.ds(h_ld + 8 * odd, y.shape[0] // 2), :]).astype(F32)
            sl = slice(MEM, MEM + cnt) if odd else slice(0, cnt)
            out_s[rows, cols] = residual(x_s[rows, cols].astype(F32), a[sl], b[sl])

        order = list(range(n_part, KT))
        for n in order:
            finish(n, _dot(lhs_o, _u2b(wo_s[n])))
            if n < KT - 1:
                side_group()
            if n == n_part:
                for n2 in range(n_part):
                    tail = _u2b(wo_s[n2, pl.ds(h_split * 64, (H - h_split) * 64), :])
                    finish(n2, _dot(lhs_b, tail) + acc[n2])
        return new_mem

    def patch_row(t, yrow):
        xr, w = load_row(t)
        bits = pltpu.bitcast(_rbf(xr + yrow), U32)
        w = jnp.where(t % 2 == 0,
                      (w & jnp.uint32(0xFFFF0000)) | (bits >> 16),
                      (w & jnp.uint32(0xFFFF)) | bits)
        for k in range(KT):
            xn_t[k, pl.ds(t // 2, 1), :] = w[:, 128 * k:128 * (k + 1)]

    def fix_copy(j, r0):
        return pltpu.make_async_copy(out_s.at[pl.ds(r0, 16), :], out_hbm.at[pl.ds(r0, 16), :],
                                     sems.at[SEM_FIX + j])

    def gather_tokens():
        for cp in ffn_copies:
            cp.wait()
        idx_s[0] = sel_s[0, 0]
        idx_s[1] = sel_s[1, 0]
        sel_row = lax.broadcasted_iota(jnp.int32, (8, D), 0)
        xs1, _ = load_row(idx_s[0])
        xs2, _ = load_row(idx_s[1])
        xsel_s[...] = jnp.where(sel_row == 0, xs1, jnp.where(sel_row == 1, xs2, 0.0))

    def apply_ffn():
        out_copy(0).wait()
        patch_row(idx_s[0], yy_s[0:1, :])
        patch_row(idx_s[1], yy_s[1:2, :])
        blks = [idx_s[j] >> 4 for j in range(2)]
        for blk in blks:
            r0 = pl.multiple_of(jnp.minimum(blk, (S - ROWS) // 16 - 1) * 16, 16)
            for n in range(KT):
                cols = pl.ds(128 * n, 128)
                out_s[pl.ds(r0, 16), cols] = residual(
                    x_s[pl.ds(r0, 16), cols].astype(F32),
                    _u2b(abuf[n, pl.ds(half_rows(r0), 8), :]).astype(F32),
                    _u2b(xn_t[n, pl.ds(half_rows(r0), 8), :]).astype(F32))
        blk1, blk2 = [jnp.minimum(blk, (S - 2 * ROWS) // 16 - 1) for blk in blks]
        blk2 = jnp.where(blk2 == blk1, jnp.where(blk1 == 0, 1, blk1 - 1), blk2)
        for j, blk in enumerate((blk1, blk2)):
            fix_copy(j, pl.multiple_of(blk * 16, 16)).start()
        out_copy(1).start()

    def body(i, carry):
        mem, y = list(carry[:KT]), list(carry[KT:])

        @pl.when((i == 1) | (i >= NIT - 2))
        def _():
            pl.when(i == 1)(gather_tokens)
            pl.when(i == NIT - 2)(lambda: out_copy(0).start())
            pl.when(i == NIT - 1)(apply_ffn)

        side = ffn_groups(i, y)
        held = {}
        for u in range(UNROLL):
            mem = one_step(i, u, mem, held, side)
        for _ in side:
            raise AssertionError("ffn groups left over")
        gate = _rbf(jax.nn.sigmoid(gate_s[:, 0:1]))
        yy_s[...] = _rbf(_rbf(jnp.concatenate(y, axis=1)) * gate)
        return tuple(mem) + tuple(y)

    for n in range(KT):
        wo_copy(n).wait()
    for cp in ffn0_copies:
        cp.wait()
    xsel_s[...] = jnp.zeros(xsel_s.shape, F32)
    mi = mem0_s[...].astype(F32)
    mip = _b2u(jnp.concatenate([mi, mi], axis=0).astype(BF))
    lax.fori_loop(0, NIT, body,
                  tuple(mip[:, 128 * k:128 * (k + 1)] for k in range(KT))
                  + (jnp.zeros((8, 512), F32), jnp.zeros((8, 512), F32)))
    out_copy(2).start()
    for j in range(2):
        fix_copy(j, 0).wait()
    out_copy(1).wait()
    out_copy(2).wait()


@jax.jit
def pallas_parallel_sum__memory_aug_recurrent_mem_tr__moe_arch_mod__prompt_kernel(
    A_x: jax.Array,
    A_mem0: jax.Array,
    A_Wq: jax.Array,
    A_Wk: jax.Array,
    A_Wv: jax.Array,
    A_Wo: jax.Array,
    A_seg_len: jax.Array,
    B_x: jax.Array,
    B_w_r: jax.Array,
    B_w_gate: jax.Array,
    B_w_up: jax.Array,
    B_w_down: jax.Array,
):
    del A_seg_len, B_x
    assert A_x.shape == (1, S, D) and A_mem0.shape == (1, MEM, D)
    assert A_Wq.shape == (D, H, DH) and A_Wo.shape == (H, DH, D)
    assert B_w_gate.shape == (D, FF) and B_w_down.shape == (FF, D)
    any_spec = pl.BlockSpec(memory_space=pl.ANY)
    out = pl.pallas_call(
        _kernel,
        out_shape=jax.ShapeDtypeStruct((S, D), BF),
        in_specs=[any_spec] * 10,
        out_specs=any_spec,
        scratch_shapes=[
            pltpu.VMEM((S, D), BF),
            pltpu.VMEM((KT, S // 2, 128), U32),
            pltpu.VMEM((KT, PRE // 2, 128), U32),
            pltpu.VMEM((KT, 16 * NSEG, 128), U32),
            pltpu.VMEM((3 * H + 2, D // 2, 128), U32),
            pltpu.VMEM((KT, H * DH // 2, 128), U32),
            pltpu.VMEM((3 * H, RING32, 128), U32),
            pltpu.VMEM((KT, S // 2, 128), U32),
            pltpu.VMEM((S, D), BF),
            pltpu.VMEM((NPQ + 1, D, 128), U32),
            pltpu.VMEM((D // 2, FF), U32),
            pltpu.VMEM((D // 2, FF), U32),
            pltpu.VMEM((FF // 2, D), U32),
            pltpu.VMEM((MEM, D), BF),
            pltpu.VMEM((D,), BF),
            pltpu.VMEM((8, D), F32),
            pltpu.VMEM((16, 128), F32),
            pltpu.VMEM((8, 128), jnp.int32),
            pltpu.VMEM((8, 128), F32),
            pltpu.VMEM((8, D), F32),
            pltpu.VMEM((8, D), F32),
            pltpu.SMEM((1,), jnp.int32),
            pltpu.SMEM((2,), jnp.int32),
            pltpu.SemaphoreType.DMA((NSEM,)),
        ],
        compiler_params=pltpu.CompilerParams(vmem_limit_bytes=126 * 1024 * 1024,
                                             disable_bounds_checks=True, disable_semaphore_checks=True),
    )(A_x.reshape(S, D), A_mem0.reshape(MEM, D), A_Wq, A_Wk, A_Wv, A_Wo.reshape(H * DH, D),
      B_w_r, B_w_gate, B_w_up, B_w_down)
    return out.reshape(1, S, D)
```

```python
import jax
import jax.numpy as jnp
from jax import lax
import jax.experimental.pallas as pl
import jax.experimental.pallas.tpu as pltpu

BF = jnp.bfloat16
U32 = jnp.uint32
F32 = jnp.float32

S = 2048
D = 1024
H = 32
DH = 128
MEM = 8
SEG = 32
NSEG = S // SEG
FF = 3584
KT = D // 128
FT = FF // 128
XS = 24
PRE = S - NSEG * XS
RING = 576
RING32 = RING // 2
NPAIR = H // 2
NPQ = 3 * NPAIR
PP = 6
NPRE = NPQ // PP
LNP = 16
SEM_SMALL, SEM_X0, SEM_X = 0, 2, 6
SEM_W0 = SEM_X + NPRE
SEM_W = SEM_W0 + PP
SEM_WO = SEM_W + NPRE
SEM_FFN0, SEM_FFN, SEM_FIX, SEM_OUT = SEM_WO + 1, SEM_WO + 2, SEM_WO + 3, SEM_WO + 5
NSEM = SEM_OUT + 3

LAG_QK = 1
LAG_PV = 4
N_PART, H_SPLIT = 4, 26
N_PART_ODD, H_SPLIT_ODD = 4, 24
K_SPLIT = 2
UNROLL = 4

REL_SCHED = {0: [(0, 0), (0, 1)], 1: [(0, 2), (0, 3)], 2: [(0, 4)], 3: [(0, 5)], 4: [(0, 6)], 5: [(0, 7)]}
REL_SCHED.update({8 * j - 2 + k: [(j, k)] for j in range(1, PP) for k in range(8)})
REL_SCHED0 = {6: [(0, k) for k in range(8)],
              13: [(1, k) for k in range(8)],
              26: [(3, k) for k in range(3)], 27: [(3, k) for k in range(3, 6)], 28: [(3, 6), (3, 7)]}
REL_SCHED0.update({8 * j - 2 + k: [(j, k)] for j in (2, 4, 5) for k in range(8)})
BARRIERS0 = {6: [1], 13: [2, 3], 26: [4, 5, 6]}
SCORE_SCHED = [1, 16, 31]
LN_SCHED = [11 * q // 4 for q in range(LNP)]
LN_LAG = 5
REL_LAG = 2
FIRST_BATCH = 6


def _b2u(x):
    return pltpu.bitcast(x, U32)


def _u2b(x):
    return pltpu.bitcast(x, BF)


def _dot(a, b):
    return jnp.dot(a, b, preferred_element_type=F32)


def _dot_nt(a, b):
    return lax.dot_general(a, b, (((1,), (1,)), ((), ())), preferred_element_type=F32)


def _after(w, dep, zero):
    if not dep:
        return w
    d = dep[0]
    for e in dep[1:]:
        d = d | e
    return jnp.concatenate([w[0:8] | (d & zero), w[8:]], axis=0)


def _rbf(x):
    return x.astype(BF).astype(F32)


def _kernel(x_hbm, mem0_hbm, wq_hbm, wk_hbm, wv_hbm, wo_hbm, wr_hbm, wg_hbm, wu_hbm, wd_hbm,
            out_hbm,
            x_s, xn_t, xn_pre, hbuf, wqkv, wo_s, ring, abuf, out_s, raw,
            wg_s, wu_s, wd_s, mem0_s, wr_s, wrf_s, r_s, sel_s, gate_s, xsel_s, yy_s, zero_s, idx_s,
            sems):
    w32 = [w.bitcast(U32) for w in (wq_hbm, wk_hbm, wv_hbm)]
    wo32 = wo_hbm.bitcast(U32)
    wg32 = wg_hbm.bitcast(U32)
    wu32 = wu_hbm.bitcast(U32)
    wd32 = wd_hbm.bitcast(U32)

    def rows_copy(r0, n, sem):
        return pltpu.make_async_copy(x_hbm.at[pl.ds(r0, n), :], x_s.at[pl.ds(r0, n), :], sems.at[sem])

    def x_first(c):
        return rows_copy(128 * c if isinstance(c, int) else pl.multiple_of(128 * c, 128), 128, SEM_X0 + c)

    def x_piece(t):
        r0 = PRE + 16 * LNP * (t - 2)
        return rows_copy(r0 if isinstance(t, int) else pl.multiple_of(r0, 256), 16 * LNP, SEM_X + t)

    def pair_copy(p):
        q = min(p, NPQ - 1)
        sem = SEM_W0 + p if p <= PP else SEM_W + (p - 1) // PP
        return pltpu.make_async_copy(w32[q // NPAIR].at[:, q % NPAIR, :], raw.at[p], sems.at[sem])

    def pairs_wait(t):
        dst = raw.at[pl.ds(PP * t + 1, PP)]
        pltpu.make_async_copy(dst, dst, sems.at[SEM_W + t]).wait()

    def wo_copy(n):
        return pltpu.make_async_copy(wo32.at[:, pl.ds(128 * n, 128)], wo_s.at[n], sems.at[SEM_WO])

    small_copies = [pltpu.make_async_copy(mem0_hbm, mem0_s, sems.at[SEM_SMALL]),
                    pltpu.make_async_copy(wr_hbm, wr_s, sems.at[SEM_SMALL + 1])]
    ffn0_copies = [
        pltpu.make_async_copy(wg32.at[:, pl.ds(0, 128)], wg_s.at[:, pl.ds(0, 128)], sems.at[SEM_FFN0]),
        pltpu.make_async_copy(wu32.at[:, pl.ds(0, 128)], wu_s.at[:, pl.ds(0, 128)], sems.at[SEM_FFN0]),
        pltpu.make_async_copy(wd32.at[pl.ds(0, 64), :], wd_s.at[pl.ds(0, 64), :], sems.at[SEM_FFN0])]
    ffn_copies = [
        pltpu.make_async_copy(wg32.at[:, pl.ds(128, FF - 128)], wg_s.at[:, pl.ds(128, FF - 128)], sems.at[SEM_FFN]),
        pltpu.make_async_copy(wu32.at[:, pl.ds(128, FF - 128)], wu_s.at[:, pl.ds(128, FF - 128)], sems.at[SEM_FFN]),
        pltpu.make_async_copy(wd32.at[pl.ds(64, FF // 2 - 64), :], wd_s.at[pl.ds(64, FF // 2 - 64), :],
                              sems.at[SEM_FFN])]

    zero_s[0] = 0
    for c in range(4):
        x_first(c).start()
        if c == 0:
            for cp in small_copies:
                cp.start()
            pair_copy(0).start()

    def queue(t0, t1):
        for t in range(t0, t1):
            for p in range(PP * t + 1, PP * t + PP + 1):
                pair_copy(p).start()
            if t >= 2:
                x_piece(t).start()

    queue(0, FIRST_BATCH)
    eps_bf = 1.0013580322265625e-05

    def score16(g, xn):
        wr = jnp.concatenate([wrf_s[...], wrf_s[...]], axis=0)
        score = _rbf(jnp.sum(xn.astype(F32) * wr, axis=1, keepdims=True))
        r_s[...] = jnp.where(lane16 == g, score, r_s[...])

    def layernorm16(rq, dst_ref, dst_row, not_before=None):
        rq = rq if isinstance(rq, int) else pl.multiple_of(rq, 16)
        xf = x_s[pl.ds(rq, 16), :].astype(F32)
        if not_before is not None:
            x0 = _after(pltpu.bitcast(xf[:, 0:128], U32), [not_before], zero_box[0])
            xf = jnp.concatenate([pltpu.bitcast(x0, F32), xf[:, 128:]], axis=1)
        mean = jnp.sum(xf, axis=1, keepdims=True) * (1.0 / D)
        cen = xf - mean
        var = jnp.sum(cen * cen, axis=1, keepdims=True) * (1.0 / D)
        v = _rbf(_rbf(var) + eps_bf)
        rs = lax.rsqrt(v)
        sd = v * rs
        sd = _rbf(sd + 0.5 * rs * (v - sd * sd))
        inv = pl.reciprocal(sd, approx=True)
        inv = inv * (2.0 - sd * inv)
        xn = (_rbf(xf - _rbf(mean)) * inv).astype(BF)
        if dst_ref is hbuf:
            score16(rq // 16, xn)
        xp = _b2u(xn)
        hq = rq // 2 if isinstance(rq, int) else pl.multiple_of(rq // 2, 8)
        dst_row = dst_row if isinstance(dst_row, int) else pl.multiple_of(dst_row, 8)
        for k in range(KT):
            if dst_ref is hbuf:
                xn_t[k, pl.ds(hq, 8), :] = xp[:, 128 * k:128 * (k + 1)]
            dst_ref[k, pl.ds(dst_row, 8), :] = xp[:, 128 * k:128 * (k + 1)]

    zero_box = [None]

    def fresh_zero():
        zero_box[0] = jnp.full((8, 128), zero_s[0], jnp.int32).astype(U32)

    r_s[...] = jnp.full(r_s.shape, -jnp.inf, F32)
    lane16 = lax.broadcasted_iota(jnp.int32, (16, 128), 1)

    x_first(0).wait()
    for q in range(8):
        layernorm16(16 * q, xn_pre, 8 * q)


    def relayout(src, dst, j, k, not_before=None):
        a = src[j, pl.ds(128 * k, 64, stride=2), :]
        if not_before is not None:
            a = a | jnp.concatenate([not_before & zero_box[0]] * 8, axis=0)
        b = src[j, pl.ds(128 * k + 1, 64, stride=2), :]
        rows = pl.ds(64 * k, 64)
        dst[2 * j, rows, :] = (a & jnp.uint32(0xFFFF)) | (b << 16)
        dst[2 * j + 1, rows, :] = (a >> 16) | (b & jnp.uint32(0xFFFF0000))

    def pre_dot(w_view, ring_view, h, row, dep=None):
        lhs = jnp.concatenate([_u2b(xn_pre[kk, pl.ds(row, 64), :]) for kk in range(KT)], axis=1)
        y = _dot(lhs, _u2b(_after(w_view[h], dep, zero_box[0])))
        yp = _b2u(y.astype(BF))
        ring_view[h, pl.ds(32 + row, 64), :] = yp
        return yp[0:8]

    for c in small_copies:
        c.wait()
    pair_copy(0).wait()
    for k in range(8):
        relayout(raw, wqkv, 0, k)
    wrf_s[...] = jnp.broadcast_to(wr_s[...].astype(F32).reshape(1, D), (8, D))

    def start_body(c, carry):
        x_first(c).wait()
        row = pl.multiple_of(64 * (c - 1), 64)
        for h in range(2):
            pre_dot(wqkv, ring, h, row)
        for q in range(8):
            layernorm16(2 * row + 128 + 16 * q, xn_pre, row + 64 + 8 * q)
        return carry

    lax.fori_loop(1, PRE // 128, start_body, 0)

    def second_batch():
        queue(FIRST_BATCH, NPRE)
        for n in range(KT):
            wo_copy(n).start()
        for cp in ffn0_copies + ffn_copies:
            cp.start()

    def pre_iter(t, first):
        deps = {}
        raw_view = raw.at[pl.ds(PP * t, PP + 1)]
        w_view = wqkv.at[pl.ds(2 * PP * t, 2 * PP + 2)]
        ring_view = ring.at[pl.ds(2 * PP * t, 2 * PP)]
        done = None
        for v in range(6 if first else 0, 8 * PP):
            h, row = v // 4, 64 * (v % 4)
            if first and v < 8:
                h, row = v - 6, 192
            if v == 0 or (first and v in BARRIERS0):
                if v:
                    for p in BARRIERS0[v]:
                        pair_copy(p).wait()
                    if v == max(BARRIERS0):
                        second_batch()
                fresh_zero()
                done = None
            prev = done
            done = pre_dot(w_view, ring_view, h, row, deps.get(v))
            for jr, kr in (REL_SCHED0 if first else REL_SCHED).get(v, ()):
                relayout(raw_view, w_view, jr + 1, kr, prev)
                deps.setdefault(v + REL_LAG, []).append(w_view[2 * jr + 3, pl.ds(64 * kr + 56, 8), :])
            if first:
                continue
            if v in LN_SCHED:
                q = LNP * (t - 2) + LN_SCHED.index(v)
                hrow = pl.multiple_of(jnp.where(q < 0, XS, 32 * (q // 3) + 8 * (q % 3)), 8)
                layernorm16(PRE + 16 * q, hbuf, hrow, done if prev is not None else None)
                deps.setdefault(v + LN_LAG, []).append(hbuf[KT - 1, pl.ds(hrow, 8), :])
            if v in SCORE_SCHED:
                g = jnp.minimum(len(SCORE_SCHED) * (t - 1) + SCORE_SCHED.index(v), PRE // 16 - LNP - 1)
                rows = pl.ds(pl.multiple_of(8 * g, 8), 8)
                xp = [xn_pre[kk, rows, :] for kk in range(KT)]
                xp[0] = xp[0] | (done & zero_box[0])
                for kk in range(KT):
                    xn_t[kk, rows, :] = xp[kk]
                score16(g, _u2b(jnp.concatenate(xp, axis=1)))

    pre_iter(0, True)

    def pre_body(t, carry):
        pairs_wait(t)

        @pl.when(t >= 2)
        def _():
            x_piece(t).wait()
        pre_iter(t, False)
        return carry

    lax.fori_loop(1, NPRE, pre_body, 0)
    row = lax.broadcasted_iota(jnp.int32, (80, 80), 0)
    col = lax.broadcasted_iota(jnp.int32, (80, 80), 1)
    same_head = (jnp.where(row < 64, row >> 5, (row - 64) >> 3)
                 == jnp.where(col < 64, col >> 5, (col - 64) >> 3))
    allowed = same_head & ((col >= 64) | (row >= 64) | (col <= row))
    fill = jnp.where(same_head, -1e9, -jnp.inf).astype(F32)
    low_half = lax.broadcasted_iota(jnp.int32, (8, 128), 0) < 4
    high_half = jnp.logical_not(low_half)
    scale = DH ** -0.5

    def load_row(t):
        w = jnp.concatenate([xn_t[k, pl.ds(t // 2, 1), :] for k in range(KT)], axis=1)
        bits = jnp.where(t % 2 == 0, w << 16, w & jnp.uint32(0xFFFF0000))
        return pltpu.bitcast(bits, F32), w

    def select_tokens():
        r = r_s[...]
        tok = lane16 * 16 + lax.broadcasted_iota(jnp.int32, (16, 128), 0)

        def full(op, v):
            return op(op(v, axis=0, keepdims=True), axis=1, keepdims=True)

        top1 = full(jnp.max, r)
        idx1 = full(jnp.min, jnp.where(r == top1, tok, S - 1))
        r2 = jnp.where(tok == idx1, -jnp.inf, r)
        top2 = full(jnp.max, r2)
        idx2 = full(jnp.min, jnp.where((r2 == top2) & (tok != idx1), tok, S - 1))
        first = lax.broadcasted_iota(jnp.int32, (8, 128), 0) == 0
        gate_s[...] = jnp.where(first, top1, top2)
        sel_s[...] = jnp.where(first, idx1, idx2)

    NIT = NSEG // UNROLL
    ROWS = SEG * UNROLL

    def half_rows(r0):
        return pl.multiple_of(r0 // 2, 8)

    def residual(xf, a, b):
        return (_rbf(xf + a) + b).astype(BF)

    def out_copy(j):
        r0, n = (0, S - 2 * ROWS) if j == 0 else (S - (3 - j) * ROWS, ROWS)
        return pltpu.make_async_copy(out_s.at[pl.ds(r0, n), :], out_hbm.at[pl.ds(r0, n), :],
                                     sems.at[SEM_OUT + j])

    def ffn_groups(i, y):
        x_sel = xsel_s[...]
        live = (i >= 1) & (i < NIT - 1)
        hid = {}

        def up(w_ref, j, key):
            cols = pl.ds(pl.multiple_of(128 * j, 128), 128)
            part = _dot(x_sel[:, 0:512], _u2b(w_ref[pl.ds(0, 256), cols]).astype(F32))
            yield
            hid[key] = _rbf(_dot(x_sel[:, 512:1024], _u2b(w_ref[pl.ds(256, 256), cols]).astype(F32)) + part)
            yield

        for jj in range(2):
            j = jnp.clip(2 * (i - 1) + jj, 0, FT - 1)
            yield from up(wg_s, j, "g")
            yield from up(wu_s, j, "u")
            g = hid["g"]
            hb = jnp.where(live, _rbf(_rbf(g * _rbf(jax.nn.sigmoid(g))) * hid["u"]), 0.0)
            rows = pl.ds(pl.multiple_of(64 * j, 64), 64)
            yield
            for half in range(2):
                y[half] = _dot(hb, _u2b(wd_s[rows, pl.ds(512 * half, 512)]).astype(F32)) + y[half]
                yield

    def one_step(i, u, mem, held, side):
        odd = u % 2
        s2 = i * (UNROLL // 2) + u // 2
        h_ld = pl.multiple_of(16 * UNROLL * i, 32) + 32 * (u // 2)
        r24 = pl.multiple_of((12 * UNROLL * i) % RING32, 8) + XS * (u // 2)
        qkv_ld = pl.multiple_of((SEG * s2 + 32) % RING32, 32) + 16 * odd
        m0 = 0 if odd else XS

        def with_mem(lo, hi, m):
            if odd:
                return [jnp.where(low_half, m, lo), hi]
            return [lo, jnp.where(low_half, hi, m)]

        def store_tokens(ref, idx, base, yp):
            if odd:
                pltpu.store(ref.at[idx, pl.ds(base + 8, 8), :], yp[0:8], mask=high_half)
                ref[idx, pl.ds(base + 16, yp.shape[0] - 8), :] = yp[8:]
            else:
                ref[idx, pl.ds(base, 8), :] = yp[0:8]
                pltpu.store(ref.at[idx, pl.ds(base + 8, 8), :], yp[8:16], mask=low_half)

        lk = [_u2b(jnp.concatenate(with_mem(hbuf[k, pl.ds(h_ld + 8 * odd, 8), :],
                                            hbuf[k, pl.ds(h_ld + 8 + 8 * odd, 8), :], mem[k]), axis=0))
              for k in range(KT)]
        lhs = jnp.concatenate(lk, axis=1)

        ymem = {}
        xs = {}
        probs = {}
        parts = {}

        def proj(h):
            split = h < K_SPLIT and u > 0
            if split:
                lhs7 = jnp.concatenate(lk[:KT - 1], axis=1)
                head = [_dot(lhs7, _u2b(wqkv[m * H + h, pl.ds(0, 448), :])) for m in range(3)]
            for m in range(3):
                if split:
                    y = _dot(lk[KT - 1], _u2b(wqkv[m * H + h, pl.ds(448, 64), :])) + head[m]
                else:
                    y = _dot(lhs, _u2b(wqkv[m * H + h]))
                store_tokens(ring, m * H + h, r24, _b2u(y.astype(BF)))
                ymem[(h, m)] = y[m0:m0 + MEM]
                xs[(h, m)] = ring[m * H + h, pl.ds(qkv_ld, SEG // 2), :]

        def pair(p, m):
            a, b = 2 * p, 2 * p + 1
            mm = jnp.concatenate([ymem[(a, m)], ymem[(b, m)]], axis=0).astype(BF)
            return jnp.concatenate([_u2b(xs[(a, m)]), _u2b(xs[(b, m)]), mm], axis=0)

        def qk(p):
            sc = _dot_nt(pair(p, 0), pair(p, 1))
            sc = jnp.where(allowed, sc * scale, fill)
            e = jnp.exp(sc - jnp.max(sc, axis=1, keepdims=True))
            l = jnp.sum(e, axis=1, keepdims=True)
            r = pl.reciprocal(l, approx=True)
            r = r * (2.0 - l * r)
            probs[p] = (e * r).astype(BF)

        def pv(p):
            op = _b2u(_dot(probs[p], pair(p, 2)).astype(BF))
            om = op[32:40]
            om_sw = pltpu.roll(om, 4, axis=0)
            for j, h in enumerate((2 * p, 2 * p + 1)):
                x0, x1 = op[16 * j:16 * j + 8], op[16 * j + 8:16 * j + 16]
                m = om if j != odd else om_sw
                if odd:
                    rows = with_mem(held[h], x0, m) + [x1]
                else:
                    rows = with_mem(x0, x1, m)
                    held[h] = x1
                parts[h] = _u2b(jnp.concatenate(rows, axis=0))

        def after(t):
            for lag, fn in ((LAG_QK, qk), (LAG_PV, pv)):
                if (t - 1 - lag) % 2 == 0 and 0 <= (t - 1 - lag) // 2 < NPAIR:
                    fn((t - 1 - lag) // 2)

        def side_group():
            if odd:
                next(side, None)

        for t in range(H):
            proj(t)
            after(t)
            if u == 0 and t == 8:
                select_tokens()
        t = H
        n_part, h_split = (N_PART_ODD, H_SPLIT_ODD) if odd else (N_PART, H_SPLIT)
        lhs_a = jnp.concatenate([parts[j] for j in range(h_split)], axis=1)
        acc = []
        for n in range(n_part):
            acc.append(_dot(lhs_a, _u2b(wo_s[n, pl.ds(0, h_split * 64), :])))
            after(t)
            side_group()
            t += 1
        while t - 1 - LAG_PV <= 2 * (NPAIR - 1):
            after(t)
            t += 1
        lhs_b = jnp.concatenate([parts[j] for j in range(h_split, H)], axis=1)
        lhs_o = jnp.concatenate([lhs_a, lhs_b], axis=1)
        new_mem = [None] * KT
        pair_row = pl.multiple_of(ROWS * i, 64) + 64 * (u // 2)

        def finish(n, y):
            ym = y[m0:m0 + MEM]
            new_mem[n] = _b2u(jnp.concatenate([ym, ym], axis=0).astype(BF))
            yb = y.astype(BF)
            store_tokens(abuf, n, h_ld, _b2u(yb))
            cols = pl.ds(128 * n, 128)
            lo, cnt = (XS, 2 * SEG - XS) if odd else (0, XS)
            rows = pl.ds(pl.multiple_of(pair_row + lo, 8), cnt)
            a = yb.astype(F32)
            b = _u2b(xn_t[n, pl.ds(h_ld + 8 * odd, y.shape[0] // 2), :]).astype(F32)
            sl = slice(MEM, MEM + cnt) if odd else slice(0, cnt)
            out_s[rows, cols] = residual(x_s[rows, cols].astype(F32), a[sl], b[sl])

        order = list(range(n_part, KT))
        for n in order:
            finish(n, _dot(lhs_o, _u2b(wo_s[n])))
            if n < KT - 1:
                side_group()
            if n == n_part:
                for n2 in range(n_part):
                    tail = _u2b(wo_s[n2, pl.ds(h_split * 64, (H - h_split) * 64), :])
                    finish(n2, _dot(lhs_b, tail) + acc[n2])
        return new_mem

    def patch_row(t, yrow):
        xr, w = load_row(t)
        bits = pltpu.bitcast(_rbf(xr + yrow), U32)
        w = jnp.where(t % 2 == 0,
                      (w & jnp.uint32(0xFFFF0000)) | (bits >> 16),
                      (w & jnp.uint32(0xFFFF)) | bits)
        for k in range(KT):
            xn_t[k, pl.ds(t // 2, 1), :] = w[:, 128 * k:128 * (k + 1)]

    def fix_copy(j, r0):
        return pltpu.make_async_copy(out_s.at[pl.ds(r0, 16), :], out_hbm.at[pl.ds(r0, 16), :],
                                     sems.at[SEM_FIX + j])

    def gather_tokens():
        for cp in ffn_copies:
            cp.wait()
        idx_s[0] = sel_s[0, 0]
        idx_s[1] = sel_s[1, 0]
        sel_row = lax.broadcasted_iota(jnp.int32, (8, D), 0)
        xs1, _ = load_row(idx_s[0])
        xs2, _ = load_row(idx_s[1])
        xsel_s[...] = jnp.where(sel_row == 0, xs1, jnp.where(sel_row == 1, xs2, 0.0))

    def apply_ffn():
        out_copy(0).wait()
        patch_row(idx_s[0], yy_s[0:1, :])
        patch_row(idx_s[1], yy_s[1:2, :])
        blks = [idx_s[j] >> 4 for j in range(2)]
        for blk in blks:
            r0 = pl.multiple_of(jnp.minimum(blk, (S - ROWS) // 16 - 1) * 16, 16)
            for n in range(KT):
                cols = pl.ds(128 * n, 128)
                out_s[pl.ds(r0, 16), cols] = residual(
                    x_s[pl.ds(r0, 16), cols].astype(F32),
                    _u2b(abuf[n, pl.ds(half_rows(r0), 8), :]).astype(F32),
                    _u2b(xn_t[n, pl.ds(half_rows(r0), 8), :]).astype(F32))
        blk1, blk2 = [jnp.minimum(blk, (S - 2 * ROWS) // 16 - 1) for blk in blks]
        blk2 = jnp.where(blk2 == blk1, jnp.where(blk1 == 0, 1, blk1 - 1), blk2)
        for j, blk in enumerate((blk1, blk2)):
            fix_copy(j, pl.multiple_of(blk * 16, 16)).start()
        out_copy(1).start()

    def body(i, carry):
        mem, y = list(carry[:KT]), list(carry[KT:])

        @pl.when((i == 1) | (i >= NIT - 2))
        def _():
            pl.when(i == 1)(gather_tokens)
            pl.when(i == NIT - 2)(lambda: out_copy(0).start())
            pl.when(i == NIT - 1)(apply_ffn)

        side = ffn_groups(i, y)
        held = {}
        for u in range(UNROLL):
            mem = one_step(i, u, mem, held, side)
        for _ in side:
            raise AssertionError("ffn groups left over")
        gate = _rbf(jax.nn.sigmoid(gate_s[:, 0:1]))
        yy_s[...] = _rbf(_rbf(jnp.concatenate(y, axis=1)) * gate)
        return tuple(mem) + tuple(y)

    for n in range(KT):
        wo_copy(n).wait()
    for cp in ffn0_copies:
        cp.wait()
    xsel_s[...] = jnp.zeros(xsel_s.shape, F32)
    mi = mem0_s[...].astype(F32)
    mip = _b2u(jnp.concatenate([mi, mi], axis=0).astype(BF))
    lax.fori_loop(0, NIT, body,
                  tuple(mip[:, 128 * k:128 * (k + 1)] for k in range(KT))
                  + (jnp.zeros((8, 512), F32), jnp.zeros((8, 512), F32)))
    out_copy(2).start()
    for j in range(2):
        fix_copy(j, 0).wait()
    out_copy(1).wait()
    out_copy(2).wait()


@jax.jit
def pallas_parallel_sum__memory_aug_recurrent_mem_tr__moe_arch_mod__prompt_kernel(
    A_x: jax.Array,
    A_mem0: jax.Array,
    A_Wq: jax.Array,
    A_Wk: jax.Array,
    A_Wv: jax.Array,
    A_Wo: jax.Array,
    A_seg_len: jax.Array,
    B_x: jax.Array,
    B_w_r: jax.Array,
    B_w_gate: jax.Array,
    B_w_up: jax.Array,
    B_w_down: jax.Array,
):
    del A_seg_len, B_x
    assert A_x.shape == (1, S, D) and A_mem0.shape == (1, MEM, D)
    assert A_Wq.shape == (D, H, DH) and A_Wo.shape == (H, DH, D)
    assert B_w_gate.shape == (D, FF) and B_w_down.shape == (FF, D)
    any_spec = pl.BlockSpec(memory_space=pl.ANY)
    out = pl.pallas_call(
        _kernel,
        out_shape=jax.ShapeDtypeStruct((S, D), BF),
        in_specs=[any_spec] * 10,
        out_specs=any_spec,
        scratch_shapes=[
            pltpu.VMEM((S, D), BF),
            pltpu.VMEM((KT, S // 2, 128), U32),
            pltpu.VMEM((KT, PRE // 2, 128), U32),
            pltpu.VMEM((KT, 16 * NSEG, 128), U32),
            pltpu.VMEM((3 * H + 2, D // 2, 128), U32),
            pltpu.VMEM((KT, H * DH // 2, 128), U32),
            pltpu.VMEM((3 * H, RING32, 128), U32),
            pltpu.VMEM((KT, S // 2, 128), U32),
            pltpu.VMEM((S, D), BF),
            pltpu.VMEM((NPQ + 1, D, 128), U32),
            pltpu.VMEM((D // 2, FF), U32),
            pltpu.VMEM((D // 2, FF), U32),
            pltpu.VMEM((FF // 2, D), U32),
            pltpu.VMEM((MEM, D), BF),
            pltpu.VMEM((D,), BF),
            pltpu.VMEM((8, D), F32),
            pltpu.VMEM((16, 128), F32),
            pltpu.VMEM((8, 128), jnp.int32),
            pltpu.VMEM((8, 128), F32),
            pltpu.VMEM((8, D), F32),
            pltpu.VMEM((8, D), F32),
            pltpu.SMEM((1,), jnp.int32),
            pltpu.SMEM((2,), jnp.int32),
            pltpu.SemaphoreType.DMA((NSEM,)),
        ],
        compiler_params=pltpu.CompilerParams(vmem_limit_bytes=126 * 1024 * 1024,
                                             disable_bounds_checks=True, disable_semaphore_checks=True),
    )(A_x.reshape(S, D), A_mem0.reshape(MEM, D), A_Wq, A_Wk, A_Wv, A_Wo.reshape(H * DH, D),
      B_w_r, B_w_gate, B_w_up, B_w_down)
    return out.reshape(1, S, D)
```

```python
import jax
import jax.numpy as jnp
from jax import lax
import jax.experimental.pallas as pl
import jax.experimental.pallas.tpu as pltpu

BF = jnp.bfloat16
U32 = jnp.uint32
F32 = jnp.float32

S = 2048
D = 1024
H = 32
DH = 128
MEM = 8
SEG = 32
NSEG = S // SEG
FF = 3584
KT = D // 128
FT = FF // 128
XS = 24
PRE = S - NSEG * XS
RING = 576
RING32 = RING // 2
NPAIR = H // 2
NPQ = 3 * NPAIR
PP = 6
NPRE = NPQ // PP
LNP = 16
SEM_SMALL, SEM_X0, SEM_X = 0, 2, 6
SEM_W0 = SEM_X + NPRE
SEM_W = SEM_W0 + PP
SEM_WO = SEM_W + NPRE
SEM_FFN0, SEM_FFN, SEM_FIX, SEM_OUT = SEM_WO + 1, SEM_WO + 2, SEM_WO + 3, SEM_WO + 5
NSEM = SEM_OUT + 3

LAG_QK = 1
LAG_PV = 4
N_PART, H_SPLIT = 4, 26
N_PART_ODD, H_SPLIT_ODD = 4, 24
K_SPLIT = 2
UNROLL = 4

REL_SCHED = {0: [(0, 0), (0, 1)], 1: [(0, 2), (0, 3)], 2: [(0, 4)], 3: [(0, 5)], 4: [(0, 6)], 5: [(0, 7)]}
REL_SCHED.update({8 * j - 2 + k: [(j, k)] for j in range(1, PP) for k in range(8)})
REL_SCHED0 = {6: [(0, k) for k in range(8)],
              13: [(1, k) for k in range(8)],
              26: [(3, k) for k in range(3)], 27: [(3, k) for k in range(3, 6)], 28: [(3, 6), (3, 7)]}
REL_SCHED0.update({8 * j - 2 + k: [(j, k)] for j in (2, 4, 5) for k in range(8)})
BARRIERS0 = {6: [1], 13: [2, 3], 26: [4, 5, 6]}
SCORE_SCHED = [1, 16, 31]
LN_SCHED = [11 * q // 4 for q in range(LNP)]
LN_LAG = 5
REL_LAG = 2
FIRST_BATCH = 6


def _b2u(x):
    return pltpu.bitcast(x, U32)


def _u2b(x):
    return pltpu.bitcast(x, BF)


def _dot(a, b):
    return jnp.dot(a, b, preferred_element_type=F32)


def _dot_nt(a, b):
    return lax.dot_general(a, b, (((1,), (1,)), ((), ())), preferred_element_type=F32)


def _after(w, dep, zero):
    if not dep:
        return w
    d = dep[0]
    for e in dep[1:]:
        d = d | e
    return jnp.concatenate([w[0:8] | (d & zero), w[8:]], axis=0)


def _rbf(x):
    return x.astype(BF).astype(F32)


def _kernel(x_hbm, mem0_hbm, wq_hbm, wk_hbm, wv_hbm, wo_hbm, wr_hbm, wg_hbm, wu_hbm, wd_hbm,
            out_hbm,
            x_s, xn_t, xn_pre, hbuf, wqkv, wo_s, ring, abuf, out_s, raw,
            wg_s, wu_s, wd_s, mem0_s, wr_s, wrf_s, r_s, sel_s, gate_s, xsel_s, yy_s, zero_s, idx_s,
            sems):
    w32 = [w.bitcast(U32) for w in (wq_hbm, wk_hbm, wv_hbm)]
    wo32 = wo_hbm.bitcast(U32)
    wg32 = wg_hbm.bitcast(U32)
    wu32 = wu_hbm.bitcast(U32)
    wd32 = wd_hbm.bitcast(U32)

    def rows_copy(r0, n, sem):
        return pltpu.make_async_copy(x_hbm.at[pl.ds(r0, n), :], x_s.at[pl.ds(r0, n), :], sems.at[sem])

    def x_first(c):
        return rows_copy(128 * c if isinstance(c, int) else pl.multiple_of(128 * c, 128), 128, SEM_X0 + c)

    def x_piece(t):
        r0 = PRE + 16 * LNP * (t - 2)
        return rows_copy(r0 if isinstance(t, int) else pl.multiple_of(r0, 256), 16 * LNP, SEM_X + t)

    def pair_copy(p):
        q = min(p, NPQ - 1)
        sem = SEM_W0 + p if p <= PP else SEM_W + (p - 1) // PP
        return pltpu.make_async_copy(w32[q // NPAIR].at[:, q % NPAIR, :], raw.at[p], sems.at[sem])

    def pairs_wait(t):
        dst = raw.at[pl.ds(PP * t + 1, PP)]
        pltpu.make_async_copy(dst, dst, sems.at[SEM_W + t]).wait()

    def wo_copy(n):
        return pltpu.make_async_copy(wo32.at[:, pl.ds(128 * n, 128)], wo_s.at[n], sems.at[SEM_WO])

    small_copies = [pltpu.make_async_copy(mem0_hbm, mem0_s, sems.at[SEM_SMALL]),
                    pltpu.make_async_copy(wr_hbm, wr_s, sems.at[SEM_SMALL + 1])]
    ffn0_copies = [
        pltpu.make_async_copy(wg32.at[:, pl.ds(0, 128)], wg_s.at[:, pl.ds(0, 128)], sems.at[SEM_FFN0]),
        pltpu.make_async_copy(wu32.at[:, pl.ds(0, 128)], wu_s.at[:, pl.ds(0, 128)], sems.at[SEM_FFN0]),
        pltpu.make_async_copy(wd32.at[pl.ds(0, 64), :], wd_s.at[pl.ds(0, 64), :], sems.at[SEM_FFN0])]
    ffn_copies = [
        pltpu.make_async_copy(wg32.at[:, pl.ds(128, FF - 128)], wg_s.at[:, pl.ds(128, FF - 128)], sems.at[SEM_FFN]),
        pltpu.make_async_copy(wu32.at[:, pl.ds(128, FF - 128)], wu_s.at[:, pl.ds(128, FF - 128)], sems.at[SEM_FFN]),
        pltpu.make_async_copy(wd32.at[pl.ds(64, FF // 2 - 64), :], wd_s.at[pl.ds(64, FF // 2 - 64), :],
                              sems.at[SEM_FFN])]

    zero_s[0] = 0
    for c in range(4):
        x_first(c).start()
        if c == 0:
            for cp in small_copies:
                cp.start()
            pair_copy(0).start()

    def queue(t0, t1):
        for t in range(t0, t1):
            for p in range(PP * t + 1, PP * t + PP + 1):
                pair_copy(p).start()
            if t >= 2:
                x_piece(t).start()

    queue(0, FIRST_BATCH)
    eps_bf = 1.0013580322265625e-05

    def score16(g, xn):
        wr = jnp.concatenate([wrf_s[...], wrf_s[...]], axis=0)
        score = _rbf(jnp.sum(xn.astype(F32) * wr, axis=1, keepdims=True))
        r_s[...] = jnp.where(lane16 == g, score, r_s[...])

    def layernorm16(rq, dst_ref, dst_row, not_before=None):
        rq = rq if isinstance(rq, int) else pl.multiple_of(rq, 16)
        xf = x_s[pl.ds(rq, 16), :].astype(F32)
        if not_before is not None:
            x0 = _after(pltpu.bitcast(xf[:, 0:128], U32), [not_before], zero_box[0])
            xf = jnp.concatenate([pltpu.bitcast(x0, F32), xf[:, 128:]], axis=1)
        mean = jnp.sum(xf, axis=1, keepdims=True) * (1.0 / D)
        cen = xf - mean
        var = jnp.sum(cen * cen, axis=1, keepdims=True) * (1.0 / D)
        v = _rbf(_rbf(var) + eps_bf)
        rs = lax.rsqrt(v)
        sd = v * rs
        sd = _rbf(sd + 0.5 * rs * (v - sd * sd))
        inv = pl.reciprocal(sd, approx=True)
        inv = inv * (2.0 - sd * inv)
        xn = (_rbf(xf - _rbf(mean)) * inv).astype(BF)
        if dst_ref is hbuf:
            score16(rq // 16, xn)
        xp = _b2u(xn)
        hq = rq // 2 if isinstance(rq, int) else pl.multiple_of(rq // 2, 8)
        dst_row = dst_row if isinstance(dst_row, int) else pl.multiple_of(dst_row, 8)
        for k in range(KT):
            if dst_ref is hbuf:
                xn_t[k, pl.ds(hq, 8), :] = xp[:, 128 * k:128 * (k + 1)]
            dst_ref[k, pl.ds(dst_row, 8), :] = xp[:, 128 * k:128 * (k + 1)]

    zero_box = [None]

    def fresh_zero():
        zero_box[0] = jnp.full((8, 128), zero_s[0], jnp.int32).astype(U32)

    r_s[...] = jnp.full(r_s.shape, -jnp.inf, F32)
    lane16 = lax.broadcasted_iota(jnp.int32, (16, 128), 1)

    x_first(0).wait()
    for q in range(8):
        layernorm16(16 * q, xn_pre, 8 * q)


    def relayout(src, dst, j, k, not_before=None):
        a = src[j, pl.ds(128 * k, 64, stride=2), :]
        if not_before is not None:
            a = a | jnp.concatenate([not_before & zero_box[0]] * 8, axis=0)
        b = src[j, pl.ds(128 * k + 1, 64, stride=2), :]
        rows = pl.ds(64 * k, 64)
        dst[2 * j, rows, :] = (a & jnp.uint32(0xFFFF)) | (b << 16)
        dst[2 * j + 1, rows, :] = (a >> 16) | (b & jnp.uint32(0xFFFF0000))

    def pre_dot(w_view, ring_view, h, row, dep=None):
        lhs = jnp.concatenate([_u2b(xn_pre[kk, pl.ds(row, 64), :]) for kk in range(KT)], axis=1)
        y = _dot(lhs, _u2b(_after(w_view[h], dep, zero_box[0])))
        yp = _b2u(y.astype(BF))
        ring_view[h, pl.ds(32 + row, 64), :] = yp
        return yp[0:8]

    for c in small_copies:
        c.wait()
    pair_copy(0).wait()
    for k in range(8):
        relayout(raw, wqkv, 0, k)
    wrf_s[...] = jnp.broadcast_to(wr_s[...].astype(F32).reshape(1, D), (8, D))

    def start_body(c, carry):
        x_first(c).wait()
        row = pl.multiple_of(64 * (c - 1), 64)
        for h in range(2):
            pre_dot(wqkv, ring, h, row)
        for q in range(8):
            layernorm16(2 * row + 128 + 16 * q, xn_pre, row + 64 + 8 * q)
        return carry

    lax.fori_loop(1, PRE // 128, start_body, 0)

    def second_batch():
        queue(FIRST_BATCH, NPRE)
        for n in range(KT):
            wo_copy(n).start()
        for cp in ffn0_copies + ffn_copies:
            cp.start()

    def pre_iter(t, first):
        deps = {}
        raw_view = raw.at[pl.ds(PP * t, PP + 1)]
        w_view = wqkv.at[pl.ds(2 * PP * t, 2 * PP + 2)]
        ring_view = ring.at[pl.ds(2 * PP * t, 2 * PP)]
        done = None
        for v in range(6 if first else 0, 8 * PP):
            h, row = v // 4, 64 * (v % 4)
            if first and v < 8:
                h, row = v - 6, 192
            if v == 0 or (first and v in BARRIERS0):
                if v:
                    for p in BARRIERS0[v]:
                        pair_copy(p).wait()
                    if v == max(BARRIERS0):
                        second_batch()
                fresh_zero()
                done = None
            prev = done
            done = pre_dot(w_view, ring_view, h, row, deps.get(v))
            for jr, kr in (REL_SCHED0 if first else REL_SCHED).get(v, ()):
                relayout(raw_view, w_view, jr + 1, kr, prev)
                deps.setdefault(v + REL_LAG, []).append(w_view[2 * jr + 3, pl.ds(64 * kr + 56, 8), :])
            if first:
                continue
            if v in LN_SCHED:
                q = LNP * (t - 2) + LN_SCHED.index(v)
                hrow = pl.multiple_of(jnp.where(q < 0, XS, 32 * (q // 3) + 8 * (q % 3)), 8)
                layernorm16(PRE + 16 * q, hbuf, hrow, done if prev is not None else None)
                deps.setdefault(v + LN_LAG, []).append(hbuf[KT - 1, pl.ds(hrow, 8), :])
            if v in SCORE_SCHED:
                g = jnp.minimum(len(SCORE_SCHED) * (t - 1) + SCORE_SCHED.index(v), PRE // 16 - LNP - 1)
                rows = pl.ds(pl.multiple_of(8 * g, 8), 8)
                xp = [xn_pre[kk, rows, :] for kk in range(KT)]
                xp[0] = xp[0] | (done & zero_box[0])
                for kk in range(KT):
                    xn_t[kk, rows, :] = xp[kk]
                score16(g, _u2b(jnp.concatenate(xp, axis=1)))

    pre_iter(0, True)

    def pre_body(t, carry):
        pairs_wait(t)

        @pl.when(t >= 2)
        def _():
            x_piece(t).wait()
        pre_iter(t, False)
        return carry

    lax.fori_loop(1, NPRE, pre_body, 0)
    row = lax.broadcasted_iota(jnp.int32, (80, 80), 0)
    col = lax.broadcasted_iota(jnp.int32, (80, 80), 1)
    same_head = (jnp.where(row < 64, row >> 5, (row - 64) >> 3)
                 == jnp.where(col < 64, col >> 5, (col - 64) >> 3))
    allowed = same_head & ((col >= 64) | (row >= 64) | (col <= row))
    fill = jnp.where(same_head, -1e9, -jnp.inf).astype(F32)
    low_half = lax.broadcasted_iota(jnp.int32, (8, 128), 0) < 4
    high_half = jnp.logical_not(low_half)
    scale = DH ** -0.5

    def load_row(t):
        w = jnp.concatenate([xn_t[k, pl.ds(t // 2, 1), :] for k in range(KT)], axis=1)
        bits = jnp.where(t % 2 == 0, w << 16, w & jnp.uint32(0xFFFF0000))
        return pltpu.bitcast(bits, F32), w

    def select_tokens():
        r = r_s[...]
        tok = lane16 * 16 + lax.broadcasted_iota(jnp.int32, (16, 128), 0)

        def full(op, v):
            return op(op(v, axis=0, keepdims=True), axis=1, keepdims=True)

        top1 = full(jnp.max, r)
        idx1 = full(jnp.min, jnp.where(r == top1, tok, S - 1))
        r2 = jnp.where(tok == idx1, -jnp.inf, r)
        top2 = full(jnp.max, r2)
        idx2 = full(jnp.min, jnp.where((r2 == top2) & (tok != idx1), tok, S - 1))
        first = lax.broadcasted_iota(jnp.int32, (8, 128), 0) == 0
        gate_s[...] = jnp.where(first, top1, top2)
        sel_s[...] = jnp.where(first, idx1, idx2)

    NIT = NSEG // UNROLL
    ROWS = SEG * UNROLL

    def half_rows(r0):
        return pl.multiple_of(r0 // 2, 8)

    def residual(xf, a, b):
        return (_rbf(xf + a) + b).astype(BF)

    def out_copy(j):
        r0, n = (0, S - 2 * ROWS) if j == 0 else (S - (3 - j) * ROWS, ROWS)
        return pltpu.make_async_copy(out_s.at[pl.ds(r0, n), :], out_hbm.at[pl.ds(r0, n), :],
                                     sems.at[SEM_OUT + j])

    def ffn_groups(i, y):
        x_sel = xsel_s[...]
        live = (i >= 1) & (i < NIT - 1)
        hid = {}

        def up(w_ref, j, key):
            cols = pl.ds(pl.multiple_of(128 * j, 128), 128)
            part = _dot(x_sel[:, 0:512], _u2b(w_ref[pl.ds(0, 256), cols]).astype(F32))
            yield
            hid[key] = _rbf(_dot(x_sel[:, 512:1024], _u2b(w_ref[pl.ds(256, 256), cols]).astype(F32)) + part)
            yield

        for jj in range(2):
            j = jnp.clip(2 * (i - 1) + jj, 0, FT - 1)
            yield from up(wg_s, j, "g")
            yield from up(wu_s, j, "u")
            g = hid["g"]
            hb = jnp.where(live, _rbf(_rbf(g * _rbf(jax.nn.sigmoid(g))) * hid["u"]), 0.0)
            rows = pl.ds(pl.multiple_of(64 * j, 64), 64)
            yield
            for half in range(2):
                y[half] = _dot(hb, _u2b(wd_s[rows, pl.ds(512 * half, 512)]).astype(F32)) + y[half]
                yield

    def one_step(i, u, mem, held, side):
        odd = u % 2
        s2 = i * (UNROLL // 2) + u // 2
        h_ld = pl.multiple_of(16 * UNROLL * i, 32) + 32 * (u // 2)
        r24 = pl.multiple_of((12 * UNROLL * i) % RING32, 8) + XS * (u // 2)
        qkv_ld = pl.multiple_of((SEG * s2 + 32) % RING32, 32) + 16 * odd
        m0 = 0 if odd else XS

        def with_mem(lo, hi, m):
            if odd:
                return [jnp.where(low_half, m, lo), hi]
            return [lo, jnp.where(low_half, hi, m)]

        def store_tokens(ref, idx, base, yp):
            if odd:
                pltpu.store(ref.at[idx, pl.ds(base + 8, 8), :], yp[0:8], mask=high_half)
                ref[idx, pl.ds(base + 16, yp.shape[0] - 8), :] = yp[8:]
            else:
                ref[idx, pl.ds(base, 8), :] = yp[0:8]
                pltpu.store(ref.at[idx, pl.ds(base + 8, 8), :], yp[8:16], mask=low_half)

        lk = [_u2b(jnp.concatenate(with_mem(hbuf[k, pl.ds(h_ld + 8 * odd, 8), :],
                                            hbuf[k, pl.ds(h_ld + 8 + 8 * odd, 8), :], mem[k]), axis=0))
              for k in range(KT)]
        lhs = jnp.concatenate(lk, axis=1)

        ymem = {}
        xs = {}
        probs = {}
        parts = {}

        def proj(h):
            split = h < K_SPLIT and u > 0
            if split:
                lhs7 = jnp.concatenate(lk[:KT - 1], axis=1)
                head = [_dot(lhs7, _u2b(wqkv[m * H + h, pl.ds(0, 448), :])) for m in range(3)]
            for m in range(3):
                if split:
                    y = _dot(lk[KT - 1], _u2b(wqkv[m * H + h, pl.ds(448, 64), :])) + head[m]
                else:
                    y = _dot(lhs, _u2b(wqkv[m * H + h]))
                store_tokens(ring, m * H + h, r24, _b2u(y.astype(BF)))
                ymem[(h, m)] = y[m0:m0 + MEM]
                xs[(h, m)] = ring[m * H + h, pl.ds(qkv_ld, SEG // 2), :]

        def pair(p, m):
            a, b = 2 * p, 2 * p + 1
            mm = jnp.concatenate([ymem[(a, m)], ymem[(b, m)]], axis=0).astype(BF)
            return jnp.concatenate([_u2b(xs[(a, m)]), _u2b(xs[(b, m)]), mm], axis=0)

        def qk(p):
            sc = _dot_nt(pair(p, 0), pair(p, 1))
            sc = jnp.where(allowed, sc * scale, fill)
            e = jnp.exp(sc - jnp.max(sc, axis=1, keepdims=True))
            l = jnp.sum(e, axis=1, keepdims=True)
            r = pl.reciprocal(l, approx=True)
            r = r * (2.0 - l * r)
            probs[p] = (e * r).astype(BF)

        def pv(p):
            op = _b2u(_dot(probs[p], pair(p, 2)).astype(BF))
            om = op[32:40]
            om_sw = pltpu.roll(om, 4, axis=0)
            for j, h in enumerate((2 * p, 2 * p + 1)):
                x0, x1 = op[16 * j:16 * j + 8], op[16 * j + 8:16 * j + 16]
                m = om if j != odd else om_sw
                if odd:
                    rows = with_mem(held[h], x0, m) + [x1]
                else:
                    rows = with_mem(x0, x1, m)
                    held[h] = x1
                parts[h] = _u2b(jnp.concatenate(rows, axis=0))

        def after(t):
            for lag, fn in ((LAG_QK, qk), (LAG_PV, pv)):
                if (t - 1 - lag) % 2 == 0 and 0 <= (t - 1 - lag) // 2 < NPAIR:
                    fn((t - 1 - lag) // 2)

        def side_group():
            if odd:
                next(side, None)

        for t in range(H):
            proj(t)
            after(t)
            if u == 0 and t == 8:
                select_tokens()
        t = H
        n_part, h_split = (N_PART_ODD, H_SPLIT_ODD) if odd else (N_PART, H_SPLIT)
        lhs_a = jnp.concatenate([parts[j] for j in range(h_split)], axis=1)
        acc = []
        for n in range(n_part):
            acc.append(_dot(lhs_a, _u2b(wo_s[n, pl.ds(0, h_split * 64), :])))
            after(t)
            side_group()
            t += 1
        while t - 1 - LAG_PV <= 2 * (NPAIR - 1):
            after(t)
            t += 1
        lhs_b = jnp.concatenate([parts[j] for j in range(h_split, H)], axis=1)
        lhs_o = jnp.concatenate([lhs_a, lhs_b], axis=1)
        new_mem = [None] * KT
        pair_row = pl.multiple_of(ROWS * i, 64) + 64 * (u // 2)

        def finish(n, y):
            ym = y[m0:m0 + MEM]
            new_mem[n] = _b2u(jnp.concatenate([ym, ym], axis=0).astype(BF))
            yb = y.astype(BF)
            store_tokens(abuf, n, h_ld, _b2u(yb))
            cols = pl.ds(128 * n, 128)
            lo, cnt = (XS, 2 * SEG - XS) if odd else (0, XS)
            rows = pl.ds(pl.multiple_of(pair_row + lo, 8), cnt)
            a = yb.astype(F32)
            b = _u2b(xn_t[n, pl.ds(h_ld + 8 * odd, y.shape[0] // 2), :]).astype(F32)
            sl = slice(MEM, MEM + cnt) if odd else slice(0, cnt)
            out_s[rows, cols] = residual(x_s[rows, cols].astype(F32), a[sl], b[sl])

        order = list(range(n_part, KT))
        for n in order:
            finish(n, _dot(lhs_o, _u2b(wo_s[n])))
            if n < KT - 1:
                side_group()
            if n == n_part:
                for n2 in range(n_part):
                    tail = _u2b(wo_s[n2, pl.ds(h_split * 64, (H - h_split) * 64), :])
                    finish(n2, _dot(lhs_b, tail) + acc[n2])
        return new_mem

    def patch_row(t, yrow):
        xr, w = load_row(t)
        bits = pltpu.bitcast(_rbf(xr + yrow), U32)
        w = jnp.where(t % 2 == 0,
                      (w & jnp.uint32(0xFFFF0000)) | (bits >> 16),
                      (w & jnp.uint32(0xFFFF)) | bits)
        for k in range(KT):
            xn_t[k, pl.ds(t // 2, 1), :] = w[:, 128 * k:128 * (k + 1)]

    def fix_copy(j):
        r0 = pl.multiple_of(idx_s[2 + j] * 16, 16)
        return pltpu.make_async_copy(out_s.at[pl.ds(r0, 16), :], out_hbm.at[pl.ds(r0, 16), :],
                                     sems.at[SEM_FIX + j])

    def gather_tokens():
        for cp in ffn_copies:
            cp.wait()
        idx_s[0] = sel_s[0, 0]
        idx_s[1] = sel_s[1, 0]
        sel_row = lax.broadcasted_iota(jnp.int32, (8, D), 0)
        xs1, _ = load_row(idx_s[0])
        xs2, _ = load_row(idx_s[1])
        xsel_s[...] = jnp.where(sel_row == 0, xs1, jnp.where(sel_row == 1, xs2, 0.0))

    def apply_ffn():
        out_copy(0).wait()
        patch_row(idx_s[0], yy_s[0:1, :])
        patch_row(idx_s[1], yy_s[1:2, :])
        blks = [idx_s[j] >> 4 for j in range(2)]
        for blk in blks:
            r0 = pl.multiple_of(jnp.minimum(blk, (S - ROWS) // 16 - 1) * 16, 16)
            for n in range(KT):
                cols = pl.ds(128 * n, 128)
                out_s[pl.ds(r0, 16), cols] = residual(
                    x_s[pl.ds(r0, 16), cols].astype(F32),
                    _u2b(abuf[n, pl.ds(half_rows(r0), 8), :]).astype(F32),
                    _u2b(xn_t[n, pl.ds(half_rows(r0), 8), :]).astype(F32))
        blk1, blk2 = [jnp.minimum(blk, (S - 2 * ROWS) // 16 - 1) for blk in blks]
        blk2 = jnp.where(blk2 == blk1, jnp.where(blk1 == 0, 1, blk1 - 1), blk2)
        for j, blk in enumerate((blk1, blk2)):
            idx_s[2 + j] = blk
            fix_copy(j).start()
        out_copy(1).start()

    def body(i, carry):
        mem, y = list(carry[:KT]), list(carry[KT:])

        @pl.when((i == 1) | (i >= NIT - 2))
        def _():
            pl.when(i == 1)(gather_tokens)
            pl.when(i == NIT - 2)(lambda: out_copy(0).start())
            pl.when(i == NIT - 1)(apply_ffn)

        side = ffn_groups(i, y)
        held = {}
        for u in range(UNROLL):
            mem = one_step(i, u, mem, held, side)
        for _ in side:
            raise AssertionError("ffn groups left over")
        gate = _rbf(jax.nn.sigmoid(gate_s[:, 0:1]))
        yy_s[...] = _rbf(_rbf(jnp.concatenate(y, axis=1)) * gate)
        return tuple(mem) + tuple(y)

    for n in range(KT):
        wo_copy(n).wait()
    for cp in ffn0_copies:
        cp.wait()
    xsel_s[...] = jnp.zeros(xsel_s.shape, F32)
    mi = mem0_s[...].astype(F32)
    mip = _b2u(jnp.concatenate([mi, mi], axis=0).astype(BF))
    lax.fori_loop(0, NIT, body,
                  tuple(mip[:, 128 * k:128 * (k + 1)] for k in range(KT))
                  + (jnp.zeros((8, 512), F32), jnp.zeros((8, 512), F32)))
    out_copy(2).start()
    for j in range(2):
        fix_copy(j).wait()
    out_copy(1).wait()
    out_copy(2).wait()


@jax.jit
def pallas_parallel_sum__memory_aug_recurrent_mem_tr__moe_arch_mod__prompt_kernel(
    A_x: jax.Array,
    A_mem0: jax.Array,
    A_Wq: jax.Array,
    A_Wk: jax.Array,
    A_Wv: jax.Array,
    A_Wo: jax.Array,
    A_seg_len: jax.Array,
    B_x: jax.Array,
    B_w_r: jax.Array,
    B_w_gate: jax.Array,
    B_w_up: jax.Array,
    B_w_down: jax.Array,
):
    del A_seg_len, B_x
    assert A_x.shape == (1, S, D) and A_mem0.shape == (1, MEM, D)
    assert A_Wq.shape == (D, H, DH) and A_Wo.shape == (H, DH, D)
    assert B_w_gate.shape == (D, FF) and B_w_down.shape == (FF, D)
    any_spec = pl.BlockSpec(memory_space=pl.ANY)
    out = pl.pallas_call(
        _kernel,
        out_shape=jax.ShapeDtypeStruct((S, D), BF),
        in_specs=[any_spec] * 10,
        out_specs=any_spec,
        scratch_shapes=[
            pltpu.VMEM((S, D), BF),
            pltpu.VMEM((KT, S // 2, 128), U32),
            pltpu.VMEM((KT, PRE // 2, 128), U32),
            pltpu.VMEM((KT, 16 * NSEG, 128), U32),
            pltpu.VMEM((3 * H + 2, D // 2, 128), U32),
            pltpu.VMEM((KT, H * DH // 2, 128), U32),
            pltpu.VMEM((3 * H, RING32, 128), U32),
            pltpu.VMEM((KT, S // 2, 128), U32),
            pltpu.VMEM((S, D), BF),
            pltpu.VMEM((NPQ + 1, D, 128), U32),
            pltpu.VMEM((D // 2, FF), U32),
            pltpu.VMEM((D // 2, FF), U32),
            pltpu.VMEM((FF // 2, D), U32),
            pltpu.VMEM((MEM, D), BF),
            pltpu.VMEM((D,), BF),
            pltpu.VMEM((8, D), F32),
            pltpu.VMEM((16, 128), F32),
            pltpu.VMEM((8, 128), jnp.int32),
            pltpu.VMEM((8, 128), F32),
            pltpu.VMEM((8, D), F32),
            pltpu.VMEM((8, D), F32),
            pltpu.SMEM((1,), jnp.int32),
            pltpu.SMEM((4,), jnp.int32),
            pltpu.SemaphoreType.DMA((NSEM,)),
        ],
        compiler_params=pltpu.CompilerParams(vmem_limit_bytes=126 * 1024 * 1024,
                                             disable_bounds_checks=True, disable_semaphore_checks=True),
    )(A_x.reshape(S, D), A_mem0.reshape(MEM, D), A_Wq, A_Wk, A_Wv, A_Wo.reshape(H * DH, D),
      B_w_r, B_w_gate, B_w_up, B_w_down)
    return out.reshape(1, S, D)
```

```python
import jax
import jax.numpy as jnp
from jax import lax
import jax.experimental.pallas as pl
import jax.experimental.pallas.tpu as pltpu

BF = jnp.bfloat16
U32 = jnp.uint32
F32 = jnp.float32

S = 2048
D = 1024
H = 32
DH = 128
MEM = 8
SEG = 32
NSEG = S // SEG
FF = 3584
KT = D // 128
FT = FF // 128
XS = 24
PRE = S - NSEG * XS
RING = 576
RING32 = RING // 2
NPAIR = H // 2
NPQ = 3 * NPAIR
PP = 6
NPRE = NPQ // PP
LNP = 16
SEM_SMALL, SEM_X0, SEM_X = 0, 2, 6
SEM_W0 = SEM_X + NPRE
SEM_W = SEM_W0 + PP
SEM_WO = SEM_W + NPRE
SEM_FFN0, SEM_FFN, SEM_FIX, SEM_OUT = SEM_WO + 1, SEM_WO + 2, SEM_WO + 3, SEM_WO + 5
NSEM = SEM_OUT + 3

LAG_QK = 1
LAG_PV = 4
N_PART, H_SPLIT = 4, 26
N_PART_ODD, H_SPLIT_ODD = 4, 24
K_SPLIT = 2
UNROLL = 4

REL_SCHED = {0: [(0, 0), (0, 1)], 1: [(0, 2), (0, 3)], 2: [(0, 4)], 3: [(0, 5)], 4: [(0, 6)], 5: [(0, 7)]}
REL_SCHED.update({8 * j - 2 + k: [(j, k)] for j in range(1, PP) for k in range(8)})
REL_SCHED0 = {6: [(0, k) for k in range(8)],
              13: [(1, k) for k in range(8)],
              26: [(3, k) for k in range(3)], 27: [(3, k) for k in range(3, 6)], 28: [(3, 6), (3, 7)]}
REL_SCHED0.update({8 * j - 2 + k: [(j, k)] for j in (2, 4, 5) for k in range(8)})
BARRIERS0 = {6: [1], 13: [2, 3], 26: [4, 5, 6]}
SCORE_SCHED = [1, 16, 31]
LN_SCHED = [11 * q // 4 for q in range(LNP)]
LN_LAG = 5
REL_LAG = 2
FIRST_BATCH = 6


def _b2u(x):
    return pltpu.bitcast(x, U32)


def _u2b(x):
    return pltpu.bitcast(x, BF)


def _dot(a, b):
    return jnp.dot(a, b, preferred_element_type=F32)


def _dot_nt(a, b):
    return lax.dot_general(a, b, (((1,), (1,)), ((), ())), preferred_element_type=F32)


def _after(w, dep, zero):
    if not dep:
        return w
    d = dep[0]
    for e in dep[1:]:
        d = d | e
    return jnp.concatenate([w[0:8] | (d & zero), w[8:]], axis=0)


def _rbf(x):
    return x.astype(BF).astype(F32)


def _kernel(x_hbm, mem0_hbm, wq_hbm, wk_hbm, wv_hbm, wo_hbm, wr_hbm, wg_hbm, wu_hbm, wd_hbm,
            out_hbm,
            x_s, xn_t, xn_pre, hbuf, wqkv, wo_s, ring, abuf, out_s, raw,
            wg_s, wu_s, wd_s, mem0_s, wr_s, wrf_s, r_s, sel_s, gate_s, xsel_s, yy_s, zero_s, idx_s,
            sems):
    w32 = [w.bitcast(U32) for w in (wq_hbm, wk_hbm, wv_hbm)]
    wo32 = wo_hbm.bitcast(U32)
    wg32 = wg_hbm.bitcast(U32)
    wu32 = wu_hbm.bitcast(U32)
    wd32 = wd_hbm.bitcast(U32)

    def rows_copy(r0, n, sem):
        return pltpu.make_async_copy(x_hbm.at[pl.ds(r0, n), :], x_s.at[pl.ds(r0, n), :], sems.at[sem])

    def x_first(c):
        return rows_copy(128 * c if isinstance(c, int) else pl.multiple_of(128 * c, 128), 128, SEM_X0 + c)

    def x_piece(t):
        r0 = PRE + 16 * LNP * (t - 2)
        return rows_copy(r0 if isinstance(t, int) else pl.multiple_of(r0, 256), 16 * LNP, SEM_X + t)

    def pair_copy(p):
        q = min(p, NPQ - 1)
        sem = SEM_W0 + p if p <= PP else SEM_W + (p - 1) // PP
        return pltpu.make_async_copy(w32[q // NPAIR].at[:, q % NPAIR, :], raw.at[p], sems.at[sem])

    def pairs_wait(t):
        dst = raw.at[pl.ds(PP * t + 1, PP)]
        pltpu.make_async_copy(dst, dst, sems.at[SEM_W + t]).wait()

    def wo_copy(n):
        return pltpu.make_async_copy(wo32.at[:, pl.ds(128 * n, 128)], wo_s.at[n], sems.at[SEM_WO])

    small_copies = [pltpu.make_async_copy(mem0_hbm, mem0_s, sems.at[SEM_SMALL]),
                    pltpu.make_async_copy(wr_hbm, wr_s, sems.at[SEM_SMALL + 1])]
    ffn0_copies = [
        pltpu.make_async_copy(wg32.at[:, pl.ds(0, 128)], wg_s.at[:, pl.ds(0, 128)], sems.at[SEM_FFN0]),
        pltpu.make_async_copy(wu32.at[:, pl.ds(0, 128)], wu_s.at[:, pl.ds(0, 128)], sems.at[SEM_FFN0]),
        pltpu.make_async_copy(wd32.at[pl.ds(0, 64), :], wd_s.at[pl.ds(0, 64), :], sems.at[SEM_FFN0])]
    ffn_copies = [
        pltpu.make_async_copy(wg32.at[:, pl.ds(128, FF - 128)], wg_s.at[:, pl.ds(128, FF - 128)], sems.at[SEM_FFN]),
        pltpu.make_async_copy(wu32.at[:, pl.ds(128, FF - 128)], wu_s.at[:, pl.ds(128, FF - 128)], sems.at[SEM_FFN]),
        pltpu.make_async_copy(wd32.at[pl.ds(64, FF // 2 - 64), :], wd_s.at[pl.ds(64, FF // 2 - 64), :],
                              sems.at[SEM_FFN])]

    zero_s[0] = 0
    for c in range(4):
        x_first(c).start()
        if c == 0:
            for cp in small_copies:
                cp.start()
            pair_copy(0).start()

    def queue(t0, t1):
        for t in range(t0, t1):
            for p in range(PP * t + 1, PP * t + PP + 1):
                pair_copy(p).start()
            if t >= 2:
                x_piece(t).start()

    queue(0, FIRST_BATCH)
    eps_bf = 1.0013580322265625e-05

    def score16(g, xn):
        wr = jnp.concatenate([wrf_s[...], wrf_s[...]], axis=0)
        score = _rbf(jnp.sum(xn.astype(F32) * wr, axis=1, keepdims=True))
        r_s[...] = jnp.where(lane16 == g, score, r_s[...])

    def layernorm16(rq, dst_ref, dst_row, not_before=None):
        rq = rq if isinstance(rq, int) else pl.multiple_of(rq, 16)
        xf = x_s[pl.ds(rq, 16), :].astype(F32)
        if not_before is not None:
            x0 = _after(pltpu.bitcast(xf[:, 0:128], U32), [not_before], zero_box[0])
            xf = jnp.concatenate([pltpu.bitcast(x0, F32), xf[:, 128:]], axis=1)
        mean = jnp.sum(xf, axis=1, keepdims=True) * (1.0 / D)
        cen = xf - mean
        var = jnp.sum(cen * cen, axis=1, keepdims=True) * (1.0 / D)
        sd = _rbf(jnp.sqrt(_rbf(_rbf(var) + eps_bf)))
        xn = (_rbf(xf - _rbf(mean)) * (1.0 / sd)).astype(BF)
        if dst_ref is hbuf:
            score16(rq // 16, xn)
        xp = _b2u(xn)
        hq = rq // 2 if isinstance(rq, int) else pl.multiple_of(rq // 2, 8)
        dst_row = dst_row if isinstance(dst_row, int) else pl.multiple_of(dst_row, 8)
        for k in range(KT):
            xn_t[k, pl.ds(hq, 8), :] = xp[:, 128 * k:128 * (k + 1)]
            dst_ref[k, pl.ds(dst_row, 8), :] = xp[:, 128 * k:128 * (k + 1)]

    zero_box = [None]

    def fresh_zero():
        zero_box[0] = jnp.full((8, 128), zero_s[0], jnp.int32).astype(U32)

    r_s[...] = jnp.full(r_s.shape, -jnp.inf, F32)
    lane16 = lax.broadcasted_iota(jnp.int32, (16, 128), 1)

    x_first(0).wait()
    for q in range(8):
        layernorm16(16 * q, xn_pre, 8 * q)


    def relayout(src, dst, j, k, not_before=None):
        a = src[j, pl.ds(128 * k, 64, stride=2), :]
        if not_before is not None:
            a = a | jnp.concatenate([not_before & zero_box[0]] * 8, axis=0)
        b = src[j, pl.ds(128 * k + 1, 64, stride=2), :]
        rows = pl.ds(64 * k, 64)
        dst[2 * j, rows, :] = (a & jnp.uint32(0xFFFF)) | (b << 16)
        dst[2 * j + 1, rows, :] = (a >> 16) | (b & jnp.uint32(0xFFFF0000))

    def pre_dot(w_view, ring_view, h, row, dep=None):
        lhs = jnp.concatenate([_u2b(xn_pre[kk, pl.ds(row, 64), :]) for kk in range(KT)], axis=1)
        y = _dot(lhs, _u2b(_after(w_view[h], dep, zero_box[0])))
        yp = _b2u(y.astype(BF))
        ring_view[h, pl.ds(32 + row, 64), :] = yp
        return yp[0:8]

    for c in small_copies:
        c.wait()
    pair_copy(0).wait()
    for k in range(8):
        relayout(raw, wqkv, 0, k)
    wrf_s[...] = jnp.broadcast_to(wr_s[...].astype(F32).reshape(1, D), (8, D))

    def start_body(c, carry):
        x_first(c).wait()
        row = pl.multiple_of(64 * (c - 1), 64)
        for h in range(2):
            pre_dot(wqkv, ring, h, row)
        for q in range(8):
            layernorm16(2 * row + 128 + 16 * q, xn_pre, row + 64 + 8 * q)
        return carry

    lax.fori_loop(1, PRE // 128, start_body, 0)

    def second_batch():
        queue(FIRST_BATCH, NPRE)
        for n in range(KT):
            wo_copy(n).start()
        for cp in ffn0_copies + ffn_copies:
            cp.start()

    def pre_iter(t, first):
        deps = {}
        raw_view = raw.at[pl.ds(PP * t, PP + 1)]
        w_view = wqkv.at[pl.ds(2 * PP * t, 2 * PP + 2)]
        ring_view = ring.at[pl.ds(2 * PP * t, 2 * PP)]
        done = None
        for v in range(6 if first else 0, 8 * PP):
            h, row = v // 4, 64 * (v % 4)
            if first and v < 8:
                h, row = v - 6, 192
            if v == 0 or (first and v in BARRIERS0):
                if v:
                    for p in BARRIERS0[v]:
                        pair_copy(p).wait()
                    if v == max(BARRIERS0):
                        second_batch()
                fresh_zero()
                done = None
            prev = done
            done = pre_dot(w_view, ring_view, h, row, deps.get(v))
            for jr, kr in (REL_SCHED0 if first else REL_SCHED).get(v, ()):
                relayout(raw_view, w_view, jr + 1, kr, prev)
                deps.setdefault(v + REL_LAG, []).append(w_view[2 * jr + 3, pl.ds(64 * kr + 56, 8), :])
            if first:
                continue
            if v in LN_SCHED:
                q = LNP * (t - 2) + LN_SCHED.index(v)
                hrow = pl.multiple_of(jnp.where(q < 0, XS, 32 * (q // 3) + 8 * (q % 3)), 8)
                layernorm16(PRE + 16 * q, hbuf, hrow, done if prev is not None else None)
                deps.setdefault(v + LN_LAG, []).append(hbuf[KT - 1, pl.ds(hrow, 8), :])
            if v in SCORE_SCHED:
                g = jnp.minimum(len(SCORE_SCHED) * (t - 1) + SCORE_SCHED.index(v), PRE // 16 - LNP - 1)
                rows = pl.ds(pl.multiple_of(8 * g, 8), 8)
                xp = [xn_pre[kk, rows, :] for kk in range(KT)]
                xp[0] = xp[0] | (done & zero_box[0])
                score16(g, _u2b(jnp.concatenate(xp, axis=1)))

    pre_iter(0, True)

    def pre_body(t, carry):
        pairs_wait(t)

        @pl.when(t >= 2)
        def _():
            x_piece(t).wait()
        pre_iter(t, False)
        return carry

    lax.fori_loop(1, NPRE, pre_body, 0)
    row = lax.broadcasted_iota(jnp.int32, (80, 80), 0)
    col = lax.broadcasted_iota(jnp.int32, (80, 80), 1)
    same_head = (jnp.where(row < 64, row >> 5, (row - 64) >> 3)
                 == jnp.where(col < 64, col >> 5, (col - 64) >> 3))
    allowed = same_head & ((col >= 64) | (row >= 64) | (col <= row))
    fill = jnp.where(same_head, -1e9, -jnp.inf).astype(F32)
    low_half = lax.broadcasted_iota(jnp.int32, (8, 128), 0) < 4
    high_half = jnp.logical_not(low_half)
    scale = DH ** -0.5

    def load_row(t):
        w = jnp.concatenate([xn_t[k, pl.ds(t // 2, 1), :] for k in range(KT)], axis=1)
        bits = jnp.where(t % 2 == 0, w << 16, w & jnp.uint32(0xFFFF0000))
        return pltpu.bitcast(bits, F32), w

    def select_tokens():
        r = r_s[...]
        tok = lane16 * 16 + lax.broadcasted_iota(jnp.int32, (16, 128), 0)

        def full(op, v):
            return op(op(v, axis=0, keepdims=True), axis=1, keepdims=True)

        top1 = full(jnp.max, r)
        idx1 = full(jnp.min, jnp.where(r == top1, tok, S - 1))
        r2 = jnp.where(tok == idx1, -jnp.inf, r)
        top2 = full(jnp.max, r2)
        idx2 = full(jnp.min, jnp.where((r2 == top2) & (tok != idx1), tok, S - 1))
        first = lax.broadcasted_iota(jnp.int32, (8, 128), 0) == 0
        gate_s[...] = jnp.where(first, top1, top2)
        sel_s[...] = jnp.where(first, idx1, idx2)

    NIT = NSEG // UNROLL
    ROWS = SEG * UNROLL

    def half_rows(r0):
        return pl.multiple_of(r0 // 2, 8)

    def residual(xf, a, b):
        return (_rbf(xf + a) + b).astype(BF)

    def out_copy(j):
        r0, n = (0, S - 2 * ROWS) if j == 0 else (S - (3 - j) * ROWS, ROWS)
        return pltpu.make_async_copy(out_s.at[pl.ds(r0, n), :], out_hbm.at[pl.ds(r0, n), :],
                                     sems.at[SEM_OUT + j])

    def ffn_groups(i, y):
        x_sel = xsel_s[...]
        live = (i >= 1) & (i < NIT - 1)
        hid = {}

        def up(w_ref, j, key):
            cols = pl.ds(pl.multiple_of(128 * j, 128), 128)
            part = _dot(x_sel[:, 0:512], _u2b(w_ref[pl.ds(0, 256), cols]).astype(F32))
            yield
            hid[key] = _rbf(_dot(x_sel[:, 512:1024], _u2b(w_ref[pl.ds(256, 256), cols]).astype(F32)) + part)
            yield

        for jj in range(2):
            j = jnp.clip(2 * (i - 1) + jj, 0, FT - 1)
            yield from up(wg_s, j, "g")
            yield from up(wu_s, j, "u")
            g = hid["g"]
            hb = jnp.where(live, _rbf(_rbf(g * _rbf(jax.nn.sigmoid(g))) * hid["u"]), 0.0)
            rows = pl.ds(pl.multiple_of(64 * j, 64), 64)
            yield
            for half in range(2):
                y[half] = _dot(hb, _u2b(wd_s[rows, pl.ds(512 * half, 512)]).astype(F32)) + y[half]
                yield

    def one_step(i, u, mem, held, side):
        odd = u % 2
        s2 = i * (UNROLL // 2) + u // 2
        h_ld = pl.multiple_of(16 * UNROLL * i, 32) + 32 * (u // 2)
        r24 = pl.multiple_of((12 * UNROLL * i) % RING32, 8) + XS * (u // 2)
        qkv_ld = pl.multiple_of((SEG * s2 + 32) % RING32, 32) + 16 * odd
        m0 = 0 if odd else XS

        def with_mem(lo, hi, m):
            if odd:
                return [jnp.where(low_half, m, lo), hi]
            return [lo, jnp.where(low_half, hi, m)]

        def store_tokens(ref, idx, base, yp):
            if odd:
                pltpu.store(ref.at[idx, pl.ds(base + 8, 8), :], yp[0:8], mask=high_half)
                ref[idx, pl.ds(base + 16, yp.shape[0] - 8), :] = yp[8:]
            else:
                ref[idx, pl.ds(base, 8), :] = yp[0:8]
                pltpu.store(ref.at[idx, pl.ds(base + 8, 8), :], yp[8:16], mask=low_half)

        lk = [_u2b(jnp.concatenate(with_mem(hbuf[k, pl.ds(h_ld + 8 * odd, 8), :],
                                            hbuf[k, pl.ds(h_ld + 8 + 8 * odd, 8), :], mem[k]), axis=0))
              for k in range(KT)]
        lhs = jnp.concatenate(lk, axis=1)

        ymem = {}
        xs = {}
        probs = {}
        parts = {}

        def proj(h):
            split = h < K_SPLIT and u > 0
            if split:
                lhs7 = jnp.concatenate(lk[:KT - 1], axis=1)
                head = [_dot(lhs7, _u2b(wqkv[m * H + h, pl.ds(0, 448), :])) for m in range(3)]
            for m in range(3):
                if split:
                    y = _dot(lk[KT - 1], _u2b(wqkv[m * H + h, pl.ds(448, 64), :])) + head[m]
                else:
                    y = _dot(lhs, _u2b(wqkv[m * H + h]))
                store_tokens(ring, m * H + h, r24, _b2u(y.astype(BF)))
                ymem[(h, m)] = y[m0:m0 + MEM]
                xs[(h, m)] = ring[m * H + h, pl.ds(qkv_ld, SEG // 2), :]

        def pair(p, m):
            a, b = 2 * p, 2 * p + 1
            mm = jnp.concatenate([ymem[(a, m)], ymem[(b, m)]], axis=0).astype(BF)
            return jnp.concatenate([_u2b(xs[(a, m)]), _u2b(xs[(b, m)]), mm], axis=0)

        def qk(p):
            sc = _dot_nt(pair(p, 0), pair(p, 1))
            sc = jnp.where(allowed, sc * scale, fill)
            e = jnp.exp(sc - jnp.max(sc, axis=1, keepdims=True))
            l = jnp.sum(e, axis=1, keepdims=True)
            r = pl.reciprocal(l, approx=True)
            r = r * (2.0 - l * r)
            probs[p] = (e * r).astype(BF)

        def pv(p):
            op = _b2u(_dot(probs[p], pair(p, 2)).astype(BF))
            om = op[32:40]
            om_sw = pltpu.roll(om, 4, axis=0)
            for j, h in enumerate((2 * p, 2 * p + 1)):
                x0, x1 = op[16 * j:16 * j + 8], op[16 * j + 8:16 * j + 16]
                m = om if j != odd else om_sw
                if odd:
                    rows = with_mem(held[h], x0, m) + [x1]
                else:
                    rows = with_mem(x0, x1, m)
                    held[h] = x1
                parts[h] = _u2b(jnp.concatenate(rows, axis=0))

        def after(t):
            for lag, fn in ((LAG_QK, qk), (LAG_PV, pv)):
                if (t - 1 - lag) % 2 == 0 and 0 <= (t - 1 - lag) // 2 < NPAIR:
                    fn((t - 1 - lag) // 2)

        def side_group():
            if odd:
                next(side, None)

        for t in range(H):
            proj(t)
            after(t)
            if u == 0 and t == 8:
                select_tokens()
        t = H
        n_part, h_split = (N_PART_ODD, H_SPLIT_ODD) if odd else (N_PART, H_SPLIT)
        lhs_a = jnp.concatenate([parts[j] for j in range(h_split)], axis=1)
        acc = []
        for n in range(n_part):
            acc.append(_dot(lhs_a, _u2b(wo_s[n, pl.ds(0, h_split * 64), :])))
            after(t)
            side_group()
            t += 1
        while t - 1 - LAG_PV <= 2 * (NPAIR - 1):
            after(t)
            t += 1
        lhs_b = jnp.concatenate([parts[j] for j in range(h_split, H)], axis=1)
        lhs_o = jnp.concatenate([lhs_a, lhs_b], axis=1)
        new_mem = [None] * KT
        pair_row = pl.multiple_of(ROWS * i, 64) + 64 * (u // 2)

        def finish(n, y):
            ym = y[m0:m0 + MEM]
            new_mem[n] = _b2u(jnp.concatenate([ym, ym], axis=0).astype(BF))
            yb = y.astype(BF)
            store_tokens(abuf, n, h_ld, _b2u(yb))
            cols = pl.ds(128 * n, 128)
            lo, cnt = (XS, 2 * SEG - XS) if odd else (0, XS)
            rows = pl.ds(pl.multiple_of(pair_row + lo, 8), cnt)
            a = yb.astype(F32)
            b = _u2b(xn_t[n, pl.ds(h_ld + 8 * odd, y.shape[0] // 2), :]).astype(F32)
            sl = slice(MEM, MEM + cnt) if odd else slice(0, cnt)
            out_s[rows, cols] = residual(x_s[rows, cols].astype(F32), a[sl], b[sl])

        order = list(range(n_part, KT))
        for n in order:
            finish(n, _dot(lhs_o, _u2b(wo_s[n])))
            if n < KT - 1:
                side_group()
            if n == n_part:
                for n2 in range(n_part):
                    tail = _u2b(wo_s[n2, pl.ds(h_split * 64, (H - h_split) * 64), :])
                    finish(n2, _dot(lhs_b, tail) + acc[n2])
        return new_mem

    def patch_row(t, yrow):
        xr, w = load_row(t)
        bits = pltpu.bitcast(_rbf(xr + yrow), U32)
        w = jnp.where(t % 2 == 0,
                      (w & jnp.uint32(0xFFFF0000)) | (bits >> 16),
                      (w & jnp.uint32(0xFFFF)) | bits)
        for k in range(KT):
            xn_t[k, pl.ds(t // 2, 1), :] = w[:, 128 * k:128 * (k + 1)]

    def fix_copy(j):
        r0 = pl.multiple_of(idx_s[2 + j] * 16, 16)
        return pltpu.make_async_copy(out_s.at[pl.ds(r0, 16), :], out_hbm.at[pl.ds(r0, 16), :],
                                     sems.at[SEM_FIX + j])

    def gather_tokens():
        for cp in ffn_copies:
            cp.wait()
        idx_s[0] = sel_s[0, 0]
        idx_s[1] = sel_s[1, 0]
        sel_row = lax.broadcasted_iota(jnp.int32, (8, D), 0)
        xs1, _ = load_row(idx_s[0])
        xs2, _ = load_row(idx_s[1])
        xsel_s[...] = jnp.where(sel_row == 0, xs1, jnp.where(sel_row == 1, xs2, 0.0))

    def apply_ffn():
        out_copy(0).wait()
        patch_row(idx_s[0], yy_s[0:1, :])
        patch_row(idx_s[1], yy_s[1:2, :])
        blks = [idx_s[j] >> 4 for j in range(2)]
        for blk in blks:
            r0 = pl.multiple_of(jnp.minimum(blk, (S - ROWS) // 16 - 1) * 16, 16)
            for n in range(KT):
                cols = pl.ds(128 * n, 128)
                out_s[pl.ds(r0, 16), cols] = residual(
                    x_s[pl.ds(r0, 16), cols].astype(F32),
                    _u2b(abuf[n, pl.ds(half_rows(r0), 8), :]).astype(F32),
                    _u2b(xn_t[n, pl.ds(half_rows(r0), 8), :]).astype(F32))
        blk1, blk2 = [jnp.minimum(blk, (S - 2 * ROWS) // 16 - 1) for blk in blks]
        blk2 = jnp.where(blk2 == blk1, jnp.where(blk1 == 0, 1, blk1 - 1), blk2)
        for j, blk in enumerate((blk1, blk2)):
            idx_s[2 + j] = blk
            fix_copy(j).start()
        out_copy(1).start()

    def body(i, carry):
        mem, y = list(carry[:KT]), list(carry[KT:])

        @pl.when((i == 1) | (i >= NIT - 2))
        def _():
            pl.when(i == 1)(gather_tokens)
            pl.when(i == NIT - 2)(lambda: out_copy(0).start())
            pl.when(i == NIT - 1)(apply_ffn)

        side = ffn_groups(i, y)
        held = {}
        for u in range(UNROLL):
            mem = one_step(i, u, mem, held, side)
        for _ in side:
            raise AssertionError("ffn groups left over")
        gate = _rbf(jax.nn.sigmoid(gate_s[:, 0:1]))
        yy_s[...] = _rbf(_rbf(jnp.concatenate(y, axis=1)) * gate)
        return tuple(mem) + tuple(y)

    for n in range(KT):
        wo_copy(n).wait()
    for cp in ffn0_copies:
        cp.wait()
    xsel_s[...] = jnp.zeros(xsel_s.shape, F32)
    mi = mem0_s[...].astype(F32)
    mip = _b2u(jnp.concatenate([mi, mi], axis=0).astype(BF))
    lax.fori_loop(0, NIT, body,
                  tuple(mip[:, 128 * k:128 * (k + 1)] for k in range(KT))
                  + (jnp.zeros((8, 512), F32), jnp.zeros((8, 512), F32)))
    out_copy(2).start()
    for j in range(2):
        fix_copy(j).wait()
    out_copy(1).wait()
    out_copy(2).wait()


@jax.jit
def pallas_parallel_sum__memory_aug_recurrent_mem_tr__moe_arch_mod__prompt_kernel(
    A_x: jax.Array,
    A_mem0: jax.Array,
    A_Wq: jax.Array,
    A_Wk: jax.Array,
    A_Wv: jax.Array,
    A_Wo: jax.Array,
    A_seg_len: jax.Array,
    B_x: jax.Array,
    B_w_r: jax.Array,
    B_w_gate: jax.Array,
    B_w_up: jax.Array,
    B_w_down: jax.Array,
):
    del A_seg_len, B_x
    assert A_x.shape == (1, S, D) and A_mem0.shape == (1, MEM, D)
    assert A_Wq.shape == (D, H, DH) and A_Wo.shape == (H, DH, D)
    assert B_w_gate.shape == (D, FF) and B_w_down.shape == (FF, D)
    any_spec = pl.BlockSpec(memory_space=pl.ANY)
    out = pl.pallas_call(
        _kernel,
        out_shape=jax.ShapeDtypeStruct((S, D), BF),
        in_specs=[any_spec] * 10,
        out_specs=any_spec,
        scratch_shapes=[
            pltpu.VMEM((S, D), BF),
            pltpu.VMEM((KT, S // 2, 128), U32),
            pltpu.VMEM((KT, PRE // 2, 128), U32),
            pltpu.VMEM((KT, 16 * NSEG, 128), U32),
            pltpu.VMEM((3 * H + 2, D // 2, 128), U32),
            pltpu.VMEM((KT, H * DH // 2, 128), U32),
            pltpu.VMEM((3 * H, RING32, 128), U32),
            pltpu.VMEM((KT, S // 2, 128), U32),
            pltpu.VMEM((S, D), BF),
            pltpu.VMEM((NPQ + 1, D, 128), U32),
            pltpu.VMEM((D // 2, FF), U32),
            pltpu.VMEM((D // 2, FF), U32),
            pltpu.VMEM((FF // 2, D), U32),
            pltpu.VMEM((MEM, D), BF),
            pltpu.VMEM((D,), BF),
            pltpu.VMEM((8, D), F32),
            pltpu.VMEM((16, 128), F32),
            pltpu.VMEM((8, 128), jnp.int32),
            pltpu.VMEM((8, 128), F32),
            pltpu.VMEM((8, D), F32),
            pltpu.VMEM((8, D), F32),
            pltpu.SMEM((1,), jnp.int32),
            pltpu.SMEM((4,), jnp.int32),
            pltpu.SemaphoreType.DMA((NSEM,)),
        ],
        compiler_params=pltpu.CompilerParams(vmem_limit_bytes=126 * 1024 * 1024,
                                             disable_bounds_checks=True, disable_semaphore_checks=True),
    )(A_x.reshape(S, D), A_mem0.reshape(MEM, D), A_Wq, A_Wk, A_Wv, A_Wo.reshape(H * DH, D),
      B_w_r, B_w_gate, B_w_up, B_w_down)
    return out.reshape(1, S, D)
```
